```python
import jax
import jax.numpy as jnp

def _softmax(x, axis=-1):
    return jax.nn.softmax(x, axis=axis)

def _gelu(x):
    return jax.nn.gelu(x, approximate=True)

def _silu(x):
    return jax.nn.silu(x)

def _sigmoid(x):
    return jax.nn.sigmoid(x)

def _layernorm(x, axis=-1, eps=1e-05):
    m = jnp.mean(x, axis=axis, keepdims=True)
    v = jnp.var(x, axis=axis, keepdims=True)
    return (x - m) / jnp.sqrt(v + eps)

def _scatter_add(tgt, idx, src, axis=0):
    return tgt.at[idx].add(src)

def _segment_sum(src, seg, n):
    return jax.ops.segment_sum(src, seg, n)

class _Rng:

    def __init__(self, key):
        self._k = key

    def _next(self):
        self._k, sub = jax.random.split(self._k)
        return sub

    def normal(self, shape):
        return jax.random.normal(self._next(), shape, dtype=jnp.bfloat16)

    def randint(self, lo, hi, shape):
        return jax.random.randint(self._next(), shape, lo, hi, dtype=jnp.int32)

    def uniform(self, shape, lo=0.0, hi=1.0):
        return jax.random.uniform(self._next(), shape, jnp.bfloat16, lo, hi)

    def permutation(self, n):
        return jax.random.permutation(self._next(), n)
kernel_name = 'adaLN_cond__memory_aug_recurrent_mem_tr__moe_arch_mod__prompt'

def setup_inputs():
    _rng = _Rng(jax.random.key(int.from_bytes(__import__("os").urandom(4), "little")))
    _w = lambda a: (lambda t: t.astype(jnp.bfloat16) if jnp.issubdtype(t.dtype, jnp.floating) else t)(jnp.asarray(a))

    def _A_setup():
        B, S, Dm = (1, 2048, 1024)
        H, Dh = (32, 128)
        M, seg = (8, 32)
        seg = min(seg, S)
        S = S // seg * seg
        return {'x': _w((lambda *s: _rng.normal(s) * 0.05)(B, S, Dm)), 'mem0': _w((lambda *s: _rng.normal(s) * 0.05)(B, M, Dm)), 'Wq': _w((lambda *s: _rng.normal(s) * 0.05)(Dm, H, Dh) * Dm ** (-0.5)), 'Wk': _w((lambda *s: _rng.normal(s) * 0.05)(Dm, H, Dh) * Dm ** (-0.5)), 'Wv': _w((lambda *s: _rng.normal(s) * 0.05)(Dm, H, Dh) * Dm ** (-0.5)), 'Wo': _w((lambda *s: _rng.normal(s) * 0.05)(H, Dh, Dm) * (H * Dh) ** (-0.5)), 'seg_len': seg}
    _A_in = _A_setup()

    def _B_setup():
        B, S, D, F, C = (1, 2048, 1024, 3584, 2)
        return {'x': _w((lambda *s: _rng.normal(s) * 0.05)(B, S, D)), 'w_r': _w((lambda *s: _rng.normal(s) * 0.05)(D)), 'w_gate': _w((lambda *s: _rng.normal(s) * 0.05)(D, F)), 'w_up': _w((lambda *s: _rng.normal(s) * 0.05)(D, F)), 'w_down': _w((lambda *s: _rng.normal(s) * 0.05)(F, D))}
    _B_in = _B_setup()
    return {'A_x': _A_in['x'], 'A_mem0': _A_in['mem0'], 'A_Wq': _A_in['Wq'], 'A_Wk': _A_in['Wk'], 'A_Wv': _A_in['Wv'], 'A_Wo': _A_in['Wo'], 'A_seg_len': _A_in['seg_len'], 'B_x': _B_in['x'], 'B_w_r': _B_in['w_r'], 'B_w_gate': _B_in['w_gate'], 'B_w_up': _B_in['w_up'], 'B_w_down': _B_in['w_down'], 'c': _w((lambda *s: _rng.normal(s) * 0.05)(1, 1024)), 'w_mod': _w((lambda *s: _rng.normal(s) * 0.05)(1024, 6 * 1024) * 1024 ** (-0.5))}

def reference(A_x, A_mem0, A_Wq, A_Wk, A_Wv, A_Wo, A_seg_len, B_x, B_w_r, B_w_gate, B_w_up, B_w_down, c, w_mod):

    def _A_ref(x, mem0, Wq, Wk, Wv, Wo, seg_len):
        B, S, Dm = x.shape
        H, Dh = (Wq.shape[1], Wq.shape[2])
        M = mem0.shape[1]
        scale = Dh ** (-0.5)
        n_seg = S // seg_len
        L = M + seg_len
        idx = jnp.arange(L)
        mask = (idx[:, None] < M) | (idx[:, None] >= idx[None, :])
        mem = mem0
        outs = []
        for s in range(n_seg):
            xs = x[:, s * seg_len:(s + 1) * seg_len, :].copy()
            h = jnp.concatenate([mem, xs], axis=1)
            q = jnp.einsum('btd,dhe->bhte', h, Wq)
            k = jnp.einsum('btd,dhe->bhte', h, Wk)
            v = jnp.einsum('btd,dhe->bhte', h, Wv)
            scores = jnp.einsum('bhqe,bhke->bhqk', q, k) * scale
            scores = jnp.where(mask[None, None], scores, -1000000000.0)
            p = _softmax(scores, axis=-1)
            o = jnp.einsum('bhqk,bhke->bhqe', p, v)
            o = jnp.einsum('bhte,hed->btd', o, Wo)
            mem = o[:, :M, :].copy()
            outs.append(o[:, M:, :])
        return jnp.concatenate(outs, axis=1)

    def _B_ref(x, w_r, w_gate, w_up, w_down):
        B, S, D = x.shape
        C = 2
        r = x @ w_r
        idx = jnp.argsort(-r, axis=-1)[:, :C]
        idx_e = jnp.repeat(idx.reshape(B, C, 1), D, axis=2)
        x_sel = jnp.take_along_axis(x, idx_e, axis=1)
        g = _silu(x_sel @ w_gate)
        u = x_sel @ w_up
        y = g * u @ w_down
        r_sel = _sigmoid(jnp.take_along_axis(r, idx, axis=1))
        y = y * r_sel.reshape(B, C, 1)
        b_off = (jnp.arange(B) * S).reshape(B, 1)
        flat_idx = (idx + b_off).reshape(B * C)
        zero = (x * 0.0).reshape(B * S, D)
        upd = _scatter_add(zero, flat_idx, y.reshape(B * C, D), axis=0)
        return x + upd.reshape(B, S, D)
    x = A_x
    mod = (_silu(c) @ w_mod).reshape(c.shape[0], 6, 1, -1)
    sa, ca, ga, sb, cb, gb = (mod[:, 0].copy(), mod[:, 1].copy(), mod[:, 2].copy(), mod[:, 3].copy(), mod[:, 4].copy(), mod[:, 5].copy())
    h = _layernorm(x, axis=-1) * (1 + ca) + sa
    x = x + ga * _A_ref(h, A_mem0, A_Wq, A_Wk, A_Wv, A_Wo, A_seg_len)
    h = _layernorm(x, axis=-1) * (1 + cb) + sb
    x = x + gb * _B_ref(h, B_w_r, B_w_gate, B_w_up, B_w_down)
    return x
```

```python
import jax
import jax.numpy as jnp
from jax import lax
import jax.experimental.pallas as pl
import jax.experimental.pallas.tpu as pltpu

BF16 = jnp.bfloat16
F32 = jnp.float32
U32 = jnp.uint32

S = 2048
D = 1024
H = 32
E = 128
M = 8
SEG = 32
NSEG = S // SEG
NPAIR = H // 2
F = 3584
DB = D // 128
FB = F // 128
GP = 8
NCHUNK = 3 * NPAIR // GP
PR = 2 * SEG + 2 * M
LAG = 8
EPS = 1e-5
SCALE = E ** (-0.5)


def _rb(v):
    return v.astype(BF16).astype(F32)


def _dot(a, b):
    return jnp.dot(a, b, preferred_element_type=F32)


def _bf(words):
    return pltpu.bitcast(words, BF16)


def _pk(v):
    return pltpu.bitcast(v.astype(BF16), U32)


def _ln_mod(x, scale1p, shift):
    m = jnp.mean(x, axis=-1, keepdims=True)
    xc = x - m
    var = jnp.mean(xc * xc, axis=-1, keepdims=True)
    sd = _rb(jnp.sqrt(_rb(_rb(var) + EPS)))
    n = _rb(_rb(x - _rb(m)) * (1.0 / sd))
    return _rb(_rb(n * scale1p) + shift)


def _fill_matrix():
    i = lax.broadcasted_iota(jnp.int32, (PR, PR), 0)
    j = lax.broadcasted_iota(jnp.int32, (PR, PR), 1)

    def head(t):
        return jnp.where(t < 2 * SEG, t >> 5, (t - 2 * SEG) >> 3)

    def pos(t):
        r = t & (SEG - 1)
        return jnp.where(t < 2 * SEG, jnp.where(r < M, r, r + M), M + (t & (M - 1)))

    same = head(i) == head(j)
    pi = pos(i)
    ok = jnp.where(pi < M, 1, jnp.where(pi >= pos(j), 1, 0))
    return jnp.where(same, jnp.where(ok == 1, 0.0, -1e9), -3e38).astype(F32)


def _kernel(x_hbm, mem0_ref, wq_hbm, wk_hbm, wv_hbm, wo_hbm, wr_ref, wg_hbm, wu_hbm, wd_hbm,
            c_ref, wmod_hbm, out_hbm,
            x_v, w_v, wo_v, cache, odef, lhs_v, o_s, a_all, x1_v, out_v, r_v, mod_v, fill_v,
            sem_x, sem_wo, sem_out):

    x_head = pltpu.make_async_copy(x_hbm.at[:, pl.ds(0, M), :], x_v.at[:, pl.ds(0, M), :], sem_x.at[0])
    x_tail = pltpu.make_async_copy(x_hbm.at[:, pl.ds(M, SEG - M), :], x_v.at[:, pl.ds(M, SEG - M), :],
                                   sem_x.at[1])
    wo_w = wo_hbm.bitcast(U32)
    wo_cps = [pltpu.make_async_copy(wo_w.at[:, pl.ds(j * 128, 128)], wo_v.at[j], sem_wo.at[j])
              for j in range(DB)]

    def mod_row(k):
        return mod_v[k, 0:1, :]

    def prologue(stage, wmod_v, hc, sem_st, sem_mod):
        mod_cps = [pltpu.make_async_copy(wmod_hbm.at[:, pl.ds(k * D, D)], wmod_v.at[k], sem_mod.at[k])
                   for k in range(6)]
        st_cps = []
        for m_i, w_hbm in enumerate((wq_hbm, wk_hbm, wv_hbm)):
            wb = w_hbm.bitcast(U32)
            for g in range(NPAIR // GP):
                ci = m_i * (NPAIR // GP) + g
                st_cps.append(pltpu.make_async_copy(wb.at[:, pl.ds(g * GP, GP), :], stage.at[ci],
                                                    sem_st.at[ci]))
        x_head.start()
        mod_cps[0].start()
        mod_cps[1].start()
        for cp in st_cps:
            cp.start()
        x_tail.start()
        for cp in wo_cps:
            cp.start()
        for cp in mod_cps[2:]:
            cp.start()

        fill_v[...] = _fill_matrix()
        odef[:, pl.ds(0, SEG), :] = jnp.zeros((H, SEG, E), BF16)
        a_all[0] = jnp.zeros((SEG, D), BF16)

        c = c_ref[...].astype(F32)
        sc = (c * jax.nn.sigmoid(c)).astype(BF16)
        sc = jnp.broadcast_to(sc, (16, D))

        def do_mod(k):
            mod_cps[k].wait()
            v = _rb(_dot(sc, wmod_v[k]))[0:8]
            if k in (1, 4):
                v = _rb(1.0 + v)
            mod_v[k] = v

        do_mod(0)
        do_mod(1)
        x_head.wait()
        for b in range(4):
            xb = x_v[pl.ds(b * 16, 16), pl.ds(0, M), :].astype(F32).reshape(128, D)
            hb = _ln_mod(xb, mod_row(1), mod_row(0)).astype(BF16)
            for j in range(DB):
                hc[j, pl.ds(b * 64, 64), :] = _pk(hb[:, j * 128:(j + 1) * 128])

        s2 = stage.reshape(NCHUNK * D * GP, E)
        PPI = 4

        def pro_body(i, carry):
            ci = i // (GP // PPI)

            @pl.when(i % (GP // PPI) == 0)
            def _():
                pltpu.make_async_copy(stage.at[ci], stage.at[ci], sem_st.at[ci]).wait()

            for t in range(PPI):
                gp = i * PPI + t
                base = ci * (D * GP) + (gp % GP)
                b = s2[pl.ds(base, D, stride=GP), :]
                w1 = pltpu.bitcast(b << 16, F32).astype(BF16)
                w2 = pltpu.bitcast(b & jnp.uint32(0xFFFF0000), F32).astype(BF16)
                w_v[2 * gp] = _pk(w1)
                w_v[2 * gp + 1] = _pk(w2)
                hcv = jnp.concatenate([_bf(hc[j]) for j in range(DB)], axis=1)
                r1 = _dot(hcv, w1).reshape(NSEG, M, E)
                r2 = _dot(hcv, w2).reshape(NSEG, M, E)
                cache[gp] = _pk(jnp.concatenate([r1, r2], axis=1).reshape(NSEG * 2 * M, E))
            return carry

        lax.fori_loop(0, 3 * NPAIR // PPI, pro_body, 0)

        for k in range(2, 6):
            do_mod(k)

    pl.run_scoped(
        prologue,
        pltpu.VMEM((NCHUNK, D, GP, E), U32),
        pltpu.VMEM((6, D, D), BF16),
        pltpu.VMEM((DB, NSEG * M // 2, E), U32),
        pltpu.SemaphoreType.DMA((NCHUNK,)),
        pltpu.SemaphoreType.DMA((6,)),
    )

    x_tail.wait()
    for cp in wo_cps:
        cp.wait()

    def ln1_tail(seg):
        xt = x_v[seg, pl.ds(M, SEG - M), :].astype(F32)
        return _ln_mod(xt, mod_row(1), mod_row(0)).astype(BF16)

    lhs_v[pl.ds(0, M), :] = mem0_ref[...]
    lhs_v[pl.ds(M, SEG - M), :] = ln1_tail(0)

    def post(seg, r0, nr):
        rows = pl.ds(r0, nr)
        x = x_v[seg, rows, :].astype(F32)
        a = a_all[seg, rows, :].astype(F32)
        x1 = _rb(x + _rb(mod_row(2) * a))
        h2 = _ln_mod(x1, mod_row(4), mod_row(3))
        r = jnp.sum(h2 * wr_ref[...].astype(F32), axis=-1, keepdims=True)
        r_v[seg, rows, :] = _rb(r)
        x1_v[seg, rows, :] = x1.astype(BF16)
        o = x1 + _rb(mod_row(5) * h2)
        out_v[seg, rows, :] = o.astype(BF16)
        return o, r

    def deferred_lhs(grp):
        row0 = pl.multiple_of(grp * SEG, SEG)
        return jnp.concatenate([odef[h, pl.ds(row0, SEG), :] for h in range(H)], axis=1)

    def deferred(lhs, grp, j):
        res = _dot(lhs, _bf(wo_v[j])).astype(BF16).reshape(4, M, 128)
        col0 = j * 128
        if not isinstance(j, int):
            col0 = pl.multiple_of(col0, 128)
        a_all[pl.ds(grp * 4, 4), pl.ds(0, M), pl.ds(col0, 128)] = res

    def out_copy(seg):
        return pltpu.make_async_copy(out_v.at[seg], out_hbm.at[seg], sem_out)

    def fold(v):
        t = v[:, 0:128]
        for j in range(1, DB):
            t = t + v[:, j * 128:(j + 1) * 128]
        return t

    def main(wg_v, wu_v, wd_v, sem_moe):
        moe_cps = []
        wg_w, wu_w, wd_w = wg_hbm.bitcast(U32), wu_hbm.bitcast(U32), wd_hbm.bitcast(U32)
        for j in range(FB):
            moe_cps.append(pltpu.make_async_copy(wg_w.at[:, pl.ds(j * 128, 128)], wg_v.at[j], sem_moe.at[0]))
            moe_cps.append(pltpu.make_async_copy(wu_w.at[:, pl.ds(j * 128, 128)], wu_v.at[j], sem_moe.at[1]))
        for j in range(DB):
            moe_cps.append(pltpu.make_async_copy(wd_w.at[:, pl.ds(j * 128, 128)], wd_v.at[j], sem_moe.at[2]))
        for cp in moe_cps:
            cp.start()

        def step(s, carry):
            @pl.when(s > LAG)
            def _():
                out_copy(s - LAG - 1).start()

            lhs = lhs_v[...]
            pseg = jnp.maximum(s - LAG, 0)
            nseg = jnp.minimum(s + 1, NSEG - 1)
            grp = jnp.maximum(s // 4 - 1, 0)
            row0 = pl.multiple_of(s * M, M)

            def side(p):
                if p % 2 == 0 or p // 2 >= 7:
                    return None
                i = p // 2
                if i < 4:
                    o, r = post(pseg, i * 8, 8)
                    return fold(o) + r
                r0 = (i - 3) * 8
                xt = x_v[nseg, pl.ds(r0, 8), :].astype(F32)
                h = _ln_mod(xt, mod_row(1), mod_row(0))
                lhs_v[pl.ds(r0, 8), :] = h.astype(BF16)
                return fold(h)

            def proj(m_i, p):
                g = m_i * NPAIR + p
                return jnp.concatenate(
                    [_dot(lhs, _bf(w_v[2 * g])).astype(BF16), _dot(lhs, _bf(w_v[2 * g + 1])).astype(BF16),
                     _bf(cache[g, pl.ds(row0, M), :])], axis=0)

            def probs(p, q, k):
                sc = lax.dot_general(q, k, (((1,), (1,)), ((), ())), preferred_element_type=F32) * SCALE
                fm = fill_v[...]
                tok = side(p)
                if tok is not None:
                    top = fm[0:8]
                    fm = jnp.concatenate([jnp.where(top > 1.0, tok[:, 0:PR], top), fm[8:]], axis=0)
                sc = jnp.where(fm == 0.0, sc, fm)
                e = jnp.exp(sc - jnp.max(sc, axis=-1, keepdims=True))
                return (e * (1.0 / jnp.sum(e, axis=-1, keepdims=True))).astype(BF16)

            def attend(p, pr, v):
                o = _dot(pr, v)
                o_s[2 * p] = _pk(o[0:SEG])
                o_s[2 * p + 1] = _pk(o[SEG:2 * SEG])
                odef[2 * p, pl.ds(row0, M), :] = o[2 * SEG:2 * SEG + M].astype(BF16)
                odef[2 * p + 1, pl.ds(row0, M), :] = o[2 * SEG + M:].astype(BF16)

            dl = deferred_lhs(grp)
            qs, ks, vs, ps = {}, {}, {}, {}
            for p in range(NPAIR):
                qs[p] = proj(0, p)
                if p >= 1:
                    ps[p - 1] = probs(p - 1, qs.pop(p - 1), ks.pop(p - 1))
                ks[p] = proj(1, p)
                if p >= 2:
                    attend(p - 2, ps.pop(p - 2), vs.pop(p - 2))
                vs[p] = proj(2, p)
            L = NPAIR - 1
            deferred(dl, grp, (s % 4) * 2)
            ps[L] = probs(L, qs.pop(L), ks.pop(L))
            attend(L - 1, ps.pop(L - 1), vs.pop(L - 1))
            deferred(dl, grp, (s % 4) * 2 + 1)

            KC = 2
            HC = H // KC
            acc = [None] * DB
            for kc in range(KC):
                ol = jnp.concatenate([_bf(o_s[kc * HC + h]) for h in range(HC)], axis=1)
                for j in range(DB):
                    part = _dot(ol, _bf(wo_v[j, pl.ds(kc * HC * E // 2, HC * E // 2), :]))
                    acc[j] = part if kc == 0 else acc[j] + part
                    if kc == 0 and j == 2:
                        attend(L, ps.pop(L), vs.pop(L))
            a = jnp.concatenate(acc, axis=1)
            lhs_v[pl.ds(0, M), :] = a[0:M].astype(BF16)
            a_all[s, pl.ds(M, SEG - M), :] = a[M:].astype(BF16)
            return carry

        lax.fori_loop(0, NSEG, step, 0)

        out_copy(NSEG - LAG - 1).start()
        dl = deferred_lhs(NSEG // 4 - 1)
        for j in range(DB):
            deferred(dl, NSEG // 4 - 1, j)
        for seg in range(NSEG - LAG, NSEG):
            post(seg, 0, SEG)
            out_copy(seg).start()

        r = r_v[...].reshape(S, 1)
        idx = lax.broadcasted_iota(jnp.int32, (S, 1), 0)
        m1 = jnp.max(r, axis=0, keepdims=True)
        i1v = jnp.min(jnp.where(r == m1, idx, S - 1), axis=0, keepdims=True)
        r2 = jnp.where(idx == i1v, -jnp.inf, r)
        m2 = jnp.max(r2, axis=0, keepdims=True)
        i2v = jnp.min(jnp.where((r2 == m2) & (idx != i1v), idx, S - 1), axis=0, keepdims=True)
        i1 = i1v[0, 0]
        i2 = i2v[0, 0]

        def tile_of(i):
            return i >> 5, pl.multiple_of(((i >> 3) & 3) * 8, 8)

        sel = [tile_of(i1), tile_of(i2)]
        x1s = jnp.concatenate([x1_v[sg, pl.ds(r0, 8), :].astype(F32) for sg, r0 in sel], axis=0)
        h2s = _ln_mod(x1s, mod_row(4), mod_row(3))
        h2b = h2s.astype(BF16)
        for k, buf in enumerate((wg_v, wu_v, wd_v)):
            pltpu.make_async_copy(buf, buf, sem_moe.at[k]).wait()
        gus = []
        for j in range(FB):
            g = _rb(_dot(h2b, _bf(wg_v[j])))
            g = _rb(g * jax.nn.sigmoid(g))
            u = _rb(_dot(h2b, _bf(wu_v[j])))
            gus.append((g * u).astype(BF16))
        gu = jnp.concatenate(gus, axis=1)
        y = jnp.concatenate([_rb(_dot(gu, _bf(wd_v[j]))) for j in range(DB)], axis=1)
        rows = lax.broadcasted_iota(jnp.int32, (16, 1), 0)
        rs = _rb(jax.nn.sigmoid(jnp.where(rows < 8, m1, m2)))
        y = _rb(y * rs)
        full = (x1s + _rb(mod_row(5) * _rb(h2s + y)))

        pltpu.make_async_copy(out_v, out_v, sem_out).wait()
        r8 = lax.broadcasted_iota(jnp.int32, (8, 1), 0)
        for t, (i, (sg, r0)) in enumerate(zip((i1, i2), sel)):
            old = out_v[sg, pl.ds(r0, 8), :].astype(F32)
            new = jnp.where(r8 == (i & 7), full[t * 8:(t + 1) * 8], old)
            out_v[sg, pl.ds(r0, 8), :] = new.astype(BF16)
        for sg, r0 in sel:
            cp = pltpu.make_async_copy(out_v.at[sg, pl.ds(r0, 8), :], out_hbm.at[sg, pl.ds(r0, 8), :], sem_out)
            cp.start()
            cp.wait()

    pl.run_scoped(
        main,
        pltpu.VMEM((FB, D // 2, 128), U32),
        pltpu.VMEM((FB, D // 2, 128), U32),
        pltpu.VMEM((DB, F // 2, 128), U32),
        pltpu.SemaphoreType.DMA((3,)),
    )


@jax.jit
def pallas_adaLN_cond__memory_aug_recurrent_mem_tr__moe_arch_mod__prompt_kernel(
    A_x: jax.Array,
    A_mem0: jax.Array,
    A_Wq: jax.Array,
    A_Wk: jax.Array,
    A_Wv: jax.Array,
    A_Wo: jax.Array,
    A_seg_len: jax.Array,
    B_x: jax.Array,
    B_w_r: jax.Array,
    B_w_gate: jax.Array,
    B_w_up: jax.Array,
    B_w_down: jax.Array,
    c: jax.Array,
    w_mod: jax.Array,
):
    del A_seg_len, B_x
    assert A_x.shape == (1, S, D) and A_mem0.shape == (1, M, D) and A_Wq.shape == (D, H, E)
    hbm = pl.BlockSpec(memory_space=pl.ANY)
    vmem = pl.BlockSpec(memory_space=pltpu.VMEM)
    out = pl.pallas_call(
        _kernel,
        out_shape=jax.ShapeDtypeStruct((NSEG, SEG, D), BF16),
        in_specs=[hbm, vmem, hbm, hbm, hbm, hbm, vmem, hbm, hbm, hbm, vmem, hbm],
        out_specs=hbm,
        scratch_shapes=[
            pltpu.VMEM((NSEG, SEG, D), BF16),
            pltpu.VMEM((3 * H, D // 2, E), U32),
            pltpu.VMEM((DB, H * E // 2, 128), U32),
            pltpu.VMEM((3 * NPAIR, NSEG * M, E), U32),
            pltpu.VMEM((H, NSEG * M, E), BF16),
            pltpu.VMEM((SEG, D), BF16),
            pltpu.VMEM((H, SEG // 2, E), U32),
            pltpu.VMEM((NSEG, SEG, D), BF16),
            pltpu.VMEM((NSEG, SEG, D), BF16),
            pltpu.VMEM((NSEG, SEG, D), BF16),
            pltpu.VMEM((NSEG, SEG, 1), F32),
            pltpu.VMEM((6, 8, D), F32),
            pltpu.VMEM((PR, PR), F32),
            pltpu.SemaphoreType.DMA((2,)),
            pltpu.SemaphoreType.DMA((DB,)),
            pltpu.SemaphoreType.DMA,
        ],
        compiler_params=pltpu.CompilerParams(vmem_limit_bytes=120 * 1024 * 1024),
    )(
        A_x.reshape(NSEG, SEG, D),
        A_mem0.reshape(M, D),
        A_Wq, A_Wk, A_Wv,
        A_Wo.reshape(H * E, D),
        B_w_r.reshape(1, D),
        B_w_gate, B_w_up, B_w_down,
        c, w_mod,
    )
    return out.reshape(1, S, D)
```

```python
import jax
import jax.numpy as jnp
from jax import lax
import jax.experimental.pallas as pl
import jax.experimental.pallas.tpu as pltpu

BF16 = jnp.bfloat16
F32 = jnp.float32
U32 = jnp.uint32

S = 2048
D = 1024
H = 32
E = 128
M = 8
SEG = 32
NSEG = S // SEG
NPAIR = H // 2
F = 3584
DB = D // 128
FB = F // 128
GP = 8
NCHUNK = 3 * NPAIR // GP
PR = 2 * SEG + 2 * M
LAG = 8
SEM_X = 0
SEM_WO = SEM_X + 2
SEM_MOD = SEM_WO + DB
SEM_ST = SEM_MOD + 6
SEM_MOE = SEM_ST + NCHUNK
SEM_OUT = SEM_MOE + 3
NSEM = SEM_OUT + 1
EPS = 1e-5
SCALE = E ** (-0.5)


def _rb(v):
    return v.astype(BF16).astype(F32)


def _dot(a, b):
    return jnp.dot(a, b, preferred_element_type=F32)


def _recip(x):
    r = pl.reciprocal(x, approx=True)
    return r * (2.0 - x * r)


def _bf(words):
    return pltpu.bitcast(words, BF16)


def _pk(v):
    return pltpu.bitcast(v.astype(BF16), U32)


def _ln_mod(x, scale1p, shift):
    m = jnp.mean(x, axis=-1, keepdims=True)
    xc = x - m
    var = jnp.mean(xc * xc, axis=-1, keepdims=True)
    sd = _rb(jnp.sqrt(_rb(_rb(var) + EPS)))
    n = _rb(_rb(x - _rb(m)) * (1.0 / sd))
    return _rb(_rb(n * scale1p) + shift)


def _fill_matrix():
    i = lax.broadcasted_iota(jnp.int32, (PR, PR), 0)
    j = lax.broadcasted_iota(jnp.int32, (PR, PR), 1)

    def head(t):
        return jnp.where(t < 2 * SEG, t >> 5, (t - 2 * SEG) >> 3)

    def pos(t):
        r = t & (SEG - 1)
        return jnp.where(t < 2 * SEG, jnp.where(r < M, r, r + M), M + (t & (M - 1)))

    same = head(i) == head(j)
    pi = pos(i)
    ok = jnp.where(pi < M, 1, jnp.where(pi >= pos(j), 1, 0))
    return jnp.where(same, jnp.where(ok == 1, 0.0, -1e9), -3e38).astype(F32)


def _kernel(x_hbm, mem0_ref, wq_hbm, wk_hbm, wv_hbm, wo_hbm, wr_ref, wg_hbm, wu_hbm, wd_hbm,
            c_ref, wmod_hbm, out_hbm,
            x_v, w_v, wo_v, cache, odef, lhs_v, o_s, a_all, x1_v, out_v, r_v, mod_v, fill_v,
            sems):

    x_head = pltpu.make_async_copy(x_hbm.at[:, pl.ds(0, M), :], x_v.at[:, pl.ds(0, M), :], sems.at[SEM_X])
    x_tail = pltpu.make_async_copy(x_hbm.at[:, pl.ds(M, SEG - M), :], x_v.at[:, pl.ds(M, SEG - M), :],
                                   sems.at[SEM_X + 1])
    wo_w = wo_hbm.bitcast(U32)
    wo_cps = [pltpu.make_async_copy(wo_w.at[:, pl.ds(j * 128, 128)], wo_v.at[j], sems.at[SEM_WO + j])
              for j in range(DB)]

    def mod_row(k):
        return mod_v[k, 0:1, :]

    def prologue(stage, wmod_v, hc):
        mod_cps = [pltpu.make_async_copy(wmod_hbm.at[:, pl.ds(k * D, D)], wmod_v.at[k], sems.at[SEM_MOD + k])
                   for k in range(6)]
        st_cps = []
        for m_i, w_hbm in enumerate((wq_hbm, wk_hbm, wv_hbm)):
            wb = w_hbm.bitcast(U32)
            for g in range(NPAIR // GP):
                ci = m_i * (NPAIR // GP) + g
                st_cps.append(pltpu.make_async_copy(wb.at[:, pl.ds(g * GP, GP), :], stage.at[ci],
                                                    sems.at[SEM_ST + ci]))
        x_head.start()
        mod_cps[0].start()
        mod_cps[1].start()
        for cp in st_cps:
            cp.start()
        x_tail.start()
        for cp in wo_cps:
            cp.start()
        for cp in mod_cps[2:]:
            cp.start()

        fill_v[...] = _fill_matrix()
        odef[:, pl.ds(0, SEG), :] = jnp.zeros((H, SEG, E), BF16)
        a_all[0] = jnp.zeros((SEG, D), BF16)

        c = c_ref[...].astype(F32)
        sc = (c * jax.nn.sigmoid(c)).astype(BF16)
        sc = jnp.broadcast_to(sc, (16, D))

        def do_mod(k):
            mod_cps[k].wait()
            v = _rb(_dot(sc, wmod_v[k]))[0:8]
            if k in (1, 4):
                v = _rb(1.0 + v)
            mod_v[k] = v

        do_mod(0)
        do_mod(1)
        x_head.wait()
        for b in range(4):
            xb = x_v[pl.ds(b * 16, 16), pl.ds(0, M), :].astype(F32).reshape(128, D)
            hb = _ln_mod(xb, mod_row(1), mod_row(0)).astype(BF16)
            for j in range(DB):
                hc[j, pl.ds(b * 64, 64), :] = _pk(hb[:, j * 128:(j + 1) * 128])

        s2 = stage.reshape(NCHUNK * D * GP, E)
        PPI = 4

        def pro_body(i, carry):
            ci = i // (GP // PPI)

            @pl.when(i % (GP // PPI) == 0)
            def _():
                pltpu.make_async_copy(stage.at[ci], stage.at[ci], sems.at[SEM_ST + ci]).wait()

            for t in range(PPI):
                gp = i * PPI + t
                base = ci * (D * GP) + (gp % GP)
                b = s2[pl.ds(base, D, stride=GP), :]
                w1 = pltpu.bitcast(b << 16, F32).astype(BF16)
                w2 = pltpu.bitcast(b & jnp.uint32(0xFFFF0000), F32).astype(BF16)
                w_v[2 * gp] = _pk(w1)
                w_v[2 * gp + 1] = _pk(w2)
                hcv = jnp.concatenate([_bf(hc[j]) for j in range(DB)], axis=1)
                r1 = _dot(hcv, w1).reshape(NSEG, M, E)
                r2 = _dot(hcv, w2).reshape(NSEG, M, E)
                cache[gp] = _pk(jnp.concatenate([r1, r2], axis=1).reshape(NSEG * 2 * M, E))
            return carry

        lax.fori_loop(0, 3 * NPAIR // PPI, pro_body, 0)

        for k in range(2, 6):
            do_mod(k)

    pl.run_scoped(
        prologue,
        pltpu.VMEM((NCHUNK, D, GP, E), U32),
        pltpu.VMEM((6, D, D), BF16),
        pltpu.VMEM((DB, NSEG * M // 2, E), U32),
    )

    x_tail.wait()
    for cp in wo_cps:
        cp.wait()

    def ln1_tail(seg):
        xt = x_v[seg, pl.ds(M, SEG - M), :].astype(F32)
        return _ln_mod(xt, mod_row(1), mod_row(0)).astype(BF16)

    lhs_v[pl.ds(0, M), :] = mem0_ref[...]
    lhs_v[pl.ds(M, SEG - M), :] = ln1_tail(0)

    def post(seg, r0, nr):
        rows = pl.ds(r0, nr)
        x = x_v[seg, rows, :].astype(F32)
        a = a_all[seg, rows, :].astype(F32)
        x1 = _rb(x + _rb(mod_row(2) * a))
        h2 = _ln_mod(x1, mod_row(4), mod_row(3))
        r = jnp.sum(h2 * wr_ref[...].astype(F32), axis=-1, keepdims=True)
        r_v[seg, rows, :] = _rb(r)
        x1_v[seg, rows, :] = x1.astype(BF16)
        o = x1 + _rb(mod_row(5) * h2)
        out_v[seg, rows, :] = o.astype(BF16)
        return o, r

    def deferred_lhs(grp):
        row0 = pl.multiple_of(grp * SEG, SEG)
        return jnp.concatenate([odef[h, pl.ds(row0, SEG), :] for h in range(H)], axis=1)

    def deferred(lhs, grp, j):
        res = _dot(lhs, _bf(wo_v[j])).astype(BF16).reshape(4, M, 128)
        col0 = j * 128
        if not isinstance(j, int):
            col0 = pl.multiple_of(col0, 128)
        a_all[pl.ds(grp * 4, 4), pl.ds(0, M), pl.ds(col0, 128)] = res

    def out_copy(seg):
        return pltpu.make_async_copy(out_v.at[seg], out_hbm.at[seg], sems.at[SEM_OUT])

    def fold(v):
        t = v[:, 0:128]
        for j in range(1, DB):
            t = t + v[:, j * 128:(j + 1) * 128]
        return t

    def main(wg_v, wu_v, wd_v):
        moe_cps = []
        wg_w, wu_w, wd_w = wg_hbm.bitcast(U32), wu_hbm.bitcast(U32), wd_hbm.bitcast(U32)
        for j in range(FB):
            moe_cps.append(pltpu.make_async_copy(wg_w.at[:, pl.ds(j * 128, 128)], wg_v.at[j], sems.at[SEM_MOE]))
            moe_cps.append(pltpu.make_async_copy(wu_w.at[:, pl.ds(j * 128, 128)], wu_v.at[j], sems.at[SEM_MOE + 1]))
        for j in range(DB):
            moe_cps.append(pltpu.make_async_copy(wd_w.at[:, pl.ds(j * 128, 128)], wd_v.at[j], sems.at[SEM_MOE + 2]))
        for cp in moe_cps:
            cp.start()

        def step(s, carry):
            @pl.when(s > LAG)
            def _():
                out_copy(s - LAG - 1).start()

            lhs = lhs_v[...]
            pseg = jnp.maximum(s - LAG, 0)
            nseg = jnp.minimum(s + 1, NSEG - 1)
            grp = jnp.maximum(s // 4 - 1, 0)
            row0 = pl.multiple_of(s * M, M)

            def side(p):
                if p % 2 == 0 or p // 2 >= 7:
                    return None
                i = p // 2
                if i < 4:
                    o, r = post(pseg, i * 8, 8)
                    return fold(o) + r
                r0 = (i - 3) * 8
                xt = x_v[nseg, pl.ds(r0, 8), :].astype(F32)
                h = _ln_mod(xt, mod_row(1), mod_row(0))
                lhs_v[pl.ds(r0, 8), :] = h.astype(BF16)
                return fold(h)

            def proj(m_i, p):
                g = m_i * NPAIR + p
                return jnp.concatenate(
                    [_dot(lhs, _bf(w_v[2 * g])).astype(BF16), _dot(lhs, _bf(w_v[2 * g + 1])).astype(BF16),
                     _bf(cache[g, pl.ds(row0, M), :])], axis=0)

            def probs(p, q, k):
                sc = lax.dot_general(q, k, (((1,), (1,)), ((), ())), preferred_element_type=F32) * SCALE
                fm = fill_v[...]
                tok = side(p)
                if tok is not None:
                    top = fm[0:8]
                    fm = jnp.concatenate([jnp.where(top > 1.0, tok[:, 0:PR], top), fm[8:]], axis=0)
                sc = jnp.where(fm == 0.0, sc, fm)
                e = jnp.exp(sc - jnp.max(sc, axis=-1, keepdims=True))
                return e.astype(BF16), _recip(jnp.sum(e, axis=-1, keepdims=True))

            def attend(p, pr, v):
                o = _dot(pr[0], v) * pr[1]
                o_s[2 * p] = _pk(o[0:SEG])
                o_s[2 * p + 1] = _pk(o[SEG:2 * SEG])
                odef[2 * p, pl.ds(row0, M), :] = o[2 * SEG:2 * SEG + M].astype(BF16)
                odef[2 * p + 1, pl.ds(row0, M), :] = o[2 * SEG + M:].astype(BF16)

            for t in range(2):
                deferred(deferred_lhs(grp), grp, (s % 4) * 2 + t)
            qs, ks, vs, ps = {}, {}, {}, {}
            PL = 3
            for p in range(NPAIR):
                qs[p] = proj(0, p)
                if p >= 1:
                    ps[p - 1] = probs(p - 1, qs.pop(p - 1), ks.pop(p - 1))
                ks[p] = proj(1, p)
                if p >= PL:
                    attend(p - PL, ps.pop(p - PL), vs.pop(p - PL))
                vs[p] = proj(2, p)
            L = NPAIR - 1

            HA = 24
            acc = [None] * DB
            for h0, h1 in ((0, HA), (HA, H)):
                ol = jnp.concatenate([_bf(o_s[h]) for h in range(h0, h1)], axis=1)
                for j in range(DB):
                    part = _dot(ol, _bf(wo_v[j, pl.ds(h0 * E // 2, (h1 - h0) * E // 2), :]))
                    acc[j] = part if h0 == 0 else part + acc[j]
                    if h0 == 0 and j == 0:
                        ps[L] = probs(L, qs.pop(L), ks.pop(L))
                        attend(L - 2, ps.pop(L - 2), vs.pop(L - 2))
                    if h0 == 0 and j == 2:
                        attend(L - 1, ps.pop(L - 1), vs.pop(L - 1))
                    if h0 == 0 and j == 5:
                        attend(L, ps.pop(L), vs.pop(L))
            a = jnp.concatenate(acc, axis=1)
            lhs_v[pl.ds(0, M), :] = a[0:M].astype(BF16)
            a_all[s, pl.ds(M, SEG - M), :] = a[M:].astype(BF16)
            return carry

        lax.fori_loop(0, NSEG, step, 0)

        out_copy(NSEG - LAG - 1).start()
        dl = deferred_lhs(NSEG // 4 - 1)
        for j in range(DB):
            deferred(dl, NSEG // 4 - 1, j)
        for seg in range(NSEG - LAG, NSEG):
            post(seg, 0, SEG)
            out_copy(seg).start()

        r = r_v[...].reshape(S, 1)
        idx = lax.broadcasted_iota(jnp.int32, (S, 1), 0)
        m1 = jnp.max(r, axis=0, keepdims=True)
        i1v = jnp.min(jnp.where(r == m1, idx, S - 1), axis=0, keepdims=True)
        r2 = jnp.where(idx == i1v, -jnp.inf, r)
        m2 = jnp.max(r2, axis=0, keepdims=True)
        i2v = jnp.min(jnp.where((r2 == m2) & (idx != i1v), idx, S - 1), axis=0, keepdims=True)
        i1 = i1v[0, 0]
        i2 = i2v[0, 0]

        def tile_of(i):
            return i >> 5, pl.multiple_of(((i >> 3) & 3) * 8, 8)

        sel = [tile_of(i1), tile_of(i2)]
        x1s = jnp.concatenate([x1_v[sg, pl.ds(r0, 8), :].astype(F32) for sg, r0 in sel], axis=0)
        h2s = _ln_mod(x1s, mod_row(4), mod_row(3))
        h2b = h2s.astype(BF16)
        for k, buf in enumerate((wg_v, wu_v, wd_v)):
            pltpu.make_async_copy(buf, buf, sems.at[SEM_MOE + k]).wait()
        gus = []
        for j in range(FB):
            g = _rb(_dot(h2b, _bf(wg_v[j])))
            g = _rb(g * jax.nn.sigmoid(g))
            u = _rb(_dot(h2b, _bf(wu_v[j])))
            gus.append((g * u).astype(BF16))
        gu = jnp.concatenate(gus, axis=1)
        y = jnp.concatenate([_rb(_dot(gu, _bf(wd_v[j]))) for j in range(DB)], axis=1)
        rows = lax.broadcasted_iota(jnp.int32, (16, 1), 0)
        rs = _rb(jax.nn.sigmoid(jnp.where(rows < 8, m1, m2)))
        y = _rb(y * rs)
        full = (x1s + _rb(mod_row(5) * _rb(h2s + y)))

        pltpu.make_async_copy(out_v, out_v, sems.at[SEM_OUT]).wait()
        r8 = lax.broadcasted_iota(jnp.int32, (8, 1), 0)
        for t, (i, (sg, r0)) in enumerate(zip((i1, i2), sel)):
            old = out_v[sg, pl.ds(r0, 8), :].astype(F32)
            new = jnp.where(r8 == (i & 7), full[t * 8:(t + 1) * 8], old)
            out_v[sg, pl.ds(r0, 8), :] = new.astype(BF16)
        for sg, r0 in sel:
            cp = pltpu.make_async_copy(out_v.at[sg, pl.ds(r0, 8), :], out_hbm.at[sg, pl.ds(r0, 8), :], sems.at[SEM_OUT])
            cp.start()
            cp.wait()

    pl.run_scoped(
        main,
        pltpu.VMEM((FB, D // 2, 128), U32),
        pltpu.VMEM((FB, D // 2, 128), U32),
        pltpu.VMEM((DB, F // 2, 128), U32),
    )


@jax.jit
def pallas_adaLN_cond__memory_aug_recurrent_mem_tr__moe_arch_mod__prompt_kernel(
    A_x: jax.Array,
    A_mem0: jax.Array,
    A_Wq: jax.Array,
    A_Wk: jax.Array,
    A_Wv: jax.Array,
    A_Wo: jax.Array,
    A_seg_len: jax.Array,
    B_x: jax.Array,
    B_w_r: jax.Array,
    B_w_gate: jax.Array,
    B_w_up: jax.Array,
    B_w_down: jax.Array,
    c: jax.Array,
    w_mod: jax.Array,
):
    del A_seg_len, B_x
    assert A_x.shape == (1, S, D) and A_mem0.shape == (1, M, D) and A_Wq.shape == (D, H, E)
    hbm = pl.BlockSpec(memory_space=pl.ANY)
    vmem = pl.BlockSpec(memory_space=pltpu.VMEM)
    out = pl.pallas_call(
        _kernel,
        out_shape=jax.ShapeDtypeStruct((NSEG, SEG, D), BF16),
        in_specs=[hbm, vmem, hbm, hbm, hbm, hbm, vmem, hbm, hbm, hbm, vmem, hbm],
        out_specs=hbm,
        scratch_shapes=[
            pltpu.VMEM((NSEG, SEG, D), BF16),
            pltpu.VMEM((3 * H, D // 2, E), U32),
            pltpu.VMEM((DB, H * E // 2, 128), U32),
            pltpu.VMEM((3 * NPAIR, NSEG * M, E), U32),
            pltpu.VMEM((H, NSEG * M, E), BF16),
            pltpu.VMEM((SEG, D), BF16),
            pltpu.VMEM((H, SEG // 2, E), U32),
            pltpu.VMEM((NSEG, SEG, D), BF16),
            pltpu.VMEM((NSEG, SEG, D), BF16),
            pltpu.VMEM((NSEG, SEG, D), BF16),
            pltpu.VMEM((NSEG, SEG, 1), F32),
            pltpu.VMEM((6, 8, D), F32),
            pltpu.VMEM((PR, PR), F32),
            pltpu.SemaphoreType.DMA((NSEM,)),
        ],
        compiler_params=pltpu.CompilerParams(vmem_limit_bytes=120 * 1024 * 1024),
    )(
        A_x.reshape(NSEG, SEG, D),
        A_mem0.reshape(M, D),
        A_Wq, A_Wk, A_Wv,
        A_Wo.reshape(H * E, D),
        B_w_r.reshape(1, D),
        B_w_gate, B_w_up, B_w_down,
        c, w_mod,
    )
    return out.reshape(1, S, D)
```

```python
import jax
import jax.numpy as jnp
from jax import lax
import jax.experimental.pallas as pl
import jax.experimental.pallas.tpu as pltpu

BF16 = jnp.bfloat16
F32 = jnp.float32
U32 = jnp.uint32

S = 2048
D = 1024
H = 32
E = 128
M = 8
SEG = 32
NSEG = S // SEG
NPAIR = H // 2
F = 3584
DB = D // 128
FB = F // 128
GP = 8
NCHUNK = 3 * NPAIR // GP
PR = 2 * SEG + 2 * M
LAG = 8
SEM_X = 0
SEM_WO = SEM_X + 2
SEM_MOD = SEM_WO + DB
SEM_ST = SEM_MOD + 6
SEM_MOE = SEM_ST + NCHUNK
SEM_OUT = SEM_MOE + 3
NSEM = SEM_OUT + 1
EPS = 1e-5
SCALE = E ** (-0.5)


def _rb(v):
    return v.astype(BF16).astype(F32)


def _dot(a, b):
    return jnp.dot(a, b, preferred_element_type=F32)


def _recip(x):
    r = pl.reciprocal(x, approx=True)
    return r * (2.0 - x * r)


def _bf(words):
    return pltpu.bitcast(words, BF16)


def _pk(v):
    return pltpu.bitcast(v.astype(BF16), U32)


def _ln_mod(x, scale1p, shift):
    m = jnp.mean(x, axis=-1, keepdims=True)
    xc = x - m
    var = jnp.mean(xc * xc, axis=-1, keepdims=True)
    sd = _rb(jnp.sqrt(_rb(_rb(var) + EPS)))
    n = _rb(_rb(x - _rb(m)) * (1.0 / sd))
    return _rb(_rb(n * scale1p) + shift)


def _fill_matrix():
    i = lax.broadcasted_iota(jnp.int32, (PR, PR), 0)
    j = lax.broadcasted_iota(jnp.int32, (PR, PR), 1)

    def head(t):
        return jnp.where(t < 2 * SEG, t >> 5, (t - 2 * SEG) >> 3)

    def pos(t):
        r = t & (SEG - 1)
        return jnp.where(t < 2 * SEG, jnp.where(r < M, r, r + M), M + (t & (M - 1)))

    same = head(i) == head(j)
    pi = pos(i)
    ok = jnp.where(pi < M, 1, jnp.where(pi >= pos(j), 1, 0))
    return jnp.where(same, jnp.where(ok == 1, 0.0, -1e9), -3e38).astype(F32)


def _kernel(x_hbm, mem0_ref, wq_hbm, wk_hbm, wv_hbm, wo_hbm, wr_ref, wg_hbm, wu_hbm, wd_hbm,
            c_ref, wmod_hbm, out_hbm,
            x_v, w_v, wo_v, cache, odef, lhs_v, nxt_v, qkv_s, o_s, a_all, x1_v, out_v, r_v, mod_v, fill_v,
            sems):

    x_head = pltpu.make_async_copy(x_hbm.at[:, pl.ds(0, M), :], x_v.at[:, pl.ds(0, M), :], sems.at[SEM_X])
    x_tail = pltpu.make_async_copy(x_hbm.at[:, pl.ds(M, SEG - M), :], x_v.at[:, pl.ds(M, SEG - M), :],
                                   sems.at[SEM_X + 1])
    wo_w = wo_hbm.bitcast(U32)
    wo_cps = [pltpu.make_async_copy(wo_w.at[:, pl.ds(j * 128, 128)], wo_v.at[j], sems.at[SEM_WO + j])
              for j in range(DB)]

    def mod_row(k, rows=8):
        v = mod_v[k]
        return v if rows == 8 else jnp.concatenate([v] * (rows // 8), axis=0)

    w_w = w_v.bitcast(U32)
    cache_w = cache.bitcast(U32)
    lhs_w = lhs_v.bitcast(U32)
    qkv_w = qkv_s.bitcast(U32)
    o_w = o_s.bitcast(U32)
    odef_w = odef.bitcast(U32)

    def prologue(stage, wmod_v, hc):
        mod_cps = [pltpu.make_async_copy(wmod_hbm.at[:, pl.ds(k * D, D)], wmod_v.at[k], sems.at[SEM_MOD + k])
                   for k in range(6)]
        st_cps = []
        for m_i, w_hbm in enumerate((wq_hbm, wk_hbm, wv_hbm)):
            wb = w_hbm.bitcast(U32)
            for g in range(NPAIR // GP):
                ci = m_i * (NPAIR // GP) + g
                st_cps.append(pltpu.make_async_copy(wb.at[:, pl.ds(g * GP, GP), :], stage.at[ci],
                                                    sems.at[SEM_ST + ci]))
        x_head.start()
        mod_cps[0].start()
        mod_cps[1].start()
        for cp in st_cps:
            cp.start()
        x_tail.start()
        for cp in wo_cps:
            cp.start()
        for cp in mod_cps[2:]:
            cp.start()

        fill_v[...] = _fill_matrix()
        odef[:, pl.ds(0, SEG), :] = jnp.zeros((H, SEG, E), BF16)
        a_all[0] = jnp.zeros((SEG, D), BF16)

        c = c_ref[...].astype(F32)
        sc = (c * jax.nn.sigmoid(c)).astype(BF16)
        sc = jnp.broadcast_to(sc, (16, D))

        def do_mod(k):
            mod_cps[k].wait()
            v = _rb(_dot(sc, wmod_v[k]))[0:8]
            if k in (1, 4):
                v = _rb(1.0 + v)
            mod_v[k] = v

        do_mod(0)
        do_mod(1)
        x_head.wait()
        for b in range(4):
            xb = x_v[pl.ds(b * 16, 16), pl.ds(0, M), :].astype(F32).reshape(128, D)
            hb = _ln_mod(xb, mod_row(1, 128), mod_row(0, 128)).astype(BF16)
            for j in range(DB):
                hc[j, pl.ds(b * 128, 128), :] = hb[:, j * 128:(j + 1) * 128]

        hc_w = hc.bitcast(U32)
        s2 = stage.reshape(NCHUNK * D * GP, E)
        PPI = 4

        def pro_body(i, carry):
            ci = i // (GP // PPI)

            @pl.when(i % (GP // PPI) == 0)
            def _():
                pltpu.make_async_copy(stage.at[ci], stage.at[ci], sems.at[SEM_ST + ci]).wait()

            for t in range(PPI):
                gp = i * PPI + t
                base = ci * (D * GP) + (gp % GP)
                b = s2[pl.ds(base, D, stride=GP), :]
                w_v[2 * gp] = pltpu.bitcast(b << 16, F32).astype(BF16)
                w_v[2 * gp + 1] = pltpu.bitcast(b & jnp.uint32(0xFFFF0000), F32).astype(BF16)
                hcv = jnp.concatenate([_bf(hc_w[j]) for j in range(DB)], axis=1)
                r1 = _dot(hcv, _bf(w_w[2 * gp])).reshape(NSEG, M, E)
                r2 = _dot(hcv, _bf(w_w[2 * gp + 1])).reshape(NSEG, M, E)
                cache[gp] = jnp.concatenate([r1, r2], axis=1).reshape(NSEG * 2 * M, E).astype(BF16)
            return carry

        lax.fori_loop(0, 3 * NPAIR // PPI, pro_body, 0)

        for k in range(2, 6):
            do_mod(k)
        mod_v[6] = jnp.broadcast_to(wr_ref[...].astype(F32), (8, D))

    pl.run_scoped(
        prologue,
        pltpu.VMEM((NCHUNK, D, GP, E), U32),
        pltpu.VMEM((6, D, D), BF16),
        pltpu.VMEM((DB, NSEG * M, E), BF16),
    )

    x_tail.wait()
    for cp in wo_cps:
        cp.wait()

    def put_rows(dst, r0, v):
        for j in range(DB):
            dst[j, pl.ds(r0, 8), :] = v[:, j * 128:(j + 1) * 128].astype(BF16)

    def ln1(seg, r0):
        xt = x_v[seg, pl.ds(r0, 8), :].astype(F32)
        return _ln_mod(xt, mod_row(1), mod_row(0))

    put_rows(lhs_v, 0, mem0_ref[...].astype(F32))
    for r0 in range(M, SEG, 8):
        put_rows(lhs_v, r0, ln1(0, r0))

    def post(seg, r0, nr):
        rows = pl.ds(r0, nr)
        x = x_v[seg, rows, :].astype(F32)
        a = a_all[seg, rows, :].astype(F32)
        x1 = _rb(x + _rb(mod_row(2, nr) * a))
        h2 = _ln_mod(x1, mod_row(4, nr), mod_row(3, nr))
        r = jnp.sum(h2 * mod_row(6, nr), axis=-1, keepdims=True)
        r_v[seg, rows, :] = _rb(r)
        x1_v[seg, rows, :] = x1.astype(BF16)
        o = x1 + _rb(mod_row(5, nr) * h2)
        out_v[seg, rows, :] = o.astype(BF16)
        return o, r

    def deferred_lhs(grp):
        row0 = pl.multiple_of(grp * (SEG // 2), SEG // 2)
        return jnp.concatenate([_bf(odef_w[h, pl.ds(row0, SEG // 2), :]) for h in range(H)], axis=1)

    def deferred(lhs, grp, j):
        res = _dot(lhs, _bf(wo_v[j])).astype(BF16).reshape(4, M, 128)
        col0 = j * 128
        if not isinstance(j, int):
            col0 = pl.multiple_of(col0, 128)
        a_all[pl.ds(grp * 4, 4), pl.ds(0, M), pl.ds(col0, 128)] = res

    def out_copy(seg):
        return pltpu.make_async_copy(out_v.at[seg], out_hbm.at[seg], sems.at[SEM_OUT])

    def fold(v):
        t = v[:, 0:128]
        for j in range(1, DB):
            t = t + v[:, j * 128:(j + 1) * 128]
        return t

    def main(wg_v, wu_v, wd_v):
        moe_cps = []
        wg_w, wu_w, wd_w = wg_hbm.bitcast(U32), wu_hbm.bitcast(U32), wd_hbm.bitcast(U32)
        for j in range(FB):
            moe_cps.append(pltpu.make_async_copy(wg_w.at[:, pl.ds(j * 128, 128)], wg_v.at[j], sems.at[SEM_MOE]))
            moe_cps.append(pltpu.make_async_copy(wu_w.at[:, pl.ds(j * 128, 128)], wu_v.at[j], sems.at[SEM_MOE + 1]))
        for j in range(DB):
            moe_cps.append(pltpu.make_async_copy(wd_w.at[:, pl.ds(j * 128, 128)], wd_v.at[j], sems.at[SEM_MOE + 2]))
        for cp in moe_cps:
            cp.start()

        def step(s, carry):
            @pl.when(s > LAG)
            def _():
                out_copy(s - LAG - 1).start()

            lhs = jnp.concatenate([_bf(lhs_w[j]) for j in range(DB)], axis=1)
            pseg = jnp.maximum(s - LAG, 0)
            nseg = jnp.minimum(s + 1, NSEG - 1)
            grp = jnp.maximum(s // 4 - 1, 0)
            row0 = pl.multiple_of(s * M, M)

            def side(p):
                if p % 2 == 0 or p // 2 >= 7:
                    return None
                i = p // 2
                if i < 4:
                    o, r = post(pseg, i * 8, 8)
                    return fold(o) + r
                r0 = (i - 3) * 8
                h = ln1(nseg, r0)
                put_rows(lhs_v, r0, h)
                return fold(h)

            def proj(m_i, p):
                g = m_i * NPAIR + p
                for t in range(2):
                    qkv_s[g, pl.ds(t * SEG, SEG), :] = _dot(lhs, _bf(w_w[2 * g + t])).astype(BF16)

            def rows_of(m_i, p):
                g = m_i * NPAIR + p
                return jnp.concatenate([_bf(qkv_w[g]), _bf(cache_w[g, pl.ds(row0, M), :])], axis=0)

            def probs(p):
                q = rows_of(0, p)
                k = rows_of(1, p)
                sc = lax.dot_general(q, k, (((1,), (1,)), ((), ())), preferred_element_type=F32) * SCALE
                fm = fill_v[...]
                tok = side(p)
                if tok is not None:
                    top = fm[0:8]
                    fm = jnp.concatenate([jnp.where(top > 1.0, tok[:, 0:PR], top), fm[8:]], axis=0)
                sc = jnp.where(fm == 0.0, sc, fm)
                e = jnp.exp(sc - jnp.max(sc, axis=-1, keepdims=True))
                return e.astype(BF16), _recip(jnp.sum(e, axis=-1, keepdims=True))

            def attend(p, pr):
                o = _dot(pr[0], rows_of(2, p)) * pr[1]
                o_s[2 * p] = o[0:SEG].astype(BF16)
                o_s[2 * p + 1] = o[SEG:2 * SEG].astype(BF16)
                odef[2 * p, pl.ds(row0, M), :] = o[2 * SEG:2 * SEG + M].astype(BF16)
                odef[2 * p + 1, pl.ds(row0, M), :] = o[2 * SEG + M:].astype(BF16)

            for t in range(2):
                deferred(deferred_lhs(grp), grp, (s % 4) * 2 + t)
            ps = {}
            for pa in range(0, NPAIR, 2):
                pb = pa + 1
                proj(0, pa)
                proj(1, pa)
                proj(0, pb)
                proj(1, pb)
                proj(2, pa)
                proj(2, pb)
                ps[pa] = probs(pa)
                ps[pb] = probs(pb)
                if pa >= 2:
                    attend(pa - 2, ps.pop(pa - 2))
                    attend(pb - 2, ps.pop(pb - 2))
            L = NPAIR - 1

            HA = 24
            acc = [None] * DB
            for h0, h1 in ((0, HA), (HA, H)):
                for j in range(DB):
                    ol = jnp.concatenate([_bf(o_w[h]) for h in range(h0, h1)], axis=1)
                    part = _dot(ol, _bf(wo_v[j, pl.ds(h0 * E // 2, (h1 - h0) * E // 2), :]))
                    if h0 == 0:
                        acc[j] = part
                    else:
                        a = part + acc[j]
                        lhs_v[j, pl.ds(0, M), :] = a[0:M].astype(BF16)
                        a_all[s, pl.ds(M, SEG - M), pl.ds(j * 128, 128)] = a[M:].astype(BF16)
                    if h0 == 0 and j == 4:
                        attend(L - 1, ps.pop(L - 1))
                        attend(L, ps.pop(L))
            return carry

        def multi(i, carry):
            for u in range(4):
                step(i * 4 + u, carry)
            return carry

        lax.fori_loop(0, NSEG // 4, multi, 0)

        out_copy(NSEG - LAG - 1).start()
        dl = deferred_lhs(NSEG // 4 - 1)
        for j in range(DB):
            deferred(dl, NSEG // 4 - 1, j)
        for seg in range(NSEG - LAG, NSEG):
            post(seg, 0, SEG)
            out_copy(seg).start()

        r = r_v[...].reshape(S, 1)
        idx = lax.broadcasted_iota(jnp.int32, (S, 1), 0)
        m1 = jnp.max(r, axis=0, keepdims=True)
        i1v = jnp.min(jnp.where(r == m1, idx, S - 1), axis=0, keepdims=True)
        r2 = jnp.where(idx == i1v, -jnp.inf, r)
        m2 = jnp.max(r2, axis=0, keepdims=True)
        i2v = jnp.min(jnp.where((r2 == m2) & (idx != i1v), idx, S - 1), axis=0, keepdims=True)
        i1 = i1v[0, 0]
        i2 = i2v[0, 0]

        def tile_of(i):
            return i >> 5, pl.multiple_of(((i >> 3) & 3) * 8, 8)

        sel = [tile_of(i1), tile_of(i2)]
        x1s = jnp.concatenate([x1_v[sg, pl.ds(r0, 8), :].astype(F32) for sg, r0 in sel], axis=0)
        h2s = _ln_mod(x1s, mod_row(4, 16), mod_row(3, 16))
        h2b = h2s.astype(BF16)
        for k, buf in enumerate((wg_v, wu_v, wd_v)):
            pltpu.make_async_copy(buf, buf, sems.at[SEM_MOE + k]).wait()
        gus = []
        for j in range(FB):
            g = _rb(_dot(h2b, _bf(wg_v[j])))
            g = _rb(g * jax.nn.sigmoid(g))
            u = _rb(_dot(h2b, _bf(wu_v[j])))
            gus.append((g * u).astype(BF16))
        gu = jnp.concatenate(gus, axis=1)
        y = jnp.concatenate([_rb(_dot(gu, _bf(wd_v[j]))) for j in range(DB)], axis=1)
        rows = lax.broadcasted_iota(jnp.int32, (16, 1), 0)
        rs = _rb(jax.nn.sigmoid(jnp.where(rows < 8, m1, m2)))
        y = _rb(y * rs)
        full = (x1s + _rb(mod_row(5, 16) * _rb(h2s + y)))

        pltpu.make_async_copy(out_v, out_v, sems.at[SEM_OUT]).wait()
        r8 = lax.broadcasted_iota(jnp.int32, (8, 1), 0)
        for t, (i, (sg, r0)) in enumerate(zip((i1, i2), sel)):
            old = out_v[sg, pl.ds(r0, 8), :].astype(F32)
            new = jnp.where(r8 == (i & 7), full[t * 8:(t + 1) * 8], old)
            out_v[sg, pl.ds(r0, 8), :] = new.astype(BF16)
        for sg, r0 in sel:
            cp = pltpu.make_async_copy(out_v.at[sg, pl.ds(r0, 8), :], out_hbm.at[sg, pl.ds(r0, 8), :], sems.at[SEM_OUT])
            cp.start()
            cp.wait()

    pl.run_scoped(
        main,
        pltpu.VMEM((FB, D // 2, 128), U32),
        pltpu.VMEM((FB, D // 2, 128), U32),
        pltpu.VMEM((DB, F // 2, 128), U32),
    )


@jax.jit
def pallas_adaLN_cond__memory_aug_recurrent_mem_tr__moe_arch_mod__prompt_kernel(
    A_x: jax.Array,
    A_mem0: jax.Array,
    A_Wq: jax.Array,
    A_Wk: jax.Array,
    A_Wv: jax.Array,
    A_Wo: jax.Array,
    A_seg_len: jax.Array,
    B_x: jax.Array,
    B_w_r: jax.Array,
    B_w_gate: jax.Array,
    B_w_up: jax.Array,
    B_w_down: jax.Array,
    c: jax.Array,
    w_mod: jax.Array,
):
    del A_seg_len, B_x
    assert A_x.shape == (1, S, D) and A_mem0.shape == (1, M, D) and A_Wq.shape == (D, H, E)
    hbm = pl.BlockSpec(memory_space=pl.ANY)
    vmem = pl.BlockSpec(memory_space=pltpu.VMEM)
    out = pl.pallas_call(
        _kernel,
        out_shape=jax.ShapeDtypeStruct((NSEG, SEG, D), BF16),
        in_specs=[hbm, vmem, hbm, hbm, hbm, hbm, vmem, hbm, hbm, hbm, vmem, hbm],
        out_specs=hbm,
        scratch_shapes=[
            pltpu.VMEM((NSEG, SEG, D), BF16),
            pltpu.VMEM((3 * H, D, E), BF16),
            pltpu.VMEM((DB, H * E // 2, 128), U32),
            pltpu.VMEM((3 * NPAIR, NSEG * 2 * M, E), BF16),
            pltpu.VMEM((H, NSEG * M, E), BF16),
            pltpu.VMEM((DB, SEG, 128), BF16),
            pltpu.VMEM((DB, SEG, 128), BF16),
            pltpu.VMEM((3 * NPAIR, 2 * SEG, E), BF16),
            pltpu.VMEM((H, SEG, E), BF16),
            pltpu.VMEM((NSEG, SEG, D), BF16),
            pltpu.VMEM((NSEG, SEG, D), BF16),
            pltpu.VMEM((NSEG, SEG, D), BF16),
            pltpu.VMEM((NSEG, SEG, 1), F32),
            pltpu.VMEM((7, 8, D), F32),
            pltpu.VMEM((PR, PR), F32),
            pltpu.SemaphoreType.DMA((NSEM,)),
        ],
        compiler_params=pltpu.CompilerParams(vmem_limit_bytes=120 * 1024 * 1024, disable_bounds_checks=True),
    )(
        A_x.reshape(NSEG, SEG, D),
        A_mem0.reshape(M, D),
        A_Wq, A_Wk, A_Wv,
        A_Wo.reshape(H * E, D),
        B_w_r.reshape(1, D),
        B_w_gate, B_w_up, B_w_down,
        c, w_mod,
    )
    return out.reshape(1, S, D)
```

```python
import jax
import jax.numpy as jnp
from jax import lax
import jax.experimental.pallas as pl
import jax.experimental.pallas.tpu as pltpu

BF16 = jnp.bfloat16
F32 = jnp.float32
U32 = jnp.uint32

S = 2048
D = 1024
H = 32
E = 128
M = 8
SEG = 32
NSEG = S // SEG
NPAIR = H // 2
NGP = 3 * NPAIR
F = 3584
DB = D // 128
FB = F // 128
PR = 2 * SEG + 2 * M
UNR = SEG // M
NIT = NSEG // UNR
PEEL = 3
PPI = 5
EARLY = 18
EPS = 1e-5
SCALE = E ** (-0.5)

SEM_SMALL = 0
SEM_X = SEM_SMALL + 3
SEM_MOD = SEM_X + 3
SEM_ST = SEM_MOD + 2
SEM_WO = SEM_ST + 1 + (NGP - PEEL) // PPI
SEM_MOE = SEM_WO + 1
SEM_OUT = SEM_MOE + 3
NSEM = SEM_OUT + 3


def _rb(v):
    return v.astype(BF16).astype(F32)


def _dot(a, b):
    return jnp.dot(a, b, preferred_element_type=F32)


def _recip(x):
    r = pl.reciprocal(x, approx=True)
    return r * (2.0 - x * r)


def _bf(words):
    return pltpu.bitcast(words, BF16)


def _ln(x):
    m = jnp.mean(x, axis=-1, keepdims=True)
    xc = x - m
    var = jnp.mean(xc * xc, axis=-1, keepdims=True)
    sd = _rb(jnp.sqrt(_rb(_rb(var) + EPS)))
    return _rb(_rb(x - _rb(m)) * (1.0 / sd))


def _ln_mod(x, scale1p, shift):
    return _rb(_rb(_ln(x) * scale1p) + shift)


def _fill_matrix():
    i = lax.broadcasted_iota(jnp.int32, (PR, PR), 0)
    j = lax.broadcasted_iota(jnp.int32, (PR, PR), 1)

    def head(t):
        return jnp.where(t < 2 * SEG, t >> 5, (t - 2 * SEG) >> 3)

    def pos(t):
        r = t & (SEG - 1)
        return jnp.where(t < 2 * SEG, jnp.where(r < M, r, r + M), M + (t & (M - 1)))

    same = head(i) == head(j)
    pi = pos(i)
    ok = jnp.where(pi < M, 1, jnp.where(pi >= pos(j), 1, 0))
    return jnp.where(same, jnp.where(ok == 1, 0.0, -1e9), -3e38).astype(F32)


def _kernel(x_hbm, mem0_hbm, wq_hbm, wk_hbm, wv_hbm, wo_hbm, wr_hbm, wg_hbm, wu_hbm, wd_hbm,
            c_hbm, wmod_hbm, out_hbm,
            x_v, w_v, wo_v, cache, odef, lhs_v, qkv_s, o_s, a_all, x1_v, out_v, r_v, mod_v, fill_v,
            mem0_v, wr_v, c_v, sems):
    w_w = w_v.bitcast(U32)
    cache_w = cache.bitcast(U32)
    lhs_w = lhs_v.bitcast(U32)
    qkv_w = qkv_s.bitcast(U32)
    o_w = o_s.bitcast(U32)
    odef_w = odef.bitcast(U32)

    def copy(src, dst, sem):
        return pltpu.make_async_copy(src, dst, sems.at[sem])

    def wait_all(buf, sem):
        copy(buf, buf, sem).wait()

    def mod_row(k, rows=8):
        v = mod_v[k]
        return v if rows == 8 else jnp.concatenate([v] * (rows // 8), axis=0)

    def put_rows(dst, r0, v):
        for j in range(DB):
            dst[j, pl.ds(r0, v.shape[0]), :] = v[:, j * 128:(j + 1) * 128].astype(BF16)

    def ln1(seg, r0):
        xt = x_v[seg, pl.ds(r0, 8), :].astype(F32)
        return _ln_mod(xt, mod_row(1), mod_row(0))

    x_tail = copy(x_hbm.at[pl.ds(1, NSEG - 1), pl.ds(M, SEG - M), :],
                  x_v.at[pl.ds(1, NSEG - 1), pl.ds(M, SEG - M), :], SEM_X + 2)

    def prologue(stage, wmod_v, hc, n_v):
        wmod_w = wmod_hbm.bitcast(U32)
        small = [copy(c_hbm, c_v, SEM_SMALL), copy(mem0_hbm, mem0_v, SEM_SMALL + 1),
                 copy(wr_hbm, wr_v, SEM_SMALL + 2)]
        x_head = copy(x_hbm.at[:, pl.ds(0, M), :], x_v.at[:, pl.ds(0, M), :], SEM_X)
        x_seg0 = copy(x_hbm.at[0, pl.ds(M, SEG - M), :], x_v.at[0, pl.ds(M, SEG - M), :], SEM_X + 1)
        for cp in small:
            cp.start()
        x_head.start()
        x_seg0.start()
        for k in (1, 0):
            for j in range(DB):
                copy(wmod_w.at[:, pl.ds(k * D + j * 128, 128)], wmod_v.at[k, j], SEM_MOD + k).start()
        slab_cps = []
        for m_i, w_hbm in enumerate((wq_hbm, wk_hbm, wv_hbm)):
            wb = w_hbm.bitcast(U32)
            for p in range(NPAIR):
                gp = m_i * NPAIR + p
                batch = 0 if gp < PEEL else 1 + (gp - PEEL) // PPI
                slab_cps.append(copy(wb.at[:, p, :], stage.at[gp], SEM_ST + batch))
        for cp in slab_cps[:EARLY]:
            cp.start()

        fill_v[...] = _fill_matrix()
        a_all[pl.ds(0, UNR + 1)] = jnp.zeros((UNR + 1, SEG, D), BF16)
        r_v[...] = jnp.zeros(r_v.shape, F32)

        for cp in small:
            cp.wait()
        c = c_v[...].astype(F32)
        sc = jnp.broadcast_to(_rb(c * jax.nn.sigmoid(c)), (16, D))
        zero = jnp.zeros((M, E), F32)
        for h in range(H):
            blk = sc[0:M, (h % DB) * 128:(h % DB + 1) * 128]
            odef[h, pl.ds(0, SEG), :] = jnp.concatenate(
                [blk if c_ == h // DB else zero for c_ in range(4)], axis=0).astype(BF16)
        sc = sc.astype(BF16)
        mod_v[6] = jnp.broadcast_to(wr_v[...].astype(F32), (8, D))
        put_rows(lhs_v, 0, mem0_v[...].astype(F32))

        def do_mod(k):
            wait_all(wmod_v.at[k], SEM_MOD + k)
            v = jnp.concatenate([_dot(sc, _bf(wmod_v[k, j])) for j in range(DB)], axis=1)
            v = _rb(v[0:8])
            mod_v[k] = _rb(1.0 + v) if k == 1 else v

        x_head.wait()
        x_seg0.wait()
        NB = 16
        RB = NSEG * M // NB
        for b in range(NB):
            xb = x_v[pl.ds(b * (NSEG // NB), NSEG // NB), pl.ds(0, M), :].astype(F32).reshape(RB, D)
            n_v[pl.ds(b * RB, RB), :] = _ln(xb)
        n_v[pl.ds(NSEG * M, SEG - M), :] = _ln(x_v[0, pl.ds(M, SEG - M), :].astype(F32))
        do_mod(1)
        for b in range(NB):
            n_v[pl.ds(b * RB, RB), :] = _rb(n_v[pl.ds(b * RB, RB), :] * mod_row(1, RB))
        n_v[pl.ds(NSEG * M, SEG - M), :] = _rb(n_v[pl.ds(NSEG * M, SEG - M), :] * mod_row(1, SEG - M))
        do_mod(0)
        for b in range(NB):
            put_rows(hc, b * RB, n_v[pl.ds(b * RB, RB), :] + mod_row(0, RB))
        put_rows(lhs_v, M, n_v[pl.ds(NSEG * M, SEG - M), :] + mod_row(0, SEG - M))

        hc_w = hc.bitcast(U32)

        def slab(gp):
            b = stage[gp]
            w_v[2 * gp] = pltpu.bitcast(b << 16, F32).astype(BF16)
            w_v[2 * gp + 1] = pltpu.bitcast(b & jnp.uint32(0xFFFF0000), F32).astype(BF16)
            hcv = jnp.concatenate([_bf(hc_w[j]) for j in range(DB)], axis=1)
            r1 = _dot(hcv, _bf(w_w[2 * gp])).reshape(NSEG, M, E)
            r2 = _dot(hcv, _bf(w_w[2 * gp + 1])).reshape(NSEG, M, E)
            cache[gp] = jnp.concatenate([r1, r2], axis=1).reshape(NSEG * 2 * M, E).astype(BF16)

        wait_all(stage.at[pl.ds(0, PEEL)], SEM_ST)
        for cp in slab_cps[EARLY:]:
            cp.start()
        x_tail.start()
        for gp in range(PEEL):
            slab(gp)

        def pro_body(i, carry):
            g0 = PEEL + i * PPI
            wait_all(stage.at[pl.ds(g0, PPI)], SEM_ST + 1 + i)

            @pl.when(i == 3)
            def _():
                wo_w = wo_hbm.bitcast(U32)
                for j in range(DB):
                    for c_ in range(4):
                        copy(wmod_w.at[:, pl.ds((2 + c_) * D + j * 128, 128)],
                             wo_v.at[j, pl.ds(c_ * (D // 2), D // 2), :], SEM_WO).start()
                for j in range(DB):
                    copy(wo_w.at[:, pl.ds(j * 128, 128)], wo_v.at[DB + j], SEM_WO).start()

            for t in range(PPI):
                slab(g0 + t)
            return carry

        lax.fori_loop(0, (NGP - PEEL) // PPI, pro_body, 0)

    pl.run_scoped(
        prologue,
        pltpu.VMEM((NGP, D, E), U32),
        pltpu.VMEM((2, DB, D // 2, 128), U32),
        pltpu.VMEM((DB, NSEG * M, E), BF16),
        pltpu.VMEM((NSEG * M + SEG - M, D), F32),
    )

    lane = lax.broadcasted_iota(jnp.int32, (8, 2 * 128), 1)

    def post(seg, q):
        rows = pl.ds(8 * q, 8)
        x = x_v[seg, rows, :].astype(F32)
        a = a_all[seg + UNR, rows, :].astype(F32)
        x1 = _rb(x + _rb(mod_row(2) * a))
        h2 = _ln_mod(x1, mod_row(4), mod_row(3))
        r = jnp.sum(h2 * mod_row(6), axis=-1, keepdims=True)
        r_v[...] = jnp.where(lane == seg * 4 + q, _rb(r), r_v[...])
        x1_v[seg, rows, :] = x1.astype(BF16)
        o = x1 + _rb(mod_row(5) * h2)
        out_v[seg, rows, :] = o.astype(BF16)
        return o, r

    def deferred(blk, wsel, j):
        row0 = blk * (SEG // 2)
        if not isinstance(blk, int):
            row0 = pl.multiple_of(row0, SEG // 2)
        lhs = jnp.concatenate([_bf(odef_w[h, pl.ds(row0, SEG // 2), :]) for h in range(H)], axis=1)
        res = _dot(lhs, _bf(wo_v[wsel + j])).astype(BF16).reshape(UNR, M, 128)
        a_all[pl.ds(blk * UNR, UNR), pl.ds(0, M), pl.ds(j * 128, 128)] = res

    def out_copy(grp):
        return copy(out_v.at[pl.ds(grp * UNR, UNR)], out_hbm.at[pl.ds(grp * UNR, UNR)], SEM_OUT)

    def fold(v):
        t = v[:, 0:128]
        for j in range(1, DB):
            t = t + v[:, j * 128:(j + 1) * 128]
        return t

    def main(wg_v, wu_v, wd_v):
        wg_w, wu_w, wd_w = wg_hbm.bitcast(U32), wu_hbm.bitcast(U32), wd_hbm.bitcast(U32)
        for j in range(FB):
            copy(wg_w.at[:, pl.ds(j * 128, 128)], wg_v.at[j], SEM_MOE).start()
            copy(wu_w.at[:, pl.ds(j * 128, 128)], wu_v.at[j], SEM_MOE + 1).start()
        for j in range(DB):
            copy(wd_w.at[:, pl.ds(j * 128, 128)], wd_v.at[j], SEM_MOE + 2).start()
        x_tail.wait()
        wait_all(wo_v, SEM_WO)

        def step(it, u):
            s = it * UNR + u
            lhs = jnp.concatenate([_bf(lhs_w[j]) for j in range(DB)], axis=1)
            nseg = jnp.minimum(s + 1, NSEG - 1)
            crow = pl.multiple_of(s * M, M)
            orow = pl.multiple_of((s + UNR) * M, M)

            def side(p):
                if p % 2 == 0 or p // 2 >= 7:
                    return None
                i = p // 2
                if i < 4:
                    lag = 2 * UNR if i == 0 else UNR
                    o, r = post(jnp.maximum(s - lag, 0), i)
                    return fold(o) + r
                r0 = (i - 3) * 8
                h = ln1(nseg, r0)
                put_rows(lhs_v, r0, h)
                return fold(h)

            def proj(m_i, p):
                g = m_i * NPAIR + p
                for t in range(2):
                    qkv_s[g, pl.ds(t * SEG, SEG), :] = _dot(lhs, _bf(w_w[2 * g + t])).astype(BF16)

            def rows_of(m_i, p):
                g = m_i * NPAIR + p
                return jnp.concatenate([_bf(qkv_w[g]), _bf(cache_w[g, pl.ds(crow, M), :])], axis=0)

            def probs(p):
                q = rows_of(0, p)
                k = rows_of(1, p)
                sc = lax.dot_general(q, k, (((1,), (1,)), ((), ())), preferred_element_type=F32) * SCALE
                fm = fill_v[...]
                tok = side(p)
                if tok is not None:
                    top = fm[0:8]
                    fm = jnp.concatenate([jnp.where(top > 1.0, tok[:, 0:PR], top), fm[8:]], axis=0)
                sc = jnp.where(fm == 0.0, sc, fm)
                e = jnp.exp(sc - jnp.max(sc, axis=-1, keepdims=True))
                return e.astype(BF16), _recip(jnp.sum(e, axis=-1, keepdims=True))

            def attend(p, pr):
                o = _dot(pr[0], rows_of(2, p)) * pr[1]
                o_s[2 * p] = o[0:SEG].astype(BF16)
                o_s[2 * p + 1] = o[SEG:2 * SEG].astype(BF16)
                odef[2 * p, pl.ds(orow, M), :] = o[2 * SEG:2 * SEG + M].astype(BF16)
                odef[2 * p + 1, pl.ds(orow, M), :] = o[2 * SEG + M:].astype(BF16)

            wsel = jnp.where(it == 0, 0, DB)
            for t in range(DB // UNR):
                deferred(it, wsel, u * (DB // UNR) + t)
            ps = {}
            for pa in range(0, NPAIR, 2):
                pb = pa + 1
                proj(0, pa)
                proj(1, pa)
                proj(0, pb)
                proj(1, pb)
                proj(2, pa)
                proj(2, pb)
                ps[pa] = probs(pa)
                ps[pb] = probs(pb)
                if pa >= 2:
                    attend(pa - 2, ps.pop(pa - 2))
                    attend(pb - 2, ps.pop(pb - 2))
            L = NPAIR - 1

            HA = 24
            acc = [None] * DB
            for h0, h1 in ((0, HA), (HA, H)):
                for j in range(DB):
                    ol = jnp.concatenate([_bf(o_w[h]) for h in range(h0, h1)], axis=1)
                    part = _dot(ol, _bf(wo_v[DB + j, pl.ds(h0 * E // 2, (h1 - h0) * E // 2), :]))
                    if h0 == 0:
                        acc[j] = part
                    else:
                        a = part + acc[j]
                        lhs_v[j, pl.ds(0, M), :] = a[0:M].astype(BF16)
                        a_all[s + UNR, pl.ds(M, SEG - M), pl.ds(j * 128, 128)] = a[M:].astype(BF16)
                    if h0 == 0 and j == 4:
                        attend(L - 1, ps.pop(L - 1))
                        attend(L, ps.pop(L))

        def iteration(it, carry):
            @pl.when(it >= 3)
            def _():
                out_copy(it - 3).start()

            for c_ in range(4):
                v = a_all[c_, pl.ds(0, M), :].astype(F32)
                mod_v[2 + c_] = _rb(1.0 + v) if c_ == 2 else v
            for u in range(UNR):
                step(it, u)
            return carry

        lax.fori_loop(0, NIT, iteration, 0)

        out_copy(NIT - 3).start()
        for j in range(DB):
            deferred(NIT, DB, j)
        for seg in range(NSEG - 2 * UNR, NSEG - UNR):
            post(seg, 0)
        out_copy(NIT - 2).start()
        for seg in range(NSEG - UNR, NSEG):
            for q in (1, 2, 3):
                post(seg, q)
        for seg in range(NSEG - UNR, NSEG):
            post(seg, 0)
        out_copy(NIT - 1).start()

        def all_max(v):
            return jnp.max(jnp.max(v, axis=1, keepdims=True), axis=0, keepdims=True)

        def all_min(v):
            return jnp.min(jnp.min(v, axis=1, keepdims=True), axis=0, keepdims=True)

        r = r_v[...]
        idx = (lane * 8 + lax.broadcasted_iota(jnp.int32, r.shape, 0)).astype(F32)
        m1 = all_max(r)
        i1v = all_min(jnp.where(r == m1, idx, S - 1.0))
        r2 = jnp.where(idx == i1v, -jnp.inf, r)
        m2 = all_max(r2)
        i2v = all_min(jnp.where(r2 == m2, jnp.where(idx == i1v, S - 1.0, idx), S - 1.0))
        i1 = i1v.astype(jnp.int32)[0, 0]
        i2 = i2v.astype(jnp.int32)[0, 0]

        def tile_of(i):
            return i >> 5, pl.multiple_of(((i >> 3) & 3) * 8, 8)

        sel = [tile_of(i1), tile_of(i2)]
        for k, buf in enumerate((wg_v, wu_v, wd_v)):
            wait_all(buf, SEM_MOE + k)
        x1s = jnp.concatenate([x1_v[sg, pl.ds(r0, 8), :].astype(F32) for sg, r0 in sel], axis=0)
        h2s = _ln_mod(x1s, mod_row(4, 16), mod_row(3, 16))
        h2b = h2s.astype(BF16)
        gus = []
        for j in range(FB):
            g = _rb(_dot(h2b, _bf(wg_v[j])))
            g = _rb(g * jax.nn.sigmoid(g))
            u = _rb(_dot(h2b, _bf(wu_v[j])))
            gus.append(g * u)
        gu = jnp.concatenate(gus, axis=1).astype(BF16)
        y = jnp.concatenate([_rb(_dot(gu, _bf(wd_v[j]))) for j in range(DB)], axis=1)
        rows = lax.broadcasted_iota(jnp.int32, (16, 1), 0)
        rs = _rb(jax.nn.sigmoid(jnp.where(rows < 8, m1, m2)))
        y = _rb(y * rs)
        full = x1s + _rb(mod_row(5, 16) * _rb(h2s + y))

        wait_all(out_v, SEM_OUT)
        r8 = lax.broadcasted_iota(jnp.int32, (8, 1), 0)
        for t, (i, (sg, r0)) in enumerate(zip((i1, i2), sel)):
            old = out_v[sg, pl.ds(r0, 8), :].astype(F32)
            new = jnp.where(r8 == (i & 7), full[t * 8:(t + 1) * 8], old)
            out_v[sg, pl.ds(r0, 8), :] = new.astype(BF16)
        fix = [copy(out_v.at[sg, pl.ds(r0, 8), :], out_hbm.at[sg, pl.ds(r0, 8), :], SEM_OUT + 1 + t)
               for t, (sg, r0) in enumerate(sel)]
        differ = (i1 >> 3) != (i2 >> 3)
        fix[0].start()

        @pl.when(differ)
        def _():
            fix[1].start()
            fix[1].wait()

        fix[0].wait()

    pl.run_scoped(
        main,
        pltpu.VMEM((FB, D // 2, 128), U32),
        pltpu.VMEM((FB, D // 2, 128), U32),
        pltpu.VMEM((DB, F // 2, 128), U32),
    )


@jax.jit
def pallas_adaLN_cond__memory_aug_recurrent_mem_tr__moe_arch_mod__prompt_kernel(
    A_x: jax.Array,
    A_mem0: jax.Array,
    A_Wq: jax.Array,
    A_Wk: jax.Array,
    A_Wv: jax.Array,
    A_Wo: jax.Array,
    A_seg_len: jax.Array,
    B_x: jax.Array,
    B_w_r: jax.Array,
    B_w_gate: jax.Array,
    B_w_up: jax.Array,
    B_w_down: jax.Array,
    c: jax.Array,
    w_mod: jax.Array,
):
    del A_seg_len, B_x
    assert A_x.shape == (1, S, D) and A_mem0.shape == (1, M, D) and A_Wq.shape == (D, H, E)
    hbm = pl.BlockSpec(memory_space=pl.ANY)
    out = pl.pallas_call(
        _kernel,
        out_shape=jax.ShapeDtypeStruct((NSEG, SEG, D), BF16),
        in_specs=[hbm] * 12,
        out_specs=hbm,
        scratch_shapes=[
            pltpu.VMEM((NSEG, SEG, D), BF16),
            pltpu.VMEM((3 * H, D, E), BF16),
            pltpu.VMEM((2 * DB, H * E // 2, 128), U32),
            pltpu.VMEM((NGP, NSEG * 2 * M, E), BF16),
            pltpu.VMEM((H, (NSEG + UNR) * M, E), BF16),
            pltpu.VMEM((DB, SEG, 128), BF16),
            pltpu.VMEM((NGP, 2 * SEG, E), BF16),
            pltpu.VMEM((H, SEG, E), BF16),
            pltpu.VMEM((NSEG + UNR, SEG, D), BF16),
            pltpu.VMEM((NSEG, SEG, D), BF16),
            pltpu.VMEM((NSEG, SEG, D), BF16),
            pltpu.VMEM((8, S // 8), F32),
            pltpu.VMEM((7, 8, D), F32),
            pltpu.VMEM((PR, PR), F32),
            pltpu.VMEM((M, D), BF16),
            pltpu.VMEM((1, D), BF16),
            pltpu.VMEM((1, D), BF16),
            pltpu.SemaphoreType.DMA((NSEM,)),
        ],
        compiler_params=pltpu.CompilerParams(
            vmem_limit_bytes=120 * 1024 * 1024, disable_bounds_checks=True),
    )(
        A_x.reshape(NSEG, SEG, D),
        A_mem0.reshape(M, D),
        A_Wq, A_Wk, A_Wv,
        A_Wo.reshape(H * E, D),
        B_w_r.reshape(1, D),
        B_w_gate, B_w_up, B_w_down,
        c, w_mod,
    )
    return out.reshape(1, S, D)
```

```python
import jax
import jax.numpy as jnp
from jax import lax
import jax.experimental.pallas as pl
import jax.experimental.pallas.tpu as pltpu

BF16 = jnp.bfloat16
F32 = jnp.float32
U32 = jnp.uint32

S = 2048
D = 1024
H = 32
E = 128
M = 8
SEG = 32
NSEG = S // SEG
NPAIR = H // 2
NGP = 3 * NPAIR
F = 3584
DB = D // 128
FB = F // 128
PR = 2 * SEG + 2 * M
UNR = SEG // M
NIT = NSEG // UNR
PEEL = 3
PPI = 5
EARLY = 18
EPS = 1e-5
SCALE = E ** (-0.5)

SEM_SMALL = 0
SEM_X = SEM_SMALL + 3
SEM_MOD = SEM_X + 3
SEM_ST = SEM_MOD + 2
SEM_WO = SEM_ST + 1 + (NGP - PEEL) // PPI
SEM_MOE = SEM_WO + 1
SEM_OUT = SEM_MOE + 3
NSEM = SEM_OUT + 3


def _rb(v):
    return v.astype(BF16).astype(F32)


def _dot(a, b):
    return jnp.dot(a, b, preferred_element_type=F32)


def _recip(x):
    r = pl.reciprocal(x, approx=True)
    return r * (2.0 - x * r)


def _bf(words):
    return pltpu.bitcast(words, BF16)


def _ln(x):
    m = jnp.mean(x, axis=-1, keepdims=True)
    xc = x - m
    var = jnp.mean(xc * xc, axis=-1, keepdims=True)
    sd = _rb(jnp.sqrt(_rb(_rb(var) + EPS)))
    return _rb(_rb(x - _rb(m)) * (1.0 / sd))


def _ln_mod(x, scale1p, shift):
    return _rb(_rb(_ln(x) * scale1p) + shift)


def _fill_matrix():
    i = lax.broadcasted_iota(jnp.int32, (PR, PR), 0)
    j = lax.broadcasted_iota(jnp.int32, (PR, PR), 1)

    def head(t):
        return jnp.where(t < 2 * SEG, t >> 5, (t - 2 * SEG) >> 3)

    def pos(t):
        r = t & (SEG - 1)
        return jnp.where(t < 2 * SEG, jnp.where(r < M, r, r + M), M + (t & (M - 1)))

    same = head(i) == head(j)
    pi = pos(i)
    ok = jnp.where(pi < M, 1, jnp.where(pi >= pos(j), 1, 0))
    return jnp.where(same, jnp.where(ok == 1, 0.0, -1e9), -3e38).astype(F32)


def _kernel(x_hbm, mem0_hbm, wq_hbm, wk_hbm, wv_hbm, wo_hbm, wr_hbm, wg_hbm, wu_hbm, wd_hbm,
            c_hbm, wmod_hbm, out_hbm,
            x_v, w_v, wo_v, cache, odef, lhs_v, qkv_s, o_s, a_all, x1_v, out_v, r_v, mod_v, fill_v,
            mem0_v, wr_v, c_v, sems):
    w_w = w_v.bitcast(U32)
    cache_w = cache.bitcast(U32)
    lhs_w = lhs_v.bitcast(U32)
    qkv_w = qkv_s.bitcast(U32)
    o_w = o_s.bitcast(U32)
    odef_w = odef.bitcast(U32)

    def copy(src, dst, sem):
        return pltpu.make_async_copy(src, dst, sems.at[sem])

    def wait_all(buf, sem):
        copy(buf, buf, sem).wait()

    def mod_row(k, rows=8):
        v = mod_v[k]
        return v if rows == 8 else jnp.concatenate([v] * (rows // 8), axis=0)

    def put_rows(dst, r0, v):
        for j in range(DB):
            dst[j, pl.ds(r0, v.shape[0]), :] = v[:, j * 128:(j + 1) * 128].astype(BF16)

    def ln1(seg, r0):
        xt = x_v[seg, pl.ds(r0, 8), :].astype(F32)
        return _ln_mod(xt, mod_row(1), mod_row(0))

    x_tail = copy(x_hbm.at[pl.ds(1, NSEG - 1), pl.ds(M, SEG - M), :],
                  x_v.at[pl.ds(1, NSEG - 1), pl.ds(M, SEG - M), :], SEM_X + 2)

    def prologue(stage, wmod_v, hc, n_v):
        wmod_w = wmod_hbm.bitcast(U32)
        small = [copy(c_hbm, c_v, SEM_SMALL), copy(mem0_hbm, mem0_v, SEM_SMALL + 1),
                 copy(wr_hbm, wr_v, SEM_SMALL + 2)]
        x_head = copy(x_hbm.at[:, pl.ds(0, M), :], x_v.at[:, pl.ds(0, M), :], SEM_X)
        x_seg0 = copy(x_hbm.at[0, pl.ds(M, SEG - M), :], x_v.at[0, pl.ds(M, SEG - M), :], SEM_X + 1)
        for cp in small:
            cp.start()
        x_head.start()
        x_seg0.start()
        for k in (1, 0):
            for j in range(DB):
                copy(wmod_w.at[:, pl.ds(k * D + j * 128, 128)], wmod_v.at[k, j], SEM_MOD + k).start()
        slab_cps = []
        for m_i, w_hbm in enumerate((wq_hbm, wk_hbm, wv_hbm)):
            wb = w_hbm.bitcast(U32)
            for p in range(NPAIR):
                gp = m_i * NPAIR + p
                batch = 0 if gp < PEEL else 1 + (gp - PEEL) // PPI
                slab_cps.append(copy(wb.at[:, p, :], stage.at[gp], SEM_ST + batch))
        for cp in slab_cps[:EARLY]:
            cp.start()

        fill_v[...] = _fill_matrix()
        a_all[pl.ds(0, UNR + 1)] = jnp.zeros((UNR + 1, SEG, D), BF16)
        r_v[...] = jnp.zeros(r_v.shape, F32)
        qkv_s[0] = jnp.zeros((2 * SEG, E), BF16)
        o_s[0] = jnp.zeros((SEG, E), BF16)

        for cp in small:
            cp.wait()
        c = c_v[...].astype(F32)
        sc = jnp.broadcast_to(_rb(c * jax.nn.sigmoid(c)), (16, D))
        zero = jnp.zeros((M, E), F32)
        for h in range(H):
            blk = sc[0:M, (h % DB) * 128:(h % DB + 1) * 128]
            odef[h, pl.ds(0, SEG), :] = jnp.concatenate(
                [blk if c_ == h // DB else zero for c_ in range(4)], axis=0).astype(BF16)
        sc = sc.astype(BF16)
        mod_v[6] = jnp.broadcast_to(wr_v[...].astype(F32), (8, D))
        put_rows(lhs_v, 0, mem0_v[...].astype(F32))

        def do_mod(k):
            wait_all(wmod_v.at[k], SEM_MOD + k)
            v = jnp.concatenate([_dot(sc, _bf(wmod_v[k, j])) for j in range(DB)], axis=1)
            v = _rb(v[0:8])
            mod_v[k] = _rb(1.0 + v) if k == 1 else v

        x_head.wait()
        x_seg0.wait()
        NB = 16
        RB = NSEG * M // NB
        for b in range(NB):
            xb = x_v[pl.ds(b * (NSEG // NB), NSEG // NB), pl.ds(0, M), :].astype(F32).reshape(RB, D)
            n_v[pl.ds(b * RB, RB), :] = _ln(xb)
        n_v[pl.ds(NSEG * M, SEG - M), :] = _ln(x_v[0, pl.ds(M, SEG - M), :].astype(F32))
        do_mod(1)
        for b in range(NB):
            n_v[pl.ds(b * RB, RB), :] = _rb(n_v[pl.ds(b * RB, RB), :] * mod_row(1, RB))
        n_v[pl.ds(NSEG * M, SEG - M), :] = _rb(n_v[pl.ds(NSEG * M, SEG - M), :] * mod_row(1, SEG - M))
        do_mod(0)
        for b in range(NB):
            put_rows(hc, b * RB, n_v[pl.ds(b * RB, RB), :] + mod_row(0, RB))
        put_rows(lhs_v, M, n_v[pl.ds(NSEG * M, SEG - M), :] + mod_row(0, SEG - M))

        hc_w = hc.bitcast(U32)

        def slab(gp):
            b = stage[gp]
            w_v[2 * gp] = pltpu.bitcast(b << 16, F32).astype(BF16)
            w_v[2 * gp + 1] = pltpu.bitcast(b & jnp.uint32(0xFFFF0000), F32).astype(BF16)
            hcv = jnp.concatenate([_bf(hc_w[j]) for j in range(DB)], axis=1)
            r1 = _dot(hcv, _bf(w_w[2 * gp])).reshape(NSEG, M, E)
            r2 = _dot(hcv, _bf(w_w[2 * gp + 1])).reshape(NSEG, M, E)
            cache[gp] = jnp.concatenate([r1, r2], axis=1).reshape(NSEG * 2 * M, E).astype(BF16)

        wait_all(stage.at[pl.ds(0, PEEL)], SEM_ST)
        for cp in slab_cps[EARLY:]:
            cp.start()
        x_tail.start()
        for gp in range(PEEL):
            slab(gp)

        def pro_body(i, carry):
            g0 = PEEL + i * PPI
            wait_all(stage.at[pl.ds(g0, PPI)], SEM_ST + 1 + i)

            @pl.when(i == 3)
            def _():
                wo_w = wo_hbm.bitcast(U32)
                for j in range(DB):
                    for c_ in range(4):
                        copy(wmod_w.at[:, pl.ds((2 + c_) * D + j * 128, 128)],
                             wo_v.at[j, pl.ds(c_ * (D // 2), D // 2), :], SEM_WO).start()
                for j in range(DB):
                    copy(wo_w.at[:, pl.ds(j * 128, 128)], wo_v.at[DB + j], SEM_WO).start()

            for t in range(PPI):
                slab(g0 + t)
            return carry

        lax.fori_loop(0, (NGP - PEEL) // PPI, pro_body, 0)

    pl.run_scoped(
        prologue,
        pltpu.VMEM((NGP, D, E), U32),
        pltpu.VMEM((2, DB, D // 2, 128), U32),
        pltpu.VMEM((DB, NSEG * M, E), BF16),
        pltpu.VMEM((NSEG * M + SEG - M, D), F32),
    )

    lane = lax.broadcasted_iota(jnp.int32, (8, 2 * 128), 1)

    def post(seg, q):
        rows = pl.ds(8 * q, 8)
        x = x_v[seg, rows, :].astype(F32)
        a = a_all[seg + UNR, rows, :].astype(F32)
        x1 = _rb(x + _rb(mod_row(2) * a))
        h2 = _ln_mod(x1, mod_row(4), mod_row(3))
        r = jnp.sum(h2 * mod_row(6), axis=-1, keepdims=True)
        r_v[...] = jnp.where(lane == seg * 4 + q, _rb(r), r_v[...])
        x1_v[seg, rows, :] = x1.astype(BF16)
        o = x1 + _rb(mod_row(5) * h2)
        out_v[seg, rows, :] = o.astype(BF16)
        return o, r

    def deferred(blk, wsel, j):
        row0 = blk * (SEG // 2)
        if not isinstance(blk, int):
            row0 = pl.multiple_of(row0, SEG // 2)
        lhs = jnp.concatenate([_bf(odef_w[h, pl.ds(row0, SEG // 2), :]) for h in range(H)], axis=1)
        res = _dot(lhs, _bf(wo_v[wsel + j])).astype(BF16).reshape(UNR, M, 128)
        a_all[pl.ds(blk * UNR, UNR), pl.ds(0, M), pl.ds(j * 128, 128)] = res

    def out_copy(grp):
        return copy(out_v.at[pl.ds(grp * UNR, UNR)], out_hbm.at[pl.ds(grp * UNR, UNR)], SEM_OUT)

    def fold(v):
        t = v[:, 0:128]
        for j in range(1, DB):
            t = t + v[:, j * 128:(j + 1) * 128]
        return t

    def main(wg_v, wu_v, wd_v):
        wg_w, wu_w, wd_w = wg_hbm.bitcast(U32), wu_hbm.bitcast(U32), wd_hbm.bitcast(U32)
        for j in range(FB):
            copy(wg_w.at[:, pl.ds(j * 128, 128)], wg_v.at[j], SEM_MOE).start()
            copy(wu_w.at[:, pl.ds(j * 128, 128)], wu_v.at[j], SEM_MOE + 1).start()
        for j in range(DB):
            copy(wd_w.at[:, pl.ds(j * 128, 128)], wd_v.at[j], SEM_MOE + 2).start()
        x_tail.wait()
        wait_all(wo_v, SEM_WO)

        def step(it, u):
            s = it * UNR + u
            lhs = jnp.concatenate([_bf(lhs_w[j]) for j in range(DB)], axis=1)
            nseg = jnp.minimum(s + 1, NSEG - 1)
            crow = pl.multiple_of(s * M, M)
            orow = pl.multiple_of((s + UNR) * M, M)

            def side(p):
                if p % 2 == 0 or p < 3:
                    return None
                i = p // 2 - 1
                if i < 4:
                    lag = 2 * UNR if i == 0 else UNR
                    o, r = post(jnp.maximum(s - lag, 0), i)
                    return fold(o) + r
                r0 = (i - 3) * 8
                h = ln1(nseg, r0)
                put_rows(lhs_v, r0, h)
                return fold(h)

            def proj(m_i, p):
                g = m_i * NPAIR + p
                for t in range(2):
                    qkv_s[g, pl.ds(t * SEG, SEG), :] = _dot(lhs, _bf(w_w[2 * g + t])).astype(BF16)

            def rows_of(m_i, p):
                g = m_i * NPAIR + p
                return jnp.concatenate([_bf(qkv_w[g]), _bf(cache_w[g, pl.ds(crow, M), :])], axis=0)

            def probs(p):
                q = rows_of(0, p)
                k = rows_of(1, p)
                sc = lax.dot_general(q, k, (((1,), (1,)), ((), ())), preferred_element_type=F32) * SCALE
                fm = fill_v[...]
                tok = side(p)
                if tok is not None:
                    top = fm[0:8]
                    fm = jnp.concatenate([jnp.where(top > 1.0, tok[:, 0:PR], top), fm[8:]], axis=0)
                sc = jnp.where(fm == 0.0, sc, fm)
                e = jnp.exp(sc - jnp.max(sc, axis=-1, keepdims=True))
                return (e * _recip(jnp.sum(e, axis=-1, keepdims=True))).astype(BF16)

            def attend(p, pr):
                o = _dot(pr, rows_of(2, p))
                o_s[2 * p] = o[0:SEG].astype(BF16)
                o_s[2 * p + 1] = o[SEG:2 * SEG].astype(BF16)
                odef[2 * p, pl.ds(orow, M), :] = o[2 * SEG:2 * SEG + M].astype(BF16)
                odef[2 * p + 1, pl.ds(orow, M), :] = o[2 * SEG + M:].astype(BF16)

            wsel = jnp.where(it == 0, 0, DB)
            for t in range(DB // UNR):
                deferred(it, wsel, u * (DB // UNR) + t)
            ps = {}
            for pa in range(0, NPAIR, 2):
                pb = pa + 1
                proj(0, pa)
                proj(1, pa)
                proj(0, pb)
                proj(1, pb)
                proj(2, pa)
                proj(2, pb)
                ps[pa] = probs(pa)
                ps[pb] = probs(pb)
                if pa >= 2:
                    attend(pa - 2, ps.pop(pa - 2))
                    attend(pb - 2, ps.pop(pb - 2))
            L = NPAIR - 1

            HA = 24
            acc = [None] * DB
            for h0, h1 in ((0, HA), (HA, H)):
                for j in range(DB):
                    ol = jnp.concatenate([_bf(o_w[h]) for h in range(h0, h1)], axis=1)
                    part = _dot(ol, _bf(wo_v[DB + j, pl.ds(h0 * E // 2, (h1 - h0) * E // 2), :]))
                    if h0 == 0:
                        acc[j] = part
                    else:
                        a = part + acc[j]
                        lhs_v[j, pl.ds(0, M), :] = a[0:M].astype(BF16)
                        a_all[s + UNR, pl.ds(M, SEG - M), pl.ds(j * 128, 128)] = a[M:].astype(BF16)
                    if h0 == 0 and j == 4:
                        attend(L - 1, ps.pop(L - 1))
                        attend(L, ps.pop(L))

        def iteration(it, carry):
            @pl.when(it >= 3)
            def _():
                out_copy(it - 3).start()

            for c_ in range(4):
                v = a_all[c_, pl.ds(0, M), :].astype(F32)
                mod_v[2 + c_] = _rb(1.0 + v) if c_ == 2 else v
            for u in range(UNR):
                step(it, u)
            return carry

        lax.fori_loop(0, NIT, iteration, 0)

        out_copy(NIT - 3).start()
        for j in range(DB):
            deferred(NIT, DB, j)
        for seg in range(NSEG - 2 * UNR, NSEG - UNR):
            post(seg, 0)
        out_copy(NIT - 2).start()
        for seg in range(NSEG - UNR, NSEG):
            for q in (1, 2, 3):
                post(seg, q)
        for seg in range(NSEG - UNR, NSEG):
            post(seg, 0)
        out_copy(NIT - 1).start()

        def all_max(v):
            return jnp.max(jnp.max(v, axis=1, keepdims=True), axis=0, keepdims=True)

        def all_min(v):
            return jnp.min(jnp.min(v, axis=1, keepdims=True), axis=0, keepdims=True)

        r = r_v[...]
        idx = (lane * 8 + lax.broadcasted_iota(jnp.int32, r.shape, 0)).astype(F32)
        m1 = all_max(r)
        i1v = all_min(jnp.where(r == m1, idx, S - 1.0))
        r2 = jnp.where(idx == i1v, -jnp.inf, r)
        m2 = all_max(r2)
        i2v = all_min(jnp.where(r2 == m2, jnp.where(idx == i1v, S - 1.0, idx), S - 1.0))
        i1 = i1v.astype(jnp.int32)[0, 0]
        i2 = i2v.astype(jnp.int32)[0, 0]

        def tile_of(i):
            return i >> 5, pl.multiple_of(((i >> 3) & 3) * 8, 8)

        sel = [tile_of(i1), tile_of(i2)]
        for k, buf in enumerate((wg_v, wu_v, wd_v)):
            wait_all(buf, SEM_MOE + k)
        x1s = jnp.concatenate([x1_v[sg, pl.ds(r0, 8), :].astype(F32) for sg, r0 in sel], axis=0)
        h2s = _ln_mod(x1s, mod_row(4, 16), mod_row(3, 16))
        h2b = h2s.astype(BF16)
        gus = []
        for j in range(FB):
            g = _rb(_dot(h2b, _bf(wg_v[j])))
            g = _rb(g * jax.nn.sigmoid(g))
            u = _rb(_dot(h2b, _bf(wu_v[j])))
            gus.append(g * u)
        gu = jnp.concatenate(gus, axis=1).astype(BF16)
        y = jnp.concatenate([_rb(_dot(gu, _bf(wd_v[j]))) for j in range(DB)], axis=1)
        rows = lax.broadcasted_iota(jnp.int32, (16, 1), 0)
        rs = _rb(jax.nn.sigmoid(jnp.where(rows < 8, m1, m2)))
        y = _rb(y * rs)
        full = x1s + _rb(mod_row(5, 16) * _rb(h2s + y))

        wait_all(out_v, SEM_OUT)
        r8 = lax.broadcasted_iota(jnp.int32, (8, 1), 0)
        for t, (i, (sg, r0)) in enumerate(zip((i1, i2), sel)):
            old = out_v[sg, pl.ds(r0, 8), :].astype(F32)
            new = jnp.where(r8 == (i & 7), full[t * 8:(t + 1) * 8], old)
            out_v[sg, pl.ds(r0, 8), :] = new.astype(BF16)
        fix = [copy(out_v.at[sg, pl.ds(r0, 8), :], out_hbm.at[sg, pl.ds(r0, 8), :], SEM_OUT + 1 + t)
               for t, (sg, r0) in enumerate(sel)]
        differ = (i1 >> 3) != (i2 >> 3)
        fix[0].start()

        @pl.when(differ)
        def _():
            fix[1].start()
            fix[1].wait()

        fix[0].wait()

    pl.run_scoped(
        main,
        pltpu.VMEM((FB, D // 2, 128), U32),
        pltpu.VMEM((FB, D // 2, 128), U32),
        pltpu.VMEM((DB, F // 2, 128), U32),
    )


@jax.jit
def pallas_adaLN_cond__memory_aug_recurrent_mem_tr__moe_arch_mod__prompt_kernel(
    A_x: jax.Array,
    A_mem0: jax.Array,
    A_Wq: jax.Array,
    A_Wk: jax.Array,
    A_Wv: jax.Array,
    A_Wo: jax.Array,
    A_seg_len: jax.Array,
    B_x: jax.Array,
    B_w_r: jax.Array,
    B_w_gate: jax.Array,
    B_w_up: jax.Array,
    B_w_down: jax.Array,
    c: jax.Array,
    w_mod: jax.Array,
):
    del A_seg_len, B_x
    assert A_x.shape == (1, S, D) and A_mem0.shape == (1, M, D) and A_Wq.shape == (D, H, E)
    hbm = pl.BlockSpec(memory_space=pl.ANY)
    out = pl.pallas_call(
        _kernel,
        out_shape=jax.ShapeDtypeStruct((NSEG, SEG, D), BF16),
        in_specs=[hbm] * 12,
        out_specs=hbm,
        scratch_shapes=[
            pltpu.VMEM((NSEG, SEG, D), BF16),
            pltpu.VMEM((3 * H, D, E), BF16),
            pltpu.VMEM((2 * DB, H * E // 2, 128), U32),
            pltpu.VMEM((NGP, NSEG * 2 * M, E), BF16),
            pltpu.VMEM((H, (NSEG + UNR) * M, E), BF16),
            pltpu.VMEM((DB, SEG, 128), BF16),
            pltpu.VMEM((NGP, 2 * SEG, E), BF16),
            pltpu.VMEM((H, SEG, E), BF16),
            pltpu.VMEM((NSEG + UNR, SEG, D), BF16),
            pltpu.VMEM((NSEG, SEG, D), BF16),
            pltpu.VMEM((NSEG, SEG, D), BF16),
            pltpu.VMEM((8, S // 8), F32),
            pltpu.VMEM((7, 8, D), F32),
            pltpu.VMEM((PR, PR), F32),
            pltpu.VMEM((M, D), BF16),
            pltpu.VMEM((1, D), BF16),
            pltpu.VMEM((1, D), BF16),
            pltpu.SemaphoreType.DMA((NSEM,)),
        ],
        compiler_params=pltpu.CompilerParams(
            vmem_limit_bytes=120 * 1024 * 1024, disable_bounds_checks=True),
    )(
        A_x.reshape(NSEG, SEG, D),
        A_mem0.reshape(M, D),
        A_Wq, A_Wk, A_Wv,
        A_Wo.reshape(H * E, D),
        B_w_r.reshape(1, D),
        B_w_gate, B_w_up, B_w_down,
        c, w_mod,
    )
    return out.reshape(1, S, D)
```

```python
import jax
import jax.numpy as jnp
from jax import lax
import jax.experimental.pallas as pl
import jax.experimental.pallas.tpu as pltpu

BF16 = jnp.bfloat16
F32 = jnp.float32
U32 = jnp.uint32

S = 2048
D = 1024
H = 32
E = 128
M = 8
SEG = 32
NSEG = S // SEG
NPAIR = H // 2
NGP = 3 * NPAIR
F = 3584
DB = D // 128
FB = F // 128
PR = 2 * SEG + 2 * M
UNR = SEG // M
NIT = NSEG // UNR
PEEL = 3
PPI = 5
EARLY = 18
EPS = 1e-5
SCALE = E ** (-0.5)

SEM_SMALL = 0
SEM_X = SEM_SMALL + 3
SEM_MOD = SEM_X + 3
SEM_ST = SEM_MOD + 2
SEM_WO = SEM_ST + 1 + (NGP - PEEL) // PPI
SEM_MOE = SEM_WO + 1
SEM_OUT = SEM_MOE + 3
NSEM = SEM_OUT + 3


def _rb(v):
    return v.astype(BF16).astype(F32)


def _dot(a, b):
    return jnp.dot(a, b, preferred_element_type=F32)


def _recip(x):
    r = pl.reciprocal(x, approx=True)
    return r * (2.0 - x * r)


def _bf(words):
    return pltpu.bitcast(words, BF16)


def _ln(x):
    m = jnp.mean(x, axis=-1, keepdims=True)
    xc = x - m
    var = jnp.mean(xc * xc, axis=-1, keepdims=True)
    sd = _rb(jnp.sqrt(_rb(_rb(var) + EPS)))
    return _rb(_rb(x - _rb(m)) * (1.0 / sd))


def _ln_mod(x, scale1p, shift):
    return _rb(_rb(_ln(x) * scale1p) + shift)


def _fill_matrix():
    i = lax.broadcasted_iota(jnp.int32, (PR, PR), 0)
    j = lax.broadcasted_iota(jnp.int32, (PR, PR), 1)

    def head(t):
        return jnp.where(t < 2 * SEG, t >> 5, (t - 2 * SEG) >> 3)

    def pos(t):
        r = t & (SEG - 1)
        return jnp.where(t < 2 * SEG, jnp.where(r < M, r, r + M), M + (t & (M - 1)))

    same = head(i) == head(j)
    pi = pos(i)
    ok = jnp.where(pi < M, 1, jnp.where(pi >= pos(j), 1, 0))
    return jnp.where(same, jnp.where(ok == 1, 0.0, -1e9), -3e38).astype(F32)


def _kernel(x_hbm, mem0_hbm, wq_hbm, wk_hbm, wv_hbm, wo_hbm, wr_hbm, wg_hbm, wu_hbm, wd_hbm,
            c_hbm, wmod_hbm, out_hbm,
            x_v, w_v, wo_v, cache, odef, lhs_v, qkv_s, o_s, a_all, x1_v, out_v, r_v, mod_v, fill_v,
            mem0_v, wr_v, c_v, sems):
    w_w = w_v.bitcast(U32)
    cache_w = cache.bitcast(U32)
    lhs_w = lhs_v.bitcast(U32)
    qkv_w = qkv_s.bitcast(U32)
    o_w = o_s.bitcast(U32)
    odef_w = odef.bitcast(U32)

    def copy(src, dst, sem):
        return pltpu.make_async_copy(src, dst, sems.at[sem])

    def wait_all(buf, sem):
        copy(buf, buf, sem).wait()

    def mod_row(k, rows=8):
        v = mod_v[k]
        return v if rows == 8 else jnp.concatenate([v] * (rows // 8), axis=0)

    def put_rows(dst, r0, v):
        for j in range(DB):
            dst[j, pl.ds(r0, v.shape[0]), :] = v[:, j * 128:(j + 1) * 128].astype(BF16)

    def ln1(seg, r0):
        xt = x_v[seg, pl.ds(r0, 8), :].astype(F32)
        return _ln_mod(xt, mod_row(1), mod_row(0))

    x_tail = copy(x_hbm.at[pl.ds(1, NSEG - 1), pl.ds(M, SEG - M), :],
                  x_v.at[pl.ds(1, NSEG - 1), pl.ds(M, SEG - M), :], SEM_X + 2)

    def prologue(stage, wmod_v, hc, n_v):
        wmod_w = wmod_hbm.bitcast(U32)
        small = [copy(c_hbm, c_v, SEM_SMALL), copy(mem0_hbm, mem0_v, SEM_SMALL + 1),
                 copy(wr_hbm, wr_v, SEM_SMALL + 2)]
        x_head = copy(x_hbm.at[:, pl.ds(0, M), :], x_v.at[:, pl.ds(0, M), :], SEM_X)
        x_seg0 = copy(x_hbm.at[0, pl.ds(M, SEG - M), :], x_v.at[0, pl.ds(M, SEG - M), :], SEM_X + 1)
        for cp in small:
            cp.start()
        x_head.start()
        x_seg0.start()
        for k in (1, 0):
            for j in range(DB):
                copy(wmod_w.at[:, pl.ds(k * D + j * 128, 128)], wmod_v.at[k, j], SEM_MOD + k).start()
        slab_cps = []
        for m_i, w_hbm in enumerate((wq_hbm, wk_hbm, wv_hbm)):
            wb = w_hbm.bitcast(U32)
            for p in range(NPAIR):
                gp = m_i * NPAIR + p
                batch = 0 if gp < PEEL else 1 + (gp - PEEL) // PPI
                slab_cps.append(copy(wb.at[:, p, :], stage.at[gp], SEM_ST + batch))
        for cp in slab_cps[:EARLY]:
            cp.start()

        fill_v[...] = _fill_matrix()
        a_all[pl.ds(0, UNR + 1)] = jnp.zeros((UNR + 1, SEG, D), BF16)
        r_v[...] = jnp.zeros(r_v.shape, F32)
        qkv_s[0] = jnp.zeros((2 * SEG, E), BF16)
        o_s[0] = jnp.zeros((SEG, E), BF16)

        for cp in small:
            cp.wait()
        c = c_v[...].astype(F32)
        sc = jnp.broadcast_to(_rb(c * jax.nn.sigmoid(c)), (16, D))
        zero = jnp.zeros((M, E), F32)
        for h in range(H):
            blk = sc[0:M, (h % DB) * 128:(h % DB + 1) * 128]
            odef[0, h] = jnp.concatenate(
                [blk if c_ == h // DB else zero for c_ in range(4)], axis=0).astype(BF16)
        sc = sc.astype(BF16)
        mod_v[6] = jnp.broadcast_to(wr_v[...].astype(F32), (8, D))
        put_rows(lhs_v, 0, mem0_v[...].astype(F32))

        def do_mod(k):
            wait_all(wmod_v.at[k], SEM_MOD + k)
            v = jnp.concatenate([_dot(sc, _bf(wmod_v[k, j])) for j in range(DB)], axis=1)
            v = _rb(v[0:8])
            mod_v[k] = _rb(1.0 + v) if k == 1 else v

        x_head.wait()
        x_seg0.wait()
        NB = 16
        RB = NSEG * M // NB
        for b in range(NB):
            xb = x_v[pl.ds(b * (NSEG // NB), NSEG // NB), pl.ds(0, M), :].astype(F32).reshape(RB, D)
            n_v[pl.ds(b * RB, RB), :] = _ln(xb)
        n_v[pl.ds(NSEG * M, SEG - M), :] = _ln(x_v[0, pl.ds(M, SEG - M), :].astype(F32))
        do_mod(1)
        for b in range(NB):
            n_v[pl.ds(b * RB, RB), :] = _rb(n_v[pl.ds(b * RB, RB), :] * mod_row(1, RB))
        n_v[pl.ds(NSEG * M, SEG - M), :] = _rb(n_v[pl.ds(NSEG * M, SEG - M), :] * mod_row(1, SEG - M))
        do_mod(0)
        for b in range(NB):
            put_rows(hc, b * RB, n_v[pl.ds(b * RB, RB), :] + mod_row(0, RB))
        put_rows(lhs_v, M, n_v[pl.ds(NSEG * M, SEG - M), :] + mod_row(0, SEG - M))

        hc_w = hc.bitcast(U32)

        def slab(gp):
            b = stage[gp]
            w_v[2 * gp] = pltpu.bitcast(b << 16, F32).astype(BF16)
            w_v[2 * gp + 1] = pltpu.bitcast(b & jnp.uint32(0xFFFF0000), F32).astype(BF16)
            hcv = jnp.concatenate([_bf(hc_w[j]) for j in range(DB)], axis=1)
            r1 = _dot(hcv, _bf(w_w[2 * gp])).reshape(NSEG, M, E)
            r2 = _dot(hcv, _bf(w_w[2 * gp + 1])).reshape(NSEG, M, E)
            cache[gp] = jnp.concatenate([r1, r2], axis=1).reshape(NIT, UNR * 2 * M, E).astype(BF16)

        wait_all(stage.at[pl.ds(0, PEEL)], SEM_ST)
        for cp in slab_cps[EARLY:]:
            cp.start()
        x_tail.start()
        for gp in range(PEEL):
            slab(gp)

        def pro_body(i, carry):
            g0 = PEEL + i * PPI
            wait_all(stage.at[pl.ds(g0, PPI)], SEM_ST + 1 + i)

            @pl.when(i == 3)
            def _():
                wo_w = wo_hbm.bitcast(U32)
                for j in range(DB):
                    for c_ in range(4):
                        copy(wmod_w.at[:, pl.ds((2 + c_) * D + j * 128, 128)],
                             wo_v.at[j, pl.ds(c_ * (D // 2), D // 2), :], SEM_WO).start()
                for j in range(DB):
                    copy(wo_w.at[:, pl.ds(j * 128, 128)], wo_v.at[DB + j], SEM_WO).start()

            for t in range(PPI):
                slab(g0 + t)
            return carry

        lax.fori_loop(0, (NGP - PEEL) // PPI, pro_body, 0)

    pl.run_scoped(
        prologue,
        pltpu.VMEM((NGP, D, E), U32),
        pltpu.VMEM((2, DB, D // 2, 128), U32),
        pltpu.VMEM((DB, NSEG * M, E), BF16),
        pltpu.VMEM((NSEG * M + SEG - M, D), F32),
    )

    lane = lax.broadcasted_iota(jnp.int32, (8, 2 * 128), 1)

    def post(seg, q):
        rows = pl.ds(8 * q, 8)
        x = x_v[seg, rows, :].astype(F32)
        a = a_all[seg + UNR, rows, :].astype(F32)
        x1 = _rb(x + _rb(mod_row(2) * a))
        h2 = _ln_mod(x1, mod_row(4), mod_row(3))
        r = jnp.sum(h2 * mod_row(6), axis=-1, keepdims=True)
        r_v[...] = jnp.where(lane == seg * 4 + q, _rb(r), r_v[...])
        x1_v[seg, rows, :] = x1.astype(BF16)
        o = x1 + _rb(mod_row(5) * h2)
        out_v[seg, rows, :] = o.astype(BF16)
        return o, r

    def deferred(blk, wsel, j):
        lhs = jnp.concatenate([_bf(odef_w[blk, h]) for h in range(H)], axis=1)
        res = _dot(lhs, _bf(wo_v[wsel + j])).astype(BF16).reshape(UNR, M, 128)
        a_all[pl.ds(blk * UNR, UNR), pl.ds(0, M), pl.ds(j * 128, 128)] = res

    def out_copy(grp):
        return copy(out_v.at[pl.ds(grp * UNR, UNR)], out_hbm.at[pl.ds(grp * UNR, UNR)], SEM_OUT)

    def fold(v):
        t = v[:, 0:128]
        for j in range(1, DB):
            t = t + v[:, j * 128:(j + 1) * 128]
        return t

    def main(wg_v, wu_v, wd_v):
        wg_w, wu_w, wd_w = wg_hbm.bitcast(U32), wu_hbm.bitcast(U32), wd_hbm.bitcast(U32)
        for j in range(FB):
            copy(wg_w.at[:, pl.ds(j * 128, 128)], wg_v.at[j], SEM_MOE).start()
            copy(wu_w.at[:, pl.ds(j * 128, 128)], wu_v.at[j], SEM_MOE + 1).start()
        for j in range(DB):
            copy(wd_w.at[:, pl.ds(j * 128, 128)], wd_v.at[j], SEM_MOE + 2).start()
        x_tail.wait()
        wait_all(wo_v, SEM_WO)

        def step(it, u):
            s = it * UNR + u
            lhs = jnp.concatenate([_bf(lhs_w[j]) for j in range(DB)], axis=1)
            nseg = jnp.minimum(s + 1, NSEG - 1)

            def side(p):
                if p % 2 == 0 or p < 3:
                    return None
                i = p // 2 - 1
                if i < 4:
                    lag = 2 * UNR if i == 0 else UNR
                    o, r = post(jnp.maximum(s - lag, 0), i)
                    return fold(o) + r
                r0 = (i - 3) * 8
                h = ln1(nseg, r0)
                put_rows(lhs_v, r0, h)
                return fold(h)

            def proj(m_i, p):
                g = m_i * NPAIR + p
                for t in range(2):
                    qkv_s[g, pl.ds(t * SEG, SEG), :] = _dot(lhs, _bf(w_w[2 * g + t])).astype(BF16)

            def rows_of(m_i, p):
                g = m_i * NPAIR + p
                return jnp.concatenate([_bf(qkv_w[g]), _bf(cache_w[g, it, pl.ds(u * M, M), :])], axis=0)

            def probs(p):
                q = rows_of(0, p)
                k = rows_of(1, p)
                sc = lax.dot_general(q, k, (((1,), (1,)), ((), ())), preferred_element_type=F32) * SCALE
                fm = fill_v[...]
                tok = side(p)
                if tok is not None:
                    top = fm[0:8]
                    fm = jnp.concatenate([jnp.where(top > 1.0, tok[:, 0:PR], top), fm[8:]], axis=0)
                sc = jnp.where(fm == 0.0, sc, fm)
                e = jnp.exp(sc - jnp.max(sc, axis=-1, keepdims=True))
                return (e * _recip(jnp.sum(e, axis=-1, keepdims=True))).astype(BF16)

            def attend(p, pr):
                o = _dot(pr, rows_of(2, p))
                o_s[2 * p] = o[0:SEG].astype(BF16)
                o_s[2 * p + 1] = o[SEG:2 * SEG].astype(BF16)
                odef[it + 1, 2 * p, pl.ds(u * M, M), :] = o[2 * SEG:2 * SEG + M].astype(BF16)
                odef[it + 1, 2 * p + 1, pl.ds(u * M, M), :] = o[2 * SEG + M:].astype(BF16)

            wsel = jnp.where(it == 0, 0, DB)
            for t in range(DB // UNR):
                deferred(it, wsel, u * (DB // UNR) + t)
            ps = {}
            for pa in range(0, NPAIR, 2):
                pb = pa + 1
                proj(0, pa)
                proj(1, pa)
                proj(0, pb)
                proj(1, pb)
                proj(2, pa)
                proj(2, pb)
                ps[pa] = probs(pa)
                ps[pb] = probs(pb)
                if pa >= 2:
                    attend(pa - 2, ps.pop(pa - 2))
                    attend(pb - 2, ps.pop(pb - 2))
            L = NPAIR - 1

            HA = 24
            acc = [None] * DB
            for h0, h1 in ((0, HA), (HA, H)):
                for j in range(DB):
                    ol = jnp.concatenate([_bf(o_w[h]) for h in range(h0, h1)], axis=1)
                    part = _dot(ol, _bf(wo_v[DB + j, pl.ds(h0 * E // 2, (h1 - h0) * E // 2), :]))
                    if h0 == 0:
                        acc[j] = part
                    else:
                        a = part + acc[j]
                        lhs_v[j, pl.ds(0, M), :] = a[0:M].astype(BF16)
                        a_all[s + UNR, pl.ds(M, SEG - M), pl.ds(j * 128, 128)] = a[M:].astype(BF16)
                    if h0 == 0 and j == 4:
                        attend(L - 1, ps.pop(L - 1))
                        attend(L, ps.pop(L))

        def iteration(it, carry):
            @pl.when(it >= 3)
            def _():
                out_copy(it - 3).start()

            for c_ in range(4):
                v = a_all[c_, pl.ds(0, M), :].astype(F32)
                mod_v[2 + c_] = _rb(1.0 + v) if c_ == 2 else v
            for u in range(UNR):
                step(it, u)
            return carry

        lax.fori_loop(0, NIT, iteration, 0)

        out_copy(NIT - 3).start()
        for j in range(DB):
            deferred(NIT, DB, j)
        for seg in range(NSEG - 2 * UNR, NSEG - UNR):
            post(seg, 0)
        out_copy(NIT - 2).start()
        for seg in range(NSEG - UNR, NSEG):
            for q in (1, 2, 3):
                post(seg, q)
        for seg in range(NSEG - UNR, NSEG):
            post(seg, 0)
        out_copy(NIT - 1).start()

        def all_max(v):
            return jnp.max(jnp.max(v, axis=1, keepdims=True), axis=0, keepdims=True)

        def all_min(v):
            return jnp.min(jnp.min(v, axis=1, keepdims=True), axis=0, keepdims=True)

        r = r_v[...]
        idx = (lane * 8 + lax.broadcasted_iota(jnp.int32, r.shape, 0)).astype(F32)
        m1 = all_max(r)
        i1v = all_min(jnp.where(r == m1, idx, S - 1.0))
        r2 = jnp.where(idx == i1v, -jnp.inf, r)
        m2 = all_max(r2)
        i2v = all_min(jnp.where(r2 == m2, jnp.where(idx == i1v, S - 1.0, idx), S - 1.0))
        i1 = i1v.astype(jnp.int32)[0, 0]
        i2 = i2v.astype(jnp.int32)[0, 0]

        def tile_of(i):
            return i >> 5, pl.multiple_of(((i >> 3) & 3) * 8, 8)

        sel = [tile_of(i1), tile_of(i2)]
        for k, buf in enumerate((wg_v, wu_v, wd_v)):
            wait_all(buf, SEM_MOE + k)
        x1s = jnp.concatenate([x1_v[sg, pl.ds(r0, 8), :].astype(F32) for sg, r0 in sel], axis=0)
        h2s = _ln_mod(x1s, mod_row(4, 16), mod_row(3, 16))
        h2b = h2s.astype(BF16)
        gus = []
        for j in range(FB):
            g = _rb(_dot(h2b, _bf(wg_v[j])))
            g = _rb(g * jax.nn.sigmoid(g))
            u = _rb(_dot(h2b, _bf(wu_v[j])))
            gus.append(g * u)
        gu = jnp.concatenate(gus, axis=1).astype(BF16)
        y = jnp.concatenate([_rb(_dot(gu, _bf(wd_v[j]))) for j in range(DB)], axis=1)
        rows = lax.broadcasted_iota(jnp.int32, (16, 1), 0)
        rs = _rb(jax.nn.sigmoid(jnp.where(rows < 8, m1, m2)))
        y = _rb(y * rs)
        full = x1s + _rb(mod_row(5, 16) * _rb(h2s + y))

        wait_all(out_v, SEM_OUT)
        r8 = lax.broadcasted_iota(jnp.int32, (8, 1), 0)
        for t, (i, (sg, r0)) in enumerate(zip((i1, i2), sel)):
            old = out_v[sg, pl.ds(r0, 8), :].astype(F32)
            new = jnp.where(r8 == (i & 7), full[t * 8:(t + 1) * 8], old)
            out_v[sg, pl.ds(r0, 8), :] = new.astype(BF16)
        fix = [copy(out_v.at[sg, pl.ds(r0, 8), :], out_hbm.at[sg, pl.ds(r0, 8), :], SEM_OUT + 1 + t)
               for t, (sg, r0) in enumerate(sel)]
        differ = (i1 >> 3) != (i2 >> 3)
        fix[0].start()

        @pl.when(differ)
        def _():
            fix[1].start()
            fix[1].wait()

        fix[0].wait()

    pl.run_scoped(
        main,
        pltpu.VMEM((FB, D // 2, 128), U32),
        pltpu.VMEM((FB, D // 2, 128), U32),
        pltpu.VMEM((DB, F // 2, 128), U32),
    )


@jax.jit
def pallas_adaLN_cond__memory_aug_recurrent_mem_tr__moe_arch_mod__prompt_kernel(
    A_x: jax.Array,
    A_mem0: jax.Array,
    A_Wq: jax.Array,
    A_Wk: jax.Array,
    A_Wv: jax.Array,
    A_Wo: jax.Array,
    A_seg_len: jax.Array,
    B_x: jax.Array,
    B_w_r: jax.Array,
    B_w_gate: jax.Array,
    B_w_up: jax.Array,
    B_w_down: jax.Array,
    c: jax.Array,
    w_mod: jax.Array,
):
    del A_seg_len, B_x
    assert A_x.shape == (1, S, D) and A_mem0.shape == (1, M, D) and A_Wq.shape == (D, H, E)
    hbm = pl.BlockSpec(memory_space=pl.ANY)
    out = pl.pallas_call(
        _kernel,
        out_shape=jax.ShapeDtypeStruct((NSEG, SEG, D), BF16),
        in_specs=[hbm] * 12,
        out_specs=hbm,
        scratch_shapes=[
            pltpu.VMEM((NSEG, SEG, D), BF16),
            pltpu.VMEM((3 * H, D, E), BF16),
            pltpu.VMEM((2 * DB, H * E // 2, 128), U32),
            pltpu.VMEM((NGP, NIT, UNR * 2 * M, E), BF16),
            pltpu.VMEM((NIT + 1, H, SEG, E), BF16),
            pltpu.VMEM((DB, SEG, 128), BF16),
            pltpu.VMEM((NGP, 2 * SEG, E), BF16),
            pltpu.VMEM((H, SEG, E), BF16),
            pltpu.VMEM((NSEG + UNR, SEG, D), BF16),
            pltpu.VMEM((NSEG, SEG, D), BF16),
            pltpu.VMEM((NSEG, SEG, D), BF16),
            pltpu.VMEM((8, S // 8), F32),
            pltpu.VMEM((7, 8, D), F32),
            pltpu.VMEM((PR, PR), F32),
            pltpu.VMEM((M, D), BF16),
            pltpu.VMEM((1, D), BF16),
            pltpu.VMEM((1, D), BF16),
            pltpu.SemaphoreType.DMA((NSEM,)),
        ],
        compiler_params=pltpu.CompilerParams(
            vmem_limit_bytes=120 * 1024 * 1024, disable_bounds_checks=True),
    )(
        A_x.reshape(NSEG, SEG, D),
        A_mem0.reshape(M, D),
        A_Wq, A_Wk, A_Wv,
        A_Wo.reshape(H * E, D),
        B_w_r.reshape(1, D),
        B_w_gate, B_w_up, B_w_down,
        c, w_mod,
    )
    return out.reshape(1, S, D)
```

```python
import jax
import jax.numpy as jnp
from jax import lax
import jax.experimental.pallas as pl
import jax.experimental.pallas.tpu as pltpu

BF16 = jnp.bfloat16
F32 = jnp.float32
U32 = jnp.uint32

S = 2048
D = 1024
H = 32
E = 128
M = 8
SEG = 32
NSEG = S // SEG
NPAIR = H // 2
NGP = 3 * NPAIR
F = 3584
DB = D // 128
FB = F // 128
PR = 2 * SEG + 2 * M
UNR = SEG // M
NIT = NSEG // UNR
PEEL = 3
PPI = 5
EARLY = 18
EPS = 1e-5
SCALE = E ** (-0.5)

SEM_SMALL = 0
SEM_X = SEM_SMALL + 3
SEM_MOD = SEM_X + 3
SEM_ST = SEM_MOD + 2
SEM_WO = SEM_ST + 2 + (NGP - PEEL) // PPI
SEM_MOE = SEM_WO + 1
SEM_OUT = SEM_MOE + 3
NSEM = SEM_OUT + 3


def _rb(v):
    return v.astype(BF16).astype(F32)


def _dot(a, b):
    return jnp.dot(a, b, preferred_element_type=F32)


def _recip(x):
    r = pl.reciprocal(x, approx=True)
    return r * (2.0 - x * r)


def _bf(words):
    return pltpu.bitcast(words, BF16)


def _ln(x):
    m = jnp.mean(x, axis=-1, keepdims=True)
    xc = x - m
    var = jnp.mean(xc * xc, axis=-1, keepdims=True)
    sd = _rb(jnp.sqrt(_rb(_rb(var) + EPS)))
    return _rb(_rb(x - _rb(m)) * (1.0 / sd))


def _ln_mod(x, scale1p, shift):
    return _rb(_rb(_ln(x) * scale1p) + shift)


def _fill_matrix():
    i = lax.broadcasted_iota(jnp.int32, (PR, PR), 0)
    j = lax.broadcasted_iota(jnp.int32, (PR, PR), 1)

    def head(t):
        return jnp.where(t < 2 * SEG, t >> 5, (t - 2 * SEG) >> 3)

    def pos(t):
        r = t & (SEG - 1)
        return jnp.where(t < 2 * SEG, jnp.where(r < M, r, r + M), M + (t & (M - 1)))

    same = head(i) == head(j)
    pi = pos(i)
    ok = jnp.where(pi < M, 1, jnp.where(pi >= pos(j), 1, 0))
    return jnp.where(same, jnp.where(ok == 1, 0.0, -1e9), -3e38).astype(F32)


def _kernel(x_hbm, mem0_hbm, wq_hbm, wk_hbm, wv_hbm, wo_hbm, wr_hbm, wg_hbm, wu_hbm, wd_hbm,
            c_hbm, wmod_hbm, out_hbm,
            x_v, w_v, wo_v, cache, odef, lhs_v, qkv_s, o_s, a_all, x1_v, out_v, r_v, mod_v, fill_v,
            mem0_v, wr_v, c_v, sems):
    w_w = w_v.bitcast(U32)
    cache_w = cache.bitcast(U32)
    lhs_w = lhs_v.bitcast(U32)
    qkv_w = qkv_s.bitcast(U32)
    o_w = o_s.bitcast(U32)
    odef_w = odef.bitcast(U32)

    def copy(src, dst, sem):
        return pltpu.make_async_copy(src, dst, sems.at[sem])

    def wait_all(buf, sem):
        copy(buf, buf, sem).wait()

    def mod_row(k, rows=8):
        v = mod_v[k]
        return v if rows == 8 else jnp.concatenate([v] * (rows // 8), axis=0)

    def put_rows(dst, r0, v):
        for j in range(DB):
            dst[j, pl.ds(r0, v.shape[0]), :] = v[:, j * 128:(j + 1) * 128].astype(BF16)

    def ln1(seg, r0):
        xt = x_v[seg, pl.ds(r0, 8), :].astype(F32)
        return _ln_mod(xt, mod_row(1), mod_row(0))

    x_tail = copy(x_hbm.at[pl.ds(1, NSEG - 1), pl.ds(M, SEG - M), :],
                  x_v.at[pl.ds(1, NSEG - 1), pl.ds(M, SEG - M), :], SEM_X + 2)

    def prologue(stage, wmod_v, hc, n_v):
        wmod_w = wmod_hbm.bitcast(U32)
        small = [copy(c_hbm, c_v, SEM_SMALL), copy(mem0_hbm, mem0_v, SEM_SMALL + 1),
                 copy(wr_hbm, wr_v, SEM_SMALL + 2)]
        x_head = copy(x_hbm.at[:, pl.ds(0, M), :], x_v.at[:, pl.ds(0, M), :], SEM_X)
        x_seg0 = copy(x_hbm.at[0, pl.ds(M, SEG - M), :], x_v.at[0, pl.ds(M, SEG - M), :], SEM_X + 1)
        for cp in small:
            cp.start()
        x_head.start()
        x_seg0.start()
        mod_cps = [copy(wmod_hbm.at[:, pl.ds(k * D, D)], wmod_v.at[k], SEM_MOD + k) for k in range(2)]
        mod_cps[1].start()
        mod_cps[0].start()
        slab_cps = []
        for m_i, w_hbm in enumerate((wq_hbm, wk_hbm, wv_hbm)):
            wb = w_hbm.bitcast(U32)
            for p in range(NPAIR):
                gp = m_i * NPAIR + p
                batch = min(gp, 1) if gp < PEEL else 2 + (gp - PEEL) // PPI
                slab_cps.append(copy(wb.at[:, p, :], stage.at[gp], SEM_ST + batch))
        for cp in slab_cps[:EARLY]:
            cp.start()

        fill_v[...] = _fill_matrix()
        a_all[pl.ds(0, UNR + 1)] = jnp.zeros((UNR + 1, SEG, D), BF16)
        r_v[...] = jnp.zeros(r_v.shape, F32)
        qkv_s[0] = jnp.zeros((2 * SEG, E), BF16)
        o_s[0] = jnp.zeros((SEG, E), BF16)

        for cp in small:
            cp.wait()
        c = c_v[...].astype(F32)
        sc = jnp.broadcast_to(_rb(c * jax.nn.sigmoid(c)), (16, D))
        zero = jnp.zeros((M, E), F32)
        for h in range(H):
            blk = sc[0:M, (h % DB) * 128:(h % DB + 1) * 128]
            odef[0, h] = jnp.concatenate(
                [blk if c_ == h // DB else zero for c_ in range(4)], axis=0).astype(BF16)
        sc = sc.astype(BF16)
        mod_v[6] = jnp.broadcast_to(wr_v[...].astype(F32).reshape(1, D), (8, D))
        put_rows(lhs_v, 0, mem0_v[...].astype(F32))

        def do_mod(k):
            mod_cps[k].wait()
            v = _rb(_dot(sc, wmod_v[k])[0:8])
            mod_v[k] = _rb(1.0 + v) if k == 1 else v

        x_head.wait()
        x_seg0.wait()
        NB = 16
        RB = NSEG * M // NB
        for b in range(NB):
            xb = x_v[pl.ds(b * (NSEG // NB), NSEG // NB), pl.ds(0, M), :].astype(F32).reshape(RB, D)
            n_v[pl.ds(b * RB, RB), :] = _ln(xb)
        n_v[pl.ds(NSEG * M, SEG - M), :] = _ln(x_v[0, pl.ds(M, SEG - M), :].astype(F32))
        do_mod(1)
        for b in range(NB):
            n_v[pl.ds(b * RB, RB), :] = _rb(n_v[pl.ds(b * RB, RB), :] * mod_row(1, RB))
        n_v[pl.ds(NSEG * M, SEG - M), :] = _rb(n_v[pl.ds(NSEG * M, SEG - M), :] * mod_row(1, SEG - M))
        do_mod(0)
        for b in range(NB):
            put_rows(hc, b * RB, n_v[pl.ds(b * RB, RB), :] + mod_row(0, RB))
        put_rows(lhs_v, M, n_v[pl.ds(NSEG * M, SEG - M), :] + mod_row(0, SEG - M))

        hc_w = hc.bitcast(U32)

        def slab(gp):
            b = stage[gp]
            w_v[2 * gp] = pltpu.bitcast(b << 16, F32).astype(BF16)
            w_v[2 * gp + 1] = pltpu.bitcast(b & jnp.uint32(0xFFFF0000), F32).astype(BF16)
            hcv = jnp.concatenate([_bf(hc_w[j]) for j in range(DB)], axis=1)
            r1 = _dot(hcv, _bf(w_w[2 * gp])).reshape(NSEG, M, E)
            r2 = _dot(hcv, _bf(w_w[2 * gp + 1])).reshape(NSEG, M, E)
            cache[gp] = jnp.concatenate([r1, r2], axis=1).reshape(NIT, UNR * 2 * M, E).astype(BF16)

        slab_cps[0].wait()
        slab(0)
        wait_all(stage.at[pl.ds(1, PEEL - 1)], SEM_ST + 1)
        for cp in slab_cps[EARLY:]:
            cp.start()
        x_tail.start()
        for gp in range(1, PEEL):
            slab(gp)

        def pro_body(i, carry):
            g0 = PEEL + i * PPI
            wait_all(stage.at[pl.ds(g0, PPI)], SEM_ST + 2 + i)

            @pl.when(i == 3)
            def _():
                wo_w = wo_hbm.bitcast(U32)
                for j in range(DB):
                    for c_ in range(4):
                        copy(wmod_w.at[:, pl.ds((2 + c_) * D + j * 128, 128)],
                             wo_v.at[j, pl.ds(c_ * (D // 2), D // 2), :], SEM_WO).start()
                for j in range(DB):
                    copy(wo_w.at[:, pl.ds(j * 128, 128)], wo_v.at[DB + j], SEM_WO).start()

            for t in range(PPI):
                slab(g0 + t)
            return carry

        lax.fori_loop(0, (NGP - PEEL) // PPI, pro_body, 0)

    pl.run_scoped(
        prologue,
        pltpu.VMEM((NGP, D, E), U32),
        pltpu.VMEM((2, D, D), BF16),
        pltpu.VMEM((DB, NSEG * M, E), BF16),
        pltpu.VMEM((NSEG * M + SEG - M, D), F32),
    )

    lane = lax.broadcasted_iota(jnp.int32, (8, 2 * 128), 1)

    def post(seg, q):
        rows = pl.ds(8 * q, 8)
        x = x_v[seg, rows, :].astype(F32)
        a = a_all[seg + UNR, rows, :].astype(F32)
        x1 = _rb(x + _rb(mod_row(2) * a))
        h2 = _ln_mod(x1, mod_row(4), mod_row(3))
        r = jnp.sum(h2 * mod_row(6), axis=-1, keepdims=True)
        r_v[...] = jnp.where(lane == seg * 4 + q, _rb(r), r_v[...])
        x1_v[seg, rows, :] = x1.astype(BF16)
        o = x1 + _rb(mod_row(5) * h2)
        out_v[seg, rows, :] = o.astype(BF16)
        return o, r

    def deferred(blk, wsel, j):
        lhs = jnp.concatenate([_bf(odef_w[blk, h]) for h in range(H)], axis=1)
        res = _dot(lhs, _bf(wo_v[wsel + j])).astype(BF16).reshape(UNR, M, 128)
        a_all[pl.ds(blk * UNR, UNR), pl.ds(0, M), pl.ds(j * 128, 128)] = res

    def out_copy(grp):
        return copy(out_v.at[pl.ds(grp * UNR, UNR)], out_hbm.at[pl.ds(grp * UNR, UNR)], SEM_OUT)

    def fold(v):
        t = v[:, 0:128]
        for j in range(1, DB):
            t = t + v[:, j * 128:(j + 1) * 128]
        return t

    def main(wg_v, wu_v, wd_v):
        wg_w, wu_w, wd_w = wg_hbm.bitcast(U32), wu_hbm.bitcast(U32), wd_hbm.bitcast(U32)
        for j in range(FB):
            copy(wg_w.at[:, pl.ds(j * 128, 128)], wg_v.at[j], SEM_MOE).start()
            copy(wu_w.at[:, pl.ds(j * 128, 128)], wu_v.at[j], SEM_MOE + 1).start()
        for j in range(DB):
            copy(wd_w.at[:, pl.ds(j * 128, 128)], wd_v.at[j], SEM_MOE + 2).start()
        x_tail.wait()
        wait_all(wo_v, SEM_WO)

        def step(it, u):
            s = it * UNR + u
            lhs = jnp.concatenate([_bf(lhs_w[j]) for j in range(DB)], axis=1)
            nseg = jnp.minimum(s + 1, NSEG - 1)

            def side(p):
                if p % 2 == 0 or p < 3:
                    return None
                i = p // 2 - 1
                if i < 4:
                    lag = 2 * UNR if i == 0 else UNR
                    o, r = post(jnp.maximum(s - lag, 0), i)
                    return fold(o) + r
                r0 = (i - 3) * 8
                h = ln1(nseg, r0)
                put_rows(lhs_v, r0, h)
                return fold(h)

            def proj(m_i, p):
                g = m_i * NPAIR + p
                for t in range(2):
                    qkv_s[g, pl.ds(t * SEG, SEG), :] = _dot(lhs, _bf(w_w[2 * g + t])).astype(BF16)

            def rows_of(m_i, p):
                g = m_i * NPAIR + p
                return jnp.concatenate([_bf(qkv_w[g]), _bf(cache_w[g, it, pl.ds(u * M, M), :])], axis=0)

            def probs(p):
                q = rows_of(0, p)
                k = rows_of(1, p)
                sc = lax.dot_general(q, k, (((1,), (1,)), ((), ())), preferred_element_type=F32) * SCALE
                fm = fill_v[...]
                tok = side(p)
                if tok is not None:
                    top = fm[0:8]
                    fm = jnp.concatenate([jnp.where(top > 1.0, tok[:, 0:PR], top), fm[8:]], axis=0)
                sc = jnp.where(fm == 0.0, sc, fm)
                e = jnp.exp(sc - jnp.max(sc, axis=-1, keepdims=True))
                return (e * _recip(jnp.sum(e, axis=-1, keepdims=True))).astype(BF16)

            def attend(p, pr):
                o = _dot(pr, rows_of(2, p))
                o_s[2 * p] = o[0:SEG].astype(BF16)
                o_s[2 * p + 1] = o[SEG:2 * SEG].astype(BF16)
                odef[it + 1, 2 * p, pl.ds(u * M, M), :] = o[2 * SEG:2 * SEG + M].astype(BF16)
                odef[it + 1, 2 * p + 1, pl.ds(u * M, M), :] = o[2 * SEG + M:].astype(BF16)

            wsel = jnp.where(it == 0, 0, DB)
            for t in range(DB // UNR):
                deferred(it, wsel, u * (DB // UNR) + t)
            ps = {}
            for pa in range(0, NPAIR, 2):
                pb = pa + 1
                proj(0, pa)
                proj(1, pa)
                proj(0, pb)
                proj(1, pb)
                proj(2, pa)
                proj(2, pb)
                ps[pa] = probs(pa)
                ps[pb] = probs(pb)
                if pa >= 2:
                    attend(pa - 2, ps.pop(pa - 2))
                    attend(pb - 2, ps.pop(pb - 2))
            L = NPAIR - 1

            HA = 24
            acc = [None] * DB
            for h0, h1 in ((0, HA), (HA, H)):
                for j in range(DB):
                    ol = jnp.concatenate([_bf(o_w[h]) for h in range(h0, h1)], axis=1)
                    part = _dot(ol, _bf(wo_v[DB + j, pl.ds(h0 * E // 2, (h1 - h0) * E // 2), :]))
                    if h0 == 0:
                        acc[j] = part
                    else:
                        a = part + acc[j]
                        lhs_v[j, pl.ds(0, M), :] = a[0:M].astype(BF16)
                        a_all[s + UNR, pl.ds(M, SEG - M), pl.ds(j * 128, 128)] = a[M:].astype(BF16)
                    if h0 == 0 and j == 4:
                        attend(L - 1, ps.pop(L - 1))
                        attend(L, ps.pop(L))

        def iteration(it, carry):
            @pl.when(it >= 3)
            def _():
                out_copy(it - 3).start()

            for c_ in range(4):
                v = a_all[c_, pl.ds(0, M), :].astype(F32)
                mod_v[2 + c_] = _rb(1.0 + v) if c_ == 2 else v
            for u in range(UNR):
                step(it, u)
            return carry

        lax.fori_loop(0, NIT, iteration, 0)

        out_copy(NIT - 3).start()
        for j in range(DB):
            deferred(NIT, DB, j)
        for seg in range(NSEG - 2 * UNR, NSEG - UNR):
            post(seg, 0)
        out_copy(NIT - 2).start()
        for seg in range(NSEG - UNR, NSEG):
            for q in (1, 2, 3):
                post(seg, q)
        for seg in range(NSEG - UNR, NSEG):
            post(seg, 0)
        out_copy(NIT - 1).start()

        def all_max(v):
            return jnp.max(jnp.max(v, axis=1, keepdims=True), axis=0, keepdims=True)

        def all_min(v):
            return jnp.min(jnp.min(v, axis=1, keepdims=True), axis=0, keepdims=True)

        r = r_v[...]
        idx = (lane * 8 + lax.broadcasted_iota(jnp.int32, r.shape, 0)).astype(F32)
        m1 = all_max(r)
        i1v = all_min(jnp.where(r == m1, idx, S - 1.0))
        r2 = jnp.where(idx == i1v, -jnp.inf, r)
        m2 = all_max(r2)
        i2v = all_min(jnp.where(r2 == m2, jnp.where(idx == i1v, S - 1.0, idx), S - 1.0))
        i1 = i1v.astype(jnp.int32)[0, 0]
        i2 = i2v.astype(jnp.int32)[0, 0]

        def tile_of(i):
            return i >> 5, pl.multiple_of(((i >> 3) & 3) * 8, 8)

        sel = [tile_of(i1), tile_of(i2)]
        for k, buf in enumerate((wg_v, wu_v, wd_v)):
            wait_all(buf, SEM_MOE + k)
        x1s = jnp.concatenate([x1_v[sg, pl.ds(r0, 8), :].astype(F32) for sg, r0 in sel], axis=0)
        h2s = _ln_mod(x1s, mod_row(4, 16), mod_row(3, 16))
        h2b = h2s.astype(BF16)
        gus = []
        for j in range(FB):
            g = _rb(_dot(h2b, _bf(wg_v[j])))
            g = _rb(g * jax.nn.sigmoid(g))
            u = _rb(_dot(h2b, _bf(wu_v[j])))
            gus.append(g * u)
        gu = jnp.concatenate(gus, axis=1).astype(BF16)
        y = jnp.concatenate([_rb(_dot(gu, _bf(wd_v[j]))) for j in range(DB)], axis=1)
        rows = lax.broadcasted_iota(jnp.int32, (16, 1), 0)
        rs = _rb(jax.nn.sigmoid(jnp.where(rows < 8, m1, m2)))
        y = _rb(y * rs)
        full = x1s + _rb(mod_row(5, 16) * _rb(h2s + y))

        copy(out_v, out_hbm, SEM_OUT).wait()
        r8 = lax.broadcasted_iota(jnp.int32, (8, 1), 0)
        for t, (i, (sg, r0)) in enumerate(zip((i1, i2), sel)):
            old = out_v[sg, pl.ds(r0, 8), :].astype(F32)
            new = jnp.where(r8 == (i & 7), full[t * 8:(t + 1) * 8], old)
            out_v[sg, pl.ds(r0, 8), :] = new.astype(BF16)
        fix = [copy(out_v.at[sg, pl.ds(r0, 8), :], out_hbm.at[sg, pl.ds(r0, 8), :], SEM_OUT + 1 + t)
               for t, (sg, r0) in enumerate(sel)]
        differ = (i1 >> 3) != (i2 >> 3)
        fix[0].start()

        @pl.when(differ)
        def _():
            fix[1].start()
            fix[1].wait()

        fix[0].wait()

    pl.run_scoped(
        main,
        pltpu.VMEM((FB, D // 2, 128), U32),
        pltpu.VMEM((FB, D // 2, 128), U32),
        pltpu.VMEM((DB, F // 2, 128), U32),
    )


@jax.jit
def pallas_adaLN_cond__memory_aug_recurrent_mem_tr__moe_arch_mod__prompt_kernel(
    A_x: jax.Array,
    A_mem0: jax.Array,
    A_Wq: jax.Array,
    A_Wk: jax.Array,
    A_Wv: jax.Array,
    A_Wo: jax.Array,
    A_seg_len: jax.Array,
    B_x: jax.Array,
    B_w_r: jax.Array,
    B_w_gate: jax.Array,
    B_w_up: jax.Array,
    B_w_down: jax.Array,
    c: jax.Array,
    w_mod: jax.Array,
):
    del A_seg_len, B_x
    assert A_x.shape == (1, S, D) and A_mem0.shape == (1, M, D) and A_Wq.shape == (D, H, E)
    hbm = pl.BlockSpec(memory_space=pl.ANY)
    out = pl.pallas_call(
        _kernel,
        out_shape=jax.ShapeDtypeStruct((NSEG, SEG, D), BF16),
        in_specs=[hbm] * 12,
        out_specs=hbm,
        scratch_shapes=[
            pltpu.VMEM((NSEG, SEG, D), BF16),
            pltpu.VMEM((3 * H, D, E), BF16),
            pltpu.VMEM((2 * DB, H * E // 2, 128), U32),
            pltpu.VMEM((NGP, NIT, UNR * 2 * M, E), BF16),
            pltpu.VMEM((NIT + 1, H, SEG, E), BF16),
            pltpu.VMEM((DB, SEG, 128), BF16),
            pltpu.VMEM((NGP, 2 * SEG, E), BF16),
            pltpu.VMEM((H, SEG, E), BF16),
            pltpu.VMEM((NSEG + UNR, SEG, D), BF16),
            pltpu.VMEM((NSEG, SEG, D), BF16),
            pltpu.VMEM((NSEG, SEG, D), BF16),
            pltpu.VMEM((8, S // 8), F32),
            pltpu.VMEM((7, 8, D), F32),
            pltpu.VMEM((PR, PR), F32),
            pltpu.VMEM((M, D), BF16),
            pltpu.VMEM((D,), BF16),
            pltpu.VMEM((1, D), BF16),
            pltpu.SemaphoreType.DMA((NSEM,)),
        ],
        compiler_params=pltpu.CompilerParams(
            vmem_limit_bytes=120 * 1024 * 1024, disable_bounds_checks=True,
            disable_semaphore_checks=True),
    )(
        A_x.reshape(NSEG, SEG, D),
        A_mem0.reshape(M, D),
        A_Wq, A_Wk, A_Wv,
        A_Wo.reshape(H * E, D),
        B_w_r,
        B_w_gate, B_w_up, B_w_down,
        c, w_mod,
    )
    return out.reshape(1, S, D)
```

```python
import jax
import jax.numpy as jnp
from jax import lax
import jax.experimental.pallas as pl
import jax.experimental.pallas.tpu as pltpu

BF16 = jnp.bfloat16
F32 = jnp.float32
U32 = jnp.uint32

S = 2048
D = 1024
H = 32
E = 128
M = 8
SEG = 32
NSEG = S // SEG
NPAIR = H // 2
NGP = 3 * NPAIR
F = 3584
DB = D // 128
FB = F // 128
PR = 2 * SEG + 2 * M
UNR = SEG // M
NIT = NSEG // UNR
PEEL = 3
PPI = 5
EARLY = 18
EPI_LATE = 6
EPI_PIECES = (0, 0, 2, 2, 2, 2, 2, 2, 2)
EPS = 1e-5
SCALE = E ** (-0.5)

SEM_SMALL = 0
SEM_X = SEM_SMALL + 3
SEM_MOD = SEM_X + 3
SEM_ST = SEM_MOD + 2
SEM_WO = SEM_ST + 2 + (NGP - PEEL) // PPI
SEM_MOE = SEM_WO + 1
SEM_OUT = SEM_MOE + 3
NSEM = SEM_OUT + 3


def _rb(v):
    return v.astype(BF16).astype(F32)


def _dot(a, b):
    return jnp.dot(a, b, preferred_element_type=F32)


def _recip(x):
    r = pl.reciprocal(x, approx=True)
    return r * (2.0 - x * r)


def _bf(words):
    return pltpu.bitcast(words, BF16)


def _ln(x):
    m = jnp.mean(x, axis=-1, keepdims=True)
    xc = x - m
    var = jnp.mean(xc * xc, axis=-1, keepdims=True)
    sd = _rb(jnp.sqrt(_rb(_rb(var) + EPS)))
    return _rb(_rb(x - _rb(m)) * (1.0 / sd))


def _ln_mod(x, scale1p, shift):
    return _rb(_rb(_ln(x) * scale1p) + shift)


def _fill_matrix():
    i = lax.broadcasted_iota(jnp.int32, (PR, PR), 0)
    j = lax.broadcasted_iota(jnp.int32, (PR, PR), 1)

    def head(t):
        return jnp.where(t < 2 * SEG, t >> 5, (t - 2 * SEG) >> 3)

    def pos(t):
        r = t & (SEG - 1)
        return jnp.where(t < 2 * SEG, jnp.where(r < M, r, r + M), M + (t & (M - 1)))

    same = head(i) == head(j)
    pi = pos(i)
    ok = jnp.where(pi < M, 1, jnp.where(pi >= pos(j), 1, 0))
    return jnp.where(same, jnp.where(ok == 1, 0.0, -1e9), -3e38).astype(F32)


def _kernel(x_hbm, mem0_hbm, wq_hbm, wk_hbm, wv_hbm, wo_hbm, wr_hbm, wg_hbm, wu_hbm, wd_hbm,
            c_hbm, wmod_hbm, out_hbm,
            x_v, w_v, wo_v, cache, odef, lhs_v, qkv_s, o_s, a_all, x1_v, h2_v, out_v, r_v, mod_v, fill_v, never_v,
            mem0_v, wr_v, c_v, sems):
    w_w = w_v.bitcast(U32)
    cache_w = cache.bitcast(U32)
    lhs_w = lhs_v.bitcast(U32)
    qkv_w = qkv_s.bitcast(U32)
    o_w = o_s.bitcast(U32)
    odef_w = odef.bitcast(U32)

    def copy(src, dst, sem):
        return pltpu.make_async_copy(src, dst, sems.at[sem])

    def wait_all(buf, sem):
        copy(buf, buf, sem).wait()

    def mod_row(k, rows=8):
        v = mod_v[k]
        return v if rows == 8 else jnp.concatenate([v] * (rows // 8), axis=0)

    def put_rows(dst, r0, v):
        for j in range(DB):
            dst[j, pl.ds(r0, v.shape[0]), :] = v[:, j * 128:(j + 1) * 128].astype(BF16)

    def ln1(seg, r0):
        xt = x_v[seg, pl.ds(r0, 8), :].astype(F32)
        return _ln_mod(xt, mod_row(1), mod_row(0))

    x_tail = copy(x_hbm.at[pl.ds(1, NSEG - 1), pl.ds(M, SEG - M), :],
                  x_v.at[pl.ds(1, NSEG - 1), pl.ds(M, SEG - M), :], SEM_X + 2)

    def prologue(stage, wmod_v, hc, n_v):
        wmod_w = wmod_hbm.bitcast(U32)
        small = [copy(c_hbm, c_v, SEM_SMALL), copy(mem0_hbm, mem0_v, SEM_SMALL + 1),
                 copy(wr_hbm, wr_v, SEM_SMALL + 2)]
        x_head = copy(x_hbm.at[:, pl.ds(0, M), :], x_v.at[:, pl.ds(0, M), :], SEM_X)
        x_seg0 = copy(x_hbm.at[0, pl.ds(M, SEG - M), :], x_v.at[0, pl.ds(M, SEG - M), :], SEM_X + 1)
        for cp in small:
            cp.start()
        x_head.start()
        x_seg0.start()
        mod_cps = [copy(wmod_hbm.at[:, pl.ds(k * D, D)], wmod_v.at[k], SEM_MOD + k) for k in range(2)]
        mod_cps[1].start()
        mod_cps[0].start()
        slab_cps = []
        for m_i, w_hbm in enumerate((wq_hbm, wk_hbm, wv_hbm)):
            wb = w_hbm.bitcast(U32)
            for p in range(NPAIR):
                gp = m_i * NPAIR + p
                batch = min(gp, 1) if gp < PEEL else 2 + (gp - PEEL) // PPI
                slab_cps.append(copy(wb.at[:, p, :], stage.at[gp], SEM_ST + batch))
        for cp in slab_cps[:EARLY]:
            cp.start()

        fill_v[...] = _fill_matrix()
        a_all[pl.ds(0, UNR + 1)] = jnp.zeros((UNR + 1, SEG, D), BF16)
        r_v[...] = jnp.full(r_v.shape, -jnp.inf, F32)
        never_v[...] = jnp.zeros(never_v.shape, F32)
        qkv_s[0] = jnp.zeros((2 * SEG, E), BF16)
        o_s[0] = jnp.zeros((SEG, E), BF16)

        for cp in small:
            cp.wait()
        c = c_v[...].astype(F32)
        sc = jnp.broadcast_to(_rb(c * jax.nn.sigmoid(c)), (16, D))
        zero = jnp.zeros((M, E), F32)
        for h in range(H):
            blk = sc[0:M, (h % DB) * 128:(h % DB + 1) * 128]
            odef[0, h] = jnp.concatenate(
                [blk if c_ == h // DB else zero for c_ in range(4)], axis=0).astype(BF16)
        sc = sc.astype(BF16)
        mod_v[6] = jnp.broadcast_to(wr_v[...].astype(F32).reshape(1, D), (8, D))
        put_rows(lhs_v, 0, mem0_v[...].astype(F32))

        def do_mod(k):
            mod_cps[k].wait()
            v = _rb(_dot(sc, wmod_v[k])[0:8])
            mod_v[k] = _rb(1.0 + v) if k == 1 else v

        x_head.wait()
        x_seg0.wait()
        NB = 16
        RB = NSEG * M // NB
        for b in range(NB):
            xb = x_v[pl.ds(b * (NSEG // NB), NSEG // NB), pl.ds(0, M), :].astype(F32).reshape(RB, D)
            n_v[pl.ds(b * RB, RB), :] = _ln(xb)
        n_v[pl.ds(NSEG * M, SEG - M), :] = _ln(x_v[0, pl.ds(M, SEG - M), :].astype(F32))
        do_mod(1)
        for b in range(NB):
            n_v[pl.ds(b * RB, RB), :] = _rb(n_v[pl.ds(b * RB, RB), :] * mod_row(1, RB))
        n_v[pl.ds(NSEG * M, SEG - M), :] = _rb(n_v[pl.ds(NSEG * M, SEG - M), :] * mod_row(1, SEG - M))
        do_mod(0)
        for b in range(NB):
            put_rows(hc, b * RB, n_v[pl.ds(b * RB, RB), :] + mod_row(0, RB))
        put_rows(lhs_v, M, n_v[pl.ds(NSEG * M, SEG - M), :] + mod_row(0, SEG - M))

        hc_w = hc.bitcast(U32)

        def slab(gp):
            b = stage[gp]
            w_v[2 * gp] = pltpu.bitcast(b << 16, F32).astype(BF16)
            w_v[2 * gp + 1] = pltpu.bitcast(b & jnp.uint32(0xFFFF0000), F32).astype(BF16)
            hcv = jnp.concatenate([_bf(hc_w[j]) for j in range(DB)], axis=1)
            r1 = _dot(hcv, _bf(w_w[2 * gp])).reshape(NSEG, M, E)
            r2 = _dot(hcv, _bf(w_w[2 * gp + 1])).reshape(NSEG, M, E)
            cache[gp] = jnp.concatenate([r1, r2], axis=1).reshape(NIT, UNR * 2 * M, E).astype(BF16)

        slab_cps[0].wait()
        slab(0)
        wait_all(stage.at[pl.ds(1, PEEL - 1)], SEM_ST + 1)
        for cp in slab_cps[EARLY:]:
            cp.start()
        x_tail.start()
        for gp in range(1, PEEL):
            slab(gp)

        def pro_body(i, carry):
            g0 = PEEL + i * PPI
            wait_all(stage.at[pl.ds(g0, PPI)], SEM_ST + 2 + i)

            @pl.when(i == 3)
            def _():
                wo_w = wo_hbm.bitcast(U32)
                for j in range(DB):
                    for c_ in range(4):
                        copy(wmod_w.at[:, pl.ds((2 + c_) * D + j * 128, 128)],
                             wo_v.at[j, pl.ds(c_ * (D // 2), D // 2), :], SEM_WO).start()
                for j in range(DB):
                    copy(wo_w.at[:, pl.ds(j * 128, 128)], wo_v.at[DB + j], SEM_WO).start()

            for t in range(PPI):
                slab(g0 + t)
            return carry

        lax.fori_loop(0, (NGP - PEEL) // PPI, pro_body, 0)

    pl.run_scoped(
        prologue,
        pltpu.VMEM((NGP, D, E), U32),
        pltpu.VMEM((2, D, D), BF16),
        pltpu.VMEM((DB, NSEG * M, E), BF16),
        pltpu.VMEM((NSEG * M + SEG - M, D), F32),
    )

    lane = lax.broadcasted_iota(jnp.int32, (8, 2 * 128), 1)

    def post(seg, q, keep=True):
        rows = pl.ds(8 * q, 8)
        x = x_v[seg, rows, :].astype(F32)
        a = a_all[seg + UNR, rows, :].astype(F32)
        x1 = _rb(x + _rb(mod_row(2) * a))
        h2 = _ln_mod(x1, mod_row(4), mod_row(3))
        r = _rb(jnp.sum(h2 * mod_row(6), axis=-1, keepdims=True))
        if keep:
            r_v[...] = jnp.where(lane == seg * 4 + q, r, r_v[...])
        x1_v[seg, rows, :] = x1.astype(BF16)
        h2_v[seg, rows, :] = h2.astype(BF16)
        o = x1 + _rb(mod_row(5) * h2)
        out_v[seg, rows, :] = o.astype(BF16)
        return o, r

    def deferred(blk, wsel, j, tok=None, tok2=None):
        words = [odef_w[blk, h] for h in range(H)]
        if tok is not None:
            top = jnp.where(never_v[...] > 1.0, pltpu.bitcast(tok, U32), words[-1][0:8])
            words[-1] = jnp.concatenate([top, words[-1][8:]], axis=0)
        lhs = jnp.concatenate([_bf(w) for w in words], axis=1)
        res = _dot(lhs, _bf(wo_v[wsel + j]))
        if tok2 is not None:
            res = jnp.concatenate([jnp.where(never_v[...] > 1.0, tok2, res[0:8]), res[8:]], axis=0)
        res = res.astype(BF16).reshape(UNR, M, 128)
        a_all[pl.ds(blk * UNR, UNR), pl.ds(0, M), pl.ds(j * 128, 128)] = res

    def out_copy(grp):
        return copy(out_v.at[pl.ds(grp * UNR, UNR)], out_hbm.at[pl.ds(grp * UNR, UNR)], SEM_OUT)

    def fold(v):
        t = v[:, 0:128]
        for j in range(1, DB):
            t = t + v[:, j * 128:(j + 1) * 128]
        return t

    def main(wg_v, wu_v, wd_v):
        wg_w, wu_w, wd_w = wg_hbm.bitcast(U32), wu_hbm.bitcast(U32), wd_hbm.bitcast(U32)
        for j in range(FB):
            copy(wg_w.at[:, pl.ds(j * 128, 128)], wg_v.at[j], SEM_MOE).start()
            copy(wu_w.at[:, pl.ds(j * 128, 128)], wu_v.at[j], SEM_MOE + 1).start()
        for j in range(DB):
            copy(wd_w.at[:, pl.ds(j * 128, 128)], wd_v.at[j], SEM_MOE + 2).start()
        x_tail.wait()
        wait_all(wo_v, SEM_WO)

        def step(it, u):
            s = it * UNR + u
            lhs = jnp.concatenate([_bf(lhs_w[j]) for j in range(DB)], axis=1)
            nseg = jnp.minimum(s + 1, NSEG - 1)

            def side(p):
                if p % 2 == 0 or p < 3:
                    return None
                i = p // 2 - 1
                if i < 4:
                    lag = 2 * UNR if i == 0 else UNR
                    o, r = post(jnp.maximum(s - lag, 0), i)
                    return fold(o) + r
                r0 = (i - 3) * 8
                h = ln1(nseg, r0)
                put_rows(lhs_v, r0, h)
                return fold(h)

            def proj(m_i, p):
                g = m_i * NPAIR + p
                for t in range(2):
                    qkv_s[g, pl.ds(t * SEG, SEG), :] = _dot(lhs, _bf(w_w[2 * g + t])).astype(BF16)

            def rows_of(m_i, p):
                g = m_i * NPAIR + p
                return jnp.concatenate([_bf(qkv_w[g]), _bf(cache_w[g, it, pl.ds(u * M, M), :])], axis=0)

            def probs(p):
                q = rows_of(0, p)
                k = rows_of(1, p)
                sc = lax.dot_general(q, k, (((1,), (1,)), ((), ())), preferred_element_type=F32) * SCALE
                fm = fill_v[...]
                tok = side(p)
                if tok is not None:
                    top = fm[0:8]
                    fm = jnp.concatenate([jnp.where(top > 1.0, tok[:, 0:PR], top), fm[8:]], axis=0)
                sc = jnp.where(fm == 0.0, sc, fm)
                e = jnp.exp(sc - jnp.max(sc, axis=-1, keepdims=True))
                return (e * _recip(jnp.sum(e, axis=-1, keepdims=True))).astype(BF16)

            def attend(p, pr):
                o = _dot(pr, rows_of(2, p))
                o_s[2 * p] = o[0:SEG].astype(BF16)
                o_s[2 * p + 1] = o[SEG:2 * SEG].astype(BF16)
                odef[it + 1, 2 * p, pl.ds(u * M, M), :] = o[2 * SEG:2 * SEG + M].astype(BF16)
                odef[it + 1, 2 * p + 1, pl.ds(u * M, M), :] = o[2 * SEG + M:].astype(BF16)

            wsel = jnp.where(it == 0, 0, DB)
            for t in range(DB // UNR):
                deferred(it, wsel, u * (DB // UNR) + t)
            ps = {}
            for pa in range(0, NPAIR, 2):
                pb = pa + 1
                proj(0, pa)
                proj(1, pa)
                proj(0, pb)
                proj(1, pb)
                proj(2, pa)
                proj(2, pb)
                ps[pa] = probs(pa)
                ps[pb] = probs(pb)
                if pa >= 2:
                    attend(pa - 2, ps.pop(pa - 2))
                    attend(pb - 2, ps.pop(pb - 2))
            L = NPAIR - 1

            HA = 24
            acc = [None] * DB
            for h0, h1 in ((0, HA), (HA, H)):
                for j in range(DB):
                    ol = jnp.concatenate([_bf(o_w[h]) for h in range(h0, h1)], axis=1)
                    part = _dot(ol, _bf(wo_v[DB + j, pl.ds(h0 * E // 2, (h1 - h0) * E // 2), :]))
                    if h0 == 0:
                        acc[j] = part
                    else:
                        a = part + acc[j]
                        lhs_v[j, pl.ds(0, M), :] = a[0:M].astype(BF16)
                        a_all[s + UNR, pl.ds(M, SEG - M), pl.ds(j * 128, 128)] = a[M:].astype(BF16)
                    if h0 == 0 and j == 4:
                        attend(L - 1, ps.pop(L - 1))
                        attend(L, ps.pop(L))

        def iteration(it, carry):
            @pl.when(it >= 3)
            def _():
                out_copy(it - 3).start()

            for c_ in range(4):
                v = a_all[c_, pl.ds(0, M), :].astype(F32)
                mod_v[2 + c_] = _rb(1.0 + v) if c_ == 2 else v
            for u in range(UNR):
                step(it, u)
            return carry

        lax.fori_loop(0, NIT, iteration, 0)

        out_copy(NIT - 3).start()
        for k, buf in enumerate((wg_v, wu_v, wd_v)):
            wait_all(buf, SEM_MOE + k)
        early = [(seg, 0) for seg in range(NSEG - 2 * UNR, NSEG - UNR)]
        early += [(seg, q) for seg in range(NSEG - UNR, NSEG) for q in (1, 2, 3)]
        r8 = lax.broadcasted_iota(jnp.int32, (8, 1), 0)
        vals, idxs = [], []

        def pieces(n):
            tok = None
            for _ in range(n):
                seg, q = early.pop(0)
                keep = len(early) >= EPI_LATE
                o, r = post(seg, q, keep)
                if not keep:
                    vals.append(r)
                    idxs.append((r8 + (seg * SEG + q * 8)).astype(F32))
                tok = fold(o) + r if tok is None else tok + fold(o) + r
            return tok

        for j in range(DB):
            deferred(NIT, DB, j, pieces(EPI_PIECES[j]), pieces(EPI_PIECES[DB]) if j == DB - 1 else None)
        out_copy(NIT - 2).start()

        def top2(vals, idx, axes):
            def red(f, v):
                for ax in axes:
                    v = f(v, axis=ax, keepdims=True)
                return v
            m1 = red(jnp.max, vals)
            i1 = red(jnp.min, jnp.where(vals == m1, idx, S - 1.0))
            rest = jnp.where(idx == i1, -jnp.inf, vals)
            m2 = red(jnp.max, rest)
            i2 = red(jnp.min, jnp.where(rest == m2, jnp.where(idx == i1, S - 1.0, idx), S - 1.0))
            return m1, i1, m2, i2

        m1, i1v, m2, i2v = top2(r_v[...], (lane * 8 + r8).astype(F32), (1, 0))
        vals.append(jnp.where(r8 == 0, m1, jnp.where(r8 == 1, m2, -jnp.inf)))
        idxs.append(jnp.where(r8 == 0, i1v, jnp.where(r8 == 1, i2v, S - 1.0)))
        for seg, q in early + [(seg, 0) for seg in range(NSEG - UNR, NSEG)]:
            vals.append(post(seg, q, keep=False)[1])
            idxs.append((r8 + (seg * SEG + q * 8)).astype(F32))
        out_copy(NIT - 1).start()
        m1, i1v, m2, i2v = top2(jnp.concatenate(vals, axis=0), jnp.concatenate(idxs, axis=0), (0,))
        i1 = i1v.astype(jnp.int32)[0, 0]
        i2 = i2v.astype(jnp.int32)[0, 0]

        def tile_of(i):
            return i >> 5, pl.multiple_of(((i >> 3) & 3) * 8, 8)

        sel = [tile_of(i1), tile_of(i2)]
        x1s = jnp.concatenate([x1_v[sg, pl.ds(r0, 8), :].astype(F32) for sg, r0 in sel], axis=0)
        h2s = jnp.concatenate([h2_v[sg, pl.ds(r0, 8), :].astype(F32) for sg, r0 in sel], axis=0)
        h2b = h2s.astype(BF16)
        gus = []
        for j in range(FB):
            g = _rb(_dot(h2b, _bf(wg_v[j])))
            g = _rb(g * jax.nn.sigmoid(g))
            u = _rb(_dot(h2b, _bf(wu_v[j])))
            gus.append(g * u)
        gu = jnp.concatenate(gus, axis=1).astype(BF16)
        y = jnp.concatenate([_rb(_dot(gu, _bf(wd_v[j]))) for j in range(DB)], axis=1)
        rows = lax.broadcasted_iota(jnp.int32, (16, 1), 0)
        rs = _rb(jax.nn.sigmoid(jnp.where(rows < 8, m1, m2)))
        y = _rb(y * rs)
        full = x1s + _rb(mod_row(5, 16) * _rb(h2s + y))

        copy(out_v, out_hbm, SEM_OUT).wait()
        for t, (i, (sg, r0)) in enumerate(zip((i1, i2), sel)):
            old = out_v[sg, pl.ds(r0, 8), :].astype(F32)
            new = jnp.where(r8 == (i & 7), full[t * 8:(t + 1) * 8], old)
            out_v[sg, pl.ds(r0, 8), :] = new.astype(BF16)
        fix = [copy(out_v.at[sg, pl.ds(r0, 8), :], out_hbm.at[sg, pl.ds(r0, 8), :], SEM_OUT + 1 + t)
               for t, (sg, r0) in enumerate(sel)]
        differ = (i1 >> 3) != (i2 >> 3)
        fix[0].start()

        @pl.when(differ)
        def _():
            fix[1].start()
            fix[1].wait()

        fix[0].wait()

    pl.run_scoped(
        main,
        pltpu.VMEM((FB, D // 2, 128), U32),
        pltpu.VMEM((FB, D // 2, 128), U32),
        pltpu.VMEM((DB, F // 2, 128), U32),
    )


@jax.jit
def pallas_adaLN_cond__memory_aug_recurrent_mem_tr__moe_arch_mod__prompt_kernel(
    A_x: jax.Array,
    A_mem0: jax.Array,
    A_Wq: jax.Array,
    A_Wk: jax.Array,
    A_Wv: jax.Array,
    A_Wo: jax.Array,
    A_seg_len: jax.Array,
    B_x: jax.Array,
    B_w_r: jax.Array,
    B_w_gate: jax.Array,
    B_w_up: jax.Array,
    B_w_down: jax.Array,
    c: jax.Array,
    w_mod: jax.Array,
):
    del A_seg_len, B_x
    assert A_x.shape == (1, S, D) and A_mem0.shape == (1, M, D) and A_Wq.shape == (D, H, E)
    hbm = pl.BlockSpec(memory_space=pl.ANY)
    out = pl.pallas_call(
        _kernel,
        out_shape=jax.ShapeDtypeStruct((NSEG, SEG, D), BF16),
        in_specs=[hbm] * 12,
        out_specs=hbm,
        scratch_shapes=[
            pltpu.VMEM((NSEG, SEG, D), BF16),
            pltpu.VMEM((3 * H, D, E), BF16),
            pltpu.VMEM((2 * DB, H * E // 2, 128), U32),
            pltpu.VMEM((NGP, NIT, UNR * 2 * M, E), BF16),
            pltpu.VMEM((NIT + 1, H, SEG, E), BF16),
            pltpu.VMEM((DB, SEG, 128), BF16),
            pltpu.VMEM((NGP, 2 * SEG, E), BF16),
            pltpu.VMEM((H, SEG, E), BF16),
            pltpu.VMEM((NSEG + UNR, SEG, D), BF16),
            pltpu.VMEM((NSEG, SEG, D), BF16),
            pltpu.VMEM((NSEG, SEG, D), BF16),
            pltpu.VMEM((NSEG, SEG, D), BF16),
            pltpu.VMEM((8, S // 8), F32),
            pltpu.VMEM((7, 8, D), F32),
            pltpu.VMEM((PR, PR), F32),
            pltpu.VMEM((8, 128), F32),
            pltpu.VMEM((M, D), BF16),
            pltpu.VMEM((D,), BF16),
            pltpu.VMEM((1, D), BF16),
            pltpu.SemaphoreType.DMA((NSEM,)),
        ],
        compiler_params=pltpu.CompilerParams(
            vmem_limit_bytes=120 * 1024 * 1024, disable_bounds_checks=True,
            disable_semaphore_checks=True),
    )(
        A_x.reshape(NSEG, SEG, D),
        A_mem0.reshape(M, D),
        A_Wq, A_Wk, A_Wv,
        A_Wo.reshape(H * E, D),
        B_w_r,
        B_w_gate, B_w_up, B_w_down,
        c, w_mod,
    )
    return out.reshape(1, S, D)
```

```python
import jax
import jax.numpy as jnp
from jax import lax
import jax.experimental.pallas as pl
import jax.experimental.pallas.tpu as pltpu

BF16 = jnp.bfloat16
F32 = jnp.float32
U32 = jnp.uint32

S = 2048
D = 1024
H = 32
E = 128
M = 8
SEG = 32
NSEG = S // SEG
NPAIR = H // 2
NGP = 3 * NPAIR
F = 3584
DB = D // 128
FB = F // 128
PR = 2 * SEG + 2 * M
UNR = SEG // M
NIT = NSEG // UNR
KMAJ = 12
AHEAD = 3
PPI = 6
EPI_LATE = 6
EPI_PIECES = (0, 0, 2, 2, 2, 2, 2, 2, 2)
EPS = 1e-5
SCALE = E ** (-0.5)

SEM_SMALL = 0
SEM_X = SEM_SMALL + 3
SEM_MOD = SEM_X + 3
SEM_WQ = SEM_MOD + DB
SEM_ST = SEM_WQ + DB
SEM_WO = SEM_ST + (NGP - KMAJ) // PPI
SEM_MOE = SEM_WO + 1
SEM_OUT = SEM_MOE + 3
NSEM = SEM_OUT + 3


def _rb(v):
    return v.astype(BF16).astype(F32)


def _dot(a, b):
    return jnp.dot(a, b, preferred_element_type=F32)


def _recip(x):
    r = pl.reciprocal(x, approx=True)
    return r * (2.0 - x * r)


def _bf(words):
    return pltpu.bitcast(words, BF16)


def _ln(x):
    m = jnp.mean(x, axis=-1, keepdims=True)
    xc = x - m
    var = jnp.mean(xc * xc, axis=-1, keepdims=True)
    sd = _rb(jnp.sqrt(_rb(_rb(var) + EPS)))
    return _rb(_rb(x - _rb(m)) * (1.0 / sd))


def _ln_mod(x, scale1p, shift):
    return _rb(_rb(_ln(x) * scale1p) + shift)


def _fill_matrix():
    i = lax.broadcasted_iota(jnp.int32, (PR, PR), 0)
    j = lax.broadcasted_iota(jnp.int32, (PR, PR), 1)

    def head(t):
        return jnp.where(t < 2 * SEG, t >> 5, (t - 2 * SEG) >> 3)

    def pos(t):
        r = t & (SEG - 1)
        return jnp.where(t < 2 * SEG, jnp.where(r < M, r, r + M), M + (t & (M - 1)))

    same = head(i) == head(j)
    pi = pos(i)
    ok = jnp.where(pi < M, 1, jnp.where(pi >= pos(j), 1, 0))
    return jnp.where(same, jnp.where(ok == 1, 0.0, -1e9), -3e38).astype(F32)


def _kernel(x_hbm, mem0_hbm, wq_hbm, wk_hbm, wv_hbm, wo_hbm, wr_hbm, wg_hbm, wu_hbm, wd_hbm,
            c_hbm, wmod_hbm, out_hbm,
            x_v, w_v, wo_v, cache, odef, lhs_v, qkv_s, o_s, a_all, r_v, mod_v, fill_v, never_v,
            mem0_v, wr_v, c_v, sems):
    w_w = w_v.bitcast(U32)
    cache_w = cache.bitcast(U32)
    lhs_w = lhs_v.bitcast(U32)
    qkv_w = qkv_s.bitcast(U32)
    o_w = o_s.bitcast(U32)
    odef_w = odef.bitcast(U32)

    def copy(src, dst, sem):
        return pltpu.make_async_copy(src, dst, sems.at[sem])

    def wait_all(buf, sem):
        copy(buf, buf, sem).wait()

    def mod_row(k, rows=8):
        v = mod_v[k]
        return v if rows == 8 else jnp.concatenate([v] * (rows // 8), axis=0)

    def put_rows(dst, r0, v):
        for j in range(DB):
            dst[j, pl.ds(r0, v.shape[0]), :] = v[:, j * 128:(j + 1) * 128].astype(BF16)

    def ln1(seg, r0):
        xt = x_v[seg, pl.ds(r0, 8), :].astype(F32)
        return _ln_mod(xt, mod_row(1), mod_row(0))

    x_tail = copy(x_hbm.at[pl.ds(1, NSEG - 1), pl.ds(M, SEG - M), :],
                  x_v.at[pl.ds(1, NSEG - 1), pl.ds(M, SEG - M), :], SEM_X + 2)

    def prologue(stage, wmod_v, hc, n_v, acc):
        wmod_w = wmod_hbm.bitcast(U32)
        w_words = [w.bitcast(U32) for w in (wq_hbm, wk_hbm, wv_hbm)]

        def start_mod(j):
            col = j * 128 if isinstance(j, int) else pl.multiple_of(j * 128, 128)
            for k in range(2):
                copy(wmod_w.at[:, pl.ds(k * D + col, 128)], wmod_v.at[j, k], SEM_MOD + j).start()

        def start_ktile(j):
            rows = pl.ds(j * 128 if isinstance(j, int) else pl.multiple_of(j * 128, 128), 128)
            for g in range(KMAJ):
                copy(w_words[0].at[rows, g, :], stage.at[g, rows, :], SEM_WQ + j).start()

        small = [copy(c_hbm, c_v, SEM_SMALL), copy(mem0_hbm, mem0_v, SEM_SMALL + 1),
                 copy(wr_hbm, wr_v, SEM_SMALL + 2)]
        x_head = copy(x_hbm.at[:, pl.ds(0, M), :], x_v.at[:, pl.ds(0, M), :], SEM_X)
        x_seg0 = copy(x_hbm.at[0, pl.ds(M, SEG - M), :], x_v.at[0, pl.ds(M, SEG - M), :], SEM_X + 1)
        for cp in small:
            cp.start()
        x_head.start()
        x_seg0.start()
        start_mod(0)
        for j in range(AHEAD):
            start_ktile(j)
            start_mod(j + 1)
        slab_cps = [copy(w_words[g // NPAIR].at[:, g % NPAIR, :], stage.at[g], SEM_ST + (g - KMAJ) // PPI)
                    for g in range(KMAJ, NGP)]

        fill_v[...] = _fill_matrix()
        a_all[pl.ds(0, UNR + 1)] = jnp.zeros((UNR + 1, SEG, D), BF16)
        r_v[...] = jnp.full(r_v.shape, -jnp.inf, F32)
        never_v[...] = jnp.zeros(never_v.shape, F32)
        qkv_s[0] = jnp.zeros((2 * SEG, E), BF16)
        o_s[0] = jnp.zeros((SEG, E), BF16)

        def zero_acc(h, carry):
            acc[h] = jnp.zeros((NSEG * M, E), F32)
            return carry

        lax.fori_loop(0, 2 * KMAJ, zero_acc, 0)

        for cp in small:
            cp.wait()
        c = c_v[...].astype(F32)
        sc = jnp.broadcast_to(_rb(c * jax.nn.sigmoid(c)), (M, D))
        zero = jnp.zeros((M, E), F32)
        for h in range(H):
            blk = sc[:, (h % DB) * 128:(h % DB + 1) * 128]
            odef[0, h] = jnp.concatenate(
                [blk if c_ == h // DB else zero for c_ in range(4)], axis=0).astype(BF16)
        mod_v[6] = jnp.broadcast_to(wr_v[...].astype(F32).reshape(1, D), (8, D))
        put_rows(lhs_v, 0, mem0_v[...].astype(F32))

        x_head.wait()
        x_seg0.wait()
        NB = 16
        RB = NSEG * M // NB
        NR = NSEG * M + SEG - M
        for b in range(NB + 1):
            if b < NB:
                xb = x_v[pl.ds(b * (NSEG // NB), NSEG // NB), pl.ds(0, M), :].astype(F32).reshape(RB, D)
            else:
                xb = x_v[0, pl.ds(M, SEG - M), :].astype(F32)
            nb = _ln(xb)
            for j in range(DB):
                n_v[j, pl.ds(b * RB, nb.shape[0]), :] = nb[:, j * 128:(j + 1) * 128]

        hc_w = hc.bitcast(U32)

        def mod_block(j, k):
            scb = jnp.concatenate([_bf(odef_w[0, h, pl.ds(0, 8), :]) for h in range(DB)], axis=1)
            v = _rb(_dot(scb, _bf(wmod_v[j, k]))[0:8])
            return _rb(1.0 + v) if k == 1 else v

        def h_block(j, sa, ca):
            col = j * 128 if isinstance(j, int) else pl.multiple_of(j * 128, 128)
            mod_v[0, :, pl.ds(col, 128)] = sa
            mod_v[1, :, pl.ds(col, 128)] = ca
            n = n_v[j].reshape(NR // 8, 8, 128)
            hv = (_rb(n * ca[None]) + sa[None]).reshape(NR, 128).astype(BF16)
            hc[j] = hv[0:NSEG * M]
            lhs_v[j, pl.ds(M, SEG - M), :] = hv[NSEG * M:]

        def pack_pair(r1, r2):
            r = jnp.concatenate([r1.reshape(NSEG, M, E), r2.reshape(NSEG, M, E)], axis=1)
            return r.reshape(NIT, UNR * 2 * M, E).astype(BF16)

        def split_pair(b):
            return (pltpu.bitcast(b << 16, F32).astype(BF16),
                    pltpu.bitcast(b & jnp.uint32(0xFFFF0000), F32).astype(BF16))

        def q_stage(j, last):
            static = isinstance(j, int)
            k0 = j * 128 if static else pl.multiple_of(j * 128, 128)
            w0 = j * 64 if static else pl.multiple_of(j * 64, 64)
            nxt = {}
            for p in range(KMAJ):
                ws = split_pair(stage[p, pl.ds(k0, 128), :])
                rs = []
                for t in range(2):
                    h = 2 * p + t
                    w_v[h, pl.ds(k0, 128), :] = ws[t]
                    rs.append(_dot(_bf(hc_w[j]), _bf(w_w[h, pl.ds(w0, 64), :])) + acc[h])
                    if not last:
                        acc[h] = rs[t]
                if last:
                    cache[p] = pack_pair(*rs)
                elif p in (1, 3):
                    nxt[p] = mod_block(j + 1, p // 2)
            if not last:
                h_block(j + 1, nxt[1], nxt[3])

        wait_all(wmod_v.at[0], SEM_MOD)
        h_block(0, mod_block(0, 0), mod_block(0, 1))

        def wait_ktile(j):
            wait_all(stage.at[pl.ds(0, KMAJ), pl.ds(0, 128), :], SEM_WQ + j)

        def q_body(j, carry):
            wait_ktile(j)
            wait_all(wmod_v.at[0], SEM_MOD + j + 1)

            @pl.when(j + AHEAD < DB)
            def _():
                start_ktile(j + AHEAD)

            @pl.when(j + AHEAD + 1 < DB)
            def _():
                start_mod(j + AHEAD + 1)

            @pl.when(j + AHEAD == DB)
            def _():
                for cp in slab_cps[:2 * PPI]:
                    cp.start()

            q_stage(j, False)
            return carry

        lax.fori_loop(0, DB - 1, q_body, 0)
        wait_ktile(DB - 1)
        for cp in slab_cps[2 * PPI:]:
            cp.start()
        x_tail.start()
        q_stage(DB - 1, True)

        def slab(gp):
            w_v[2 * gp], w_v[2 * gp + 1] = split_pair(stage[gp])
            hcv = jnp.concatenate([_bf(hc_w[j]) for j in range(DB)], axis=1)
            cache[gp] = pack_pair(_dot(hcv, _bf(w_w[2 * gp])), _dot(hcv, _bf(w_w[2 * gp + 1])))

        def pro_body(i, carry):
            g0 = KMAJ + i * PPI
            wait_all(stage.at[pl.ds(g0, PPI)], SEM_ST + i)

            @pl.when(i == 2)
            def _():
                wo_w = wo_hbm.bitcast(U32)
                for j in range(DB):
                    for c_ in range(4):
                        copy(wmod_w.at[:, pl.ds((2 + c_) * D + j * 128, 128)],
                             wo_v.at[j, pl.ds(c_ * (D // 2), D // 2), :], SEM_WO).start()
                for j in range(DB):
                    copy(wo_w.at[:, pl.ds(j * 128, 128)], wo_v.at[DB + j], SEM_WO).start()

            for t in range(PPI):
                slab(g0 + t)
            return carry

        lax.fori_loop(0, (NGP - KMAJ) // PPI, pro_body, 0)

    pl.run_scoped(
        prologue,
        pltpu.VMEM((NGP, D, E), U32),
        pltpu.VMEM((DB, 2, D // 2, 128), U32),
        pltpu.VMEM((DB, NSEG * M, E), BF16),
        pltpu.VMEM((DB, NSEG * M + SEG - M, 128), F32),
        pltpu.VMEM((2 * KMAJ, NSEG * M, E), F32),
    )

    def main(wg_v, wu_v, wd_v, x1_v, h2_v, out_v):
        lane = lax.broadcasted_iota(jnp.int32, (8, 2 * 128), 1)

        def post(seg, q, keep=True):
            rows = pl.ds(8 * q, 8)
            x = x_v[seg, rows, :].astype(F32)
            a = a_all[seg + UNR, rows, :].astype(F32)
            x1 = _rb(x + _rb(mod_row(2) * a))
            h2 = _ln_mod(x1, mod_row(4), mod_row(3))
            r = _rb(jnp.sum(h2 * mod_row(6), axis=-1, keepdims=True))
            if keep:
                r_v[...] = jnp.where(lane == seg * 4 + q, r, r_v[...])
            x1_v[seg, rows, :] = x1.astype(BF16)
            h2_v[seg, rows, :] = h2.astype(BF16)
            o = x1 + _rb(mod_row(5) * h2)
            out_v[seg, rows, :] = o.astype(BF16)
            return o, r

        def deferred(blk, wsel, j, tok=None, tok2=None):
            words = [odef_w[blk, h] for h in range(H)]
            if tok is not None:
                top = jnp.where(never_v[...] > 1.0, pltpu.bitcast(tok, U32), words[-1][0:8])
                words[-1] = jnp.concatenate([top, words[-1][8:]], axis=0)
            lhs = jnp.concatenate([_bf(w) for w in words], axis=1)
            res = _dot(lhs, _bf(wo_v[wsel + j]))
            if tok2 is not None:
                res = jnp.concatenate([jnp.where(never_v[...] > 1.0, tok2, res[0:8]), res[8:]], axis=0)
            res = res.astype(BF16).reshape(UNR, M, 128)
            a_all[pl.ds(blk * UNR, UNR), pl.ds(0, M), pl.ds(j * 128, 128)] = res

        def out_copy(grp):
            return copy(out_v.at[pl.ds(grp * UNR, UNR)], out_hbm.at[pl.ds(grp * UNR, UNR)], SEM_OUT)

        def fold(v):
            t = v[:, 0:128]
            for j in range(1, DB):
                t = t + v[:, j * 128:(j + 1) * 128]
            return t

        wg_w, wu_w, wd_w = wg_hbm.bitcast(U32), wu_hbm.bitcast(U32), wd_hbm.bitcast(U32)
        for j in range(FB):
            copy(wg_w.at[:, pl.ds(j * 128, 128)], wg_v.at[j], SEM_MOE).start()
            copy(wu_w.at[:, pl.ds(j * 128, 128)], wu_v.at[j], SEM_MOE + 1).start()
        for j in range(DB):
            copy(wd_w.at[:, pl.ds(j * 128, 128)], wd_v.at[j], SEM_MOE + 2).start()
        x_tail.wait()
        wait_all(wo_v, SEM_WO)

        def step(it, u):
            s = it * UNR + u
            lhs = jnp.concatenate([_bf(lhs_w[j]) for j in range(DB)], axis=1)
            nseg = jnp.minimum(s + 1, NSEG - 1)

            def side(p):
                if p % 2 == 0 or p < 3:
                    return None
                i = p // 2 - 1
                if i < 4:
                    lag = 2 * UNR if i == 0 else UNR
                    o, r = post(jnp.maximum(s - lag, 0), i)
                    return fold(o) + r
                r0 = (i - 3) * 8
                h = ln1(nseg, r0)
                put_rows(lhs_v, r0, h)
                return fold(h)

            def proj(m_i, p):
                g = m_i * NPAIR + p
                for t in range(2):
                    qkv_s[g, pl.ds(t * SEG, SEG), :] = _dot(lhs, _bf(w_w[2 * g + t])).astype(BF16)

            def rows_of(m_i, p):
                g = m_i * NPAIR + p
                return jnp.concatenate([_bf(qkv_w[g]), _bf(cache_w[g, it, pl.ds(u * M, M), :])], axis=0)

            def probs(p):
                q = rows_of(0, p)
                k = rows_of(1, p)
                sc = lax.dot_general(q, k, (((1,), (1,)), ((), ())), preferred_element_type=F32) * SCALE
                fm = fill_v[...]
                tok = side(p)
                if tok is not None:
                    top = fm[0:8]
                    fm = jnp.concatenate([jnp.where(top > 1.0, tok[:, 0:PR], top), fm[8:]], axis=0)
                sc = jnp.where(fm == 0.0, sc, fm)
                e = jnp.exp(sc - jnp.max(sc, axis=-1, keepdims=True))
                return (e * _recip(jnp.sum(e, axis=-1, keepdims=True))).astype(BF16)

            def attend(p, pr):
                o = _dot(pr, rows_of(2, p))
                o_s[2 * p] = o[0:SEG].astype(BF16)
                o_s[2 * p + 1] = o[SEG:2 * SEG].astype(BF16)
                odef[it + 1, 2 * p, pl.ds(u * M, M), :] = o[2 * SEG:2 * SEG + M].astype(BF16)
                odef[it + 1, 2 * p + 1, pl.ds(u * M, M), :] = o[2 * SEG + M:].astype(BF16)

            wsel = jnp.where(it == 0, 0, DB)
            for t in range(DB // UNR):
                deferred(it, wsel, u * (DB // UNR) + t)
            ps = {}
            for pa in range(0, NPAIR, 2):
                pb = pa + 1
                proj(0, pa)
                proj(1, pa)
                proj(0, pb)
                proj(1, pb)
                proj(2, pa)
                proj(2, pb)
                ps[pa] = probs(pa)
                ps[pb] = probs(pb)
                if pa >= 2:
                    attend(pa - 2, ps.pop(pa - 2))
                    attend(pb - 2, ps.pop(pb - 2))
            L = NPAIR - 1

            HA = 24
            acc = [None] * DB
            for h0, h1 in ((0, HA), (HA, H)):
                for j in range(DB):
                    ol = jnp.concatenate([_bf(o_w[h]) for h in range(h0, h1)], axis=1)
                    part = _dot(ol, _bf(wo_v[DB + j, pl.ds(h0 * E // 2, (h1 - h0) * E // 2), :]))
                    if h0 == 0:
                        acc[j] = part
                    else:
                        a = part + acc[j]
                        lhs_v[j, pl.ds(0, M), :] = a[0:M].astype(BF16)
                        a_all[s + UNR, pl.ds(M, SEG - M), pl.ds(j * 128, 128)] = a[M:].astype(BF16)
                    if h0 == 0 and j == 4:
                        attend(L - 1, ps.pop(L - 1))
                        attend(L, ps.pop(L))

        def iteration(it, carry):
            @pl.when(it >= 3)
            def _():
                out_copy(it - 3).start()

            for c_ in range(4):
                v = a_all[c_, pl.ds(0, M), :].astype(F32)
                mod_v[2 + c_] = _rb(1.0 + v) if c_ == 2 else v
            for u in range(UNR):
                step(it, u)
            return carry

        lax.fori_loop(0, NIT, iteration, 0)

        out_copy(NIT - 3).start()
        for k, buf in enumerate((wg_v, wu_v, wd_v)):
            wait_all(buf, SEM_MOE + k)
        early = [(seg, 0) for seg in range(NSEG - 2 * UNR, NSEG - UNR)]
        early += [(seg, q) for seg in range(NSEG - UNR, NSEG) for q in (1, 2, 3)]
        r8 = lax.broadcasted_iota(jnp.int32, (8, 1), 0)
        vals, idxs = [], []

        def pieces(n):
            tok = None
            for _ in range(n):
                seg, q = early.pop(0)
                keep = len(early) >= EPI_LATE
                o, r = post(seg, q, keep)
                if not keep:
                    vals.append(r)
                    idxs.append((r8 + (seg * SEG + q * 8)).astype(F32))
                tok = fold(o) + r if tok is None else tok + fold(o) + r
            return tok

        for j in range(DB):
            deferred(NIT, DB, j, pieces(EPI_PIECES[j]), pieces(EPI_PIECES[DB]) if j == DB - 1 else None)
        out_copy(NIT - 2).start()

        def top2(vals, idx, axes):
            def red(f, v):
                for ax in axes:
                    v = f(v, axis=ax, keepdims=True)
                return v
            m1 = red(jnp.max, vals)
            i1 = red(jnp.min, jnp.where(vals == m1, idx, S - 1.0))
            rest = jnp.where(idx == i1, -jnp.inf, vals)
            m2 = red(jnp.max, rest)
            i2 = red(jnp.min, jnp.where(rest == m2, jnp.where(idx == i1, S - 1.0, idx), S - 1.0))
            return m1, i1, m2, i2

        m1, i1v, m2, i2v = top2(r_v[...], (lane * 8 + r8).astype(F32), (1, 0))
        vals.append(jnp.where(r8 == 0, m1, jnp.where(r8 == 1, m2, -jnp.inf)))
        idxs.append(jnp.where(r8 == 0, i1v, jnp.where(r8 == 1, i2v, S - 1.0)))
        for seg, q in early + [(seg, 0) for seg in range(NSEG - UNR, NSEG)]:
            vals.append(post(seg, q, keep=False)[1])
            idxs.append((r8 + (seg * SEG + q * 8)).astype(F32))
        out_copy(NIT - 1).start()
        m1, i1v, m2, i2v = top2(jnp.concatenate(vals, axis=0), jnp.concatenate(idxs, axis=0), (0,))
        i1 = i1v.astype(jnp.int32)[0, 0]
        i2 = i2v.astype(jnp.int32)[0, 0]

        def tile_of(i):
            return i >> 5, pl.multiple_of(((i >> 3) & 3) * 8, 8)

        sel = [tile_of(i1), tile_of(i2)]
        x1s = jnp.concatenate([x1_v[sg, pl.ds(r0, 8), :].astype(F32) for sg, r0 in sel], axis=0)
        h2s = jnp.concatenate([h2_v[sg, pl.ds(r0, 8), :].astype(F32) for sg, r0 in sel], axis=0)
        h2b = h2s.astype(BF16)
        gus = []
        for j in range(FB):
            g = _rb(_dot(h2b, _bf(wg_v[j])))
            g = _rb(g * jax.nn.sigmoid(g))
            u = _rb(_dot(h2b, _bf(wu_v[j])))
            gus.append(g * u)
        gu = jnp.concatenate(gus, axis=1).astype(BF16)
        y = jnp.concatenate([_rb(_dot(gu, _bf(wd_v[j]))) for j in range(DB)], axis=1)
        rows = lax.broadcasted_iota(jnp.int32, (16, 1), 0)
        rs = _rb(jax.nn.sigmoid(jnp.where(rows < 8, m1, m2)))
        y = _rb(y * rs)
        full = x1s + _rb(mod_row(5, 16) * _rb(h2s + y))

        copy(out_v, out_hbm, SEM_OUT).wait()
        for t, (i, (sg, r0)) in enumerate(zip((i1, i2), sel)):
            old = out_v[sg, pl.ds(r0, 8), :].astype(F32)
            new = jnp.where(r8 == (i & 7), full[t * 8:(t + 1) * 8], old)
            out_v[sg, pl.ds(r0, 8), :] = new.astype(BF16)
        fix = [copy(out_v.at[sg, pl.ds(r0, 8), :], out_hbm.at[sg, pl.ds(r0, 8), :], SEM_OUT + 1 + t)
               for t, (sg, r0) in enumerate(sel)]
        differ = (i1 >> 3) != (i2 >> 3)
        fix[0].start()

        @pl.when(differ)
        def _():
            fix[1].start()
            fix[1].wait()

        fix[0].wait()

    pl.run_scoped(
        main,
        pltpu.VMEM((FB, D // 2, 128), U32),
        pltpu.VMEM((FB, D // 2, 128), U32),
        pltpu.VMEM((DB, F // 2, 128), U32),
        pltpu.VMEM((NSEG, SEG, D), BF16),
        pltpu.VMEM((NSEG, SEG, D), BF16),
        pltpu.VMEM((NSEG, SEG, D), BF16),
    )


@jax.jit
def pallas_adaLN_cond__memory_aug_recurrent_mem_tr__moe_arch_mod__prompt_kernel(
    A_x: jax.Array,
    A_mem0: jax.Array,
    A_Wq: jax.Array,
    A_Wk: jax.Array,
    A_Wv: jax.Array,
    A_Wo: jax.Array,
    A_seg_len: jax.Array,
    B_x: jax.Array,
    B_w_r: jax.Array,
    B_w_gate: jax.Array,
    B_w_up: jax.Array,
    B_w_down: jax.Array,
    c: jax.Array,
    w_mod: jax.Array,
):
    del A_seg_len, B_x
    assert A_x.shape == (1, S, D) and A_mem0.shape == (1, M, D) and A_Wq.shape == (D, H, E)
    hbm = pl.BlockSpec(memory_space=pl.ANY)
    out = pl.pallas_call(
        _kernel,
        out_shape=jax.ShapeDtypeStruct((NSEG, SEG, D), BF16),
        in_specs=[hbm] * 12,
        out_specs=hbm,
        scratch_shapes=[
            pltpu.VMEM((NSEG, SEG, D), BF16),
            pltpu.VMEM((3 * H, D, E), BF16),
            pltpu.VMEM((2 * DB, H * E // 2, 128), U32),
            pltpu.VMEM((NGP, NIT, UNR * 2 * M, E), BF16),
            pltpu.VMEM((NIT + 1, H, SEG, E), BF16),
            pltpu.VMEM((DB, SEG, 128), BF16),
            pltpu.VMEM((NGP, 2 * SEG, E), BF16),
            pltpu.VMEM((H, SEG, E), BF16),
            pltpu.VMEM((NSEG + UNR, SEG, D), BF16),
            pltpu.VMEM((8, S // 8), F32),
            pltpu.VMEM((7, 8, D), F32),
            pltpu.VMEM((PR, PR), F32),
            pltpu.VMEM((8, 128), F32),
            pltpu.VMEM((M, D), BF16),
            pltpu.VMEM((D,), BF16),
            pltpu.VMEM((1, D), BF16),
            pltpu.SemaphoreType.DMA((NSEM,)),
        ],
        compiler_params=pltpu.CompilerParams(
            vmem_limit_bytes=120 * 1024 * 1024, disable_bounds_checks=True,
            disable_semaphore_checks=True),
    )(
        A_x.reshape(NSEG, SEG, D),
        A_mem0.reshape(M, D),
        A_Wq, A_Wk, A_Wv,
        A_Wo.reshape(H * E, D),
        B_w_r,
        B_w_gate, B_w_up, B_w_down,
        c, w_mod,
    )
    return out.reshape(1, S, D)
```

```python
import jax
import jax.numpy as jnp
from jax import lax
import jax.experimental.pallas as pl
import jax.experimental.pallas.tpu as pltpu

BF16 = jnp.bfloat16
F32 = jnp.float32
U32 = jnp.uint32

S = 2048
D = 1024
H = 32
E = 128
M = 8
SEG = 32
NSEG = S // SEG
NPAIR = H // 2
NGP = 3 * NPAIR
F = 3584
DB = D // 128
FB = F // 128
PR = 2 * SEG + 2 * M
UNR = SEG // M
NIT = NSEG // UNR
KMAJ = 12
AHEAD = 3
PPI = 6
EPI_LATE = 6
EPI_PIECES = (0, 0, 2, 2, 2, 2, 2, 2, 2)
EPS = 1e-5
SCALE = E ** (-0.5)

SEM_SMALL = 0
SEM_X = SEM_SMALL + 3
SEM_MOD = SEM_X + 3
SEM_WQ = SEM_MOD + DB
SEM_ST = SEM_WQ + DB
SEM_WO = SEM_ST + (NGP - KMAJ) // PPI
SEM_MOE = SEM_WO + 1
SEM_OUT = SEM_MOE + 3
NSEM = SEM_OUT + 3


def _rb(v):
    return v.astype(BF16).astype(F32)


def _dot(a, b):
    return jnp.dot(a, b, preferred_element_type=F32)


def _recip(x):
    r = pl.reciprocal(x, approx=True)
    return r * (2.0 - x * r)


def _bf(words):
    return pltpu.bitcast(words, BF16)


def _ln(x):
    m = jnp.mean(x, axis=-1, keepdims=True)
    xc = x - m
    var = jnp.mean(xc * xc, axis=-1, keepdims=True)
    sd = _rb(jnp.sqrt(_rb(_rb(var) + EPS)))
    return _rb(_rb(x - _rb(m)) * (1.0 / sd))


def _ln_mod(x, scale1p, shift):
    return _rb(_rb(_ln(x) * scale1p) + shift)


def _fill_matrix():
    i = lax.broadcasted_iota(jnp.int32, (PR, PR), 0)
    j = lax.broadcasted_iota(jnp.int32, (PR, PR), 1)

    def head(t):
        return jnp.where(t < 2 * SEG, t >> 5, (t - 2 * SEG) >> 3)

    def pos(t):
        r = t & (SEG - 1)
        return jnp.where(t < 2 * SEG, jnp.where(r < M, r, r + M), M + (t & (M - 1)))

    same = head(i) == head(j)
    pi = pos(i)
    ok = jnp.where(pi < M, 1, jnp.where(pi >= pos(j), 1, 0))
    return jnp.where(same, jnp.where(ok == 1, 0.0, -1e9), -3e38).astype(F32)


def _kernel(x_hbm, mem0_hbm, wq_hbm, wk_hbm, wv_hbm, wo_hbm, wr_hbm, wg_hbm, wu_hbm, wd_hbm,
            c_hbm, wmod_hbm, out_hbm,
            x_v, w_v, wo_v, cache, odef, lhs_v, qkv_s, o_s, a_all, r_v, mod_v, fill_v, never_v,
            mem0_v, wr_v, c_v, sems):
    w_w = w_v.bitcast(U32)
    cache_w = cache.bitcast(U32)
    lhs_w = lhs_v.bitcast(U32)
    qkv_w = qkv_s.bitcast(U32)
    o_w = o_s.bitcast(U32)
    odef_w = odef.bitcast(U32)

    def weights(h):
        return _bf(w_w[h].reshape(D // 2, E))

    def copy(src, dst, sem):
        return pltpu.make_async_copy(src, dst, sems.at[sem])

    def wait_all(buf, sem):
        copy(buf, buf, sem).wait()

    def mod_row(k, rows=8):
        v = mod_v[k]
        return v if rows == 8 else jnp.concatenate([v] * (rows // 8), axis=0)

    def put_rows(dst, r0, v):
        for j in range(DB):
            dst[j, pl.ds(r0, v.shape[0]), :] = v[:, j * 128:(j + 1) * 128].astype(BF16)

    def ln1(seg, r0):
        xt = x_v[seg, pl.ds(r0, 8), :].astype(F32)
        return _ln_mod(xt, mod_row(1), mod_row(0))

    x_tail = copy(x_hbm.at[pl.ds(1, NSEG - 1), pl.ds(M, SEG - M), :],
                  x_v.at[pl.ds(1, NSEG - 1), pl.ds(M, SEG - M), :], SEM_X + 2)

    def prologue(stage, wmod_v, hc, n_v, acc):
        wmod_w = wmod_hbm.bitcast(U32)
        w_words = [w.bitcast(U32) for w in (wq_hbm, wk_hbm, wv_hbm)]

        def start_mod(j):
            col = j * 128 if isinstance(j, int) else pl.multiple_of(j * 128, 128)
            for k in range(2):
                copy(wmod_w.at[:, pl.ds(k * D + col, 128)], wmod_v.at[j, k], SEM_MOD + j).start()

        def start_ktile(j):
            rows = pl.ds(j * 128 if isinstance(j, int) else pl.multiple_of(j * 128, 128), 128)
            for g in range(KMAJ):
                copy(w_words[0].at[rows, g, :], stage.at[g, rows, :], SEM_WQ + j).start()

        small = [copy(c_hbm, c_v, SEM_SMALL), copy(mem0_hbm, mem0_v, SEM_SMALL + 1),
                 copy(wr_hbm, wr_v, SEM_SMALL + 2)]
        x_head = copy(x_hbm.at[:, pl.ds(0, M), :], x_v.at[:, pl.ds(0, M), :], SEM_X)
        x_seg0 = copy(x_hbm.at[0, pl.ds(M, SEG - M), :], x_v.at[0, pl.ds(M, SEG - M), :], SEM_X + 1)
        for cp in small:
            cp.start()
        x_head.start()
        x_seg0.start()
        start_mod(0)
        for j in range(AHEAD):
            start_ktile(j)
            start_mod(j + 1)
        slab_cps = [copy(w_words[g // NPAIR].at[:, g % NPAIR, :], stage.at[g], SEM_ST + (g - KMAJ) // PPI)
                    for g in range(KMAJ, NGP)]

        fill_v[...] = _fill_matrix()
        a_all[pl.ds(0, UNR + 1)] = jnp.zeros((UNR + 1, SEG, D), BF16)
        r_v[...] = jnp.full(r_v.shape, -jnp.inf, F32)
        never_v[...] = jnp.zeros(never_v.shape, F32)
        qkv_s[0] = jnp.zeros((2 * SEG, E), BF16)
        o_s[0] = jnp.zeros((SEG, E), BF16)

        def zero_acc(h, carry):
            acc[h] = jnp.zeros((NSEG * M, E), F32)
            return carry

        lax.fori_loop(0, 2 * KMAJ, zero_acc, 0)

        for cp in small:
            cp.wait()
        c = c_v[...].astype(F32)
        sc = jnp.broadcast_to(_rb(c * jax.nn.sigmoid(c)), (M, D))
        zero = jnp.zeros((M, E), F32)
        for h in range(H):
            blk = sc[:, (h % DB) * 128:(h % DB + 1) * 128]
            odef[0, h] = jnp.concatenate(
                [blk if c_ == h // DB else zero for c_ in range(4)], axis=0).astype(BF16)
        mod_v[6] = jnp.broadcast_to(wr_v[...].astype(F32).reshape(1, D), (8, D))
        put_rows(lhs_v, 0, mem0_v[...].astype(F32))

        x_head.wait()
        x_seg0.wait()
        NB = 16
        RB = NSEG * M // NB
        NR = NSEG * M + SEG - M
        for b in range(NB + 1):
            if b < NB:
                xb = x_v[pl.ds(b * (NSEG // NB), NSEG // NB), pl.ds(0, M), :].astype(F32).reshape(RB, D)
            else:
                xb = x_v[0, pl.ds(M, SEG - M), :].astype(F32)
            nb = _ln(xb)
            for j in range(DB):
                n_v[j, pl.ds(b * RB, nb.shape[0]), :] = nb[:, j * 128:(j + 1) * 128]

        hc_w = hc.bitcast(U32)

        def h_block(j, k):
            scb = jnp.concatenate([_bf(odef_w[0, h, pl.ds(0, 8), :]) for h in range(DB)], axis=1)
            v = _rb(_dot(scb, _bf(wmod_v[j, k]))[0:8])
            if k == 1:
                v = _rb(1.0 + v)
            col = j * 128 if isinstance(j, int) else pl.multiple_of(j * 128, 128)
            mod_v[k, :, pl.ds(col, 128)] = v
            n = n_v[j, pl.ds(0, NR), :].reshape(NR // 8, 8, 128)
            if k == 1:
                n_v[j, pl.ds(0, NR), :] = _rb(n * v[None]).reshape(NR, 128)
            else:
                hv = (n + v[None]).reshape(NR, 128).astype(BF16)
                hc[j] = hv[0:NSEG * M]
                lhs_v[j, pl.ds(M, SEG - M), :] = hv[NSEG * M:]

        def pack_pair(r1, r2):
            r = jnp.concatenate([r1.reshape(NSEG, M, E), r2.reshape(NSEG, M, E)], axis=1)
            return r.reshape(NIT, UNR * 2 * M, E).astype(BF16)

        def split_pair(b):
            return (pltpu.bitcast(b << 16, F32).astype(BF16),
                    pltpu.bitcast(b & jnp.uint32(0xFFFF0000), F32).astype(BF16))

        def q_stage(j, last):
            static = isinstance(j, int)
            k0 = j * 128 if static else pl.multiple_of(j * 128, 128)
            for p in range(KMAJ):
                ws = split_pair(stage[p, pl.ds(k0, 128), :])
                rs = []
                for t in range(2):
                    h = 2 * p + t
                    w_v[h, j] = ws[t]
                    rs.append(_dot(_bf(hc_w[j]), _bf(w_w[h, j])) + acc[h])
                    if not last:
                        acc[h] = rs[t]
                if last:
                    cache[p] = pack_pair(*rs)
                elif p in (1, 5):
                    h_block(j + 1, 1 if p == 1 else 0)

        wait_all(wmod_v.at[0], SEM_MOD)
        h_block(0, 1)
        h_block(0, 0)

        def wait_ktile(j):
            wait_all(stage.at[pl.ds(0, KMAJ), pl.ds(0, 128), :], SEM_WQ + j)

        def q_body(j, carry):
            wait_ktile(j)
            wait_all(wmod_v.at[0], SEM_MOD + j + 1)

            @pl.when(j + AHEAD < DB)
            def _():
                start_ktile(j + AHEAD)

            @pl.when(j + AHEAD + 1 < DB)
            def _():
                start_mod(j + AHEAD + 1)

            @pl.when(j + AHEAD == DB)
            def _():
                for cp in slab_cps[:2 * PPI]:
                    cp.start()

            q_stage(j, False)
            return carry

        lax.fori_loop(0, DB - 1, q_body, 0)
        wait_ktile(DB - 1)
        for cp in slab_cps[2 * PPI:]:
            cp.start()
        x_tail.start()
        q_stage(DB - 1, True)

        def slab(gp):
            w_v[2 * gp], w_v[2 * gp + 1] = split_pair(stage[gp].reshape(DB, 128, E))
            hcv = jnp.concatenate([_bf(hc_w[j]) for j in range(DB)], axis=1)
            cache[gp] = pack_pair(_dot(hcv, weights(2 * gp)), _dot(hcv, weights(2 * gp + 1)))

        def pro_body(i, carry):
            g0 = KMAJ + i * PPI
            wait_all(stage.at[pl.ds(g0, PPI)], SEM_ST + i)

            @pl.when(i == 2)
            def _():
                wo_w = wo_hbm.bitcast(U32)
                for j in range(DB):
                    for c_ in range(4):
                        copy(wmod_w.at[:, pl.ds((2 + c_) * D + j * 128, 128)],
                             wo_v.at[j, pl.ds(c_ * (D // 2), D // 2), :], SEM_WO).start()
                for j in range(DB):
                    copy(wo_w.at[:, pl.ds(j * 128, 128)], wo_v.at[DB + j], SEM_WO).start()

            for t in range(PPI):
                slab(g0 + t)
            return carry

        lax.fori_loop(0, (NGP - KMAJ) // PPI, pro_body, 0)

    pl.run_scoped(
        prologue,
        pltpu.VMEM((NGP, D, E), U32),
        pltpu.VMEM((DB, 2, D // 2, 128), U32),
        pltpu.VMEM((DB, NSEG * M, E), BF16),
        pltpu.VMEM((DB, NSEG * M + SEG, 128), F32),
        pltpu.VMEM((2 * KMAJ, NSEG * M, E), F32),
    )

    def main(wg_v, wu_v, wd_v, x1_v, h2_v, out_v):
        lane = lax.broadcasted_iota(jnp.int32, (8, 2 * 128), 1)

        def post(seg, q, keep=True):
            rows = pl.ds(8 * q, 8)
            x = x_v[seg, rows, :].astype(F32)
            a = a_all[seg + UNR, rows, :].astype(F32)
            x1 = _rb(x + _rb(mod_row(2) * a))
            h2 = _ln_mod(x1, mod_row(4), mod_row(3))
            r = _rb(jnp.sum(h2 * mod_row(6), axis=-1, keepdims=True))
            if keep:
                r_v[...] = jnp.where(lane == seg * 4 + q, r, r_v[...])
            x1_v[seg, rows, :] = x1.astype(BF16)
            h2_v[seg, rows, :] = h2.astype(BF16)
            o = x1 + _rb(mod_row(5) * h2)
            out_v[seg, rows, :] = o.astype(BF16)
            return o, r

        def deferred(blk, wsel, j, tok=None, tok2=None):
            words = [odef_w[blk, h] for h in range(H)]
            if tok is not None:
                top = jnp.where(never_v[...] > 1.0, pltpu.bitcast(tok, U32), words[-1][0:8])
                words[-1] = jnp.concatenate([top, words[-1][8:]], axis=0)
            lhs = jnp.concatenate([_bf(w) for w in words], axis=1)
            res = _dot(lhs, _bf(wo_v[wsel + j]))
            if tok2 is not None:
                res = jnp.concatenate([jnp.where(never_v[...] > 1.0, tok2, res[0:8]), res[8:]], axis=0)
            res = res.astype(BF16).reshape(UNR, M, 128)
            a_all[pl.ds(blk * UNR, UNR), pl.ds(0, M), pl.ds(j * 128, 128)] = res

        def out_copy(grp):
            return copy(out_v.at[pl.ds(grp * UNR, UNR)], out_hbm.at[pl.ds(grp * UNR, UNR)], SEM_OUT)

        def fold(v):
            t = v[:, 0:128]
            for j in range(1, DB):
                t = t + v[:, j * 128:(j + 1) * 128]
            return t

        wg_w, wu_w, wd_w = wg_hbm.bitcast(U32), wu_hbm.bitcast(U32), wd_hbm.bitcast(U32)
        for j in range(FB):
            copy(wg_w.at[:, pl.ds(j * 128, 128)], wg_v.at[j], SEM_MOE).start()
            copy(wu_w.at[:, pl.ds(j * 128, 128)], wu_v.at[j], SEM_MOE + 1).start()
        for j in range(DB):
            copy(wd_w.at[:, pl.ds(j * 128, 128)], wd_v.at[j], SEM_MOE + 2).start()
        x_tail.wait()
        wait_all(wo_v, SEM_WO)

        def step(it, u):
            s = it * UNR + u
            lhs = jnp.concatenate([_bf(lhs_w[j]) for j in range(DB)], axis=1)
            nseg = jnp.minimum(s + 1, NSEG - 1)

            def side(p):
                if p % 2 == 0 or p < 3:
                    return None
                i = p // 2 - 1
                if i < 4:
                    lag = 2 * UNR if i == 0 else UNR
                    o, r = post(jnp.maximum(s - lag, 0), i)
                    return fold(o) + r
                r0 = (i - 3) * 8
                h = ln1(nseg, r0)
                put_rows(lhs_v, r0, h)
                return fold(h)

            def proj(m_i, p):
                g = m_i * NPAIR + p
                for t in range(2):
                    qkv_s[g, pl.ds(t * SEG, SEG), :] = _dot(lhs, weights(2 * g + t)).astype(BF16)

            def rows_of(m_i, p):
                g = m_i * NPAIR + p
                return jnp.concatenate([_bf(qkv_w[g]), _bf(cache_w[g, it, pl.ds(u * M, M), :])], axis=0)

            def probs(p):
                q = rows_of(0, p)
                k = rows_of(1, p)
                sc = lax.dot_general(q, k, (((1,), (1,)), ((), ())), preferred_element_type=F32) * SCALE
                fm = fill_v[...]
                tok = side(p)
                if tok is not None:
                    top = fm[0:8]
                    fm = jnp.concatenate([jnp.where(top > 1.0, tok[:, 0:PR], top), fm[8:]], axis=0)
                sc = jnp.where(fm == 0.0, sc, fm)
                e = jnp.exp(sc - jnp.max(sc, axis=-1, keepdims=True))
                return (e * _recip(jnp.sum(e, axis=-1, keepdims=True))).astype(BF16)

            def attend(p, pr):
                o = _dot(pr, rows_of(2, p))
                o_s[2 * p] = o[0:SEG].astype(BF16)
                o_s[2 * p + 1] = o[SEG:2 * SEG].astype(BF16)
                odef[it + 1, 2 * p, pl.ds(u * M, M), :] = o[2 * SEG:2 * SEG + M].astype(BF16)
                odef[it + 1, 2 * p + 1, pl.ds(u * M, M), :] = o[2 * SEG + M:].astype(BF16)

            wsel = jnp.where(it == 0, 0, DB)
            for t in range(DB // UNR):
                deferred(it, wsel, u * (DB // UNR) + t)
            ps = {}
            for pa in range(0, NPAIR, 2):
                pb = pa + 1
                proj(0, pa)
                proj(1, pa)
                proj(0, pb)
                proj(1, pb)
                proj(2, pa)
                proj(2, pb)
                ps[pa] = probs(pa)
                ps[pb] = probs(pb)
                if pa >= 2:
                    attend(pa - 2, ps.pop(pa - 2))
                    attend(pb - 2, ps.pop(pb - 2))
            L = NPAIR - 1

            HA = 24
            acc = [None] * DB
            for h0, h1 in ((0, HA), (HA, H)):
                for j in range(DB):
                    ol = jnp.concatenate([_bf(o_w[h]) for h in range(h0, h1)], axis=1)
                    part = _dot(ol, _bf(wo_v[DB + j, pl.ds(h0 * E // 2, (h1 - h0) * E // 2), :]))
                    if h0 == 0:
                        acc[j] = part
                    else:
                        a = part + acc[j]
                        lhs_v[j, pl.ds(0, M), :] = a[0:M].astype(BF16)
                        a_all[s + UNR, pl.ds(M, SEG - M), pl.ds(j * 128, 128)] = a[M:].astype(BF16)
                    if h0 == 0 and j == 4:
                        attend(L - 1, ps.pop(L - 1))
                        attend(L, ps.pop(L))

        def iteration(it, carry):
            @pl.when(it >= 3)
            def _():
                out_copy(it - 3).start()

            for c_ in range(4):
                v = a_all[c_, pl.ds(0, M), :].astype(F32)
                mod_v[2 + c_] = _rb(1.0 + v) if c_ == 2 else v
            for u in range(UNR):
                step(it, u)
            return carry

        lax.fori_loop(0, NIT, iteration, 0)

        out_copy(NIT - 3).start()
        for k, buf in enumerate((wg_v, wu_v, wd_v)):
            wait_all(buf, SEM_MOE + k)
        early = [(seg, 0) for seg in range(NSEG - 2 * UNR, NSEG - UNR)]
        early += [(seg, q) for seg in range(NSEG - UNR, NSEG) for q in (1, 2, 3)]
        r8 = lax.broadcasted_iota(jnp.int32, (8, 1), 0)
        vals, idxs = [], []

        def pieces(n):
            tok = None
            for _ in range(n):
                seg, q = early.pop(0)
                keep = len(early) >= EPI_LATE
                o, r = post(seg, q, keep)
                if not keep:
                    vals.append(r)
                    idxs.append((r8 + (seg * SEG + q * 8)).astype(F32))
                tok = fold(o) + r if tok is None else tok + fold(o) + r
            return tok

        for j in range(DB):
            deferred(NIT, DB, j, pieces(EPI_PIECES[j]), pieces(EPI_PIECES[DB]) if j == DB - 1 else None)
        out_copy(NIT - 2).start()

        def top2(vals, idx, axes):
            def red(f, v):
                for ax in axes:
                    v = f(v, axis=ax, keepdims=True)
                return v
            m1 = red(jnp.max, vals)
            i1 = red(jnp.min, jnp.where(vals == m1, idx, S - 1.0))
            rest = jnp.where(idx == i1, -jnp.inf, vals)
            m2 = red(jnp.max, rest)
            i2 = red(jnp.min, jnp.where(rest == m2, jnp.where(idx == i1, S - 1.0, idx), S - 1.0))
            return m1, i1, m2, i2

        m1, i1v, m2, i2v = top2(r_v[...], (lane * 8 + r8).astype(F32), (1, 0))
        vals.append(jnp.where(r8 == 0, m1, jnp.where(r8 == 1, m2, -jnp.inf)))
        idxs.append(jnp.where(r8 == 0, i1v, jnp.where(r8 == 1, i2v, S - 1.0)))
        for seg, q in early + [(seg, 0) for seg in range(NSEG - UNR, NSEG)]:
            vals.append(post(seg, q, keep=False)[1])
            idxs.append((r8 + (seg * SEG + q * 8)).astype(F32))
        out_copy(NIT - 1).start()
        m1, i1v, m2, i2v = top2(jnp.concatenate(vals, axis=0), jnp.concatenate(idxs, axis=0), (0,))
        i1 = i1v.astype(jnp.int32)[0, 0]
        i2 = i2v.astype(jnp.int32)[0, 0]

        def tile_of(i):
            return i >> 5, pl.multiple_of(((i >> 3) & 3) * 8, 8)

        sel = [tile_of(i1), tile_of(i2)]
        x1s = jnp.concatenate([x1_v[sg, pl.ds(r0, 8), :].astype(F32) for sg, r0 in sel], axis=0)
        h2s = jnp.concatenate([h2_v[sg, pl.ds(r0, 8), :].astype(F32) for sg, r0 in sel], axis=0)
        h2b = h2s.astype(BF16)
        gus = []
        for j in range(FB):
            g = _rb(_dot(h2b, _bf(wg_v[j])))
            g = _rb(g * jax.nn.sigmoid(g))
            u = _rb(_dot(h2b, _bf(wu_v[j])))
            gus.append(g * u)
        gu = jnp.concatenate(gus, axis=1).astype(BF16)
        y = jnp.concatenate([_rb(_dot(gu, _bf(wd_v[j]))) for j in range(DB)], axis=1)
        rows = lax.broadcasted_iota(jnp.int32, (16, 1), 0)
        rs = _rb(jax.nn.sigmoid(jnp.where(rows < 8, m1, m2)))
        y = _rb(y * rs)
        full = x1s + _rb(mod_row(5, 16) * _rb(h2s + y))

        copy(out_v, out_hbm, SEM_OUT).wait()
        for t, (i, (sg, r0)) in enumerate(zip((i1, i2), sel)):
            old = out_v[sg, pl.ds(r0, 8), :].astype(F32)
            new = jnp.where(r8 == (i & 7), full[t * 8:(t + 1) * 8], old)
            out_v[sg, pl.ds(r0, 8), :] = new.astype(BF16)
        fix = [copy(out_v.at[sg, pl.ds(r0, 8), :], out_hbm.at[sg, pl.ds(r0, 8), :], SEM_OUT + 1 + t)
               for t, (sg, r0) in enumerate(sel)]
        differ = (i1 >> 3) != (i2 >> 3)
        fix[0].start()

        @pl.when(differ)
        def _():
            fix[1].start()
            fix[1].wait()

        fix[0].wait()

    pl.run_scoped(
        main,
        pltpu.VMEM((FB, D // 2, 128), U32),
        pltpu.VMEM((FB, D // 2, 128), U32),
        pltpu.VMEM((DB, F // 2, 128), U32),
        pltpu.VMEM((NSEG, SEG, D), BF16),
        pltpu.VMEM((NSEG, SEG, D), BF16),
        pltpu.VMEM((NSEG, SEG, D), BF16),
    )


@jax.jit
def pallas_adaLN_cond__memory_aug_recurrent_mem_tr__moe_arch_mod__prompt_kernel(
    A_x: jax.Array,
    A_mem0: jax.Array,
    A_Wq: jax.Array,
    A_Wk: jax.Array,
    A_Wv: jax.Array,
    A_Wo: jax.Array,
    A_seg_len: jax.Array,
    B_x: jax.Array,
    B_w_r: jax.Array,
    B_w_gate: jax.Array,
    B_w_up: jax.Array,
    B_w_down: jax.Array,
    c: jax.Array,
    w_mod: jax.Array,
):
    del A_seg_len, B_x
    assert A_x.shape == (1, S, D) and A_mem0.shape == (1, M, D) and A_Wq.shape == (D, H, E)
    hbm = pl.BlockSpec(memory_space=pl.ANY)
    out = pl.pallas_call(
        _kernel,
        out_shape=jax.ShapeDtypeStruct((NSEG, SEG, D), BF16),
        in_specs=[hbm] * 12,
        out_specs=hbm,
        scratch_shapes=[
            pltpu.VMEM((NSEG, SEG, D), BF16),
            pltpu.VMEM((3 * H, DB, 128, E), BF16),
            pltpu.VMEM((2 * DB, H * E // 2, 128), U32),
            pltpu.VMEM((NGP, NIT, UNR * 2 * M, E), BF16),
            pltpu.VMEM((NIT + 1, H, SEG, E), BF16),
            pltpu.VMEM((DB, SEG, 128), BF16),
            pltpu.VMEM((NGP, 2 * SEG, E), BF16),
            pltpu.VMEM((H, SEG, E), BF16),
            pltpu.VMEM((NSEG + UNR, SEG, D), BF16),
            pltpu.VMEM((8, S // 8), F32),
            pltpu.VMEM((7, 8, D), F32),
            pltpu.VMEM((PR, PR), F32),
            pltpu.VMEM((8, 128), F32),
            pltpu.VMEM((M, D), BF16),
            pltpu.VMEM((D,), BF16),
            pltpu.VMEM((1, D), BF16),
            pltpu.SemaphoreType.DMA((NSEM,)),
        ],
        compiler_params=pltpu.CompilerParams(
            vmem_limit_bytes=120 * 1024 * 1024, disable_bounds_checks=True,
            disable_semaphore_checks=True),
    )(
        A_x.reshape(NSEG, SEG, D),
        A_mem0.reshape(M, D),
        A_Wq, A_Wk, A_Wv,
        A_Wo.reshape(H * E, D),
        B_w_r,
        B_w_gate, B_w_up, B_w_down,
        c, w_mod,
    )
    return out.reshape(1, S, D)
```

```python
import jax
import jax.numpy as jnp
from jax import lax
import jax.experimental.pallas as pl
import jax.experimental.pallas.tpu as pltpu

BF16 = jnp.bfloat16
F32 = jnp.float32
U32 = jnp.uint32

S = 2048
D = 1024
H = 32
E = 128
M = 8
SEG = 32
NSEG = S // SEG
NPAIR = H // 2
NGP = 3 * NPAIR
F = 3584
DB = D // 128
FB = F // 128
PR = 2 * SEG + 2 * M
UNR = SEG // M
NIT = NSEG // UNR
KMAJ = 12
AHEAD = 3
PPI = 6
EPI_LATE = 6
EPI_PIECES = (0, 0, 2, 2, 2, 2, 2, 2, 2)
TOK = 0
EPS = 1e-5
SCALE = E ** (-0.5)

SEM_SMALL = 0
SEM_X = SEM_SMALL + 3
SEM_MOD = SEM_X + 3
SEM_WQ = SEM_MOD + DB
SEM_ST = SEM_WQ + DB
SEM_WO = SEM_ST + (NGP - KMAJ) // PPI
SEM_MOE = SEM_WO + 1
SEM_OUT = SEM_MOE + 3
NSEM = SEM_OUT + 3


def _rb(v):
    return v.astype(BF16).astype(F32)


def _dot(a, b):
    return jnp.dot(a, b, preferred_element_type=F32)


def _recip(x):
    r = pl.reciprocal(x, approx=True)
    return r * (2.0 - x * r)


def _bf(words):
    return pltpu.bitcast(words, BF16)


def _ln(x):
    m = jnp.mean(x, axis=-1, keepdims=True)
    mb = _rb(m)
    d = x - mb
    var = jnp.mean(d * d, axis=-1, keepdims=True) - (m - mb) * (m - mb)
    inv = _recip(_rb(jnp.sqrt(_rb(_rb(jnp.maximum(var, 0.0)) + EPS))))
    return d * inv, inv


def _fill_matrix():
    i = lax.broadcasted_iota(jnp.int32, (PR, PR), 0)
    j = lax.broadcasted_iota(jnp.int32, (PR, PR), 1)

    def head(t):
        return jnp.where(t < 2 * SEG, t >> 5, (t - 2 * SEG) >> 3)

    def pos(t):
        r = t & (SEG - 1)
        return jnp.where(t < 2 * SEG, jnp.where(r < M, r, r + M), M + (t & (M - 1)))

    same = head(i) == head(j)
    pi = pos(i)
    ok = jnp.where(pi < M, 1, jnp.where(pi >= pos(j), 1, 0))
    return jnp.where(same, jnp.where(ok == 1, 0.0, -1e9), -3e38).astype(F32)


def _kernel(x_hbm, mem0_hbm, wq_hbm, wk_hbm, wv_hbm, wo_hbm, wr_hbm, wg_hbm, wu_hbm, wd_hbm,
            c_hbm, wmod_hbm, out_hbm,
            x_v, w_v, wo_v, cache, odef, lhs_v, qkv_s, o_s, a_all, r_v, mod_v, fill_v, never_v,
            mem0_v, wr_v, c_v, sems):
    w_w = w_v.bitcast(U32)
    cache_w = cache.bitcast(U32)
    lhs_w = lhs_v.bitcast(U32)
    qkv_w = qkv_s.bitcast(U32)
    o_w = o_s.bitcast(U32)
    odef_w = odef.bitcast(U32)

    def weights(h):
        return _bf(w_w[h].reshape(D // 2, E))

    def copy(src, dst, sem):
        return pltpu.make_async_copy(src, dst, sems.at[sem])

    def wait_all(buf, sem):
        copy(buf, buf, sem).wait()

    def mod_row(k, rows=8):
        v = mod_v[k]
        return v if rows == 8 else jnp.concatenate([v] * (rows // 8), axis=0)

    def put_rows(dst, r0, v):
        for j in range(DB):
            dst[j, pl.ds(r0, v.shape[0]), :] = v[:, j * 128:(j + 1) * 128].astype(BF16)

    def ln1(seg, r0):
        n, inv = _ln(x_v[seg, pl.ds(r0, 8), :].astype(F32))
        return n * mod_row(1) + mod_row(0), inv

    x_tail = copy(x_hbm.at[pl.ds(1, NSEG - 1), pl.ds(M, SEG - M), :],
                  x_v.at[pl.ds(1, NSEG - 1), pl.ds(M, SEG - M), :], SEM_X + 2)

    def prologue(stage, wmod_v, hc, n_v, acc):
        wmod_w = wmod_hbm.bitcast(U32)
        w_words = [w.bitcast(U32) for w in (wq_hbm, wk_hbm, wv_hbm)]

        def start_mod(j):
            col = j * 128 if isinstance(j, int) else pl.multiple_of(j * 128, 128)
            for k in range(2):
                copy(wmod_w.at[:, pl.ds(k * D + col, 128)], wmod_v.at[j, k], SEM_MOD + j).start()

        def start_ktile(j):
            rows = pl.ds(j * 128 if isinstance(j, int) else pl.multiple_of(j * 128, 128), 128)
            for g in range(KMAJ):
                copy(w_words[0].at[rows, g, :], stage.at[g, rows, :], SEM_WQ + j).start()

        small = [copy(c_hbm, c_v, SEM_SMALL), copy(mem0_hbm, mem0_v, SEM_SMALL + 1),
                 copy(wr_hbm, wr_v, SEM_SMALL + 2)]
        x_head = copy(x_hbm.at[:, pl.ds(0, M), :], x_v.at[:, pl.ds(0, M), :], SEM_X)
        x_seg0 = copy(x_hbm.at[0, pl.ds(M, SEG - M), :], x_v.at[0, pl.ds(M, SEG - M), :], SEM_X + 1)
        for cp in small:
            cp.start()
        x_head.start()
        x_seg0.start()
        start_mod(0)
        for j in range(AHEAD):
            start_ktile(j)
            start_mod(j + 1)
        slab_cps = [copy(w_words[g // NPAIR].at[:, g % NPAIR, :], stage.at[g], SEM_ST + (g - KMAJ) // PPI)
                    for g in range(KMAJ, NGP)]

        fill_v[...] = _fill_matrix()
        a_all[pl.ds(0, UNR + 1)] = jnp.zeros((UNR + 1, SEG, D), BF16)
        r_v[...] = jnp.full(r_v.shape, -jnp.inf, F32)
        never_v[...] = jnp.zeros(never_v.shape, F32)
        qkv_s[0] = jnp.zeros((2 * SEG, E), BF16)
        o_s[0] = jnp.zeros((SEG, E), BF16)

        def zero_acc(h, carry):
            acc[h] = jnp.zeros((NSEG * M, E), F32)
            return carry

        lax.fori_loop(0, 2 * KMAJ, zero_acc, 0)

        for cp in small:
            cp.wait()
        c = c_v[...].astype(F32)
        sc = jnp.broadcast_to(_rb(c * jax.nn.sigmoid(c)), (M, D))
        zero = jnp.zeros((M, E), F32)
        for h in range(H):
            blk = sc[:, (h % DB) * 128:(h % DB + 1) * 128]
            odef[0, h] = jnp.concatenate(
                [blk if c_ == h // DB else zero for c_ in range(4)], axis=0).astype(BF16)
        mod_v[6] = jnp.broadcast_to(wr_v[...].astype(F32).reshape(1, D), (8, D))
        put_rows(lhs_v, 0, mem0_v[...].astype(F32))

        x_head.wait()
        x_seg0.wait()
        NB = 16
        RB = NSEG * M // NB
        NR = NSEG * M + SEG - M
        for b in range(NB + 1):
            if b < NB:
                xb = x_v[pl.ds(b * (NSEG // NB), NSEG // NB), pl.ds(0, M), :].astype(F32).reshape(RB, D)
            else:
                xb = x_v[0, pl.ds(M, SEG - M), :].astype(F32)
            nb = _ln(xb)[0]
            for j in range(DB):
                n_v[j, pl.ds(b * RB, nb.shape[0]), :] = nb[:, j * 128:(j + 1) * 128]

        hc_w = hc.bitcast(U32)

        def h_block(j, k):
            scb = jnp.concatenate([_bf(odef_w[0, h, pl.ds(0, 8), :]) for h in range(DB)], axis=1)
            v = _rb(_dot(scb, _bf(wmod_v[j, k]))[0:8])
            if k == 1:
                v = _rb(1.0 + v)
            col = j * 128 if isinstance(j, int) else pl.multiple_of(j * 128, 128)
            mod_v[k, :, pl.ds(col, 128)] = v
            n = n_v[j, pl.ds(0, NR), :].reshape(NR // 8, 8, 128)
            if k == 1:
                n_v[j, pl.ds(0, NR), :] = (n * v[None]).reshape(NR, 128)
            else:
                hv = (n + v[None]).reshape(NR, 128).astype(BF16)
                hc[j] = hv[0:NSEG * M]
                lhs_v[j, pl.ds(M, SEG - M), :] = hv[NSEG * M:]

        def pack_pair(r1, r2):
            r = jnp.concatenate([r1.reshape(NSEG, M, E), r2.reshape(NSEG, M, E)], axis=1)
            return r.reshape(NIT, UNR * 2 * M, E).astype(BF16)

        def split_pair(b):
            return (pltpu.bitcast(b << 16, F32).astype(BF16),
                    pltpu.bitcast(b & jnp.uint32(0xFFFF0000), F32).astype(BF16))

        def q_stage(j, last):
            static = isinstance(j, int)
            k0 = j * 128 if static else pl.multiple_of(j * 128, 128)
            for p in range(KMAJ):
                ws = split_pair(stage[p, pl.ds(k0, 128), :])
                rs = []
                for t in range(2):
                    h = 2 * p + t
                    w_v[h, j] = ws[t]
                    rs.append(_dot(_bf(hc_w[j]), _bf(w_w[h, j])) + acc[h])
                    if not last:
                        acc[h] = rs[t]
                if last:
                    cache[p] = pack_pair(*rs)
                elif p in (1, 5):
                    h_block(j + 1, 1 if p == 1 else 0)

        wait_all(wmod_v.at[0], SEM_MOD)
        h_block(0, 1)
        h_block(0, 0)

        def wait_ktile(j):
            wait_all(stage.at[pl.ds(0, KMAJ), pl.ds(0, 128), :], SEM_WQ + j)

        def q_body(j, carry):
            wait_ktile(j)
            wait_all(wmod_v.at[0], SEM_MOD + j + 1)

            @pl.when(j + AHEAD < DB)
            def _():
                start_ktile(j + AHEAD)

            @pl.when(j + AHEAD + 1 < DB)
            def _():
                start_mod(j + AHEAD + 1)

            @pl.when(j + AHEAD == DB)
            def _():
                for cp in slab_cps[:2 * PPI]:
                    cp.start()

            q_stage(j, False)
            return carry

        lax.fori_loop(0, DB - 1, q_body, 0)
        wait_ktile(DB - 1)
        for cp in slab_cps[2 * PPI:]:
            cp.start()
        x_tail.start()
        q_stage(DB - 1, True)

        def slab(gp):
            w_v[2 * gp], w_v[2 * gp + 1] = split_pair(stage[gp].reshape(DB, 128, E))
            hcv = jnp.concatenate([_bf(hc_w[j]) for j in range(DB)], axis=1)
            cache[gp] = pack_pair(_dot(hcv, weights(2 * gp)), _dot(hcv, weights(2 * gp + 1)))

        def pro_body(i, carry):
            g0 = KMAJ + i * PPI
            wait_all(stage.at[pl.ds(g0, PPI)], SEM_ST + i)

            @pl.when(i == 2)
            def _():
                wo_w = wo_hbm.bitcast(U32)
                for j in range(DB):
                    for c_ in range(4):
                        copy(wmod_w.at[:, pl.ds((2 + c_) * D + j * 128, 128)],
                             wo_v.at[j, pl.ds(c_ * (D // 2), D // 2), :], SEM_WO).start()
                for j in range(DB):
                    copy(wo_w.at[:, pl.ds(j * 128, 128)], wo_v.at[DB + j], SEM_WO).start()

            for t in range(PPI):
                slab(g0 + t)
            return carry

        lax.fori_loop(0, (NGP - KMAJ) // PPI, pro_body, 0)

    pl.run_scoped(
        prologue,
        pltpu.VMEM((NGP, D, E), U32),
        pltpu.VMEM((DB, 2, D // 2, 128), U32),
        pltpu.VMEM((DB, NSEG * M, E), BF16),
        pltpu.VMEM((DB, NSEG * M + SEG, 128), F32),
        pltpu.VMEM((2 * KMAJ, NSEG * M, E), F32),
    )

    def main(wg_v, wu_v, wd_v, x1_v, h2_v, out_v):
        lane = lax.broadcasted_iota(jnp.int32, (8, 2 * 128), 1)

        def post(seg, q, keep=True):
            rows = pl.ds(8 * q, 8)
            x = x_v[seg, rows, :].astype(F32)
            a = a_all[seg + UNR, rows, :].astype(F32)
            x1 = _rb(x + mod_row(2) * a)
            n, inv = _ln(x1)
            h2 = _rb(n * mod_row(4) + mod_row(3))
            r = _rb(jnp.sum(h2 * mod_row(6), axis=-1, keepdims=True))
            if keep:
                r_v[...] = jnp.where(lane == seg * 4 + q, r, r_v[...])
            x1_v[seg, rows, :] = x1.astype(BF16)
            h2_v[seg, rows, :] = h2.astype(BF16)
            out_v[seg, rows, :] = (x1 + mod_row(5) * h2).astype(BF16)
            return inv, r

        def deferred(blk, wsel, j, tok=None, tok2=None):
            words = [odef_w[blk, h] for h in range(H)]
            if tok is not None:
                tok = pltpu.bitcast(jnp.broadcast_to(tok, (8, 128)), U32)
                top = jnp.where(never_v[...] > 1.0, tok, words[-1][0:8])
                words[-1] = jnp.concatenate([top, words[-1][8:]], axis=0)
            lhs = jnp.concatenate([_bf(w) for w in words], axis=1)
            res = _dot(lhs, _bf(wo_v[wsel + j]))
            if tok2 is not None:
                res = jnp.concatenate([jnp.where(never_v[...] > 1.0, tok2, res[0:8]), res[8:]], axis=0)
            res = res.astype(BF16).reshape(UNR, M, 128)
            a_all[pl.ds(blk * UNR, UNR), pl.ds(0, M), pl.ds(j * 128, 128)] = res

        def out_copy(grp):
            return copy(out_v.at[pl.ds(grp * UNR, UNR)], out_hbm.at[pl.ds(grp * UNR, UNR)], SEM_OUT)

        wg_w, wu_w, wd_w = wg_hbm.bitcast(U32), wu_hbm.bitcast(U32), wd_hbm.bitcast(U32)
        for j in range(FB):
            copy(wg_w.at[:, pl.ds(j * 128, 128)], wg_v.at[j], SEM_MOE).start()
            copy(wu_w.at[:, pl.ds(j * 128, 128)], wu_v.at[j], SEM_MOE + 1).start()
        for j in range(DB):
            copy(wd_w.at[:, pl.ds(j * 128, 128)], wd_v.at[j], SEM_MOE + 2).start()
        x_tail.wait()
        wait_all(wo_v, SEM_WO)

        def step(it, u):
            s = it * UNR + u
            lhs = jnp.concatenate([_bf(lhs_w[j]) for j in range(DB)], axis=1)
            nseg = jnp.minimum(s + 1, NSEG - 1)

            def side(p):
                if p % 2 == 0 or p < 3:
                    return None
                i = p // 2 - 1
                if i < 4:
                    lag = 2 * UNR if i == 0 else UNR
                    return post(jnp.maximum(s - lag, 0), i)[TOK]
                r0 = (i - 3) * 8
                h, inv = ln1(nseg, r0)
                put_rows(lhs_v, r0, h)
                return inv

            def proj(m_i, p):
                g = m_i * NPAIR + p
                for t in range(2):
                    qkv_s[g, pl.ds(t * SEG, SEG), :] = _dot(lhs, weights(2 * g + t)).astype(BF16)

            def rows_of(m_i, p):
                g = m_i * NPAIR + p
                return jnp.concatenate([_bf(qkv_w[g]), _bf(cache_w[g, it, pl.ds(u * M, M), :])], axis=0)

            def probs(p):
                q = rows_of(0, p)
                k = rows_of(1, p)
                sc = lax.dot_general(q, k, (((1,), (1,)), ((), ())), preferred_element_type=F32) * SCALE
                fm = fill_v[...]
                tok = side(p)
                if tok is not None:
                    top = fm[0:8]
                    fm = jnp.concatenate([jnp.where(top > 1.0, tok, top), fm[8:]], axis=0)
                sc = jnp.where(fm == 0.0, sc, fm)
                e = jnp.exp(sc - jnp.max(sc, axis=-1, keepdims=True))
                return (e * _recip(jnp.sum(e, axis=-1, keepdims=True))).astype(BF16)

            def attend(p, pr):
                o = _dot(pr, rows_of(2, p))
                o_s[2 * p] = o[0:SEG].astype(BF16)
                o_s[2 * p + 1] = o[SEG:2 * SEG].astype(BF16)
                odef[it + 1, 2 * p, pl.ds(u * M, M), :] = o[2 * SEG:2 * SEG + M].astype(BF16)
                odef[it + 1, 2 * p + 1, pl.ds(u * M, M), :] = o[2 * SEG + M:].astype(BF16)

            wsel = jnp.where(it == 0, 0, DB)
            for t in range(DB // UNR):
                deferred(it, wsel, u * (DB // UNR) + t)
            ps = {}
            for pa in range(0, NPAIR, 2):
                pb = pa + 1
                proj(0, pa)
                proj(1, pa)
                proj(0, pb)
                proj(1, pb)
                proj(2, pa)
                proj(2, pb)
                ps[pa] = probs(pa)
                ps[pb] = probs(pb)
                if pa >= 2:
                    attend(pa - 2, ps.pop(pa - 2))
                    attend(pb - 2, ps.pop(pb - 2))
            L = NPAIR - 1

            HA = 24
            acc = [None] * DB
            for h0, h1 in ((0, HA), (HA, H)):
                for j in range(DB):
                    ol = jnp.concatenate([_bf(o_w[h]) for h in range(h0, h1)], axis=1)
                    part = _dot(ol, _bf(wo_v[DB + j, pl.ds(h0 * E // 2, (h1 - h0) * E // 2), :]))
                    if h0 == 0:
                        acc[j] = part
                    else:
                        a = part + acc[j]
                        lhs_v[j, pl.ds(0, M), :] = a[0:M].astype(BF16)
                        a_all[s + UNR, pl.ds(M, SEG - M), pl.ds(j * 128, 128)] = a[M:].astype(BF16)
                    if h0 == 0 and j == 4:
                        attend(L - 1, ps.pop(L - 1))
                        attend(L, ps.pop(L))

        def iteration(it, carry):
            @pl.when(it >= 3)
            def _():
                out_copy(it - 3).start()

            for c_ in range(4):
                v = a_all[c_, pl.ds(0, M), :].astype(F32)
                mod_v[2 + c_] = _rb(1.0 + v) if c_ == 2 else v
            for u in range(UNR):
                step(it, u)
            return carry

        lax.fori_loop(0, NIT, iteration, 0)

        out_copy(NIT - 3).start()
        for k, buf in enumerate((wg_v, wu_v, wd_v)):
            wait_all(buf, SEM_MOE + k)
        early = [(seg, 0) for seg in range(NSEG - 2 * UNR, NSEG - UNR)]
        early += [(seg, q) for seg in range(NSEG - UNR, NSEG) for q in (1, 2, 3)]
        r8 = lax.broadcasted_iota(jnp.int32, (8, 1), 0)
        vals, idxs = [], []

        def pieces(n):
            tok = None
            for _ in range(n):
                seg, q = early.pop(0)
                keep = len(early) >= EPI_LATE
                r = post(seg, q, keep)[1]
                if not keep:
                    vals.append(r)
                    idxs.append((r8 + (seg * SEG + q * 8)).astype(F32))
                tok = r if tok is None else tok + r
            return tok

        for j in range(DB):
            deferred(NIT, DB, j, pieces(EPI_PIECES[j]), pieces(EPI_PIECES[DB]) if j == DB - 1 else None)
        out_copy(NIT - 2).start()

        def top2(vals, idx, axes):
            def red(f, v):
                for ax in axes:
                    v = f(v, axis=ax, keepdims=True)
                return v
            m1 = red(jnp.max, vals)
            i1 = red(jnp.min, jnp.where(vals == m1, idx, S - 1.0))
            rest = jnp.where(idx == i1, -jnp.inf, vals)
            m2 = red(jnp.max, rest)
            i2 = red(jnp.min, jnp.where(rest == m2, jnp.where(idx == i1, S - 1.0, idx), S - 1.0))
            return m1, i1, m2, i2

        m1, i1v, m2, i2v = top2(r_v[...], (lane * 8 + r8).astype(F32), (1, 0))
        vals.append(jnp.where(r8 == 0, m1, jnp.where(r8 == 1, m2, -jnp.inf)))
        idxs.append(jnp.where(r8 == 0, i1v, jnp.where(r8 == 1, i2v, S - 1.0)))
        for seg, q in early + [(seg, 0) for seg in range(NSEG - UNR, NSEG)]:
            vals.append(post(seg, q, keep=False)[1])
            idxs.append((r8 + (seg * SEG + q * 8)).astype(F32))
        out_copy(NIT - 1).start()
        m1, i1v, m2, i2v = top2(jnp.concatenate(vals, axis=0), jnp.concatenate(idxs, axis=0), (0,))
        i1 = i1v.astype(jnp.int32)[0, 0]
        i2 = i2v.astype(jnp.int32)[0, 0]

        def tile_of(i):
            return i >> 5, pl.multiple_of(((i >> 3) & 3) * 8, 8)

        sel = [tile_of(i1), tile_of(i2)]
        x1s = jnp.concatenate([x1_v[sg, pl.ds(r0, 8), :].astype(F32) for sg, r0 in sel], axis=0)
        h2s = jnp.concatenate([h2_v[sg, pl.ds(r0, 8), :].astype(F32) for sg, r0 in sel], axis=0)
        h2b = h2s.astype(BF16)
        gus = []
        for j in range(FB):
            g = _rb(_dot(h2b, _bf(wg_v[j])))
            g = _rb(g * jax.nn.sigmoid(g))
            u = _rb(_dot(h2b, _bf(wu_v[j])))
            gus.append(g * u)
        gu = jnp.concatenate(gus, axis=1).astype(BF16)
        y = jnp.concatenate([_rb(_dot(gu, _bf(wd_v[j]))) for j in range(DB)], axis=1)
        rows = lax.broadcasted_iota(jnp.int32, (16, 1), 0)
        rs = _rb(jax.nn.sigmoid(jnp.where(rows < 8, m1, m2)))
        y = _rb(y * rs)
        full = x1s + mod_row(5, 16) * _rb(h2s + y)

        copy(out_v, out_hbm, SEM_OUT).wait()
        for t, (i, (sg, r0)) in enumerate(zip((i1, i2), sel)):
            old = out_v[sg, pl.ds(r0, 8), :].astype(F32)
            new = jnp.where(r8 == (i & 7), full[t * 8:(t + 1) * 8], old)
            out_v[sg, pl.ds(r0, 8), :] = new.astype(BF16)
        fix = [copy(out_v.at[sg, pl.ds(r0, 8), :], out_hbm.at[sg, pl.ds(r0, 8), :], SEM_OUT + 1 + t)
               for t, (sg, r0) in enumerate(sel)]
        differ = (i1 >> 3) != (i2 >> 3)
        fix[0].start()

        @pl.when(differ)
        def _():
            fix[1].start()
            fix[1].wait()

        fix[0].wait()

    pl.run_scoped(
        main,
        pltpu.VMEM((FB, D // 2, 128), U32),
        pltpu.VMEM((FB, D // 2, 128), U32),
        pltpu.VMEM((DB, F // 2, 128), U32),
        pltpu.VMEM((NSEG, SEG, D), BF16),
        pltpu.VMEM((NSEG, SEG, D), BF16),
        pltpu.VMEM((NSEG, SEG, D), BF16),
    )


@jax.jit
def pallas_adaLN_cond__memory_aug_recurrent_mem_tr__moe_arch_mod__prompt_kernel(
    A_x: jax.Array,
    A_mem0: jax.Array,
    A_Wq: jax.Array,
    A_Wk: jax.Array,
    A_Wv: jax.Array,
    A_Wo: jax.Array,
    A_seg_len: jax.Array,
    B_x: jax.Array,
    B_w_r: jax.Array,
    B_w_gate: jax.Array,
    B_w_up: jax.Array,
    B_w_down: jax.Array,
    c: jax.Array,
    w_mod: jax.Array,
):
    del A_seg_len, B_x
    assert A_x.shape == (1, S, D) and A_mem0.shape == (1, M, D) and A_Wq.shape == (D, H, E)
    hbm = pl.BlockSpec(memory_space=pl.ANY)
    out = pl.pallas_call(
        _kernel,
        out_shape=jax.ShapeDtypeStruct((NSEG, SEG, D), BF16),
        in_specs=[hbm] * 12,
        out_specs=hbm,
        scratch_shapes=[
            pltpu.VMEM((NSEG, SEG, D), BF16),
            pltpu.VMEM((3 * H, DB, 128, E), BF16),
            pltpu.VMEM((2 * DB, H * E // 2, 128), U32),
            pltpu.VMEM((NGP, NIT, UNR * 2 * M, E), BF16),
            pltpu.VMEM((NIT + 1, H, SEG, E), BF16),
            pltpu.VMEM((DB, SEG, 128), BF16),
            pltpu.VMEM((NGP, 2 * SEG, E), BF16),
            pltpu.VMEM((H, SEG, E), BF16),
            pltpu.VMEM((NSEG + UNR, SEG, D), BF16),
            pltpu.VMEM((8, S // 8), F32),
            pltpu.VMEM((7, 8, D), F32),
            pltpu.VMEM((PR, PR), F32),
            pltpu.VMEM((8, 128), F32),
            pltpu.VMEM((M, D), BF16),
            pltpu.VMEM((D,), BF16),
            pltpu.VMEM((1, D), BF16),
            pltpu.SemaphoreType.DMA((NSEM,)),
        ],
        compiler_params=pltpu.CompilerParams(
            vmem_limit_bytes=120 * 1024 * 1024, disable_bounds_checks=True,
            disable_semaphore_checks=True),
    )(
        A_x.reshape(NSEG, SEG, D),
        A_mem0.reshape(M, D),
        A_Wq, A_Wk, A_Wv,
        A_Wo.reshape(H * E, D),
        B_w_r,
        B_w_gate, B_w_up, B_w_down,
        c, w_mod,
    )
    return out.reshape(1, S, D)
```

```python
import jax
import jax.numpy as jnp
from jax import lax
import jax.experimental.pallas as pl
import jax.experimental.pallas.tpu as pltpu

BF16 = jnp.bfloat16
F32 = jnp.float32
U32 = jnp.uint32

S = 2048
D = 1024
H = 32
E = 128
M = 8
SEG = 32
NSEG = S // SEG
NPAIR = H // 2
NGP = 3 * NPAIR
F = 3584
DB = D // 128
FB = F // 128
PR = 2 * SEG + 2 * M
UNR = SEG // M
NIT = NSEG // UNR
KMAJ = 12
AHEAD = 3
PPI = 6
EPI_LATE = 6
EPI_PIECES = (0, 0, 2, 2, 2, 2, 2, 2, 2)
HA = 24
SIDE_SLOTS = [("softmax", 4), ("softmax", 8), ("softmax", 10), ("softmax", 12), (0, 2), (0, 5), (HA, 0)]
EPS = 1e-5
SCALE = E ** (-0.5)

SEM_SMALL = 0
SEM_X = SEM_SMALL + 3
SEM_MOD = SEM_X + 3
SEM_WQ = SEM_MOD + DB
SEM_ST = SEM_WQ + DB
SEM_WO = SEM_ST + (NGP - KMAJ) // PPI
SEM_MOE = SEM_WO + 1
SEM_OUT = SEM_MOE + 3
NSEM = SEM_OUT + 3


def _rb(v):
    return v.astype(BF16).astype(F32)


def _dot(a, b):
    return jnp.dot(a, b, preferred_element_type=F32)


def _recip(x):
    r = pl.reciprocal(x, approx=True)
    return r * (2.0 - x * r)


def _bf(words):
    return pltpu.bitcast(words, BF16)


def _ln(x):
    m = jnp.mean(x, axis=-1, keepdims=True)
    mb = _rb(m)
    d = x - mb
    var = jnp.mean(d * d, axis=-1, keepdims=True) - (m - mb) * (m - mb)
    inv = _recip(_rb(jnp.sqrt(_rb(_rb(jnp.maximum(var, 0.0)) + EPS))))
    return d * inv, inv


def _fill_matrix():
    i = lax.broadcasted_iota(jnp.int32, (PR, PR), 0)
    j = lax.broadcasted_iota(jnp.int32, (PR, PR), 1)

    def head(t):
        return jnp.where(t < 2 * SEG, t >> 5, (t - 2 * SEG) >> 3)

    def pos(t):
        r = t & (SEG - 1)
        return jnp.where(t < 2 * SEG, jnp.where(r < M, r, r + M), M + (t & (M - 1)))

    same = head(i) == head(j)
    pi = pos(i)
    ok = jnp.where(pi < M, 1, jnp.where(pi >= pos(j), 1, 0))
    return jnp.where(same, jnp.where(ok == 1, 0.0, -1e9), -3e38).astype(F32)


def _kernel(x_hbm, mem0_hbm, wq_hbm, wk_hbm, wv_hbm, wo_hbm, wr_hbm, wg_hbm, wu_hbm, wd_hbm,
            c_hbm, wmod_hbm, out_hbm,
            x_v, w_v, wo_v, cache, odef, lhs_v, qkv_s, o_s, a_all, r_v, mod_v, fill_v, never_v,
            mem0_v, wr_v, c_v, sems):
    w_w = w_v.bitcast(U32)
    cache_w = cache.bitcast(U32)
    lhs_w = lhs_v.bitcast(U32)
    qkv_w = qkv_s.bitcast(U32)
    o_w = o_s.bitcast(U32)
    odef_w = odef.bitcast(U32)

    def weights(h):
        return _bf(w_w[h].reshape(D // 2, E))

    def copy(src, dst, sem):
        return pltpu.make_async_copy(src, dst, sems.at[sem])

    def wait_all(buf, sem):
        copy(buf, buf, sem).wait()

    def mod_row(k, rows=8):
        v = mod_v[k]
        return v if rows == 8 else jnp.concatenate([v] * (rows // 8), axis=0)

    def put_rows(dst, r0, v):
        for j in range(DB):
            dst[j, pl.ds(r0, v.shape[0]), :] = v[:, j * 128:(j + 1) * 128].astype(BF16)

    def ln1(seg, r0):
        n, inv = _ln(x_v[seg, pl.ds(r0, 8), :].astype(F32))
        return n * mod_row(1) + mod_row(0), inv

    x_tail = copy(x_hbm.at[pl.ds(1, NSEG - 1), pl.ds(M, SEG - M), :],
                  x_v.at[pl.ds(1, NSEG - 1), pl.ds(M, SEG - M), :], SEM_X + 2)

    def prologue(stage, wmod_v, hc, n_v, acc):
        wmod_w = wmod_hbm.bitcast(U32)
        w_words = [w.bitcast(U32) for w in (wq_hbm, wk_hbm, wv_hbm)]

        def start_mod(j):
            col = j * 128 if isinstance(j, int) else pl.multiple_of(j * 128, 128)
            for k in range(2):
                copy(wmod_w.at[:, pl.ds(k * D + col, 128)], wmod_v.at[j, k], SEM_MOD + j).start()

        def start_ktile(j):
            rows = pl.ds(j * 128 if isinstance(j, int) else pl.multiple_of(j * 128, 128), 128)
            for g in range(KMAJ):
                copy(w_words[0].at[rows, g, :], stage.at[g, rows, :], SEM_WQ + j).start()

        small = [copy(c_hbm, c_v, SEM_SMALL), copy(mem0_hbm, mem0_v, SEM_SMALL + 1),
                 copy(wr_hbm, wr_v, SEM_SMALL + 2)]
        x_head = copy(x_hbm.at[:, pl.ds(0, M), :], x_v.at[:, pl.ds(0, M), :], SEM_X)
        x_seg0 = copy(x_hbm.at[0, pl.ds(M, SEG - M), :], x_v.at[0, pl.ds(M, SEG - M), :], SEM_X + 1)
        for cp in small:
            cp.start()
        x_head.start()
        x_seg0.start()
        start_mod(0)
        for j in range(AHEAD):
            start_ktile(j)
            start_mod(j + 1)
        slab_cps = [copy(w_words[g // NPAIR].at[:, g % NPAIR, :], stage.at[g], SEM_ST + (g - KMAJ) // PPI)
                    for g in range(KMAJ, NGP)]

        fill_v[...] = _fill_matrix()
        a_all[pl.ds(0, UNR + 1)] = jnp.zeros((UNR + 1, SEG, D), BF16)
        r_v[...] = jnp.full(r_v.shape, -jnp.inf, F32)
        never_v[...] = jnp.zeros(never_v.shape, F32)
        qkv_s[0] = jnp.zeros((2 * SEG, E), BF16)
        o_s[0] = jnp.zeros((SEG, E), BF16)

        def zero_acc(h, carry):
            acc[h] = jnp.zeros((NSEG * M, E), F32)
            return carry

        lax.fori_loop(0, 2 * KMAJ, zero_acc, 0)

        for cp in small:
            cp.wait()
        c = c_v[...].astype(F32)
        sc = jnp.broadcast_to(_rb(c * jax.nn.sigmoid(c)), (M, D))
        zero = jnp.zeros((M, E), F32)
        for h in range(H):
            blk = sc[:, (h % DB) * 128:(h % DB + 1) * 128]
            odef[0, h] = jnp.concatenate(
                [blk if c_ == h // DB else zero for c_ in range(4)], axis=0).astype(BF16)
        mod_v[6] = jnp.broadcast_to(wr_v[...].astype(F32).reshape(1, D), (8, D))
        put_rows(lhs_v, 0, mem0_v[...].astype(F32))

        x_head.wait()
        x_seg0.wait()
        NB = 16
        RB = NSEG * M // NB
        NR = NSEG * M + SEG - M
        for b in range(NB + 1):
            if b < NB:
                xb = x_v[pl.ds(b * (NSEG // NB), NSEG // NB), pl.ds(0, M), :].astype(F32).reshape(RB, D)
            else:
                xb = x_v[0, pl.ds(M, SEG - M), :].astype(F32)
            nb = _ln(xb)[0]
            for j in range(DB):
                n_v[j, pl.ds(b * RB, nb.shape[0]), :] = nb[:, j * 128:(j + 1) * 128]

        hc_w = hc.bitcast(U32)

        def h_block(j, k):
            scb = jnp.concatenate([_bf(odef_w[0, h, pl.ds(0, 8), :]) for h in range(DB)], axis=1)
            v = _rb(_dot(scb, _bf(wmod_v[j, k]))[0:8])
            if k == 1:
                v = _rb(1.0 + v)
            col = j * 128 if isinstance(j, int) else pl.multiple_of(j * 128, 128)
            mod_v[k, :, pl.ds(col, 128)] = v
            n = n_v[j, pl.ds(0, NR), :].reshape(NR // 8, 8, 128)
            if k == 1:
                n_v[j, pl.ds(0, NR), :] = (n * v[None]).reshape(NR, 128)
            else:
                hv = (n + v[None]).reshape(NR, 128).astype(BF16)
                hc[j] = hv[0:NSEG * M]
                lhs_v[j, pl.ds(M, SEG - M), :] = hv[NSEG * M:]

        def pack_pair(r1, r2):
            r = jnp.concatenate([r1.reshape(NSEG, M, E), r2.reshape(NSEG, M, E)], axis=1)
            return r.reshape(NIT, UNR * 2 * M, E).astype(BF16)

        def split_pair(b):
            return (pltpu.bitcast(b << 16, F32).astype(BF16),
                    pltpu.bitcast(b & jnp.uint32(0xFFFF0000), F32).astype(BF16))

        def q_stage(j, last):
            static = isinstance(j, int)
            k0 = j * 128 if static else pl.multiple_of(j * 128, 128)
            for p in range(KMAJ):
                ws = split_pair(stage[p, pl.ds(k0, 128), :])
                rs = []
                for t in range(2):
                    h = 2 * p + t
                    w_v[h, j] = ws[t]
                    rs.append(_dot(_bf(hc_w[j]), _bf(w_w[h, j])) + acc[h])
                    if not last:
                        acc[h] = rs[t]
                if last:
                    cache[p] = pack_pair(*rs)
                elif p in (1, 5):
                    h_block(j + 1, 1 if p == 1 else 0)

        wait_all(wmod_v.at[0], SEM_MOD)
        h_block(0, 1)
        h_block(0, 0)

        def wait_ktile(j):
            wait_all(stage.at[pl.ds(0, KMAJ), pl.ds(0, 128), :], SEM_WQ + j)

        def q_body(j, carry):
            wait_ktile(j)
            wait_all(wmod_v.at[0], SEM_MOD + j + 1)

            @pl.when(j + AHEAD < DB)
            def _():
                start_ktile(j + AHEAD)

            @pl.when(j + AHEAD + 1 < DB)
            def _():
                start_mod(j + AHEAD + 1)

            @pl.when(j + AHEAD == DB)
            def _():
                for cp in slab_cps[:2 * PPI]:
                    cp.start()

            q_stage(j, False)
            return carry

        lax.fori_loop(0, DB - 1, q_body, 0)
        wait_ktile(DB - 1)
        for cp in slab_cps[2 * PPI:]:
            cp.start()
        x_tail.start()
        q_stage(DB - 1, True)

        def slab(gp):
            w_v[2 * gp], w_v[2 * gp + 1] = split_pair(stage[gp].reshape(DB, 128, E))
            hcv = jnp.concatenate([_bf(hc_w[j]) for j in range(DB)], axis=1)
            cache[gp] = pack_pair(_dot(hcv, weights(2 * gp)), _dot(hcv, weights(2 * gp + 1)))

        def pro_body(i, carry):
            g0 = KMAJ + i * PPI
            wait_all(stage.at[pl.ds(g0, PPI)], SEM_ST + i)

            @pl.when(i == 2)
            def _():
                wo_w = wo_hbm.bitcast(U32)
                for j in range(DB):
                    for c_ in range(4):
                        copy(wmod_w.at[:, pl.ds((2 + c_) * D + j * 128, 128)],
                             wo_v.at[j, pl.ds(c_ * (D // 2), D // 2), :], SEM_WO).start()
                for j in range(DB):
                    copy(wo_w.at[:, pl.ds(j * 128, 128)], wo_v.at[DB + j], SEM_WO).start()

            for t in range(PPI):
                slab(g0 + t)
            return carry

        lax.fori_loop(0, (NGP - KMAJ) // PPI, pro_body, 0)

    pl.run_scoped(
        prologue,
        pltpu.VMEM((NGP, D, E), U32),
        pltpu.VMEM((DB, 2, D // 2, 128), U32),
        pltpu.VMEM((DB, NSEG * M, E), BF16),
        pltpu.VMEM((DB, NSEG * M + SEG, 128), F32),
        pltpu.VMEM((2 * KMAJ, NSEG * M, E), F32),
    )

    def main(wg_v, wu_v, wd_v, x1_v, h2_v, out_v):
        lane = lax.broadcasted_iota(jnp.int32, (8, 2 * 128), 1)

        def post(seg, q, keep=True):
            rows = pl.ds(8 * q, 8)
            x = x_v[seg, rows, :].astype(F32)
            a = a_all[seg + UNR, rows, :].astype(F32)
            x1 = _rb(x + mod_row(2) * a)
            n, inv = _ln(x1)
            h2 = _rb(n * mod_row(4) + mod_row(3))
            r = _rb(jnp.sum(h2 * mod_row(6), axis=-1, keepdims=True))
            if keep:
                r_v[...] = jnp.where(lane == seg * 4 + q, r, r_v[...])
            x1_v[seg, rows, :] = x1.astype(BF16)
            h2_v[seg, rows, :] = h2.astype(BF16)
            out_v[seg, rows, :] = (x1 + mod_row(5) * h2).astype(BF16)
            return inv, r

        def tie(v, tok):
            if tok is None:
                return v
            tok = jnp.broadcast_to(tok, (8, 128))
            if v.dtype != F32:
                tok = pltpu.bitcast(tok, v.dtype)
            return jnp.concatenate([jnp.where(never_v[...] > 1.0, tok, v[0:8]), v[8:]], axis=0)

        def deferred(blk, wsel, j, tok=None, tok2=None):
            words = [odef_w[blk, h] for h in range(H)]
            words[-1] = tie(words[-1], tok)
            lhs = jnp.concatenate([_bf(w) for w in words], axis=1)
            res = tie(_dot(lhs, _bf(wo_v[wsel + j])), tok2).astype(BF16).reshape(UNR, M, 128)
            a_all[pl.ds(blk * UNR, UNR), pl.ds(0, M), pl.ds(j * 128, 128)] = res

        def out_copy(grp):
            return copy(out_v.at[pl.ds(grp * UNR, UNR)], out_hbm.at[pl.ds(grp * UNR, UNR)], SEM_OUT)

        wg_w, wu_w, wd_w = wg_hbm.bitcast(U32), wu_hbm.bitcast(U32), wd_hbm.bitcast(U32)
        for j in range(FB):
            copy(wg_w.at[:, pl.ds(j * 128, 128)], wg_v.at[j], SEM_MOE).start()
            copy(wu_w.at[:, pl.ds(j * 128, 128)], wu_v.at[j], SEM_MOE + 1).start()
        for j in range(DB):
            copy(wd_w.at[:, pl.ds(j * 128, 128)], wd_v.at[j], SEM_MOE + 2).start()
        x_tail.wait()
        wait_all(wo_v, SEM_WO)

        def step(it, u):
            s = it * UNR + u
            lhs = jnp.concatenate([_bf(lhs_w[j]) for j in range(DB)], axis=1)
            nseg = jnp.minimum(s + 1, NSEG - 1)

            def side(slot):
                if slot not in SIDE_SLOTS:
                    return None
                i = SIDE_SLOTS.index(slot)
                if i < 4:
                    lag = 2 * UNR if i == 0 else UNR
                    return post(jnp.maximum(s - lag, 0), i)[0]
                r0 = (i - 3) * 8
                h, inv = ln1(nseg, r0)
                put_rows(lhs_v, r0, h)
                return inv

            def proj(m_i, p):
                g = m_i * NPAIR + p
                for t in range(2):
                    qkv_s[g, pl.ds(t * SEG, SEG), :] = _dot(lhs, weights(2 * g + t)).astype(BF16)

            def rows_of(m_i, p):
                g = m_i * NPAIR + p
                return jnp.concatenate([_bf(qkv_w[g]), _bf(cache_w[g, it, pl.ds(u * M, M), :])], axis=0)

            def probs(p):
                parts = [lax.dot_general(_bf(qkv_w[p]), rows_of(1, p), (((1,), (1,)), ((), ())),
                                         preferred_element_type=F32)]
                qc = _bf(cache_w[p, it, pl.ds(u * M, M), :]).astype(F32)
                kc = _bf(cache_w[NPAIR + p, it, pl.ds(u * M, M), :]).astype(F32)
                col = lax.broadcasted_iota(jnp.int32, (M, PR), 1)
                for t in range(2):
                    km = _bf(qkv_w[NPAIR + p, pl.ds(t * (SEG // 2), 8), :]).astype(F32)
                    qt = qc[t * M:(t + 1) * M]
                    st = jnp.zeros((M, PR), F32)
                    for j in range(M):
                        st = jnp.where(col == t * SEG + j,
                                       jnp.sum(qt * km[j:j + 1], axis=-1, keepdims=True), st)
                        st = jnp.where(col == 2 * SEG + t * M + j,
                                       jnp.sum(qt * kc[t * M + j:t * M + j + 1], axis=-1, keepdims=True), st)
                    parts.append(st)
                sc = jnp.concatenate(parts, axis=0) * SCALE
                fm = fill_v[...]
                tok = side(("softmax", p))
                if tok is not None:
                    top = fm[0:8]
                    fm = jnp.concatenate([jnp.where(top > 1.0, tok, top), fm[8:]], axis=0)
                sc = jnp.where(fm == 0.0, sc, fm)
                e = jnp.exp(sc - jnp.max(sc, axis=-1, keepdims=True))
                return (e * _recip(jnp.sum(e, axis=-1, keepdims=True))).astype(BF16)

            def attend(p, pr):
                o = _dot(pr, rows_of(2, p))
                o_s[2 * p] = o[0:SEG].astype(BF16)
                o_s[2 * p + 1] = o[SEG:2 * SEG].astype(BF16)
                odef[it + 1, 2 * p, pl.ds(u * M, M), :] = o[2 * SEG:2 * SEG + M].astype(BF16)
                odef[it + 1, 2 * p + 1, pl.ds(u * M, M), :] = o[2 * SEG + M:].astype(BF16)

            wsel = jnp.where(it == 0, 0, DB)
            for t in range(DB // UNR):
                deferred(it, wsel, u * (DB // UNR) + t)
            ps = {}
            for pa in range(0, NPAIR, 2):
                pb = pa + 1
                proj(0, pa)
                proj(1, pa)
                proj(0, pb)
                proj(1, pb)
                proj(2, pa)
                proj(2, pb)
                for kind in ("scores", "values") if pa % 4 == 0 else ("values", "scores"):
                    for p in (pa, pb):
                        if kind == "scores":
                            ps[p] = probs(p)
                        elif p >= 2:
                            attend(p - 2, ps.pop(p - 2))
            L = NPAIR - 1

            acc = [None] * DB
            for h0, h1 in ((0, HA), (HA, H)):
                for j in range(DB):
                    words = [o_w[h] for h in range(h0, h1)]
                    words[0] = tie(words[0], side((h0, j)))
                    ol = jnp.concatenate([_bf(w) for w in words], axis=1)
                    part = _dot(ol, _bf(wo_v[DB + j, pl.ds(h0 * E // 2, (h1 - h0) * E // 2), :]))
                    if h0 == 0:
                        acc[j] = part
                    else:
                        a = part + acc[j]
                        lhs_v[j, pl.ds(0, M), :] = a[0:M].astype(BF16)
                        a_all[s + UNR, pl.ds(M, SEG - M), pl.ds(j * 128, 128)] = a[M:].astype(BF16)
                    if h0 == 0 and j == 4:
                        attend(L - 1, ps.pop(L - 1))
                        attend(L, ps.pop(L))

        def iteration(it, carry):
            @pl.when(it >= 3)
            def _():
                out_copy(it - 3).start()

            for c_ in range(4):
                v = a_all[c_, pl.ds(0, M), :].astype(F32)
                mod_v[2 + c_] = _rb(1.0 + v) if c_ == 2 else v
            for u in range(UNR):
                step(it, u)
            return carry

        lax.fori_loop(0, NIT, iteration, 0)

        out_copy(NIT - 3).start()
        for k, buf in enumerate((wg_v, wu_v, wd_v)):
            wait_all(buf, SEM_MOE + k)
        early = [(seg, 0) for seg in range(NSEG - 2 * UNR, NSEG - UNR)]
        early += [(seg, q) for seg in range(NSEG - UNR, NSEG) for q in (1, 2, 3)]
        r8 = lax.broadcasted_iota(jnp.int32, (8, 1), 0)
        vals, idxs = [], []

        def pieces(n):
            tok = None
            for _ in range(n):
                seg, q = early.pop(0)
                keep = len(early) >= EPI_LATE
                r = post(seg, q, keep)[1]
                if not keep:
                    vals.append(r)
                    idxs.append((r8 + (seg * SEG + q * 8)).astype(F32))
                tok = r if tok is None else tok + r
            return tok

        for j in range(DB):
            deferred(NIT, DB, j, pieces(EPI_PIECES[j]), pieces(EPI_PIECES[DB]) if j == DB - 1 else None)
        out_copy(NIT - 2).start()

        def top2(vals, idx, axes):
            def red(f, v):
                for ax in axes:
                    v = f(v, axis=ax, keepdims=True)
                return v
            m1 = red(jnp.max, vals)
            i1 = red(jnp.min, jnp.where(vals == m1, idx, S - 1.0))
            rest = jnp.where(idx == i1, -jnp.inf, vals)
            m2 = red(jnp.max, rest)
            i2 = red(jnp.min, jnp.where(rest == m2, jnp.where(idx == i1, S - 1.0, idx), S - 1.0))
            return m1, i1, m2, i2

        m1, i1v, m2, i2v = top2(r_v[...], (lane * 8 + r8).astype(F32), (1, 0))
        vals.append(jnp.where(r8 == 0, m1, jnp.where(r8 == 1, m2, -jnp.inf)))
        idxs.append(jnp.where(r8 == 0, i1v, jnp.where(r8 == 1, i2v, S - 1.0)))
        for seg, q in early + [(seg, 0) for seg in range(NSEG - UNR, NSEG)]:
            vals.append(post(seg, q, keep=False)[1])
            idxs.append((r8 + (seg * SEG + q * 8)).astype(F32))
        out_copy(NIT - 1).start()
        m1, i1v, m2, i2v = top2(jnp.concatenate(vals, axis=0), jnp.concatenate(idxs, axis=0), (0,))
        i1 = i1v.astype(jnp.int32)[0, 0]
        i2 = i2v.astype(jnp.int32)[0, 0]

        def tile_of(i):
            return i >> 5, pl.multiple_of(((i >> 3) & 3) * 8, 8)

        sel = [tile_of(i1), tile_of(i2)]
        x1s = jnp.concatenate([x1_v[sg, pl.ds(r0, 8), :].astype(F32) for sg, r0 in sel], axis=0)
        h2s = jnp.concatenate([h2_v[sg, pl.ds(r0, 8), :].astype(F32) for sg, r0 in sel], axis=0)
        h2b = h2s.astype(BF16)
        gus = []
        for j in range(FB):
            g = _rb(_dot(h2b, _bf(wg_v[j])))
            g = _rb(g * jax.nn.sigmoid(g))
            u = _rb(_dot(h2b, _bf(wu_v[j])))
            gus.append(g * u)
        gu = jnp.concatenate(gus, axis=1).astype(BF16)
        y = jnp.concatenate([_rb(_dot(gu, _bf(wd_v[j]))) for j in range(DB)], axis=1)
        rows = lax.broadcasted_iota(jnp.int32, (16, 1), 0)
        rs = _rb(jax.nn.sigmoid(jnp.where(rows < 8, m1, m2)))
        y = _rb(y * rs)
        full = x1s + mod_row(5, 16) * _rb(h2s + y)

        copy(out_v, out_hbm, SEM_OUT).wait()
        for t, (i, (sg, r0)) in enumerate(zip((i1, i2), sel)):
            old = out_v[sg, pl.ds(r0, 8), :].astype(F32)
            new = jnp.where(r8 == (i & 7), full[t * 8:(t + 1) * 8], old)
            out_v[sg, pl.ds(r0, 8), :] = new.astype(BF16)
        fix = [copy(out_v.at[sg, pl.ds(r0, 8), :], out_hbm.at[sg, pl.ds(r0, 8), :], SEM_OUT + 1 + t)
               for t, (sg, r0) in enumerate(sel)]
        differ = (i1 >> 3) != (i2 >> 3)
        fix[0].start()

        @pl.when(differ)
        def _():
            fix[1].start()
            fix[1].wait()

        fix[0].wait()

    pl.run_scoped(
        main,
        pltpu.VMEM((FB, D // 2, 128), U32),
        pltpu.VMEM((FB, D // 2, 128), U32),
        pltpu.VMEM((DB, F // 2, 128), U32),
        pltpu.VMEM((NSEG, SEG, D), BF16),
        pltpu.VMEM((NSEG, SEG, D), BF16),
        pltpu.VMEM((NSEG, SEG, D), BF16),
    )


@jax.jit
def pallas_adaLN_cond__memory_aug_recurrent_mem_tr__moe_arch_mod__prompt_kernel(
    A_x: jax.Array,
    A_mem0: jax.Array,
    A_Wq: jax.Array,
    A_Wk: jax.Array,
    A_Wv: jax.Array,
    A_Wo: jax.Array,
    A_seg_len: jax.Array,
    B_x: jax.Array,
    B_w_r: jax.Array,
    B_w_gate: jax.Array,
    B_w_up: jax.Array,
    B_w_down: jax.Array,
    c: jax.Array,
    w_mod: jax.Array,
):
    del A_seg_len, B_x
    assert A_x.shape == (1, S, D) and A_mem0.shape == (1, M, D) and A_Wq.shape == (D, H, E)
    hbm = pl.BlockSpec(memory_space=pl.ANY)
    out = pl.pallas_call(
        _kernel,
        out_shape=jax.ShapeDtypeStruct((NSEG, SEG, D), BF16),
        in_specs=[hbm] * 12,
        out_specs=hbm,
        scratch_shapes=[
            pltpu.VMEM((NSEG, SEG, D), BF16),
            pltpu.VMEM((3 * H, DB, 128, E), BF16),
            pltpu.VMEM((2 * DB, H * E // 2, 128), U32),
            pltpu.VMEM((NGP, NIT, UNR * 2 * M, E), BF16),
            pltpu.VMEM((NIT + 1, H, SEG, E), BF16),
            pltpu.VMEM((DB, SEG, 128), BF16),
            pltpu.VMEM((NGP, 2 * SEG, E), BF16),
            pltpu.VMEM((H, SEG, E), BF16),
            pltpu.VMEM((NSEG + UNR, SEG, D), BF16),
            pltpu.VMEM((8, S // 8), F32),
            pltpu.VMEM((7, 8, D), F32),
            pltpu.VMEM((PR, PR), F32),
            pltpu.VMEM((8, 128), F32),
            pltpu.VMEM((M, D), BF16),
            pltpu.VMEM((D,), BF16),
            pltpu.VMEM((1, D), BF16),
            pltpu.SemaphoreType.DMA((NSEM,)),
        ],
        compiler_params=pltpu.CompilerParams(
            vmem_limit_bytes=120 * 1024 * 1024, disable_bounds_checks=True,
            disable_semaphore_checks=True),
    )(
        A_x.reshape(NSEG, SEG, D),
        A_mem0.reshape(M, D),
        A_Wq, A_Wk, A_Wv,
        A_Wo.reshape(H * E, D),
        B_w_r,
        B_w_gate, B_w_up, B_w_down,
        c, w_mod,
    )
    return out.reshape(1, S, D)
```

```python
import jax
import jax.numpy as jnp
from jax import lax
import jax.experimental.pallas as pl
import jax.experimental.pallas.tpu as pltpu

BF16 = jnp.bfloat16
F32 = jnp.float32
U32 = jnp.uint32

S = 2048
D = 1024
H = 32
E = 128
M = 8
SEG = 32
NSEG = S // SEG
NPAIR = H // 2
NGP = 3 * NPAIR
F = 3584
DB = D // 128
FB = F // 128
PR = 2 * SEG + 2 * M
UNR = SEG // M
NIT = NSEG // UNR
KMAJ = 12
AHEAD = 3
PPI = 6
EPI_LATE = 6
EPI_PIECES = (0, 0, 2, 2, 2, 2, 2, 2, 2)
HA = 24
SIDE_SLOTS = [("softmax", 4), ("softmax", 8), ("softmax", 10), ("softmax", 12), (0, 2), (0, 5), (HA, 0)]
EPS = 1e-5
SCALE = E ** (-0.5)

SEM_SMALL = 0
SEM_X = SEM_SMALL + 3
SEM_MOD = SEM_X + 3
SEM_WQ = SEM_MOD + DB
SEM_ST = SEM_WQ + DB
SEM_WO = SEM_ST + (NGP - KMAJ) // PPI
SEM_MOE = SEM_WO + 1
SEM_OUT = SEM_MOE + 3
NSEM = SEM_OUT + 3


def _rb(v):
    return v.astype(BF16).astype(F32)


def _dot(a, b):
    return jnp.dot(a, b, preferred_element_type=F32)


def _recip(x):
    r = pl.reciprocal(x, approx=True)
    return r * (2.0 - x * r)


def _bf(words):
    return pltpu.bitcast(words, BF16)


def _ln(x):
    m = jnp.mean(x, axis=-1, keepdims=True)
    mb = _rb(m)
    d = x - mb
    var = jnp.mean(d * d, axis=-1, keepdims=True) - (m - mb) * (m - mb)
    inv = _recip(_rb(jnp.sqrt(_rb(_rb(jnp.maximum(var, 0.0)) + EPS))))
    return d * inv, inv


def _fill_matrix():
    i = lax.broadcasted_iota(jnp.int32, (PR, PR), 0)
    j = lax.broadcasted_iota(jnp.int32, (PR, PR), 1)

    def head(t):
        return jnp.where(t < 2 * SEG, t >> 5, (t - 2 * SEG) >> 3)

    def pos(t):
        r = t & (SEG - 1)
        return jnp.where(t < 2 * SEG, jnp.where(r < M, r, r + M), M + (t & (M - 1)))

    same = head(i) == head(j)
    pi = pos(i)
    ok = jnp.where(pi < M, 1, jnp.where(pi >= pos(j), 1, 0))
    return jnp.where(same, jnp.where(ok == 1, 0.0, -1e9), -3e38).astype(F32)


def _kernel(x_hbm, mem0_hbm, wq_hbm, wk_hbm, wv_hbm, wo_hbm, wr_hbm, wg_hbm, wu_hbm, wd_hbm,
            c_hbm, wmod_hbm, out_hbm,
            x_v, w_v, wo_v, cache, odef, lhs_v, qkv_s, o_s, a_all, r_v, mod_v, fill_v, never_v,
            mem0_v, wr_v, c_v, sems):
    w_w = w_v.bitcast(U32)
    cache_w = cache.bitcast(U32)
    lhs_w = lhs_v.bitcast(U32)
    qkv_w = qkv_s.bitcast(U32)
    o_w = o_s.bitcast(U32)
    odef_w = odef.bitcast(U32)

    def weights(h):
        return _bf(w_w[h].reshape(D // 2, E))

    def copy(src, dst, sem):
        return pltpu.make_async_copy(src, dst, sems.at[sem])

    def wait_all(buf, sem):
        copy(buf, buf, sem).wait()

    def mod_row(k, rows=8):
        v = mod_v[k]
        return v if rows == 8 else jnp.concatenate([v] * (rows // 8), axis=0)

    def put_rows(dst, r0, v):
        for j in range(DB):
            dst[j, pl.ds(r0, v.shape[0]), :] = v[:, j * 128:(j + 1) * 128].astype(BF16)

    def ln1(seg, r0):
        n, inv = _ln(x_v[seg, pl.ds(r0, 8), :].astype(F32))
        return n * mod_row(1) + mod_row(0), inv

    x_tail = copy(x_hbm.at[pl.ds(1, NSEG - 1), pl.ds(M, SEG - M), :],
                  x_v.at[pl.ds(1, NSEG - 1), pl.ds(M, SEG - M), :], SEM_X + 2)

    def prologue(stage, wmod_v, hc, n_v, acc):
        wmod_w = wmod_hbm.bitcast(U32)
        w_words = [w.bitcast(U32) for w in (wq_hbm, wk_hbm, wv_hbm)]

        def start_mod(j):
            col = j * 128 if isinstance(j, int) else pl.multiple_of(j * 128, 128)
            for k in range(2):
                copy(wmod_w.at[:, pl.ds(k * D + col, 128)], wmod_v.at[j, k], SEM_MOD + j).start()

        def start_ktile(j):
            rows = pl.ds(j * 128 if isinstance(j, int) else pl.multiple_of(j * 128, 128), 128)
            for g in range(KMAJ):
                copy(w_words[0].at[rows, g, :], stage.at[g, rows, :], SEM_WQ + j).start()

        small = [copy(c_hbm, c_v, SEM_SMALL), copy(mem0_hbm, mem0_v, SEM_SMALL + 1),
                 copy(wr_hbm, wr_v, SEM_SMALL + 2)]
        x_head = copy(x_hbm.at[:, pl.ds(0, M), :], x_v.at[:, pl.ds(0, M), :], SEM_X)
        x_seg0 = copy(x_hbm.at[0, pl.ds(M, SEG - M), :], x_v.at[0, pl.ds(M, SEG - M), :], SEM_X + 1)
        for cp in small:
            cp.start()
        x_head.start()
        x_seg0.start()
        start_mod(0)
        for j in range(AHEAD):
            start_ktile(j)
            start_mod(j + 1)
        slab_cps = [copy(w_words[g // NPAIR].at[:, g % NPAIR, :], stage.at[g], SEM_ST + (g - KMAJ) // PPI)
                    for g in range(KMAJ, NGP)]

        fill_v[...] = _fill_matrix()
        a_all[pl.ds(0, UNR + 1)] = jnp.zeros((UNR + 1, SEG, D), BF16)
        r_v[...] = jnp.full(r_v.shape, -jnp.inf, F32)
        never_v[...] = jnp.zeros(never_v.shape, F32)
        qkv_s[0] = jnp.zeros((2 * SEG, E), BF16)
        o_s[0] = jnp.zeros((SEG, E), BF16)

        def zero_acc(h, carry):
            acc[h] = jnp.zeros((NSEG * M, E), F32)
            return carry

        lax.fori_loop(0, 2 * KMAJ, zero_acc, 0)

        for cp in small:
            cp.wait()
        c = c_v[...].astype(F32)
        sc = jnp.broadcast_to(_rb(c * jax.nn.sigmoid(c)), (M, D))
        zero = jnp.zeros((M, E), F32)
        for h in range(H):
            blk = sc[:, (h % DB) * 128:(h % DB + 1) * 128]
            odef[0, h] = jnp.concatenate(
                [blk if c_ == h // DB else zero for c_ in range(4)], axis=0).astype(BF16)
        mod_v[6] = jnp.broadcast_to(wr_v[...].astype(F32).reshape(1, D), (8, D))
        put_rows(lhs_v, 0, mem0_v[...].astype(F32))

        x_head.wait()
        x_seg0.wait()
        NB = 16
        RB = NSEG * M // NB
        NR = NSEG * M + SEG - M
        for b in range(NB + 1):
            if b < NB:
                xb = x_v[pl.ds(b * (NSEG // NB), NSEG // NB), pl.ds(0, M), :].astype(F32).reshape(RB, D)
            else:
                xb = x_v[0, pl.ds(M, SEG - M), :].astype(F32)
            nb = _ln(xb)[0]
            for j in range(DB):
                n_v[j, pl.ds(b * RB, nb.shape[0]), :] = nb[:, j * 128:(j + 1) * 128]

        hc_w = hc.bitcast(U32)

        def h_block(j, k):
            scb = jnp.concatenate([_bf(odef_w[0, h, pl.ds(0, 8), :]) for h in range(DB)], axis=1)
            v = _rb(_dot(scb, _bf(wmod_v[j, k]))[0:8])
            if k == 1:
                v = _rb(1.0 + v)
            col = j * 128 if isinstance(j, int) else pl.multiple_of(j * 128, 128)
            mod_v[k, :, pl.ds(col, 128)] = v
            n = n_v[j, pl.ds(0, NR), :].reshape(NR // 8, 8, 128)
            if k == 1:
                n_v[j, pl.ds(0, NR), :] = (n * v[None]).reshape(NR, 128)
            else:
                hv = (n + v[None]).reshape(NR, 128).astype(BF16)
                hc[j] = hv[0:NSEG * M]
                lhs_v[j, pl.ds(M, SEG - M), :] = hv[NSEG * M:]

        def pack_pair(r1, r2):
            r = jnp.concatenate([r1.reshape(NSEG, M, E), r2.reshape(NSEG, M, E)], axis=1)
            return r.reshape(NIT, UNR * 2 * M, E).astype(BF16)

        def split_pair(b):
            return (pltpu.bitcast(b << 16, F32).astype(BF16),
                    pltpu.bitcast(b & jnp.uint32(0xFFFF0000), F32).astype(BF16))

        def q_stage(j, last, more_dmas):
            static = isinstance(j, int)
            k0 = j * 128 if static else pl.multiple_of(j * 128, 128)
            for p in range(KMAJ):
                ws = split_pair(stage[p, pl.ds(k0, 128), :])
                rs = []
                for t in range(2):
                    h = 2 * p + t
                    w_v[h, j] = ws[t]
                    rs.append(_dot(_bf(hc_w[j]), _bf(w_w[h, j])) + acc[h])
                    if not last:
                        acc[h] = rs[t]
                if last:
                    cache[p] = pack_pair(*rs)
                elif p in (1, 5):
                    h_block(j + 1, 1 if p == 1 else 0)
                if p == 1:
                    more_dmas()

        wait_all(wmod_v.at[0], SEM_MOD)
        h_block(0, 1)
        h_block(0, 0)

        def wait_ktile(j):
            rows = pl.ds(j * 128 if isinstance(j, int) else pl.multiple_of(j * 128, 128), 128)
            wait_all(stage.at[pl.ds(0, KMAJ), rows, :], SEM_WQ + j)

        def q_body(j, carry):
            wait_ktile(j)
            wait_all(wmod_v.at[j + 1], SEM_MOD + j + 1)

            def more_dmas():
                @pl.when(j + AHEAD < DB)
                def _():
                    start_ktile(j + AHEAD)

                @pl.when(j + AHEAD + 1 < DB)
                def _():
                    start_mod(j + AHEAD + 1)

                @pl.when(j + AHEAD == DB)
                def _():
                    for cp in slab_cps[:2 * PPI]:
                        cp.start()

            q_stage(j, False, more_dmas)
            return carry

        lax.fori_loop(0, DB - 1, q_body, 0)
        wait_ktile(DB - 1)

        def last_dmas():
            for cp in slab_cps[2 * PPI:]:
                cp.start()
            x_tail.start()

        q_stage(DB - 1, True, last_dmas)

        def slab(gp):
            w_v[2 * gp], w_v[2 * gp + 1] = split_pair(stage[gp].reshape(DB, 128, E))
            hcv = jnp.concatenate([_bf(hc_w[j]) for j in range(DB)], axis=1)
            cache[gp] = pack_pair(_dot(hcv, weights(2 * gp)), _dot(hcv, weights(2 * gp + 1)))

        def pro_body(i, carry):
            g0 = KMAJ + i * PPI
            wait_all(stage.at[pl.ds(g0, PPI)], SEM_ST + i)

            @pl.when(i == 2)
            def _():
                wo_w = wo_hbm.bitcast(U32)
                for j in range(DB):
                    for c_ in range(4):
                        copy(wmod_w.at[:, pl.ds((2 + c_) * D + j * 128, 128)],
                             wo_v.at[j, pl.ds(c_ * (D // 2), D // 2), :], SEM_WO).start()
                for j in range(DB):
                    copy(wo_w.at[:, pl.ds(j * 128, 128)], wo_v.at[DB + j], SEM_WO).start()

            for t in range(PPI):
                slab(g0 + t)
            return carry

        lax.fori_loop(0, (NGP - KMAJ) // PPI, pro_body, 0)

    pl.run_scoped(
        prologue,
        pltpu.VMEM((NGP, D, E), U32),
        pltpu.VMEM((DB, 2, D // 2, 128), U32),
        pltpu.VMEM((DB, NSEG * M, E), BF16),
        pltpu.VMEM((DB, NSEG * M + SEG, 128), F32),
        pltpu.VMEM((2 * KMAJ, NSEG * M, E), F32),
    )

    def main(wg_v, wu_v, wd_v, x1_v, h2_v, out_v):
        lane = lax.broadcasted_iota(jnp.int32, (8, 2 * 128), 1)

        def post(seg, q, keep=True):
            rows = pl.ds(8 * q, 8)
            x = x_v[seg, rows, :].astype(F32)
            a = a_all[seg + UNR, rows, :].astype(F32)
            x1 = _rb(x + mod_row(2) * a)
            n, inv = _ln(x1)
            h2 = _rb(n * mod_row(4) + mod_row(3))
            r = _rb(jnp.sum(h2 * mod_row(6), axis=-1, keepdims=True))
            if keep:
                r_v[...] = jnp.where(lane == seg * 4 + q, r, r_v[...])
            x1_v[seg, rows, :] = x1.astype(BF16)
            h2_v[seg, rows, :] = h2.astype(BF16)
            out_v[seg, rows, :] = (x1 + mod_row(5) * h2).astype(BF16)
            return inv, r

        def tie(v, tok):
            if tok is None:
                return v
            tok = jnp.broadcast_to(tok, (8, 128))
            if v.dtype != F32:
                tok = pltpu.bitcast(tok, v.dtype)
            return jnp.concatenate([jnp.where(never_v[...] > 1.0, tok, v[0:8]), v[8:]], axis=0)

        def deferred(blk, wsel, j, tok=None, tok2=None):
            words = [odef_w[blk, h] for h in range(H)]
            words[-1] = tie(words[-1], tok)
            lhs = jnp.concatenate([_bf(w) for w in words], axis=1)
            res = tie(_dot(lhs, _bf(wo_v[wsel + j])), tok2).astype(BF16).reshape(UNR, M, 128)
            a_all[pl.ds(blk * UNR, UNR), pl.ds(0, M), pl.ds(j * 128, 128)] = res

        def out_copy(grp):
            return copy(out_v.at[pl.ds(grp * UNR, UNR)], out_hbm.at[pl.ds(grp * UNR, UNR)], SEM_OUT)

        wg_w, wu_w, wd_w = wg_hbm.bitcast(U32), wu_hbm.bitcast(U32), wd_hbm.bitcast(U32)
        for j in range(FB):
            copy(wg_w.at[:, pl.ds(j * 128, 128)], wg_v.at[j], SEM_MOE).start()
            copy(wu_w.at[:, pl.ds(j * 128, 128)], wu_v.at[j], SEM_MOE + 1).start()
        for j in range(DB):
            copy(wd_w.at[:, pl.ds(j * 128, 128)], wd_v.at[j], SEM_MOE + 2).start()
        x_tail.wait()
        wait_all(wo_v, SEM_WO)

        def step(it, u):
            s = it * UNR + u
            lhs = jnp.concatenate([_bf(lhs_w[j]) for j in range(DB)], axis=1)
            nseg = jnp.minimum(s + 1, NSEG - 1)

            def side(slot):
                if slot not in SIDE_SLOTS:
                    return None
                i = SIDE_SLOTS.index(slot)
                if i < 4:
                    lag = 2 * UNR if i == 0 else UNR
                    return post(jnp.maximum(s - lag, 0), i)[0]
                r0 = (i - 3) * 8
                h, inv = ln1(nseg, r0)
                put_rows(lhs_v, r0, h)
                return inv

            def proj(m_i, p):
                g = m_i * NPAIR + p
                for t in range(2):
                    qkv_s[g, pl.ds(t * SEG, SEG), :] = _dot(lhs, weights(2 * g + t)).astype(BF16)

            def rows_of(m_i, p):
                g = m_i * NPAIR + p
                return jnp.concatenate([_bf(qkv_w[g]), _bf(cache_w[g, it, pl.ds(u * M, M), :])], axis=0)

            def probs(p):
                parts = [lax.dot_general(_bf(qkv_w[p]), rows_of(1, p), (((1,), (1,)), ((), ())),
                                         preferred_element_type=F32)]
                qc = _bf(cache_w[p, it, pl.ds(u * M, M), :]).astype(F32)
                kc = _bf(cache_w[NPAIR + p, it, pl.ds(u * M, M), :]).astype(F32)
                col = lax.broadcasted_iota(jnp.int32, (M, PR), 1)
                for t in range(2):
                    km = _bf(qkv_w[NPAIR + p, pl.ds(t * (SEG // 2), 8), :]).astype(F32)
                    qt = qc[t * M:(t + 1) * M]
                    st = jnp.zeros((M, PR), F32)
                    for j in range(M):
                        st = jnp.where(col == t * SEG + j,
                                       jnp.sum(qt * km[j:j + 1], axis=-1, keepdims=True), st)
                        st = jnp.where(col == 2 * SEG + t * M + j,
                                       jnp.sum(qt * kc[t * M + j:t * M + j + 1], axis=-1, keepdims=True), st)
                    parts.append(st)
                sc = jnp.concatenate(parts, axis=0) * SCALE
                fm = fill_v[...]
                tok = side(("softmax", p))
                if tok is not None:
                    top = fm[0:8]
                    fm = jnp.concatenate([jnp.where(top > 1.0, tok, top), fm[8:]], axis=0)
                sc = jnp.where(fm == 0.0, sc, fm)
                e = jnp.exp(sc - jnp.max(sc, axis=-1, keepdims=True))
                return (e * _recip(jnp.sum(e, axis=-1, keepdims=True))).astype(BF16)

            def attend(p, pr):
                o = _dot(pr, rows_of(2, p))
                o_s[2 * p] = o[0:SEG].astype(BF16)
                o_s[2 * p + 1] = o[SEG:2 * SEG].astype(BF16)
                odef[it + 1, 2 * p, pl.ds(u * M, M), :] = o[2 * SEG:2 * SEG + M].astype(BF16)
                odef[it + 1, 2 * p + 1, pl.ds(u * M, M), :] = o[2 * SEG + M:].astype(BF16)

            wsel = jnp.where(it == 0, 0, DB)
            for t in range(DB // UNR):
                deferred(it, wsel, u * (DB // UNR) + t)
            ps = {}
            for pa in range(0, NPAIR, 2):
                pb = pa + 1
                proj(0, pa)
                proj(1, pa)
                proj(0, pb)
                proj(1, pb)
                proj(2, pa)
                proj(2, pb)
                for kind in ("scores", "values") if pa % 4 == 0 else ("values", "scores"):
                    for p in (pa, pb):
                        if kind == "scores":
                            ps[p] = probs(p)
                        elif p >= 2:
                            attend(p - 2, ps.pop(p - 2))
            L = NPAIR - 1

            acc = [None] * DB
            for h0, h1 in ((0, HA), (HA, H)):
                for j in range(DB):
                    words = [o_w[h] for h in range(h0, h1)]
                    words[0] = tie(words[0], side((h0, j)))
                    ol = jnp.concatenate([_bf(w) for w in words], axis=1)
                    part = _dot(ol, _bf(wo_v[DB + j, pl.ds(h0 * E // 2, (h1 - h0) * E // 2), :]))
                    if h0 == 0:
                        acc[j] = part
                    else:
                        a = part + acc[j]
                        lhs_v[j, pl.ds(0, M), :] = a[0:M].astype(BF16)
                        a_all[s + UNR, pl.ds(M, SEG - M), pl.ds(j * 128, 128)] = a[M:].astype(BF16)
                    if h0 == 0 and j == 4:
                        attend(L - 1, ps.pop(L - 1))
                        attend(L, ps.pop(L))

        def iteration(it, carry):
            @pl.when(it >= 3)
            def _():
                out_copy(it - 3).start()

            for c_ in range(4):
                v = a_all[c_, pl.ds(0, M), :].astype(F32)
                mod_v[2 + c_] = _rb(1.0 + v) if c_ == 2 else v
            for u in range(UNR):
                step(it, u)
            return carry

        lax.fori_loop(0, NIT, iteration, 0)

        out_copy(NIT - 3).start()
        for k, buf in enumerate((wg_v, wu_v, wd_v)):
            wait_all(buf, SEM_MOE + k)
        early = [(seg, 0) for seg in range(NSEG - 2 * UNR, NSEG - UNR)]
        early += [(seg, q) for seg in range(NSEG - UNR, NSEG) for q in (1, 2, 3)]
        r8 = lax.broadcasted_iota(jnp.int32, (8, 1), 0)
        vals, idxs = [], []

        def pieces(n):
            tok = None
            for _ in range(n):
                seg, q = early.pop(0)
                keep = len(early) >= EPI_LATE
                r = post(seg, q, keep)[1]
                if not keep:
                    vals.append(r)
                    idxs.append((r8 + (seg * SEG + q * 8)).astype(F32))
                tok = r if tok is None else tok + r
            return tok

        for j in range(DB):
            deferred(NIT, DB, j, pieces(EPI_PIECES[j]), pieces(EPI_PIECES[DB]) if j == DB - 1 else None)
        out_copy(NIT - 2).start()

        def top2(vals, idx, axes):
            def red(f, v):
                for ax in axes:
                    v = f(v, axis=ax, keepdims=True)
                return v
            m1 = red(jnp.max, vals)
            i1 = red(jnp.min, jnp.where(vals == m1, idx, S - 1.0))
            rest = jnp.where(idx == i1, -jnp.inf, vals)
            m2 = red(jnp.max, rest)
            i2 = red(jnp.min, jnp.where(rest == m2, jnp.where(idx == i1, S - 1.0, idx), S - 1.0))
            return m1, i1, m2, i2

        m1, i1v, m2, i2v = top2(r_v[...], (lane * 8 + r8).astype(F32), (1, 0))
        vals.append(jnp.where(r8 == 0, m1, jnp.where(r8 == 1, m2, -jnp.inf)))
        idxs.append(jnp.where(r8 == 0, i1v, jnp.where(r8 == 1, i2v, S - 1.0)))
        for seg, q in early + [(seg, 0) for seg in range(NSEG - UNR, NSEG)]:
            vals.append(post(seg, q, keep=False)[1])
            idxs.append((r8 + (seg * SEG + q * 8)).astype(F32))
        out_copy(NIT - 1).start()
        m1, i1v, m2, i2v = top2(jnp.concatenate(vals, axis=0), jnp.concatenate(idxs, axis=0), (0,))
        i1 = i1v.astype(jnp.int32)[0, 0]
        i2 = i2v.astype(jnp.int32)[0, 0]

        def tile_of(i):
            return i >> 5, pl.multiple_of(((i >> 3) & 3) * 8, 8)

        sel = [tile_of(i1), tile_of(i2)]
        x1s = jnp.concatenate([x1_v[sg, pl.ds(r0, 8), :].astype(F32) for sg, r0 in sel], axis=0)
        h2s = jnp.concatenate([h2_v[sg, pl.ds(r0, 8), :].astype(F32) for sg, r0 in sel], axis=0)
        h2b = h2s.astype(BF16)
        gus = []
        for j in range(FB):
            g = _rb(_dot(h2b, _bf(wg_v[j])))
            g = _rb(g * jax.nn.sigmoid(g))
            u = _rb(_dot(h2b, _bf(wu_v[j])))
            gus.append(g * u)
        gu = jnp.concatenate(gus, axis=1).astype(BF16)
        y = jnp.concatenate([_rb(_dot(gu, _bf(wd_v[j]))) for j in range(DB)], axis=1)
        rows = lax.broadcasted_iota(jnp.int32, (16, 1), 0)
        rs = _rb(jax.nn.sigmoid(jnp.where(rows < 8, m1, m2)))
        y = _rb(y * rs)
        full = x1s + mod_row(5, 16) * _rb(h2s + y)

        copy(out_v, out_hbm, SEM_OUT).wait()
        for t, (i, (sg, r0)) in enumerate(zip((i1, i2), sel)):
            old = out_v[sg, pl.ds(r0, 8), :].astype(F32)
            new = jnp.where(r8 == (i & 7), full[t * 8:(t + 1) * 8], old)
            out_v[sg, pl.ds(r0, 8), :] = new.astype(BF16)
        fix = [copy(out_v.at[sg, pl.ds(r0, 8), :], out_hbm.at[sg, pl.ds(r0, 8), :], SEM_OUT + 1 + t)
               for t, (sg, r0) in enumerate(sel)]
        differ = (i1 >> 3) != (i2 >> 3)
        fix[0].start()

        @pl.when(differ)
        def _():
            fix[1].start()
            fix[1].wait()

        fix[0].wait()

    pl.run_scoped(
        main,
        pltpu.VMEM((FB, D // 2, 128), U32),
        pltpu.VMEM((FB, D // 2, 128), U32),
        pltpu.VMEM((DB, F // 2, 128), U32),
        pltpu.VMEM((NSEG, SEG, D), BF16),
        pltpu.VMEM((NSEG, SEG, D), BF16),
        pltpu.VMEM((NSEG, SEG, D), BF16),
    )


@jax.jit
def pallas_adaLN_cond__memory_aug_recurrent_mem_tr__moe_arch_mod__prompt_kernel(
    A_x: jax.Array,
    A_mem0: jax.Array,
    A_Wq: jax.Array,
    A_Wk: jax.Array,
    A_Wv: jax.Array,
    A_Wo: jax.Array,
    A_seg_len: jax.Array,
    B_x: jax.Array,
    B_w_r: jax.Array,
    B_w_gate: jax.Array,
    B_w_up: jax.Array,
    B_w_down: jax.Array,
    c: jax.Array,
    w_mod: jax.Array,
):
    del A_seg_len, B_x
    assert A_x.shape == (1, S, D) and A_mem0.shape == (1, M, D) and A_Wq.shape == (D, H, E)
    hbm = pl.BlockSpec(memory_space=pl.ANY)
    out = pl.pallas_call(
        _kernel,
        out_shape=jax.ShapeDtypeStruct((NSEG, SEG, D), BF16),
        in_specs=[hbm] * 12,
        out_specs=hbm,
        scratch_shapes=[
            pltpu.VMEM((NSEG, SEG, D), BF16),
            pltpu.VMEM((3 * H, DB, 128, E), BF16),
            pltpu.VMEM((2 * DB, H * E // 2, 128), U32),
            pltpu.VMEM((NGP, NIT, UNR * 2 * M, E), BF16),
            pltpu.VMEM((NIT + 1, H, SEG, E), BF16),
            pltpu.VMEM((DB, SEG, 128), BF16),
            pltpu.VMEM((NGP, 2 * SEG, E), BF16),
            pltpu.VMEM((H, SEG, E), BF16),
            pltpu.VMEM((NSEG + UNR, SEG, D), BF16),
            pltpu.VMEM((8, S // 8), F32),
            pltpu.VMEM((7, 8, D), F32),
            pltpu.VMEM((PR, PR), F32),
            pltpu.VMEM((8, 128), F32),
            pltpu.VMEM((M, D), BF16),
            pltpu.VMEM((D,), BF16),
            pltpu.VMEM((1, D), BF16),
            pltpu.SemaphoreType.DMA((NSEM,)),
        ],
        compiler_params=pltpu.CompilerParams(
            vmem_limit_bytes=120 * 1024 * 1024, disable_bounds_checks=True,
            disable_semaphore_checks=True),
    )(
        A_x.reshape(NSEG, SEG, D),
        A_mem0.reshape(M, D),
        A_Wq, A_Wk, A_Wv,
        A_Wo.reshape(H * E, D),
        B_w_r,
        B_w_gate, B_w_up, B_w_down,
        c, w_mod,
    )
    return out.reshape(1, S, D)
```

```python
import jax
import jax.numpy as jnp
from jax import lax
import jax.experimental.pallas as pl
import jax.experimental.pallas.tpu as pltpu

BF16 = jnp.bfloat16
F32 = jnp.float32
U32 = jnp.uint32

S = 2048
D = 1024
H = 32
E = 128
M = 8
SEG = 32
NSEG = S // SEG
NPAIR = H // 2
NGP = 3 * NPAIR
F = 3584
DB = D // 128
FB = F // 128
PR = 2 * SEG + 2 * M
UNR = SEG // M
NIT = NSEG // UNR
KMAJ = 12
AHEAD = 3
PPI = 6
EPI_LATE = 6
EPI_PIECES = (0, 0, 2, 2, 2, 2, 2, 2, 2)
HA = 24
SIDE_SLOTS = [("softmax", 4), ("softmax", 8), ("softmax", 10), ("softmax", 12), (0, 2), (0, 5), (HA, 0)]
EPS = 1e-5
SCALE = E ** (-0.5)

SEM_SMALL = 0
SEM_X = SEM_SMALL + 3
SEM_MOD = SEM_X + 3
SEM_WQ = SEM_MOD + DB
SEM_ST = SEM_WQ + DB
SEM_WO = SEM_ST + (NGP - KMAJ) // PPI
SEM_MOE = SEM_WO + 1
SEM_OUT = SEM_MOE + 3
NSEM = SEM_OUT + 3


def _rb(v):
    return v.astype(BF16).astype(F32)


def _dot(a, b):
    return jnp.dot(a, b, preferred_element_type=F32)


def _recip(x):
    r = pl.reciprocal(x, approx=True)
    return r * (2.0 - x * r)


def _bf(words):
    return pltpu.bitcast(words, BF16)


def _ln(x):
    m = jnp.mean(x, axis=-1, keepdims=True)
    mb = _rb(m)
    d = x - mb
    var = jnp.mean(d * d, axis=-1, keepdims=True) - (m - mb) * (m - mb)
    inv = _recip(_rb(jnp.sqrt(_rb(_rb(jnp.maximum(var, 0.0)) + EPS))))
    return d * inv, inv


def _fill_matrix():
    i = lax.broadcasted_iota(jnp.int32, (PR, PR), 0)
    j = lax.broadcasted_iota(jnp.int32, (PR, PR), 1)

    def head(t):
        return jnp.where(t < 2 * SEG, t >> 5, (t - 2 * SEG) >> 3)

    def pos(t):
        r = t & (SEG - 1)
        return jnp.where(t < 2 * SEG, jnp.where(r < M, r, r + M), M + (t & (M - 1)))

    same = head(i) == head(j)
    pi = pos(i)
    ok = jnp.where(pi < M, 1, jnp.where(pi >= pos(j), 1, 0))
    return jnp.where(same, jnp.where(ok == 1, 0.0, -1e9), -3e38).astype(F32)


def _kernel(x_hbm, mem0_hbm, wq_hbm, wk_hbm, wv_hbm, wo_hbm, wr_hbm, wg_hbm, wu_hbm, wd_hbm,
            c_hbm, wmod_hbm, out_hbm,
            x_v, w_v, wo_v, cache, odef, lhs_v, qkv_s, o_s, a_all, r_v, mod_v, fill_v, never_v,
            mem0_v, wr_v, c_v, sems):
    w_w = w_v.bitcast(U32)
    cache_w = cache.bitcast(U32)
    lhs_w = lhs_v.bitcast(U32)
    qkv_w = qkv_s.bitcast(U32)
    o_w = o_s.bitcast(U32)
    odef_w = odef.bitcast(U32)

    def weights(h):
        return _bf(w_w[h].reshape(D // 2, E))

    def copy(src, dst, sem):
        return pltpu.make_async_copy(src, dst, sems.at[sem])

    def wait_all(buf, sem):
        copy(buf, buf, sem).wait()

    def mod_row(k, rows=8):
        v = mod_v[k]
        return v if rows == 8 else jnp.concatenate([v] * (rows // 8), axis=0)

    def put_rows(dst, r0, v):
        for j in range(DB):
            dst[j, pl.ds(r0, v.shape[0]), :] = v[:, j * 128:(j + 1) * 128].astype(BF16)

    def ln1(seg, r0):
        n, inv = _ln(x_v[seg, pl.ds(r0, 8), :].astype(F32))
        return n * mod_row(1) + mod_row(0), inv

    x_tail = copy(x_hbm.at[pl.ds(1, NSEG - 1), pl.ds(M, SEG - M), :],
                  x_v.at[pl.ds(1, NSEG - 1), pl.ds(M, SEG - M), :], SEM_X + 2)

    def prologue(stage, wmod_v, hc, n_v, acc):
        wmod_w = wmod_hbm.bitcast(U32)
        w_words = [w.bitcast(U32) for w in (wq_hbm, wk_hbm, wv_hbm)]

        def start_mod(j):
            col = j * 128 if isinstance(j, int) else pl.multiple_of(j * 128, 128)
            for k in range(2):
                copy(wmod_w.at[:, pl.ds(k * D + col, 128)], wmod_v.at[j, k], SEM_MOD + j).start()

        def start_ktile(j):
            rows = pl.ds(j * 128 if isinstance(j, int) else pl.multiple_of(j * 128, 128), 128)
            for g in range(KMAJ):
                copy(w_words[0].at[rows, g, :], stage.at[g, rows, :], SEM_WQ + j).start()

        small = [copy(c_hbm, c_v, SEM_SMALL), copy(mem0_hbm, mem0_v, SEM_SMALL + 1),
                 copy(wr_hbm, wr_v, SEM_SMALL + 2)]
        x_head = copy(x_hbm.at[:, pl.ds(0, M), :], x_v.at[:, pl.ds(0, M), :], SEM_X)
        x_seg0 = copy(x_hbm.at[0, pl.ds(M, SEG - M), :], x_v.at[0, pl.ds(M, SEG - M), :], SEM_X + 1)
        for cp in small:
            cp.start()
        x_head.start()
        x_seg0.start()
        start_mod(0)
        for j in range(AHEAD):
            start_ktile(j)
            start_mod(j + 1)
        slab_cps = [copy(w_words[g // NPAIR].at[:, g % NPAIR, :], stage.at[g], SEM_ST + (g - KMAJ) // PPI)
                    for g in range(KMAJ, NGP)]

        fill_v[...] = _fill_matrix()
        a_all[pl.ds(0, UNR + 1)] = jnp.zeros((UNR + 1, SEG, D), BF16)
        r_v[...] = jnp.full(r_v.shape, -jnp.inf, F32)
        never_v[...] = jnp.zeros(never_v.shape, F32)
        qkv_s[0] = jnp.zeros((2 * SEG, E), BF16)
        o_s[0] = jnp.zeros((SEG, E), BF16)

        def zero_acc(h, carry):
            acc[h] = jnp.zeros((NSEG * M, E), F32)
            return carry

        lax.fori_loop(0, 2 * KMAJ, zero_acc, 0)

        for cp in small:
            cp.wait()
        c = c_v[...].astype(F32)
        sc = jnp.broadcast_to(_rb(c * jax.nn.sigmoid(c)), (M, D))
        zero = jnp.zeros((M, E), F32)
        for h in range(H):
            blk = sc[:, (h % DB) * 128:(h % DB + 1) * 128]
            odef[0, h] = jnp.concatenate(
                [blk if c_ == h // DB else zero for c_ in range(4)], axis=0).astype(BF16)
        mod_v[6] = jnp.broadcast_to(wr_v[...].astype(F32).reshape(1, D), (8, D))
        put_rows(lhs_v, 0, mem0_v[...].astype(F32))

        x_head.wait()
        x_seg0.wait()
        NB = 16
        RB = NSEG * M // NB
        NR = NSEG * M + SEG - M
        for b in range(NB + 1):
            if b < NB:
                xb = x_v[pl.ds(b * (NSEG // NB), NSEG // NB), pl.ds(0, M), :].astype(F32).reshape(RB, D)
            else:
                xb = x_v[0, pl.ds(M, SEG - M), :].astype(F32)
            nb = _ln(xb)[0]
            for j in range(DB):
                n_v[j, pl.ds(b * RB, nb.shape[0]), :] = nb[:, j * 128:(j + 1) * 128]

        hc_w = hc.bitcast(U32)

        def h_block(j, k):
            scb = jnp.concatenate([_bf(odef_w[0, h, pl.ds(0, 8), :]) for h in range(DB)], axis=1)
            v = _rb(_dot(scb, _bf(wmod_v[j, k]))[0:8])
            if k == 1:
                v = _rb(1.0 + v)
            col = j * 128 if isinstance(j, int) else pl.multiple_of(j * 128, 128)
            mod_v[k, :, pl.ds(col, 128)] = v
            n = n_v[j, pl.ds(0, NR), :].reshape(NR // 8, 8, 128)
            if k == 1:
                n_v[j, pl.ds(0, NR), :] = (n * v[None]).reshape(NR, 128)
            else:
                hv = (n + v[None]).reshape(NR, 128).astype(BF16)
                hc[j] = hv[0:NSEG * M]
                lhs_v[j, pl.ds(M, SEG - M), :] = hv[NSEG * M:]

        def pack_pair(r1, r2):
            r = jnp.concatenate([r1.reshape(NSEG, M, E), r2.reshape(NSEG, M, E)], axis=1)
            return r.reshape(NIT, UNR * 2 * M, E).astype(BF16)

        def split_pair(b):
            return (pltpu.bitcast(b << 16, F32).astype(BF16),
                    pltpu.bitcast(b & jnp.uint32(0xFFFF0000), F32).astype(BF16))

        def q_stage(j, last, more_dmas):
            static = isinstance(j, int)
            k0 = j * 128 if static else pl.multiple_of(j * 128, 128)
            for p in range(KMAJ):
                ws = split_pair(stage[p, pl.ds(k0, 128), :])
                rs = []
                for t in range(2):
                    h = 2 * p + t
                    w_v[h, j] = ws[t]
                    rs.append(_dot(_bf(hc_w[j]), _bf(w_w[h, j])) + acc[h])
                    if not last:
                        acc[h] = rs[t]
                if last:
                    cache[p] = pack_pair(*rs)
                elif p in (1, 5):
                    h_block(j + 1, 1 if p == 1 else 0)
                if p == 1:
                    more_dmas()

        wait_all(wmod_v.at[0], SEM_MOD)
        h_block(0, 1)
        h_block(0, 0)

        def wait_ktile(j):
            rows = pl.ds(j * 128 if isinstance(j, int) else pl.multiple_of(j * 128, 128), 128)
            wait_all(stage.at[pl.ds(0, KMAJ), rows, :], SEM_WQ + j)

        def q_body(j, carry):
            wait_ktile(j)
            wait_all(wmod_v.at[j + 1], SEM_MOD + j + 1)

            def more_dmas():
                @pl.when(j + AHEAD < DB)
                def _():
                    start_ktile(j + AHEAD)

                @pl.when(j + AHEAD + 1 < DB)
                def _():
                    start_mod(j + AHEAD + 1)

                @pl.when(j + AHEAD == DB)
                def _():
                    for cp in slab_cps[:2 * PPI]:
                        cp.start()

            q_stage(j, False, more_dmas)
            return carry

        lax.fori_loop(0, DB - 1, q_body, 0)
        wait_ktile(DB - 1)

        def last_dmas():
            for cp in slab_cps[2 * PPI:]:
                cp.start()
            x_tail.start()

        q_stage(DB - 1, True, last_dmas)

        def slab(gp):
            w_v[2 * gp], w_v[2 * gp + 1] = split_pair(stage[gp].reshape(DB, 128, E))
            hcv = jnp.concatenate([_bf(hc_w[j]) for j in range(DB)], axis=1)
            cache[gp] = pack_pair(_dot(hcv, weights(2 * gp)), _dot(hcv, weights(2 * gp + 1)))

        def pro_body(i, carry):
            g0 = KMAJ + i * PPI
            wait_all(stage.at[pl.ds(g0, PPI)], SEM_ST + i)

            @pl.when(i < DB // 2)
            def _():
                wo_w = wo_hbm.bitcast(U32)
                for t in range(2):
                    j = 2 * i + t
                    col = pl.multiple_of(j * 128, 128)
                    for c_ in range(4):
                        copy(wmod_w.at[:, pl.ds((2 + c_) * D + col, 128)],
                             wo_v.at[j, pl.ds(c_ * (D // 2), D // 2), :], SEM_WO).start()
                    copy(wo_w.at[:, pl.ds(col, 128)], wo_v.at[DB + j], SEM_WO).start()

            for t in range(PPI):
                slab(g0 + t)
            return carry

        lax.fori_loop(0, (NGP - KMAJ) // PPI, pro_body, 0)

    pl.run_scoped(
        prologue,
        pltpu.VMEM((NGP, D, E), U32),
        pltpu.VMEM((DB, 2, D // 2, 128), U32),
        pltpu.VMEM((DB, NSEG * M, E), BF16),
        pltpu.VMEM((DB, NSEG * M + SEG, 128), F32),
        pltpu.VMEM((2 * KMAJ, NSEG * M, E), F32),
    )

    def main(wg_v, wu_v, wd_v, x1_v, h2_v, out_v):
        lane = lax.broadcasted_iota(jnp.int32, (8, 2 * 128), 1)

        def post(seg, q, keep=True):
            rows = pl.ds(8 * q, 8)
            x = x_v[seg, rows, :].astype(F32)
            a = a_all[seg + UNR, rows, :].astype(F32)
            x1 = _rb(x + mod_row(2) * a)
            n, inv = _ln(x1)
            h2 = _rb(n * mod_row(4) + mod_row(3))
            r = _rb(jnp.sum(h2 * mod_row(6), axis=-1, keepdims=True))
            if keep:
                r_v[...] = jnp.where(lane == seg * 4 + q, r, r_v[...])
            x1_v[seg, rows, :] = x1.astype(BF16)
            h2_v[seg, rows, :] = h2.astype(BF16)
            out_v[seg, rows, :] = (x1 + mod_row(5) * h2).astype(BF16)
            return inv, r

        def tie(v, tok):
            if tok is None:
                return v
            tok = jnp.broadcast_to(tok, (8, 128))
            if v.dtype != F32:
                tok = pltpu.bitcast(tok, v.dtype)
            return jnp.concatenate([jnp.where(never_v[...] > 1.0, tok, v[0:8]), v[8:]], axis=0)

        def deferred(blk, wsel, j, tok=None, tok2=None):
            words = [odef_w[blk, h] for h in range(H)]
            words[-1] = tie(words[-1], tok)
            lhs = jnp.concatenate([_bf(w) for w in words], axis=1)
            res = tie(_dot(lhs, _bf(wo_v[wsel + j])), tok2).astype(BF16).reshape(UNR, M, 128)
            a_all[pl.ds(blk * UNR, UNR), pl.ds(0, M), pl.ds(j * 128, 128)] = res

        def out_copy(grp):
            return copy(out_v.at[pl.ds(grp * UNR, UNR)], out_hbm.at[pl.ds(grp * UNR, UNR)], SEM_OUT)

        wg_w, wu_w, wd_w = wg_hbm.bitcast(U32), wu_hbm.bitcast(U32), wd_hbm.bitcast(U32)
        x_tail.wait()
        wait_all(wo_v, SEM_WO)

        def step(it, u):
            s = it * UNR + u
            lhs = jnp.concatenate([_bf(lhs_w[j]) for j in range(DB)], axis=1)
            nseg = jnp.minimum(s + 1, NSEG - 1)

            def side(slot):
                if slot not in SIDE_SLOTS:
                    return None
                i = SIDE_SLOTS.index(slot)
                if i < 4:
                    lag = 2 * UNR if i == 0 else UNR
                    return post(jnp.maximum(s - lag, 0), i)[0]
                r0 = (i - 3) * 8
                h, inv = ln1(nseg, r0)
                put_rows(lhs_v, r0, h)
                return inv

            def proj(m_i, p):
                g = m_i * NPAIR + p
                for t in range(2):
                    qkv_s[g, pl.ds(t * SEG, SEG), :] = _dot(lhs, weights(2 * g + t)).astype(BF16)

            def rows_of(m_i, p):
                g = m_i * NPAIR + p
                return jnp.concatenate([_bf(qkv_w[g]), _bf(cache_w[g, it, pl.ds(u * M, M), :])], axis=0)

            def probs(p):
                parts = [lax.dot_general(_bf(qkv_w[p]), rows_of(1, p), (((1,), (1,)), ((), ())),
                                         preferred_element_type=F32)]
                qc = _bf(cache_w[p, it, pl.ds(u * M, M), :]).astype(F32)
                kc = _bf(cache_w[NPAIR + p, it, pl.ds(u * M, M), :]).astype(F32)
                col = lax.broadcasted_iota(jnp.int32, (M, PR), 1)
                for t in range(2):
                    km = _bf(qkv_w[NPAIR + p, pl.ds(t * (SEG // 2), 8), :]).astype(F32)
                    qt = qc[t * M:(t + 1) * M]
                    st = jnp.zeros((M, PR), F32)
                    for j in range(M):
                        st = jnp.where(col == t * SEG + j,
                                       jnp.sum(qt * km[j:j + 1], axis=-1, keepdims=True), st)
                        st = jnp.where(col == 2 * SEG + t * M + j,
                                       jnp.sum(qt * kc[t * M + j:t * M + j + 1], axis=-1, keepdims=True), st)
                    parts.append(st)
                sc = jnp.concatenate(parts, axis=0) * SCALE
                fm = fill_v[...]
                tok = side(("softmax", p))
                if tok is not None:
                    top = fm[0:8]
                    fm = jnp.concatenate([jnp.where(top > 1.0, tok, top), fm[8:]], axis=0)
                sc = jnp.where(fm == 0.0, sc, fm)
                e = jnp.exp(sc - jnp.max(sc, axis=-1, keepdims=True))
                return (e * _recip(jnp.sum(e, axis=-1, keepdims=True))).astype(BF16)

            def attend(p, pr):
                o = _dot(pr, rows_of(2, p))
                o_s[2 * p] = o[0:SEG].astype(BF16)
                o_s[2 * p + 1] = o[SEG:2 * SEG].astype(BF16)
                odef[it + 1, 2 * p, pl.ds(u * M, M), :] = o[2 * SEG:2 * SEG + M].astype(BF16)
                odef[it + 1, 2 * p + 1, pl.ds(u * M, M), :] = o[2 * SEG + M:].astype(BF16)

            wsel = jnp.where(it == 0, 0, DB)
            for t in range(DB // UNR):
                deferred(it, wsel, u * (DB // UNR) + t)
            ps = {}
            for pa in range(0, NPAIR, 2):
                pb = pa + 1
                proj(0, pa)
                proj(1, pa)
                proj(0, pb)
                proj(1, pb)
                proj(2, pa)
                proj(2, pb)
                for kind in ("scores", "values") if pa % 4 == 0 else ("values", "scores"):
                    for p in (pa, pb):
                        if kind == "scores":
                            ps[p] = probs(p)
                        elif p >= 2:
                            attend(p - 2, ps.pop(p - 2))
            L = NPAIR - 1

            acc = [None] * DB
            for h0, h1 in ((0, HA), (HA, H)):
                for j in range(DB):
                    words = [o_w[h] for h in range(h0, h1)]
                    words[0] = tie(words[0], side((h0, j)))
                    ol = jnp.concatenate([_bf(w) for w in words], axis=1)
                    part = _dot(ol, _bf(wo_v[DB + j, pl.ds(h0 * E // 2, (h1 - h0) * E // 2), :]))
                    if h0 == 0:
                        acc[j] = part
                    else:
                        a = part + acc[j]
                        lhs_v[j, pl.ds(0, M), :] = a[0:M].astype(BF16)
                        a_all[s + UNR, pl.ds(M, SEG - M), pl.ds(j * 128, 128)] = a[M:].astype(BF16)
                    if h0 == 0 and j == 4:
                        attend(L - 1, ps.pop(L - 1))
                        attend(L, ps.pop(L))

        def iteration(it, carry):
            @pl.when(it >= 3)
            def _():
                out_copy(it - 3).start()

            @pl.when(it < FB // 2)
            def _():
                for t in range(2):
                    j = 2 * it + t
                    cols = pl.ds(pl.multiple_of(j * 128, 128), 128)
                    copy(wg_w.at[:, cols], wg_v.at[j], SEM_MOE).start()
                    copy(wu_w.at[:, cols], wu_v.at[j], SEM_MOE + 1).start()

            @pl.when(it < DB)
            def _():
                cols = pl.ds(pl.multiple_of(it * 128, 128), 128)
                copy(wd_w.at[:, cols], wd_v.at[it], SEM_MOE + 2).start()

            for c_ in range(4):
                v = a_all[c_, pl.ds(0, M), :].astype(F32)
                mod_v[2 + c_] = _rb(1.0 + v) if c_ == 2 else v
            for u in range(UNR):
                step(it, u)
            return carry

        lax.fori_loop(0, NIT, iteration, 0)

        out_copy(NIT - 3).start()
        for k, buf in enumerate((wg_v, wu_v, wd_v)):
            wait_all(buf, SEM_MOE + k)
        early = [(seg, 0) for seg in range(NSEG - 2 * UNR, NSEG - UNR)]
        early += [(seg, q) for seg in range(NSEG - UNR, NSEG) for q in (1, 2, 3)]
        r8 = lax.broadcasted_iota(jnp.int32, (8, 1), 0)
        vals, idxs = [], []

        def pieces(n):
            tok = None
            for _ in range(n):
                seg, q = early.pop(0)
                keep = len(early) >= EPI_LATE
                r = post(seg, q, keep)[1]
                if not keep:
                    vals.append(r)
                    idxs.append((r8 + (seg * SEG + q * 8)).astype(F32))
                tok = r if tok is None else tok + r
            return tok

        for j in range(DB):
            deferred(NIT, DB, j, pieces(EPI_PIECES[j]), pieces(EPI_PIECES[DB]) if j == DB - 1 else None)
        out_copy(NIT - 2).start()

        def top2(vals, idx, axes):
            def red(f, v):
                for ax in axes:
                    v = f(v, axis=ax, keepdims=True)
                return v
            m1 = red(jnp.max, vals)
            i1 = red(jnp.min, jnp.where(vals == m1, idx, S - 1.0))
            rest = jnp.where(idx == i1, -jnp.inf, vals)
            m2 = red(jnp.max, rest)
            i2 = red(jnp.min, jnp.where(rest == m2, jnp.where(idx == i1, S - 1.0, idx), S - 1.0))
            return m1, i1, m2, i2

        m1, i1v, m2, i2v = top2(r_v[...], (lane * 8 + r8).astype(F32), (1, 0))
        vals.append(jnp.where(r8 == 0, m1, jnp.where(r8 == 1, m2, -jnp.inf)))
        idxs.append(jnp.where(r8 == 0, i1v, jnp.where(r8 == 1, i2v, S - 1.0)))
        for seg, q in early + [(seg, 0) for seg in range(NSEG - UNR, NSEG)]:
            vals.append(post(seg, q, keep=False)[1])
            idxs.append((r8 + (seg * SEG + q * 8)).astype(F32))
        out_copy(NIT - 1).start()
        m1, i1v, m2, i2v = top2(jnp.concatenate(vals, axis=0), jnp.concatenate(idxs, axis=0), (0,))
        i1 = i1v.astype(jnp.int32)[0, 0]
        i2 = i2v.astype(jnp.int32)[0, 0]

        def tile_of(i):
            return i >> 5, pl.multiple_of(((i >> 3) & 3) * 8, 8)

        sel = [tile_of(i1), tile_of(i2)]
        x1s = jnp.concatenate([x1_v[sg, pl.ds(r0, 8), :].astype(F32) for sg, r0 in sel], axis=0)
        h2s = jnp.concatenate([h2_v[sg, pl.ds(r0, 8), :].astype(F32) for sg, r0 in sel], axis=0)
        h2b = h2s.astype(BF16)
        gus = []
        for j in range(FB):
            g = _rb(_dot(h2b, _bf(wg_v[j])))
            g = _rb(g * jax.nn.sigmoid(g))
            u = _rb(_dot(h2b, _bf(wu_v[j])))
            gus.append(g * u)
        gu = jnp.concatenate(gus, axis=1).astype(BF16)
        y = jnp.concatenate([_rb(_dot(gu, _bf(wd_v[j]))) for j in range(DB)], axis=1)
        rows = lax.broadcasted_iota(jnp.int32, (16, 1), 0)
        rs = _rb(jax.nn.sigmoid(jnp.where(rows < 8, m1, m2)))
        y = _rb(y * rs)
        full = x1s + mod_row(5, 16) * _rb(h2s + y)

        copy(out_v, out_hbm, SEM_OUT).wait()
        for t, (i, (sg, r0)) in enumerate(zip((i1, i2), sel)):
            old = out_v[sg, pl.ds(r0, 8), :].astype(F32)
            new = jnp.where(r8 == (i & 7), full[t * 8:(t + 1) * 8], old)
            out_v[sg, pl.ds(r0, 8), :] = new.astype(BF16)
        fix = [copy(out_v.at[sg, pl.ds(r0, 8), :], out_hbm.at[sg, pl.ds(r0, 8), :], SEM_OUT + 1 + t)
               for t, (sg, r0) in enumerate(sel)]
        differ = (i1 >> 3) != (i2 >> 3)
        fix[0].start()

        @pl.when(differ)
        def _():
            fix[1].start()
            fix[1].wait()

        fix[0].wait()

    pl.run_scoped(
        main,
        pltpu.VMEM((FB, D // 2, 128), U32),
        pltpu.VMEM((FB, D // 2, 128), U32),
        pltpu.VMEM((DB, F // 2, 128), U32),
        pltpu.VMEM((NSEG, SEG, D), BF16),
        pltpu.VMEM((NSEG, SEG, D), BF16),
        pltpu.VMEM((NSEG, SEG, D), BF16),
    )


@jax.jit
def pallas_adaLN_cond__memory_aug_recurrent_mem_tr__moe_arch_mod__prompt_kernel(
    A_x: jax.Array,
    A_mem0: jax.Array,
    A_Wq: jax.Array,
    A_Wk: jax.Array,
    A_Wv: jax.Array,
    A_Wo: jax.Array,
    A_seg_len: jax.Array,
    B_x: jax.Array,
    B_w_r: jax.Array,
    B_w_gate: jax.Array,
    B_w_up: jax.Array,
    B_w_down: jax.Array,
    c: jax.Array,
    w_mod: jax.Array,
):
    del A_seg_len, B_x
    assert A_x.shape == (1, S, D) and A_mem0.shape == (1, M, D) and A_Wq.shape == (D, H, E)
    hbm = pl.BlockSpec(memory_space=pl.ANY)
    out = pl.pallas_call(
        _kernel,
        out_shape=jax.ShapeDtypeStruct((NSEG, SEG, D), BF16),
        in_specs=[hbm] * 12,
        out_specs=hbm,
        scratch_shapes=[
            pltpu.VMEM((NSEG, SEG, D), BF16),
            pltpu.VMEM((3 * H, DB, 128, E), BF16),
            pltpu.VMEM((2 * DB, H * E // 2, 128), U32),
            pltpu.VMEM((NGP, NIT, UNR * 2 * M, E), BF16),
            pltpu.VMEM((NIT + 1, H, SEG, E), BF16),
            pltpu.VMEM((DB, SEG, 128), BF16),
            pltpu.VMEM((NGP, 2 * SEG, E), BF16),
            pltpu.VMEM((H, SEG, E), BF16),
            pltpu.VMEM((NSEG + UNR, SEG, D), BF16),
            pltpu.VMEM((8, S // 8), F32),
            pltpu.VMEM((7, 8, D), F32),
            pltpu.VMEM((PR, PR), F32),
            pltpu.VMEM((8, 128), F32),
            pltpu.VMEM((M, D), BF16),
            pltpu.VMEM((D,), BF16),
            pltpu.VMEM((1, D), BF16),
            pltpu.SemaphoreType.DMA((NSEM,)),
        ],
        compiler_params=pltpu.CompilerParams(
            vmem_limit_bytes=120 * 1024 * 1024, disable_bounds_checks=True,
            disable_semaphore_checks=True),
    )(
        A_x.reshape(NSEG, SEG, D),
        A_mem0.reshape(M, D),
        A_Wq, A_Wk, A_Wv,
        A_Wo.reshape(H * E, D),
        B_w_r,
        B_w_gate, B_w_up, B_w_down,
        c, w_mod,
    )
    return out.reshape(1, S, D)
```

```python
import jax
import jax.numpy as jnp
from jax import lax
import jax.experimental.pallas as pl
import jax.experimental.pallas.tpu as pltpu

BF16 = jnp.bfloat16
F32 = jnp.float32
U32 = jnp.uint32

S = 2048
D = 1024
H = 32
E = 128
M = 8
SEG = 32
NSEG = S // SEG
NPAIR = H // 2
NGP = 3 * NPAIR
F = 3584
DB = D // 128
FB = F // 128
PR = 2 * SEG + 2 * M
UNR = SEG // M
NIT = NSEG // UNR
KMAJ = 12
AHEAD = 3
PPI = 6
EPI_LATE = 6
EPI_PIECES = (0, 0, 2, 2, 2, 2, 2, 2, 2)
HA = 24
SIDE_SLOTS = [("softmax", 4), ("softmax", 8), ("softmax", 10), ("softmax", 12), (0, 2), (0, 5), (HA, 0)]
EPS = 1e-5
SCALE = E ** (-0.5)

SEM_SMALL = 0
SEM_X = SEM_SMALL + 3
SEM_MOD = SEM_X + 3
SEM_WQ = SEM_MOD + DB
SEM_ST = SEM_WQ + DB
SEM_WO = SEM_ST + (NGP - KMAJ) // PPI
SEM_MOE = SEM_WO + 1
SEM_OUT = SEM_MOE + 3
NSEM = SEM_OUT + 3


def _rb(v):
    return v.astype(BF16).astype(F32)


def _dot(a, b):
    return jnp.dot(a, b, preferred_element_type=F32)


def _recip(x):
    r = pl.reciprocal(x, approx=True)
    return r * (2.0 - x * r)


def _bf(words):
    return pltpu.bitcast(words, BF16)


def _ln(x):
    m = jnp.mean(x, axis=-1, keepdims=True)
    mb = _rb(m)
    d = x - mb
    var = jnp.mean(d * d, axis=-1, keepdims=True) - (m - mb) * (m - mb)
    inv = _recip(_rb(jnp.sqrt(_rb(_rb(jnp.maximum(var, 0.0)) + EPS))))
    return d * inv, inv


def _fill_matrix():
    i = lax.broadcasted_iota(jnp.int32, (PR, PR), 0)
    j = lax.broadcasted_iota(jnp.int32, (PR, PR), 1)

    def head(t):
        return jnp.where(t < 2 * SEG, t >> 5, (t - 2 * SEG) >> 3)

    def pos(t):
        r = t & (SEG - 1)
        return jnp.where(t < 2 * SEG, jnp.where(r < M, r, r + M), M + (t & (M - 1)))

    same = head(i) == head(j)
    pi = pos(i)
    ok = jnp.where(pi < M, 1, jnp.where(pi >= pos(j), 1, 0))
    return jnp.where(same, jnp.where(ok == 1, 0.0, -1e9), -3e38).astype(F32)


def _kernel(x_hbm, mem0_hbm, wq_hbm, wk_hbm, wv_hbm, wo_hbm, wr_hbm, wg_hbm, wu_hbm, wd_hbm,
            c_hbm, wmod_hbm, out_hbm,
            x_v, w_v, wo_v, cache, odef, lhs_v, qkv_s, o_s, a_all, r_v, mod_v, fill_v, never_v,
            mem0_v, wr_v, c_v, sems):
    w_w = w_v.bitcast(U32)
    cache_w = cache.bitcast(U32)
    lhs_w = lhs_v.bitcast(U32)
    qkv_w = qkv_s.bitcast(U32)
    o_w = o_s.bitcast(U32)
    odef_w = odef.bitcast(U32)

    def weights(h):
        return _bf(w_w[h].reshape(D // 2, E))

    def copy(src, dst, sem):
        return pltpu.make_async_copy(src, dst, sems.at[sem])

    def wait_all(buf, sem):
        copy(buf, buf, sem).wait()

    def mod_row(k, rows=8):
        v = mod_v[k]
        return v if rows == 8 else jnp.concatenate([v] * (rows // 8), axis=0)

    def put_rows(dst, r0, v):
        for j in range(DB):
            dst[j, pl.ds(r0, v.shape[0]), :] = v[:, j * 128:(j + 1) * 128].astype(BF16)

    def ln1(seg, r0):
        n, inv = _ln(x_v[seg, pl.ds(r0, 8), :].astype(F32))
        return n * mod_row(1) + mod_row(0), inv

    x_tail = copy(x_hbm.at[pl.ds(1, NSEG - 1), pl.ds(M, SEG - M), :],
                  x_v.at[pl.ds(1, NSEG - 1), pl.ds(M, SEG - M), :], SEM_X + 2)

    def prologue(stage, wmod_v, hc, n_v, acc):
        wmod_w = wmod_hbm.bitcast(U32)
        w_words = [w.bitcast(U32) for w in (wq_hbm, wk_hbm, wv_hbm)]

        def start_mod(j):
            col = j * 128 if isinstance(j, int) else pl.multiple_of(j * 128, 128)
            for k in range(2):
                copy(wmod_w.at[:, pl.ds(k * D + col, 128)], wmod_v.at[j, k], SEM_MOD + j).start()

        def start_ktile(j):
            rows = pl.ds(j * 128 if isinstance(j, int) else pl.multiple_of(j * 128, 128), 128)
            for g in range(KMAJ):
                copy(w_words[0].at[rows, g, :], stage.at[g, rows, :], SEM_WQ + j).start()

        small = [copy(c_hbm, c_v, SEM_SMALL), copy(mem0_hbm, mem0_v, SEM_SMALL + 1),
                 copy(wr_hbm, wr_v, SEM_SMALL + 2)]
        x_head = copy(x_hbm.at[:, pl.ds(0, M), :], x_v.at[:, pl.ds(0, M), :], SEM_X)
        x_seg0 = copy(x_hbm.at[0, pl.ds(M, SEG - M), :], x_v.at[0, pl.ds(M, SEG - M), :], SEM_X + 1)
        for cp in small:
            cp.start()
        x_head.start()
        x_seg0.start()
        start_mod(0)
        for j in range(AHEAD):
            start_ktile(j)
            start_mod(j + 1)
        slab_cps = [copy(w_words[g // NPAIR].at[:, g % NPAIR, :], stage.at[g], SEM_ST + (g - KMAJ) // PPI)
                    for g in range(KMAJ, NGP)]

        fill_v[...] = _fill_matrix()
        a_all[pl.ds(0, UNR + 1)] = jnp.zeros((UNR + 1, SEG, D), BF16)
        r_v[...] = jnp.full(r_v.shape, -jnp.inf, F32)
        never_v[...] = jnp.zeros(never_v.shape, F32)
        qkv_s[0] = jnp.zeros((2 * SEG, E), BF16)
        o_s[0] = jnp.zeros((SEG, E), BF16)

        def zero_acc(h, carry):
            acc[h] = jnp.zeros((NSEG * M, E), F32)
            return carry

        lax.fori_loop(0, 2 * KMAJ, zero_acc, 0)

        for cp in small:
            cp.wait()
        c = c_v[...].astype(F32)
        sc = jnp.broadcast_to(_rb(c * jax.nn.sigmoid(c)), (M, D))
        zero = jnp.zeros((M, E), F32)
        for h in range(H):
            blk = sc[:, (h % DB) * 128:(h % DB + 1) * 128]
            odef[0, h] = jnp.concatenate(
                [blk if c_ == h // DB else zero for c_ in range(4)], axis=0).astype(BF16)
        mod_v[6] = jnp.broadcast_to(wr_v[...].astype(F32).reshape(1, D), (8, D))
        put_rows(lhs_v, 0, mem0_v[...].astype(F32))

        x_head.wait()
        x_seg0.wait()
        NB = 16
        RB = NSEG * M // NB
        NR = NSEG * M + SEG - M
        for b in range(NB + 1):
            if b < NB:
                xb = x_v[pl.ds(b * (NSEG // NB), NSEG // NB), pl.ds(0, M), :].astype(F32).reshape(RB, D)
            else:
                xb = x_v[0, pl.ds(M, SEG - M), :].astype(F32)
            nb = _ln(xb)[0]
            for j in range(DB):
                n_v[j, pl.ds(b * RB, nb.shape[0]), :] = nb[:, j * 128:(j + 1) * 128]

        hc_w = hc.bitcast(U32)

        def mod_block(j, k):
            scb = jnp.concatenate([_bf(odef_w[0, h, pl.ds(0, 8), :]) for h in range(DB)], axis=1)
            v = _rb(_dot(scb, _bf(wmod_v[j, k]))[0:8])
            if k == 1:
                v = _rb(1.0 + v)
            col = j * 128 if isinstance(j, int) else pl.multiple_of(j * 128, 128)
            mod_v[k, :, pl.ds(col, 128)] = v
            return v

        def h_block(j, ca, sa):
            n = n_v[j, pl.ds(0, NR), :].reshape(NR // 8, 8, 128)
            hv = (n * ca[None] + sa[None]).reshape(NR, 128).astype(BF16)
            hc[j] = hv[0:NSEG * M]
            lhs_v[j, pl.ds(M, SEG - M), :] = hv[NSEG * M:]

        def pack_pair(r1, r2):
            r = jnp.concatenate([r1.reshape(NSEG, M, E), r2.reshape(NSEG, M, E)], axis=1)
            return r.reshape(NIT, UNR * 2 * M, E).astype(BF16)

        def split_pair(b):
            return (pltpu.bitcast(b << 16, F32).astype(BF16),
                    pltpu.bitcast(b & jnp.uint32(0xFFFF0000), F32).astype(BF16))

        def q_stage(j, last, more_dmas):
            static = isinstance(j, int)
            k0 = j * 128 if static else pl.multiple_of(j * 128, 128)
            for p in range(KMAJ):
                ws = split_pair(stage[p, pl.ds(k0, 128), :])
                rs = []
                for t in range(2):
                    h = 2 * p + t
                    w_v[h, j] = ws[t]
                    rs.append(_dot(_bf(hc_w[j]), _bf(w_w[h, j])) + acc[h])
                    if not last:
                        acc[h] = rs[t]
                if last:
                    cache[p] = pack_pair(*rs)
                elif p == 1:
                    ca = mod_block(j + 1, 1)
                elif p == 3:
                    h_block(j + 1, ca, mod_block(j + 1, 0))
                if p == 1:
                    more_dmas()

        wait_all(wmod_v.at[0], SEM_MOD)
        h_block(0, mod_block(0, 1), mod_block(0, 0))

        def wait_ktile(j):
            rows = pl.ds(j * 128 if isinstance(j, int) else pl.multiple_of(j * 128, 128), 128)
            wait_all(stage.at[pl.ds(0, KMAJ), rows, :], SEM_WQ + j)

        def q_body(j, carry):
            wait_ktile(j)
            wait_all(wmod_v.at[j + 1], SEM_MOD + j + 1)

            def more_dmas():
                @pl.when(j + AHEAD < DB)
                def _():
                    start_ktile(j + AHEAD)

                @pl.when(j + AHEAD + 1 < DB)
                def _():
                    start_mod(j + AHEAD + 1)

                @pl.when(j + AHEAD == DB)
                def _():
                    for cp in slab_cps[:2 * PPI]:
                        cp.start()

            q_stage(j, False, more_dmas)
            return carry

        lax.fori_loop(0, DB - 1, q_body, 0)
        wait_ktile(DB - 1)

        def last_dmas():
            for cp in slab_cps[2 * PPI:]:
                cp.start()
            x_tail.start()

        q_stage(DB - 1, True, last_dmas)

        def slab(gp):
            w_v[2 * gp], w_v[2 * gp + 1] = split_pair(stage[gp].reshape(DB, 128, E))
            hcv = jnp.concatenate([_bf(hc_w[j]) for j in range(DB)], axis=1)
            cache[gp] = pack_pair(_dot(hcv, weights(2 * gp)), _dot(hcv, weights(2 * gp + 1)))

        def pro_body(i, carry):
            g0 = KMAJ + i * PPI
            wait_all(stage.at[pl.ds(g0, PPI)], SEM_ST + i)

            @pl.when(i < DB // 2)
            def _():
                wo_w = wo_hbm.bitcast(U32)
                for t in range(2):
                    j = 2 * i + t
                    col = pl.multiple_of(j * 128, 128)
                    for c_ in range(4):
                        copy(wmod_w.at[:, pl.ds((2 + c_) * D + col, 128)],
                             wo_v.at[j, pl.ds(c_ * (D // 2), D // 2), :], SEM_WO).start()
                    copy(wo_w.at[:, pl.ds(col, 128)], wo_v.at[DB + j], SEM_WO).start()

            for t in range(PPI):
                slab(g0 + t)
            return carry

        lax.fori_loop(0, (NGP - KMAJ) // PPI, pro_body, 0)

    pl.run_scoped(
        prologue,
        pltpu.VMEM((NGP, D, E), U32),
        pltpu.VMEM((DB, 2, D // 2, 128), U32),
        pltpu.VMEM((DB, NSEG * M, E), BF16),
        pltpu.VMEM((DB, NSEG * M + SEG, 128), F32),
        pltpu.VMEM((2 * KMAJ, NSEG * M, E), F32),
    )

    def main(wg_v, wu_v, wd_v, x1_v, h2_v, out_v):
        lane = lax.broadcasted_iota(jnp.int32, (8, 2 * 128), 1)

        def post(seg, q, keep=True):
            rows = pl.ds(8 * q, 8)
            x = x_v[seg, rows, :].astype(F32)
            a = a_all[seg + UNR, rows, :].astype(F32)
            x1 = _rb(x + mod_row(2) * a)
            n, inv = _ln(x1)
            h2 = _rb(n * mod_row(4) + mod_row(3))
            r = _rb(jnp.sum(h2 * mod_row(6), axis=-1, keepdims=True))
            if keep:
                r_v[...] = jnp.where(lane == seg * 4 + q, r, r_v[...])
            x1_v[seg, rows, :] = x1.astype(BF16)
            h2_v[seg, rows, :] = h2.astype(BF16)
            out_v[seg, rows, :] = (x1 + mod_row(5) * h2).astype(BF16)
            return inv, r

        def tie(v, tok):
            if tok is None:
                return v
            tok = jnp.broadcast_to(tok, (8, 128))
            if v.dtype != F32:
                tok = pltpu.bitcast(tok, v.dtype)
            return jnp.concatenate([jnp.where(never_v[...] > 1.0, tok, v[0:8]), v[8:]], axis=0)

        def deferred(blk, wsel, j, tok=None, tok2=None):
            words = [odef_w[blk, h] for h in range(H)]
            words[-1] = tie(words[-1], tok)
            lhs = jnp.concatenate([_bf(w) for w in words], axis=1)
            res = tie(_dot(lhs, _bf(wo_v[wsel + j])), tok2).astype(BF16).reshape(UNR, M, 128)
            a_all[pl.ds(blk * UNR, UNR), pl.ds(0, M), pl.ds(j * 128, 128)] = res

        def out_copy(grp):
            return copy(out_v.at[pl.ds(grp * UNR, UNR)], out_hbm.at[pl.ds(grp * UNR, UNR)], SEM_OUT)

        wg_w, wu_w, wd_w = wg_hbm.bitcast(U32), wu_hbm.bitcast(U32), wd_hbm.bitcast(U32)
        x_tail.wait()
        wait_all(wo_v, SEM_WO)

        def step(it, u):
            s = it * UNR + u
            lhs = jnp.concatenate([_bf(lhs_w[j]) for j in range(DB)], axis=1)
            nseg = jnp.minimum(s + 1, NSEG - 1)

            def side(slot):
                if slot not in SIDE_SLOTS:
                    return None
                i = SIDE_SLOTS.index(slot)
                if i < 4:
                    lag = 2 * UNR if i == 0 else UNR
                    return post(jnp.maximum(s - lag, 0), i)[0]
                r0 = (i - 3) * 8
                h, inv = ln1(nseg, r0)
                put_rows(lhs_v, r0, h)
                return inv

            def proj(m_i, p):
                g = m_i * NPAIR + p
                for t in range(2):
                    qkv_s[g, pl.ds(t * SEG, SEG), :] = _dot(lhs, weights(2 * g + t)).astype(BF16)

            def rows_of(m_i, p):
                g = m_i * NPAIR + p
                return jnp.concatenate([_bf(qkv_w[g]), _bf(cache_w[g, it, pl.ds(u * M, M), :])], axis=0)

            def probs(p):
                parts = [lax.dot_general(_bf(qkv_w[p]), rows_of(1, p), (((1,), (1,)), ((), ())),
                                         preferred_element_type=F32)]
                qc = _bf(cache_w[p, it, pl.ds(u * M, M), :]).astype(F32)
                kc = _bf(cache_w[NPAIR + p, it, pl.ds(u * M, M), :]).astype(F32)
                col = lax.broadcasted_iota(jnp.int32, (M, PR), 1)
                for t in range(2):
                    km = _bf(qkv_w[NPAIR + p, pl.ds(t * (SEG // 2), 8), :]).astype(F32)
                    qt = qc[t * M:(t + 1) * M]
                    st = jnp.zeros((M, PR), F32)
                    for j in range(M):
                        st = jnp.where(col == t * SEG + j,
                                       jnp.sum(qt * km[j:j + 1], axis=-1, keepdims=True), st)
                        st = jnp.where(col == 2 * SEG + t * M + j,
                                       jnp.sum(qt * kc[t * M + j:t * M + j + 1], axis=-1, keepdims=True), st)
                    parts.append(st)
                sc = jnp.concatenate(parts, axis=0) * SCALE
                fm = fill_v[...]
                tok = side(("softmax", p))
                if tok is not None:
                    top = fm[0:8]
                    fm = jnp.concatenate([jnp.where(top > 1.0, tok, top), fm[8:]], axis=0)
                sc = jnp.where(fm == 0.0, sc, fm)
                e = jnp.exp(sc - jnp.max(sc, axis=-1, keepdims=True))
                return (e * _recip(jnp.sum(e, axis=-1, keepdims=True))).astype(BF16)

            def attend(p, pr):
                o = _dot(pr, rows_of(2, p))
                o_s[2 * p] = o[0:SEG].astype(BF16)
                o_s[2 * p + 1] = o[SEG:2 * SEG].astype(BF16)
                odef[it + 1, 2 * p, pl.ds(u * M, M), :] = o[2 * SEG:2 * SEG + M].astype(BF16)
                odef[it + 1, 2 * p + 1, pl.ds(u * M, M), :] = o[2 * SEG + M:].astype(BF16)

            wsel = jnp.where(it == 0, 0, DB)
            for t in range(DB // UNR):
                deferred(it, wsel, u * (DB // UNR) + t)
            ps = {}
            for pa in range(0, NPAIR, 2):
                pb = pa + 1
                proj(0, pa)
                proj(1, pa)
                proj(0, pb)
                proj(1, pb)
                proj(2, pa)
                proj(2, pb)
                for kind in ("scores", "values") if pa % 4 == 0 else ("values", "scores"):
                    for p in (pa, pb):
                        if kind == "scores":
                            ps[p] = probs(p)
                        elif p >= 2:
                            attend(p - 2, ps.pop(p - 2))
            L = NPAIR - 1

            acc = [None] * DB
            for h0, h1 in ((0, HA), (HA, H)):
                for j in range(DB):
                    words = [o_w[h] for h in range(h0, h1)]
                    words[0] = tie(words[0], side((h0, j)))
                    ol = jnp.concatenate([_bf(w) for w in words], axis=1)
                    part = _dot(ol, _bf(wo_v[DB + j, pl.ds(h0 * E // 2, (h1 - h0) * E // 2), :]))
                    if h0 == 0:
                        acc[j] = part
                    else:
                        a = part + acc[j]
                        lhs_v[j, pl.ds(0, M), :] = a[0:M].astype(BF16)
                        a_all[s + UNR, pl.ds(M, SEG - M), pl.ds(j * 128, 128)] = a[M:].astype(BF16)
                    if h0 == 0 and j == 4:
                        attend(L - 1, ps.pop(L - 1))
                        attend(L, ps.pop(L))

        def iteration(it, carry):
            @pl.when(it >= 3)
            def _():
                out_copy(it - 3).start()

            @pl.when(it < FB // 2)
            def _():
                for t in range(2):
                    j = 2 * it + t
                    cols = pl.ds(pl.multiple_of(j * 128, 128), 128)
                    copy(wg_w.at[:, cols], wg_v.at[j], SEM_MOE).start()
                    copy(wu_w.at[:, cols], wu_v.at[j], SEM_MOE + 1).start()

            @pl.when(it < DB)
            def _():
                cols = pl.ds(pl.multiple_of(it * 128, 128), 128)
                copy(wd_w.at[:, cols], wd_v.at[it], SEM_MOE + 2).start()

            for c_ in range(4):
                v = a_all[c_, pl.ds(0, M), :].astype(F32)
                mod_v[2 + c_] = _rb(1.0 + v) if c_ == 2 else v
            for u in range(UNR):
                step(it, u)
            return carry

        lax.fori_loop(0, NIT, iteration, 0)

        out_copy(NIT - 3).start()
        for k, buf in enumerate((wg_v, wu_v, wd_v)):
            wait_all(buf, SEM_MOE + k)
        early = [(seg, 0) for seg in range(NSEG - 2 * UNR, NSEG - UNR)]
        early += [(seg, q) for seg in range(NSEG - UNR, NSEG) for q in (1, 2, 3)]
        r8 = lax.broadcasted_iota(jnp.int32, (8, 1), 0)
        vals, idxs = [], []

        def pieces(n):
            tok = None
            for _ in range(n):
                seg, q = early.pop(0)
                keep = len(early) >= EPI_LATE
                r = post(seg, q, keep)[1]
                if not keep:
                    vals.append(r)
                    idxs.append((r8 + (seg * SEG + q * 8)).astype(F32))
                tok = r if tok is None else tok + r
            return tok

        for j in range(DB):
            deferred(NIT, DB, j, pieces(EPI_PIECES[j]), pieces(EPI_PIECES[DB]) if j == DB - 1 else None)
        out_copy(NIT - 2).start()

        def top2(vals, idx, axes):
            def red(f, v):
                for ax in axes:
                    v = f(v, axis=ax, keepdims=True)
                return v
            m1 = red(jnp.max, vals)
            i1 = red(jnp.min, jnp.where(vals == m1, idx, S - 1.0))
            rest = jnp.where(idx == i1, -jnp.inf, vals)
            m2 = red(jnp.max, rest)
            i2 = red(jnp.min, jnp.where(rest == m2, jnp.where(idx == i1, S - 1.0, idx), S - 1.0))
            return m1, i1, m2, i2

        m1, i1v, m2, i2v = top2(r_v[...], (lane * 8 + r8).astype(F32), (1, 0))
        vals.append(jnp.where(r8 == 0, m1, jnp.where(r8 == 1, m2, -jnp.inf)))
        idxs.append(jnp.where(r8 == 0, i1v, jnp.where(r8 == 1, i2v, S - 1.0)))
        for seg, q in early + [(seg, 0) for seg in range(NSEG - UNR, NSEG)]:
            vals.append(post(seg, q, keep=False)[1])
            idxs.append((r8 + (seg * SEG + q * 8)).astype(F32))
        out_copy(NIT - 1).start()
        m1, i1v, m2, i2v = top2(jnp.concatenate(vals, axis=0), jnp.concatenate(idxs, axis=0), (0,))
        i1 = i1v.astype(jnp.int32)[0, 0]
        i2 = i2v.astype(jnp.int32)[0, 0]

        def tile_of(i):
            return i >> 5, pl.multiple_of(((i >> 3) & 3) * 8, 8)

        sel = [tile_of(i1), tile_of(i2)]
        x1s = jnp.concatenate([x1_v[sg, pl.ds(r0, 8), :].astype(F32) for sg, r0 in sel], axis=0)
        h2s = jnp.concatenate([h2_v[sg, pl.ds(r0, 8), :].astype(F32) for sg, r0 in sel], axis=0)
        h2b = h2s.astype(BF16)
        gus = []
        for j in range(FB):
            g = _rb(_dot(h2b, _bf(wg_v[j])))
            g = _rb(g * jax.nn.sigmoid(g))
            u = _rb(_dot(h2b, _bf(wu_v[j])))
            gus.append(g * u)
        gu = jnp.concatenate(gus, axis=1).astype(BF16)
        y = jnp.concatenate([_rb(_dot(gu, _bf(wd_v[j]))) for j in range(DB)], axis=1)
        rows = lax.broadcasted_iota(jnp.int32, (16, 1), 0)
        rs = _rb(jax.nn.sigmoid(jnp.where(rows < 8, m1, m2)))
        y = _rb(y * rs)
        full = x1s + mod_row(5, 16) * _rb(h2s + y)

        copy(out_v, out_hbm, SEM_OUT).wait()
        for t, (i, (sg, r0)) in enumerate(zip((i1, i2), sel)):
            old = out_v[sg, pl.ds(r0, 8), :].astype(F32)
            new = jnp.where(r8 == (i & 7), full[t * 8:(t + 1) * 8], old)
            out_v[sg, pl.ds(r0, 8), :] = new.astype(BF16)
        fix = [copy(out_v.at[sg, pl.ds(r0, 8), :], out_hbm.at[sg, pl.ds(r0, 8), :], SEM_OUT + 1 + t)
               for t, (sg, r0) in enumerate(sel)]
        differ = (i1 >> 3) != (i2 >> 3)
        fix[0].start()

        @pl.when(differ)
        def _():
            fix[1].start()
            fix[1].wait()

        fix[0].wait()

    pl.run_scoped(
        main,
        pltpu.VMEM((FB, D // 2, 128), U32),
        pltpu.VMEM((FB, D // 2, 128), U32),
        pltpu.VMEM((DB, F // 2, 128), U32),
        pltpu.VMEM((NSEG, SEG, D), BF16),
        pltpu.VMEM((NSEG, SEG, D), BF16),
        pltpu.VMEM((NSEG, SEG, D), BF16),
    )


@jax.jit
def pallas_adaLN_cond__memory_aug_recurrent_mem_tr__moe_arch_mod__prompt_kernel(
    A_x: jax.Array,
    A_mem0: jax.Array,
    A_Wq: jax.Array,
    A_Wk: jax.Array,
    A_Wv: jax.Array,
    A_Wo: jax.Array,
    A_seg_len: jax.Array,
    B_x: jax.Array,
    B_w_r: jax.Array,
    B_w_gate: jax.Array,
    B_w_up: jax.Array,
    B_w_down: jax.Array,
    c: jax.Array,
    w_mod: jax.Array,
):
    del A_seg_len, B_x
    assert A_x.shape == (1, S, D) and A_mem0.shape == (1, M, D) and A_Wq.shape == (D, H, E)
    hbm = pl.BlockSpec(memory_space=pl.ANY)
    out = pl.pallas_call(
        _kernel,
        out_shape=jax.ShapeDtypeStruct((NSEG, SEG, D), BF16),
        in_specs=[hbm] * 12,
        out_specs=hbm,
        scratch_shapes=[
            pltpu.VMEM((NSEG, SEG, D), BF16),
            pltpu.VMEM((3 * H, DB, 128, E), BF16),
            pltpu.VMEM((2 * DB, H * E // 2, 128), U32),
            pltpu.VMEM((NGP, NIT, UNR * 2 * M, E), BF16),
            pltpu.VMEM((NIT + 1, H, SEG, E), BF16),
            pltpu.VMEM((DB, SEG, 128), BF16),
            pltpu.VMEM((NGP, 2 * SEG, E), BF16),
            pltpu.VMEM((H, SEG, E), BF16),
            pltpu.VMEM((NSEG + UNR, SEG, D), BF16),
            pltpu.VMEM((8, S // 8), F32),
            pltpu.VMEM((7, 8, D), F32),
            pltpu.VMEM((PR, PR), F32),
            pltpu.VMEM((8, 128), F32),
            pltpu.VMEM((M, D), BF16),
            pltpu.VMEM((D,), BF16),
            pltpu.VMEM((1, D), BF16),
            pltpu.SemaphoreType.DMA((NSEM,)),
        ],
        compiler_params=pltpu.CompilerParams(
            vmem_limit_bytes=120 * 1024 * 1024, disable_bounds_checks=True,
            disable_semaphore_checks=True),
    )(
        A_x.reshape(NSEG, SEG, D),
        A_mem0.reshape(M, D),
        A_Wq, A_Wk, A_Wv,
        A_Wo.reshape(H * E, D),
        B_w_r,
        B_w_gate, B_w_up, B_w_down,
        c, w_mod,
    )
    return out.reshape(1, S, D)
```

```python
import jax
import jax.numpy as jnp
from jax import lax
import jax.experimental.pallas as pl
import jax.experimental.pallas.tpu as pltpu

BF16 = jnp.bfloat16
F32 = jnp.float32
U32 = jnp.uint32

S = 2048
D = 1024
H = 32
E = 128
M = 8
SEG = 32
NSEG = S // SEG
NPAIR = H // 2
NGP = 3 * NPAIR
F = 3584
DB = D // 128
FB = F // 128
PR = 2 * SEG + 2 * M
UNR = SEG // M
NIT = NSEG // UNR
KMAJ = 12
AHEAD = 3
PPI = 6
EPI_LATE = 6
EPI_PIECES = (0, 0, 2, 2, 2, 2, 2, 2, 2)
HA = 24
SIDE_SLOTS = [("softmax", 4), ("softmax", 8), ("softmax", 10), ("softmax", 12), (0, 2), (0, 5), (HA, 0)]
EPS = 1e-5
SCALE = E ** (-0.5)

SEM_SMALL = 0
SEM_X = SEM_SMALL + 3
SEM_MOD = SEM_X + 3
SEM_WQ = SEM_MOD + DB
SEM_ST = SEM_WQ + DB
SEM_WO = SEM_ST + (NGP - KMAJ) // PPI
SEM_MOE = SEM_WO + 1
SEM_OUT = SEM_MOE + 3
NSEM = SEM_OUT + 3


def _rb(v):
    return v.astype(BF16).astype(F32)


def _dot(a, b):
    return jnp.dot(a, b, preferred_element_type=F32)


def _recip(x):
    r = pl.reciprocal(x, approx=True)
    return r * (2.0 - x * r)


def _bf(words):
    return pltpu.bitcast(words, BF16)


def _ln(x):
    m = jnp.mean(x, axis=-1, keepdims=True)
    mb = _rb(m)
    d = x - mb
    var = jnp.mean(d * d, axis=-1, keepdims=True) - (m - mb) * (m - mb)
    inv = _recip(_rb(jnp.sqrt(_rb(_rb(jnp.maximum(var, 0.0)) + EPS))))
    return d * inv, inv


def _fill_matrix():
    i = lax.broadcasted_iota(jnp.int32, (PR, PR), 0)
    j = lax.broadcasted_iota(jnp.int32, (PR, PR), 1)

    def head(t):
        return jnp.where(t < 2 * SEG, t >> 5, (t - 2 * SEG) >> 3)

    def pos(t):
        r = t & (SEG - 1)
        return jnp.where(t < 2 * SEG, jnp.where(r < M, r, r + M), M + (t & (M - 1)))

    same = head(i) == head(j)
    pi = pos(i)
    ok = jnp.where(pi < M, 1, jnp.where(pi >= pos(j), 1, 0))
    return jnp.where(same, jnp.where(ok == 1, 0.0, -1e9), -3e38).astype(F32)


def _kernel(x_hbm, mem0_hbm, wq_hbm, wk_hbm, wv_hbm, wo_hbm, wr_hbm, wg_hbm, wu_hbm, wd_hbm,
            c_hbm, wmod_hbm, out_hbm,
            x_v, w_v, wo_v, cache, odef, lhs_v, qkv_s, o_s, a_all, r_v, mod_v, fill_v, never_v,
            mem0_v, wr_v, c_v, sems):
    w_w = w_v.bitcast(U32)
    cache_w = cache.bitcast(U32)
    lhs_w = lhs_v.bitcast(U32)
    qkv_w = qkv_s.bitcast(U32)
    o_w = o_s.bitcast(U32)
    odef_w = odef.bitcast(U32)

    def weights(h):
        return _bf(w_w[h].reshape(D // 2, E))

    def copy(src, dst, sem):
        return pltpu.make_async_copy(src, dst, sems.at[sem])

    def wait_all(buf, sem):
        copy(buf, buf, sem).wait()

    def mod_row(k, rows=8):
        v = mod_v[k]
        return v if rows == 8 else jnp.concatenate([v] * (rows // 8), axis=0)

    def put_rows(dst, r0, v):
        for j in range(DB):
            dst[j, pl.ds(r0, v.shape[0]), :] = v[:, j * 128:(j + 1) * 128].astype(BF16)

    def ln1(seg, r0):
        n, inv = _ln(x_v[seg, pl.ds(r0, 8), :].astype(F32))
        return n * mod_row(1) + mod_row(0), inv

    x_tail = copy(x_hbm.at[pl.ds(1, NSEG - 1), pl.ds(M, SEG - M), :],
                  x_v.at[pl.ds(1, NSEG - 1), pl.ds(M, SEG - M), :], SEM_X + 2)

    def prologue(stage, wmod_v, hc, n_v, acc):
        wmod_w = wmod_hbm.bitcast(U32)
        w_words = [w.bitcast(U32) for w in (wq_hbm, wk_hbm, wv_hbm)]

        def start_mod(j):
            col = j * 128 if isinstance(j, int) else pl.multiple_of(j * 128, 128)
            for k in range(2):
                copy(wmod_w.at[:, pl.ds(k * D + col, 128)], wmod_v.at[j, k], SEM_MOD + j).start()

        def start_ktile(j):
            rows = pl.ds(j * 128 if isinstance(j, int) else pl.multiple_of(j * 128, 128), 128)
            for g in range(KMAJ):
                copy(w_words[0].at[rows, g, :], stage.at[g, rows, :], SEM_WQ + j).start()

        small = [copy(c_hbm, c_v, SEM_SMALL), copy(mem0_hbm, mem0_v, SEM_SMALL + 1),
                 copy(wr_hbm, wr_v, SEM_SMALL + 2)]
        x_head = copy(x_hbm.at[:, pl.ds(0, M), :], x_v.at[:, pl.ds(0, M), :], SEM_X)
        x_seg0 = copy(x_hbm.at[0, pl.ds(M, SEG - M), :], x_v.at[0, pl.ds(M, SEG - M), :], SEM_X + 1)
        for cp in small:
            cp.start()
        x_head.start()
        x_seg0.start()
        start_mod(0)
        for j in range(AHEAD):
            start_ktile(j)
            start_mod(j + 1)
        slab_cps = [copy(w_words[g // NPAIR].at[:, g % NPAIR, :], stage.at[g], SEM_ST + (g - KMAJ) // PPI)
                    for g in range(KMAJ, NGP)]

        fill_v[...] = _fill_matrix()
        a_all[pl.ds(0, UNR + 1)] = jnp.zeros((UNR + 1, SEG, D), BF16)
        r_v[...] = jnp.full(r_v.shape, -jnp.inf, F32)
        never_v[...] = jnp.zeros(never_v.shape, F32)
        qkv_s[0] = jnp.zeros((2 * SEG, E), BF16)
        o_s[0] = jnp.zeros((SEG, E), BF16)

        def zero_acc(h, carry):
            acc[h] = jnp.zeros((NSEG * M, E), F32)
            return carry

        lax.fori_loop(0, 2 * KMAJ, zero_acc, 0)

        for cp in small:
            cp.wait()
        c = c_v[...].astype(F32)
        sc = jnp.broadcast_to(_rb(c * jax.nn.sigmoid(c)), (M, D))
        zero = jnp.zeros((M, E), F32)
        for h in range(H):
            blk = sc[:, (h % DB) * 128:(h % DB + 1) * 128]
            odef[0, h] = jnp.concatenate(
                [blk if c_ == h // DB else zero for c_ in range(4)], axis=0).astype(BF16)
        mod_v[6] = jnp.broadcast_to(wr_v[...].astype(F32).reshape(1, D), (8, D))
        put_rows(lhs_v, 0, mem0_v[...].astype(F32))

        x_head.wait()
        x_seg0.wait()
        NB = 16
        RB = NSEG * M // NB
        NR = NSEG * M + SEG - M
        for b in range(NB + 1):
            if b < NB:
                xb = x_v[pl.ds(b * (NSEG // NB), NSEG // NB), pl.ds(0, M), :].astype(F32).reshape(RB, D)
            else:
                xb = x_v[0, pl.ds(M, SEG - M), :].astype(F32)
            nb = _ln(xb)[0]
            for j in range(DB):
                n_v[j, pl.ds(b * RB, nb.shape[0]), :] = nb[:, j * 128:(j + 1) * 128]

        hc_w = hc.bitcast(U32)

        def mod_block(j, k, src=None):
            scb = jnp.concatenate([_bf(odef_w[0, h, pl.ds(0, 8), :]) for h in range(DB)], axis=1)
            v = _rb(_dot(scb, _bf(wmod_v[j if src is None else src, k]))[0:8])
            if k == 1:
                v = _rb(1.0 + v)
            col = j * 128 if isinstance(j, int) else pl.multiple_of(j * 128, 128)
            mod_v[k, :, pl.ds(col, 128)] = v
            return v

        def h_block(j, ca, sa):
            n = n_v[j, pl.ds(0, NR), :].reshape(NR // 8, 8, 128)
            hv = (n * ca[None] + sa[None]).reshape(NR, 128).astype(BF16)
            hc[j] = hv[0:NSEG * M]
            lhs_v[j, pl.ds(M, SEG - M), :] = hv[NSEG * M:]

        def pack_pair(r1, r2):
            r = jnp.concatenate([r1.reshape(NSEG, M, E), r2.reshape(NSEG, M, E)], axis=1)
            return r.reshape(NIT, UNR * 2 * M, E).astype(BF16)

        def split_pair(b):
            return (pltpu.bitcast(b << 16, F32).astype(BF16),
                    pltpu.bitcast(b & jnp.uint32(0xFFFF0000), F32).astype(BF16))

        def q_stage(j, last, more_dmas):
            static = isinstance(j, int)
            k0 = j * 128 if static else pl.multiple_of(j * 128, 128)
            src = None if last else jnp.where(j == 0, 0, j + 1)
            for p in range(KMAJ):
                ws = split_pair(stage[p, pl.ds(k0, 128), :])
                rs = []
                for t in range(2):
                    h = 2 * p + t
                    w_v[h, j] = ws[t]
                    rs.append(_dot(_bf(hc_w[j]), _bf(w_w[h, j])) + acc[h])
                    if not last:
                        acc[h] = rs[t]
                if last:
                    cache[p] = pack_pair(*rs)
                elif p == 1:
                    ca = mod_block(j + 1, 1, src)
                elif p == 3:
                    h_block(j + 1, ca, mod_block(j + 1, 0, src))
                if p == 1:
                    more_dmas()

        wait_all(wmod_v.at[0], SEM_MOD)
        h_block(0, mod_block(0, 1), mod_block(0, 0))

        def wait_ktile(j):
            rows = pl.ds(j * 128 if isinstance(j, int) else pl.multiple_of(j * 128, 128), 128)
            wait_all(stage.at[pl.ds(0, KMAJ), rows, :], SEM_WQ + j)

        def q_body(j, carry):
            @pl.when(j == 1)
            def _():
                wait_all(wmod_v.at[1], SEM_MOD + 1)
                h_block(1, mod_block(1, 1), mod_block(1, 0))

            wait_ktile(j)

            @pl.when(j > 0)
            def _():
                wait_all(wmod_v.at[j + 1], SEM_MOD + j + 1)

            def more_dmas():
                @pl.when(j + AHEAD < DB)
                def _():
                    start_ktile(j + AHEAD)

                @pl.when(j + AHEAD + 1 < DB)
                def _():
                    start_mod(j + AHEAD + 1)

                @pl.when(j + AHEAD == DB)
                def _():
                    for cp in slab_cps[:2 * PPI]:
                        cp.start()

            q_stage(j, False, more_dmas)
            return carry

        lax.fori_loop(0, DB - 1, q_body, 0)
        wait_ktile(DB - 1)

        def last_dmas():
            for cp in slab_cps[2 * PPI:]:
                cp.start()
            x_tail.start()

        q_stage(DB - 1, True, last_dmas)

        def slab(gp):
            w_v[2 * gp], w_v[2 * gp + 1] = split_pair(stage[gp].reshape(DB, 128, E))
            hcv = jnp.concatenate([_bf(hc_w[j]) for j in range(DB)], axis=1)
            cache[gp] = pack_pair(_dot(hcv, weights(2 * gp)), _dot(hcv, weights(2 * gp + 1)))

        def pro_body(i, carry):
            g0 = KMAJ + i * PPI
            wait_all(stage.at[pl.ds(g0, PPI)], SEM_ST + i)

            @pl.when(i < DB // 2)
            def _():
                wo_w = wo_hbm.bitcast(U32)
                for t in range(2):
                    j = 2 * i + t
                    col = pl.multiple_of(j * 128, 128)
                    for c_ in range(4):
                        copy(wmod_w.at[:, pl.ds((2 + c_) * D + col, 128)],
                             wo_v.at[j, pl.ds(c_ * (D // 2), D // 2), :], SEM_WO).start()
                    copy(wo_w.at[:, pl.ds(col, 128)], wo_v.at[DB + j], SEM_WO).start()

            for t in range(PPI):
                slab(g0 + t)
            return carry

        lax.fori_loop(0, (NGP - KMAJ) // PPI, pro_body, 0)

    pl.run_scoped(
        prologue,
        pltpu.VMEM((NGP, D, E), U32),
        pltpu.VMEM((DB, 2, D // 2, 128), U32),
        pltpu.VMEM((DB, NSEG * M, E), BF16),
        pltpu.VMEM((DB, NSEG * M + SEG, 128), F32),
        pltpu.VMEM((2 * KMAJ, NSEG * M, E), F32),
    )

    def main(wg_v, wu_v, wd_v, x1_v, h2_v, out_v):
        lane = lax.broadcasted_iota(jnp.int32, (8, 2 * 128), 1)

        def post(seg, q, keep=True):
            rows = pl.ds(8 * q, 8)
            x = x_v[seg, rows, :].astype(F32)
            a = a_all[seg + UNR, rows, :].astype(F32)
            x1 = _rb(x + mod_row(2) * a)
            n, inv = _ln(x1)
            h2 = _rb(n * mod_row(4) + mod_row(3))
            r = _rb(jnp.sum(h2 * mod_row(6), axis=-1, keepdims=True))
            if keep:
                r_v[...] = jnp.where(lane == seg * 4 + q, r, r_v[...])
            x1_v[seg, rows, :] = x1.astype(BF16)
            h2_v[seg, rows, :] = h2.astype(BF16)
            out_v[seg, rows, :] = (x1 + mod_row(5) * h2).astype(BF16)
            return inv, r

        def tie(v, tok):
            if tok is None:
                return v
            tok = jnp.broadcast_to(tok, (8, 128))
            if v.dtype != F32:
                tok = pltpu.bitcast(tok, v.dtype)
            return jnp.concatenate([jnp.where(never_v[...] > 1.0, tok, v[0:8]), v[8:]], axis=0)

        def deferred(blk, wsel, j, tok=None, tok2=None):
            words = [odef_w[blk, h] for h in range(H)]
            words[-1] = tie(words[-1], tok)
            lhs = jnp.concatenate([_bf(w) for w in words], axis=1)
            res = tie(_dot(lhs, _bf(wo_v[wsel + j])), tok2).astype(BF16).reshape(UNR, M, 128)
            a_all[pl.ds(blk * UNR, UNR), pl.ds(0, M), pl.ds(j * 128, 128)] = res

        def out_copy(grp):
            return copy(out_v.at[pl.ds(grp * UNR, UNR)], out_hbm.at[pl.ds(grp * UNR, UNR)], SEM_OUT)

        wg_w, wu_w, wd_w = wg_hbm.bitcast(U32), wu_hbm.bitcast(U32), wd_hbm.bitcast(U32)
        x_tail.wait()
        wait_all(wo_v, SEM_WO)

        def step(it, u):
            s = it * UNR + u
            lhs = jnp.concatenate([_bf(lhs_w[j]) for j in range(DB)], axis=1)
            nseg = jnp.minimum(s + 1, NSEG - 1)

            def side(slot):
                if slot not in SIDE_SLOTS:
                    return None
                i = SIDE_SLOTS.index(slot)
                if i < 4:
                    lag = 2 * UNR if i == 0 else UNR
                    return post(jnp.maximum(s - lag, 0), i)[0]
                r0 = (i - 3) * 8
                h, inv = ln1(nseg, r0)
                put_rows(lhs_v, r0, h)
                return inv

            def proj(m_i, p):
                g = m_i * NPAIR + p
                for t in range(2):
                    qkv_s[g, pl.ds(t * SEG, SEG), :] = _dot(lhs, weights(2 * g + t)).astype(BF16)

            def rows_of(m_i, p):
                g = m_i * NPAIR + p
                return jnp.concatenate([_bf(qkv_w[g]), _bf(cache_w[g, it, pl.ds(u * M, M), :])], axis=0)

            def probs(p):
                parts = [lax.dot_general(_bf(qkv_w[p]), rows_of(1, p), (((1,), (1,)), ((), ())),
                                         preferred_element_type=F32)]
                qc = _bf(cache_w[p, it, pl.ds(u * M, M), :]).astype(F32)
                kc = _bf(cache_w[NPAIR + p, it, pl.ds(u * M, M), :]).astype(F32)
                col = lax.broadcasted_iota(jnp.int32, (M, PR), 1)
                for t in range(2):
                    km = _bf(qkv_w[NPAIR + p, pl.ds(t * (SEG // 2), 8), :]).astype(F32)
                    qt = qc[t * M:(t + 1) * M]
                    st = jnp.zeros((M, PR), F32)
                    for j in range(M):
                        st = jnp.where(col == t * SEG + j,
                                       jnp.sum(qt * km[j:j + 1], axis=-1, keepdims=True), st)
                        st = jnp.where(col == 2 * SEG + t * M + j,
                                       jnp.sum(qt * kc[t * M + j:t * M + j + 1], axis=-1, keepdims=True), st)
                    parts.append(st)
                sc = jnp.concatenate(parts, axis=0) * SCALE
                fm = fill_v[...]
                tok = side(("softmax", p))
                if tok is not None:
                    top = fm[0:8]
                    fm = jnp.concatenate([jnp.where(top > 1.0, tok, top), fm[8:]], axis=0)
                sc = jnp.where(fm == 0.0, sc, fm)
                e = jnp.exp(sc - jnp.max(sc, axis=-1, keepdims=True))
                return (e * _recip(jnp.sum(e, axis=-1, keepdims=True))).astype(BF16)

            def attend(p, pr):
                o = _dot(pr, rows_of(2, p))
                o_s[2 * p] = o[0:SEG].astype(BF16)
                o_s[2 * p + 1] = o[SEG:2 * SEG].astype(BF16)
                odef[it + 1, 2 * p, pl.ds(u * M, M), :] = o[2 * SEG:2 * SEG + M].astype(BF16)
                odef[it + 1, 2 * p + 1, pl.ds(u * M, M), :] = o[2 * SEG + M:].astype(BF16)

            wsel = jnp.where(it == 0, 0, DB)
            for t in range(DB // UNR):
                deferred(it, wsel, u * (DB // UNR) + t)
            ps = {}
            for pa in range(0, NPAIR, 2):
                pb = pa + 1
                proj(0, pa)
                proj(1, pa)
                proj(0, pb)
                proj(1, pb)
                proj(2, pa)
                proj(2, pb)
                for kind in ("scores", "values") if pa % 4 == 0 else ("values", "scores"):
                    for p in (pa, pb):
                        if kind == "scores":
                            ps[p] = probs(p)
                        elif p >= 2:
                            attend(p - 2, ps.pop(p - 2))
            L = NPAIR - 1

            acc = [None] * DB
            for h0, h1 in ((0, HA), (HA, H)):
                for j in range(DB):
                    words = [o_w[h] for h in range(h0, h1)]
                    words[0] = tie(words[0], side((h0, j)))
                    ol = jnp.concatenate([_bf(w) for w in words], axis=1)
                    part = _dot(ol, _bf(wo_v[DB + j, pl.ds(h0 * E // 2, (h1 - h0) * E // 2), :]))
                    if h0 == 0:
                        acc[j] = part
                    else:
                        a = part + acc[j]
                        lhs_v[j, pl.ds(0, M), :] = a[0:M].astype(BF16)
                        a_all[s + UNR, pl.ds(M, SEG - M), pl.ds(j * 128, 128)] = a[M:].astype(BF16)
                    if h0 == 0 and j == 4:
                        attend(L - 1, ps.pop(L - 1))
                        attend(L, ps.pop(L))

        def iteration(it, carry):
            @pl.when(it >= 3)
            def _():
                out_copy(it - 3).start()

            @pl.when(it < FB // 2)
            def _():
                for t in range(2):
                    j = 2 * it + t
                    cols = pl.ds(pl.multiple_of(j * 128, 128), 128)
                    copy(wg_w.at[:, cols], wg_v.at[j], SEM_MOE).start()
                    copy(wu_w.at[:, cols], wu_v.at[j], SEM_MOE + 1).start()

            @pl.when(it < DB)
            def _():
                cols = pl.ds(pl.multiple_of(it * 128, 128), 128)
                copy(wd_w.at[:, cols], wd_v.at[it], SEM_MOE + 2).start()

            for c_ in range(4):
                v = a_all[c_, pl.ds(0, M), :].astype(F32)
                mod_v[2 + c_] = _rb(1.0 + v) if c_ == 2 else v
            for u in range(UNR):
                step(it, u)
            return carry

        lax.fori_loop(0, NIT, iteration, 0)

        out_copy(NIT - 3).start()
        for k, buf in enumerate((wg_v, wu_v, wd_v)):
            wait_all(buf, SEM_MOE + k)
        early = [(seg, 0) for seg in range(NSEG - 2 * UNR, NSEG - UNR)]
        early += [(seg, q) for seg in range(NSEG - UNR, NSEG) for q in (1, 2, 3)]
        r8 = lax.broadcasted_iota(jnp.int32, (8, 1), 0)
        vals, idxs = [], []

        def pieces(n):
            tok = None
            for _ in range(n):
                seg, q = early.pop(0)
                keep = len(early) >= EPI_LATE
                r = post(seg, q, keep)[1]
                if not keep:
                    vals.append(r)
                    idxs.append((r8 + (seg * SEG + q * 8)).astype(F32))
                tok = r if tok is None else tok + r
            return tok

        for j in range(DB):
            deferred(NIT, DB, j, pieces(EPI_PIECES[j]), pieces(EPI_PIECES[DB]) if j == DB - 1 else None)
        out_copy(NIT - 2).start()

        def top2(vals, idx, axes):
            def red(f, v):
                for ax in axes:
                    v = f(v, axis=ax, keepdims=True)
                return v
            m1 = red(jnp.max, vals)
            i1 = red(jnp.min, jnp.where(vals == m1, idx, S - 1.0))
            rest = jnp.where(idx == i1, -jnp.inf, vals)
            m2 = red(jnp.max, rest)
            i2 = red(jnp.min, jnp.where(rest == m2, jnp.where(idx == i1, S - 1.0, idx), S - 1.0))
            return m1, i1, m2, i2

        m1, i1v, m2, i2v = top2(r_v[...], (lane * 8 + r8).astype(F32), (1, 0))
        vals.append(jnp.where(r8 == 0, m1, jnp.where(r8 == 1, m2, -jnp.inf)))
        idxs.append(jnp.where(r8 == 0, i1v, jnp.where(r8 == 1, i2v, S - 1.0)))
        for seg, q in early + [(seg, 0) for seg in range(NSEG - UNR, NSEG)]:
            vals.append(post(seg, q, keep=False)[1])
            idxs.append((r8 + (seg * SEG + q * 8)).astype(F32))
        out_copy(NIT - 1).start()
        m1, i1v, m2, i2v = top2(jnp.concatenate(vals, axis=0), jnp.concatenate(idxs, axis=0), (0,))
        i1 = i1v.astype(jnp.int32)[0, 0]
        i2 = i2v.astype(jnp.int32)[0, 0]

        def tile_of(i):
            return i >> 5, pl.multiple_of(((i >> 3) & 3) * 8, 8)

        sel = [tile_of(i1), tile_of(i2)]
        x1s = jnp.concatenate([x1_v[sg, pl.ds(r0, 8), :].astype(F32) for sg, r0 in sel], axis=0)
        h2s = jnp.concatenate([h2_v[sg, pl.ds(r0, 8), :].astype(F32) for sg, r0 in sel], axis=0)
        h2b = h2s.astype(BF16)
        gus = []
        for j in range(FB):
            g = _rb(_dot(h2b, _bf(wg_v[j])))
            g = _rb(g * jax.nn.sigmoid(g))
            u = _rb(_dot(h2b, _bf(wu_v[j])))
            gus.append(g * u)
        gu = jnp.concatenate(gus, axis=1).astype(BF16)
        y = jnp.concatenate([_rb(_dot(gu, _bf(wd_v[j]))) for j in range(DB)], axis=1)
        rows = lax.broadcasted_iota(jnp.int32, (16, 1), 0)
        rs = _rb(jax.nn.sigmoid(jnp.where(rows < 8, m1, m2)))
        y = _rb(y * rs)
        full = x1s + mod_row(5, 16) * _rb(h2s + y)

        copy(out_v, out_hbm, SEM_OUT).wait()
        for t, (i, (sg, r0)) in enumerate(zip((i1, i2), sel)):
            old = out_v[sg, pl.ds(r0, 8), :].astype(F32)
            new = jnp.where(r8 == (i & 7), full[t * 8:(t + 1) * 8], old)
            out_v[sg, pl.ds(r0, 8), :] = new.astype(BF16)
        fix = [copy(out_v.at[sg, pl.ds(r0, 8), :], out_hbm.at[sg, pl.ds(r0, 8), :], SEM_OUT + 1 + t)
               for t, (sg, r0) in enumerate(sel)]
        differ = (i1 >> 3) != (i2 >> 3)
        fix[0].start()

        @pl.when(differ)
        def _():
            fix[1].start()
            fix[1].wait()

        fix[0].wait()

    pl.run_scoped(
        main,
        pltpu.VMEM((FB, D // 2, 128), U32),
        pltpu.VMEM((FB, D // 2, 128), U32),
        pltpu.VMEM((DB, F // 2, 128), U32),
        pltpu.VMEM((NSEG, SEG, D), BF16),
        pltpu.VMEM((NSEG, SEG, D), BF16),
        pltpu.VMEM((NSEG, SEG, D), BF16),
    )


@jax.jit
def pallas_adaLN_cond__memory_aug_recurrent_mem_tr__moe_arch_mod__prompt_kernel(
    A_x: jax.Array,
    A_mem0: jax.Array,
    A_Wq: jax.Array,
    A_Wk: jax.Array,
    A_Wv: jax.Array,
    A_Wo: jax.Array,
    A_seg_len: jax.Array,
    B_x: jax.Array,
    B_w_r: jax.Array,
    B_w_gate: jax.Array,
    B_w_up: jax.Array,
    B_w_down: jax.Array,
    c: jax.Array,
    w_mod: jax.Array,
):
    del A_seg_len, B_x
    assert A_x.shape == (1, S, D) and A_mem0.shape == (1, M, D) and A_Wq.shape == (D, H, E)
    hbm = pl.BlockSpec(memory_space=pl.ANY)
    out = pl.pallas_call(
        _kernel,
        out_shape=jax.ShapeDtypeStruct((NSEG, SEG, D), BF16),
        in_specs=[hbm] * 12,
        out_specs=hbm,
        scratch_shapes=[
            pltpu.VMEM((NSEG, SEG, D), BF16),
            pltpu.VMEM((3 * H, DB, 128, E), BF16),
            pltpu.VMEM((2 * DB, H * E // 2, 128), U32),
            pltpu.VMEM((NGP, NIT, UNR * 2 * M, E), BF16),
            pltpu.VMEM((NIT + 1, H, SEG, E), BF16),
            pltpu.VMEM((DB, SEG, 128), BF16),
            pltpu.VMEM((NGP, 2 * SEG, E), BF16),
            pltpu.VMEM((H, SEG, E), BF16),
            pltpu.VMEM((NSEG + UNR, SEG, D), BF16),
            pltpu.VMEM((8, S // 8), F32),
            pltpu.VMEM((7, 8, D), F32),
            pltpu.VMEM((PR, PR), F32),
            pltpu.VMEM((8, 128), F32),
            pltpu.VMEM((M, D), BF16),
            pltpu.VMEM((D,), BF16),
            pltpu.VMEM((1, D), BF16),
            pltpu.SemaphoreType.DMA((NSEM,)),
        ],
        compiler_params=pltpu.CompilerParams(
            vmem_limit_bytes=120 * 1024 * 1024, disable_bounds_checks=True,
            disable_semaphore_checks=True),
    )(
        A_x.reshape(NSEG, SEG, D),
        A_mem0.reshape(M, D),
        A_Wq, A_Wk, A_Wv,
        A_Wo.reshape(H * E, D),
        B_w_r,
        B_w_gate, B_w_up, B_w_down,
        c, w_mod,
    )
    return out.reshape(1, S, D)
```

```python
import jax
import jax.numpy as jnp
from jax import lax
import jax.experimental.pallas as pl
import jax.experimental.pallas.tpu as pltpu

BF16 = jnp.bfloat16
F32 = jnp.float32
U32 = jnp.uint32

S = 2048
D = 1024
H = 32
E = 128
M = 8
SEG = 32
NSEG = S // SEG
NPAIR = H // 2
NGP = 3 * NPAIR
F = 3584
DB = D // 128
FB = F // 128
PR = 2 * SEG + 2 * M
UNR = 4
NIT = NSEG // UNR
KMAJ = 12
AHEAD = 3
PPI = 6
NSPLIT = 2
KEARLY = 6
HA = 24
SIDE_SLOTS = [("softmax", 4), ("softmax", 8), ("softmax", 10), ("softmax", 12), (0, 2), (0, 5), (HA, 0)]
EPS = 1e-5
SCALE = E ** (-0.5)

SEM_SMALL = 0
SEM_X = SEM_SMALL + 3
SEM_MOD = SEM_X + 3
SEM_MOD2 = SEM_MOD + DB
SEM_WQ = SEM_MOD2 + 4
SEM_ST = SEM_WQ + DB
SEM_WO = SEM_ST + (NGP - KMAJ) // PPI
SEM_MOE = SEM_WO + 1
SEM_OUT = SEM_MOE + 2
NSEM = SEM_OUT + 3


def _rb(v):
    return v.astype(BF16).astype(F32)


def _dot(a, b):
    return jnp.dot(a, b, preferred_element_type=F32)


def _recip(x):
    r = pl.reciprocal(x, approx=True)
    return r * (2.0 - x * r)


def _bf(words):
    return pltpu.bitcast(words, BF16)


def _ln(x):
    m = jnp.mean(x, axis=-1, keepdims=True)
    mb = _rb(m)
    d = x - mb
    var = jnp.mean(d * d, axis=-1, keepdims=True) - (m - mb) * (m - mb)
    inv = _recip(_rb(jnp.sqrt(_rb(_rb(jnp.maximum(var, 0.0)) + EPS))))
    return d * inv, inv


def _fill_matrix():
    i = lax.broadcasted_iota(jnp.int32, (PR, PR), 0)
    j = lax.broadcasted_iota(jnp.int32, (PR, PR), 1)

    def head(t):
        return jnp.where(t < 2 * SEG, t >> 5, (t - 2 * SEG) >> 3)

    def pos(t):
        r = t & (SEG - 1)
        return jnp.where(t < 2 * SEG, jnp.where(r < M, r, r + M), M + (t & (M - 1)))

    same = head(i) == head(j)
    pi = pos(i)
    ok = jnp.where(pi < M, 1, jnp.where(pi >= pos(j), 1, 0))
    return jnp.where(same, jnp.where(ok == 1, 0.0, -1e9), -3e38).astype(F32)


def _kernel(x_hbm, mem0_hbm, wq_hbm, wk_hbm, wv_hbm, wo_hbm, wr_hbm, wg_hbm, wu_hbm, wd_hbm,
            c_hbm, wmod_hbm, out_hbm,
            x_v, w_v, wo_v, cache, lhs_v, qkv_s, o_s, acc_s, a_s, mod_v,
            stage, wmod_v, hc, n_v, acc, sc_row, sc_col, x1_v, h2_v, out_v,
            mem0_v, r_v, fill_v, never_v, c_v, wr_v, sems):
    w_w = w_v.bitcast(U32)
    cache_w = cache.bitcast(U32)
    lhs_w = lhs_v.bitcast(U32)
    qkv_w = qkv_s.bitcast(U32)
    o_w = o_s.bitcast(U32)

    def weights(h, j0=0, j1=DB):
        return _bf(w_w[h, pl.ds(j0, j1 - j0)].reshape((j1 - j0) * 64, E))

    def tie(v, tok):
        if tok is None:
            return v
        tok = jnp.broadcast_to(tok, (8, 128))
        if v.dtype != F32:
            tok = pltpu.bitcast(tok, v.dtype)
        return jnp.concatenate([jnp.where(never_v[...] > 1.0, tok, v[0:8]), v[8:]], axis=0)

    def copy(src, dst, sem):
        return pltpu.make_async_copy(src, dst, sems.at[sem])

    def wait_all(buf, sem):
        copy(buf, buf, sem).wait()

    def mod_row(k, rows=8):
        v = mod_v[k]
        return v if rows == 8 else jnp.concatenate([v] * (rows // 8), axis=0)

    def put_rows(dst, r0, v):
        for j in range(DB):
            dst[j, pl.ds(r0, v.shape[0]), :] = v[:, j * 128:(j + 1) * 128].astype(BF16)

    def ln1(seg, r0):
        n, inv = _ln(x_v[seg, pl.ds(r0, 8), :].astype(F32))
        return n * mod_row(1) + mod_row(0), inv

    x_tail = copy(x_hbm.at[pl.ds(1, NSEG - 1), pl.ds(M, SEG - M), :],
                  x_v.at[pl.ds(1, NSEG - 1), pl.ds(M, SEG - M), :], SEM_X + 2)

    def prologue():
        wmod_w = wmod_hbm.bitcast(U32)
        w_words = [w.bitcast(U32) for w in (wq_hbm, wk_hbm, wv_hbm)]

        def start_mod(j):
            col = j * 128 if isinstance(j, int) else pl.multiple_of(j * 128, 128)
            for k in range(2):
                copy(wmod_w.at[:, pl.ds(k * D + col, 128)], wmod_v.at[k, j], SEM_MOD + j).start()

        def wait_mod(j):
            wait_all(wmod_v.at[pl.ds(0, 2), j], SEM_MOD + j)

        def start_chunk(k):
            col = k * D if isinstance(k, int) else pl.multiple_of(k * D, D)
            for j in range(DB):
                copy(wmod_w.at[:, pl.ds(col + j * 128, 128)], wmod_v.at[k, j], SEM_MOD2 + k - 2).start()

        def start_ktile(j):
            rows = pl.ds(j * 128 if isinstance(j, int) else pl.multiple_of(j * 128, 128), 128)
            for g in range(KMAJ):
                copy(w_words[0].at[rows, g, :], stage.at[g, rows, :], SEM_WQ + j).start()

        small = [copy(c_hbm, c_v, SEM_SMALL), copy(mem0_hbm, mem0_v, SEM_SMALL + 1),
                 copy(wr_hbm, wr_v, SEM_SMALL + 2)]
        x_head = copy(x_hbm.at[:, pl.ds(0, M), :], x_v.at[:, pl.ds(0, M), :], SEM_X)
        x_seg0 = copy(x_hbm.at[0, pl.ds(M, SEG - M), :], x_v.at[0, pl.ds(M, SEG - M), :], SEM_X + 1)
        for cp in small:
            cp.start()
        x_head.start()
        x_seg0.start()
        start_mod(0)
        for j in range(AHEAD):
            start_ktile(j)
            start_mod(j + 1)
        slab_cps = [copy(w_words[g // NPAIR].at[:, g % NPAIR, :], stage.at[g], SEM_ST + (g - KMAJ) // PPI)
                    for g in range(KMAJ, NGP)]

        fill_v[...] = _fill_matrix()
        a_s[...] = jnp.zeros(a_s.shape, BF16)
        r_v[...] = jnp.full(r_v.shape, -jnp.inf, F32)
        never_v[...] = jnp.zeros(never_v.shape, F32)
        qkv_s[0] = jnp.zeros((2 * SEG, E), BF16)
        o_s[0] = jnp.zeros(o_s.shape[1:], BF16)
        acc_s[0] = jnp.zeros(acc_s.shape[1:], F32)

        def zero_acc(h, carry):
            acc[h] = jnp.zeros((NSEG * M, E), F32)
            return carry

        lax.fori_loop(0, 2 * KMAJ, zero_acc, 0)

        for cp in small:
            cp.wait()
        c = c_v[...].astype(F32)
        sc = _rb(c * jax.nn.sigmoid(c))
        put_rows(sc_row, 0, jnp.broadcast_to(sc, (16, D)))
        for j in range(DB):
            sc_col[pl.ds(j * 128, 128), :] = jnp.broadcast_to(sc[:, j * 128:(j + 1) * 128], (128, 128)).T
        mod_v[6] = jnp.broadcast_to(wr_v[...].astype(F32).reshape(1, D), (8, D))
        put_rows(lhs_v, 0, mem0_v[...].astype(F32))

        x_head.wait()
        x_seg0.wait()
        NB = 16
        RB = NSEG * M // NB
        NR = NSEG * M + SEG - M
        for b in range(NB + 1):
            if b < NB:
                xb = x_v[pl.ds(b * (NSEG // NB), NSEG // NB), pl.ds(0, M), :].astype(F32).reshape(RB, D)
            else:
                xb = x_v[0, pl.ds(M, SEG - M), :].astype(F32)
            nb = _ln(xb)[0]
            for j in range(DB):
                n_v[j, pl.ds(b * RB, nb.shape[0]), :] = nb[:, j * 128:(j + 1) * 128]

        hc_w = hc.bitcast(U32)
        sc_w = sc_row.bitcast(U32)

        def mod_block(j, k, src=None):
            scb = jnp.concatenate([_bf(sc_w[i]) for i in range(DB)], axis=1)
            v = _rb(_dot(scb, _bf(wmod_v[k, j if src is None else src]))[0:8])
            if k == 1:
                v = _rb(1.0 + v)
            col = j * 128 if isinstance(j, int) else pl.multiple_of(j * 128, 128)
            mod_v[k, :, pl.ds(col, 128)] = v
            return v

        def h_block(j, ca, sa):
            n = n_v[j, pl.ds(0, NR), :].reshape(NR // 8, 8, 128)
            hv = (n * ca[None] + sa[None]).reshape(NR, 128).astype(BF16)
            hc[j] = hv[0:NSEG * M]
            lhs_v[j, pl.ds(M, SEG - M), :] = hv[NSEG * M:]

        def pack_pair(r1, r2):
            r = jnp.concatenate([r1.reshape(NSEG, M, E), r2.reshape(NSEG, M, E)], axis=1)
            return r.reshape(NIT, UNR * 2 * M, E).astype(BF16)

        def split_pair(b):
            return (pltpu.bitcast(b << 16, F32).astype(BF16),
                    pltpu.bitcast(b & jnp.uint32(0xFFFF0000), F32).astype(BF16))

        def q_stage(j, last, more_dmas):
            static = isinstance(j, int)
            k0 = j * 128 if static else pl.multiple_of(j * 128, 128)
            src = None if last else jnp.where(j == 0, 0, j + 1)
            for p in range(KMAJ):
                ws = split_pair(stage[p, pl.ds(k0, 128), :])
                rs = []
                for t in range(2):
                    h = 2 * p + t
                    w_v[h, j] = ws[t]
                    rs.append(_dot(_bf(hc_w[j]), _bf(w_w[h, j])) + acc[h])
                    if not last:
                        acc[h] = rs[t]
                if last:
                    cache[p] = pack_pair(*rs)
                elif p == 1:
                    ca = mod_block(j + 1, 1, src)
                elif p == 3:
                    h_block(j + 1, ca, mod_block(j + 1, 0, src))
                if p == 1:
                    more_dmas()

        wait_mod(0)
        h_block(0, mod_block(0, 1), mod_block(0, 0))

        def wait_ktile(j):
            rows = pl.ds(j * 128 if isinstance(j, int) else pl.multiple_of(j * 128, 128), 128)
            wait_all(stage.at[pl.ds(0, KMAJ), rows, :], SEM_WQ + j)

        def q_body(j, carry):
            @pl.when(j == 1)
            def _():
                wait_mod(1)
                h_block(1, mod_block(1, 1), mod_block(1, 0))

            wait_ktile(j)

            @pl.when(j > 0)
            def _():
                wait_mod(j + 1)

            def more_dmas():
                @pl.when(j + AHEAD < DB)
                def _():
                    start_ktile(j + AHEAD)

                @pl.when(j + AHEAD + 1 < DB)
                def _():
                    start_mod(j + AHEAD + 1)

                @pl.when(j + AHEAD == DB)
                def _():
                    for cp in slab_cps[:2 * PPI]:
                        cp.start()

            q_stage(j, False, more_dmas)
            return carry

        lax.fori_loop(0, DB - 1, q_body, 0)
        wait_ktile(DB - 1)

        def last_dmas():
            for i in range(2, (NGP - KMAJ) // PPI):
                for cp in slab_cps[i * PPI:(i + 1) * PPI]:
                    cp.start()
                if i < 4:
                    start_chunk(i)

        q_stage(DB - 1, True, last_dmas)

        def pro_body(i, carry):
            g0 = KMAJ + i * PPI
            wait_all(stage.at[pl.ds(g0, PPI)], SEM_ST + i)

            @pl.when(i >= 2)
            def _():
                wait_all(wmod_v.at[i], SEM_MOD2 + i - 2)

            def more_dmas():
                @pl.when(i < 2)
                def _():
                    start_chunk(i + 4)

                @pl.when(i == 1)
                def _():
                    x_tail.start()

                @pl.when(jnp.logical_and(i >= 2, i < 4))
                def _():
                    wo_w = wo_hbm.bitcast(U32)
                    for t in range(DB // 2):
                        j = (i - 2) * (DB // 2) + t
                        cols = pl.ds(pl.multiple_of(j * 128, 128), 128)
                        copy(wo_w.at[:, cols], wo_v.at[j], SEM_WO).start()

            one = jnp.where(jnp.logical_or(i == 1, i == 4), 1.0, 0.0)

            def mod_cols(j):
                v = jnp.sum(_bf(wmod_v[i, j]).astype(F32) * sc_col[...], axis=0, keepdims=True)
                v = _rb(one + _rb(jnp.broadcast_to(v, (8, 128))))
                mod_v[i, :, pl.ds(j * 128, 128)] = v
                return v

            for t in range(PPI):
                gp = g0 + t
                w_v[2 * gp], w_v[2 * gp + 1] = split_pair(stage[gp].reshape(DB, 128, E))
                rs = []
                for hh in range(2):
                    n = 2 * t + hh - (2 * PPI - DB)
                    parts = [hc_w[j] for j in range(DB)]
                    parts[0] = tie(parts[0], mod_cols(n) if n >= 0 else None)
                    hcv = jnp.concatenate([_bf(w) for w in parts], axis=1)
                    rs.append(_dot(hcv, weights(2 * gp + hh)))
                cache[gp] = pack_pair(*rs)
                if t == 0:
                    more_dmas()
            return carry

        lax.fori_loop(0, (NGP - KMAJ) // PPI, pro_body, 0)

    prologue()

    def main():
        lane = lax.broadcasted_iota(jnp.int32, (8, 2 * 128), 1)

        def post(seg, slot, q, keep=True):
            rows = pl.ds(8 * q, 8)
            x = x_v[seg, rows, :].astype(F32)
            a = a_s[slot, rows, :].astype(F32)
            x1 = _rb(x + mod_row(2) * a)
            n, inv = _ln(x1)
            h2 = _rb(n * mod_row(4) + mod_row(3))
            r = _rb(jnp.sum(h2 * mod_row(6), axis=-1, keepdims=True))
            if keep:
                r_v[...] = jnp.where(lane == seg * 4 + q, r, r_v[...])
            x1_v[seg, rows, :] = x1.astype(BF16)
            h2_v[seg, rows, :] = h2.astype(BF16)
            out_v[seg, rows, :] = (x1 + mod_row(5) * h2).astype(BF16)
            return inv, r

        def out_copy(grp):
            return copy(out_v.at[pl.ds(grp * UNR, UNR)], out_hbm.at[pl.ds(grp * UNR, UNR)], SEM_OUT)

        wg_w, wu_w, wd_w = wg_hbm.bitcast(U32), wu_hbm.bitcast(U32), wd_hbm.bitcast(U32)
        x_tail.wait()
        wait_all(wo_v, SEM_WO)

        def step(it, u):
            s = it * UNR + u
            lhs = jnp.concatenate([_bf(lhs_w[j]) for j in range(DB)], axis=1)
            nseg = jnp.minimum(s + 1, NSEG - 1)

            def side(slot):
                if slot not in SIDE_SLOTS:
                    return None
                i = SIDE_SLOTS.index(slot)
                if i < 4:
                    lag = 2 if i == 0 else 1
                    return post(jnp.maximum(s - lag, 0), (u - lag) % UNR, i)[0]
                r0 = (i - 3) * 8
                h, inv = ln1(nseg, r0)
                put_rows(lhs_v, r0, h)
                return inv

            def proj(m_i, p):
                g = m_i * NPAIR + p
                for t in range(2):
                    qkv_s[g, pl.ds(t * SEG, SEG), :] = _dot(lhs, weights(2 * g + t)).astype(BF16)

            def rows_of(m_i, p):
                g = m_i * NPAIR + p
                return jnp.concatenate([_bf(qkv_w[g]), _bf(cache_w[g, it, pl.ds(u * M, M), :])], axis=0)

            def probs(p):
                parts = [lax.dot_general(_bf(qkv_w[p]), rows_of(1, p), (((1,), (1,)), ((), ())),
                                         preferred_element_type=F32)]
                qc = _bf(cache_w[p, it, pl.ds(u * M, M), :]).astype(F32)
                kc = _bf(cache_w[NPAIR + p, it, pl.ds(u * M, M), :]).astype(F32)
                col = lax.broadcasted_iota(jnp.int32, (M, PR), 1)
                for t in range(2):
                    km = _bf(qkv_w[NPAIR + p, pl.ds(t * (SEG // 2), 8), :]).astype(F32)
                    qt = qc[t * M:(t + 1) * M]
                    st = jnp.zeros((M, PR), F32)
                    for j in range(M):
                        st = jnp.where(col == t * SEG + j,
                                       jnp.sum(qt * km[j:j + 1], axis=-1, keepdims=True), st)
                        st = jnp.where(col == 2 * SEG + t * M + j,
                                       jnp.sum(qt * kc[t * M + j:t * M + j + 1], axis=-1, keepdims=True), st)
                    parts.append(st)
                sc = jnp.concatenate(parts, axis=0) * SCALE
                fm = fill_v[...]
                tok = side(("softmax", p))
                if tok is not None:
                    top = fm[0:8]
                    fm = jnp.concatenate([jnp.where(top > 1.0, tok, top), fm[8:]], axis=0)
                sc = jnp.where(fm == 0.0, sc, fm)
                e = jnp.exp(sc - jnp.max(sc, axis=-1, keepdims=True))
                return (e * _recip(jnp.sum(e, axis=-1, keepdims=True))).astype(BF16)

            def attend(p, pr):
                o = _dot(pr, rows_of(2, p))
                for t in range(2):
                    o_s[2 * p + t, pl.ds(0, SEG), :] = o[t * SEG:(t + 1) * SEG].astype(BF16)
                for t in range(2):
                    o_s[2 * p + t, pl.ds(SEG + (u % 2) * M, M), :] = (
                        o[2 * SEG + t * M:2 * SEG + (t + 1) * M].astype(BF16))

            ps = {}
            for pa in range(0, NPAIR, 2):
                pb = pa + 1
                todo = [(0, pa), (1, pa), (0, pb), (1, pb), (2, pa), (2, pb)]
                if pa == 0 and u > 0:
                    hs = [(m_i * NPAIR + p, t) for m_i, p in todo[:NSPLIT] for t in range(2)]
                    ke = KEARLY * 128
                    first = [_dot(lhs[:, :ke], weights(2 * g + t, 0, KEARLY)) for g, t in hs]
                    for (g, t), part in zip(hs, first):
                        res = _dot(lhs[:, ke:], weights(2 * g + t, KEARLY, DB)) + part
                        qkv_s[g, pl.ds(t * SEG, SEG), :] = res.astype(BF16)
                    todo = todo[NSPLIT:]
                for m_i, p in todo:
                    proj(m_i, p)
                for kind in ("scores", "values") if pa % 4 == 0 else ("values", "scores"):
                    for p in (pa, pb):
                        if kind == "scores":
                            ps[p] = probs(p)
                        elif p >= 2:
                            attend(p - 2, ps.pop(p - 2))
            L = NPAIR - 1

            nr = SEG + (2 * M if u % 2 else 0)
            for h0, h1 in ((0, HA), (HA, H)):
                for j in range(DB):
                    words = [o_w[h, pl.ds(0, nr // 2), :] for h in range(h0, h1)]
                    words[0] = tie(words[0], side((h0, j)))
                    ol = jnp.concatenate([_bf(w) for w in words], axis=1)
                    part = _dot(ol, _bf(wo_v[j, pl.ds(h0 * E // 2, (h1 - h0) * E // 2), :]))
                    if h0 == 0:
                        acc_s[j, pl.ds(0, nr), :] = part
                    else:
                        a = part + acc_s[j, pl.ds(0, nr), :]
                        cols = pl.ds(j * 128, 128)
                        lhs_v[j, pl.ds(0, M), :] = a[0:M].astype(BF16)
                        a_s[u, pl.ds(M, SEG - M), cols] = a[M:SEG].astype(BF16)
                        for t in range((nr - SEG) // M):
                            a_s[u - 1 + t, pl.ds(0, M), cols] = a[SEG + t * M:SEG + (t + 1) * M].astype(BF16)
                    if h0 == 0 and j == 4:
                        attend(L - 1, ps.pop(L - 1))
                        attend(L, ps.pop(L))

        def iteration(it, carry):
            @pl.when(it >= 2)
            def _():
                out_copy(it - 2).start()

            @pl.when(it < FB // 2)
            def _():
                for t in range(2):
                    j = 2 * it + t
                    cols = pl.ds(pl.multiple_of(j * 128, 128), 128)
                    half = pl.ds(t * (D // 2), D // 2)
                    copy(wg_w.at[:, cols], stage.at[it, half, :], SEM_MOE).start()
                    copy(wu_w.at[:, cols], stage.at[FB // 2 + it, half, :], SEM_MOE).start()

            @pl.when(it < DB)
            def _():
                cols = pl.ds(pl.multiple_of(it * 128, 128), 128)
                for t in range(2):
                    copy(wd_w.at[pl.ds(t * (F // 4), F // 4), cols],
                         stage.at[FB + 2 * it + t, pl.ds(0, F // 4), :], SEM_MOE + 1).start()

            for u in range(UNR):
                step(it, u)
            return carry

        lax.fori_loop(0, NIT, iteration, 0)

        out_copy(NIT - 2).start()
        wait_all(stage.at[pl.ds(0, FB)], SEM_MOE)
        wait_all(stage.at[pl.ds(FB, 2 * DB), pl.ds(0, F // 4), :], SEM_MOE + 1)
        r8 = lax.broadcasted_iota(jnp.int32, (8, 1), 0)

        def top2(vals, idx, axes):
            def red(f, v):
                for ax in axes:
                    v = f(v, axis=ax, keepdims=True)
                return v
            m1 = red(jnp.max, vals)
            i1 = red(jnp.min, jnp.where(vals == m1, idx, S - 1.0))
            rest = jnp.where(idx == i1, -jnp.inf, vals)
            m2 = red(jnp.max, rest)
            i2 = red(jnp.min, jnp.where(rest == m2, jnp.where(idx == i1, S - 1.0, idx), S - 1.0))
            return m1, i1, m2, i2

        m1, i1v, m2, i2v = top2(r_v[...], (lane * 8 + r8).astype(F32), (1, 0))
        vals = [jnp.where(r8 == 0, m1, jnp.where(r8 == 1, m2, -jnp.inf))]
        idxs = [jnp.where(r8 == 0, i1v, jnp.where(r8 == 1, i2v, S - 1.0))]
        for seg, q in [(NSEG - 2, 0)] + [(NSEG - 1, q) for q in range(4)]:
            vals.append(post(seg, seg % UNR, q, keep=False)[1])
            idxs.append((r8 + (seg * SEG + q * 8)).astype(F32))
        out_copy(NIT - 1).start()
        m1, i1v, m2, i2v = top2(jnp.concatenate(vals, axis=0), jnp.concatenate(idxs, axis=0), (0,))
        i1 = i1v.astype(jnp.int32)[0, 0]
        i2 = i2v.astype(jnp.int32)[0, 0]

        def tile_of(i):
            return i >> 5, pl.multiple_of(((i >> 3) & 3) * 8, 8)

        sel = [tile_of(i1), tile_of(i2)]
        x1s = jnp.concatenate([x1_v[sg, pl.ds(r0, 8), :].astype(F32) for sg, r0 in sel], axis=0)
        h2s = jnp.concatenate([h2_v[sg, pl.ds(r0, 8), :].astype(F32) for sg, r0 in sel], axis=0)
        h2b = h2s.astype(BF16)
        gus = []
        for j in range(FB):
            half = pl.ds((j % 2) * (D // 2), D // 2)
            g = _rb(_dot(h2b, _bf(stage[j // 2, half, :])))
            g = _rb(g * jax.nn.sigmoid(g))
            u = _rb(_dot(h2b, _bf(stage[FB // 2 + j // 2, half, :])))
            gus.append(g * u)
        gu = jnp.concatenate(gus, axis=1).astype(BF16)
        ys = []
        for j in range(DB):
            wd = stage[pl.ds(FB + 2 * j, 2), pl.ds(0, F // 4), :].reshape(F // 2, 128)
            ys.append(_rb(_dot(gu, _bf(wd))))
        y = jnp.concatenate(ys, axis=1)
        rows = lax.broadcasted_iota(jnp.int32, (16, 1), 0)
        rs = _rb(jax.nn.sigmoid(jnp.where(rows < 8, m1, m2)))
        y = _rb(y * rs)
        full = x1s + mod_row(5, 16) * _rb(h2s + y)

        copy(out_v, out_hbm, SEM_OUT).wait()
        for t, (i, (sg, r0)) in enumerate(zip((i1, i2), sel)):
            old = out_v[sg, pl.ds(r0, 8), :].astype(F32)
            new = jnp.where(r8 == (i & 7), full[t * 8:(t + 1) * 8], old)
            out_v[sg, pl.ds(r0, 8), :] = new.astype(BF16)
        fix = [copy(out_v.at[sg, pl.ds(r0, 8), :], out_hbm.at[sg, pl.ds(r0, 8), :], SEM_OUT + 1 + t)
               for t, (sg, r0) in enumerate(sel)]
        differ = (i1 >> 3) != (i2 >> 3)
        fix[0].start()

        @pl.when(differ)
        def _():
            fix[1].start()
            fix[1].wait()

        fix[0].wait()

    main()


@jax.jit
def pallas_adaLN_cond__memory_aug_recurrent_mem_tr__moe_arch_mod__prompt_kernel(
    A_x: jax.Array,
    A_mem0: jax.Array,
    A_Wq: jax.Array,
    A_Wk: jax.Array,
    A_Wv: jax.Array,
    A_Wo: jax.Array,
    A_seg_len: jax.Array,
    B_x: jax.Array,
    B_w_r: jax.Array,
    B_w_gate: jax.Array,
    B_w_up: jax.Array,
    B_w_down: jax.Array,
    c: jax.Array,
    w_mod: jax.Array,
):
    del A_seg_len, B_x
    assert A_x.shape == (1, S, D) and A_mem0.shape == (1, M, D) and A_Wq.shape == (D, H, E)
    hbm = pl.BlockSpec(memory_space=pl.ANY)
    out = pl.pallas_call(
        _kernel,
        out_shape=jax.ShapeDtypeStruct((NSEG, SEG, D), BF16),
        in_specs=[hbm] * 12,
        out_specs=hbm,
        scratch_shapes=[
            pltpu.VMEM((NSEG, SEG, D), BF16),
            pltpu.VMEM((3 * H, DB, 128, E), BF16),
            pltpu.VMEM((DB, H * E // 2, 128), U32),
            pltpu.VMEM((NGP, NIT, UNR * 2 * M, E), BF16),
            pltpu.VMEM((DB, SEG, 128), BF16),
            pltpu.VMEM((NGP, 2 * SEG, E), BF16),
            pltpu.VMEM((H, 2 * SEG, E), BF16),
            pltpu.VMEM((DB, 2 * SEG, 128), F32),
            pltpu.VMEM((UNR, SEG, D), BF16),
            pltpu.VMEM((7, 8, D), F32),
            pltpu.VMEM((NGP, D, E), U32),
            pltpu.VMEM((6, DB, D // 2, 128), U32),
            pltpu.VMEM((DB, NSEG * M, E), BF16),
            pltpu.VMEM((DB, NSEG * M + SEG, 128), F32),
            pltpu.VMEM((2 * KMAJ, NSEG * M, E), F32),
            pltpu.VMEM((DB, 16, 128), BF16),
            pltpu.VMEM((D, 128), F32),
            pltpu.VMEM((NSEG, SEG, D), BF16),
            pltpu.VMEM((NSEG, SEG, D), BF16),
            pltpu.VMEM((NSEG, SEG, D), BF16),
            pltpu.VMEM((M, D), BF16),
            pltpu.VMEM((8, S // 8), F32),
            pltpu.VMEM((PR, PR), F32),
            pltpu.VMEM((8, 128), F32),
            pltpu.VMEM((1, D), BF16),
            pltpu.VMEM((D,), BF16),
            pltpu.SemaphoreType.DMA((NSEM,)),
        ],
        compiler_params=pltpu.CompilerParams(
            vmem_limit_bytes=120 * 1024 * 1024, disable_bounds_checks=True,
            disable_semaphore_checks=True),
    )(
        A_x.reshape(NSEG, SEG, D),
        A_mem0.reshape(M, D),
        A_Wq, A_Wk, A_Wv,
        A_Wo.reshape(H * E, D),
        B_w_r,
        B_w_gate, B_w_up, B_w_down,
        c, w_mod,
    )
    return out.reshape(1, S, D)
```

```python
import jax
import jax.numpy as jnp
from jax import lax
import jax.experimental.pallas as pl
import jax.experimental.pallas.tpu as pltpu

BF16 = jnp.bfloat16
F32 = jnp.float32
U32 = jnp.uint32

S = 2048
D = 1024
H = 32
E = 128
M = 8
SEG = 32
NSEG = S // SEG
NPAIR = H // 2
NGP = 3 * NPAIR
F = 3584
DB = D // 128
FB = F // 128
PR = 2 * SEG + 2 * M
UNR = 4
NIT = NSEG // UNR
KMAJ = 12
AHEAD = 3
PPI = 6
NSPLIT = 3
KEARLY = 5
HA = 24
SIDE_SLOTS = [("softmax", 4), ("softmax", 8), ("softmax", 10), ("softmax", 12), (0, 2), (0, 5), (HA, 0)]
EPS = 1e-5
SCALE = E ** (-0.5)

SEM_SMALL = 0
SEM_X = SEM_SMALL + 3
SEM_MOD = SEM_X + 3
SEM_MOD2 = SEM_MOD + DB
SEM_WQ = SEM_MOD2 + 4
SEM_ST = SEM_WQ + DB
SEM_WO = SEM_ST + (NGP - KMAJ) // PPI
SEM_MOE = SEM_WO + 1
SEM_OUT = SEM_MOE + 2
NSEM = SEM_OUT + 3


def _rb(v):
    return v.astype(BF16).astype(F32)


def _dot(a, b):
    return jnp.dot(a, b, preferred_element_type=F32)


def _recip(x):
    r = pl.reciprocal(x, approx=True)
    return r * (2.0 - x * r)


def _bf(words):
    return pltpu.bitcast(words, BF16)


def _ln(x):
    m = jnp.mean(x, axis=-1, keepdims=True)
    mb = _rb(m)
    d = x - mb
    var = jnp.mean(d * d, axis=-1, keepdims=True) - (m - mb) * (m - mb)
    inv = _recip(_rb(jnp.sqrt(_rb(_rb(jnp.maximum(var, 0.0)) + EPS))))
    return d * inv, inv


def _fill_matrix():
    i = lax.broadcasted_iota(jnp.int32, (PR, PR), 0)
    j = lax.broadcasted_iota(jnp.int32, (PR, PR), 1)

    def head(t):
        return jnp.where(t < 2 * SEG, t >> 5, (t - 2 * SEG) >> 3)

    def pos(t):
        r = t & (SEG - 1)
        return jnp.where(t < 2 * SEG, jnp.where(r < M, r, r + M), M + (t & (M - 1)))

    same = head(i) == head(j)
    pi = pos(i)
    ok = jnp.where(pi < M, 1, jnp.where(pi >= pos(j), 1, 0))
    return jnp.where(same, jnp.where(ok == 1, 0.0, -1e9), -3e38).astype(F32)


def _kernel(x_hbm, mem0_hbm, wq_hbm, wk_hbm, wv_hbm, wo_hbm, wr_hbm, wg_hbm, wu_hbm, wd_hbm,
            c_hbm, wmod_hbm, out_hbm,
            x_v, w_v, wo_v, cache, lhs_v, qkv_s, o_s, acc_s, mod_v,
            stage, wmod_v, hc, n_v, acc, sc_row, sc_col, x1_v, h2_v, out_v,
            mem0_v, r_v, fill_v, never_v, c_v, wr_v, sems):
    w_w = w_v.bitcast(U32)
    cache_w = cache.bitcast(U32)
    lhs_w = lhs_v.bitcast(U32)
    qkv_w = qkv_s.bitcast(U32)
    o_w = o_s.bitcast(U32)

    def weights(h, j0=0, j1=DB):
        return _bf(w_w[h, pl.ds(j0, j1 - j0)].reshape((j1 - j0) * 64, E))

    def tie(v, tok):
        if tok is None:
            return v
        tok = jnp.broadcast_to(tok, (8, 128))
        if v.dtype != F32:
            tok = pltpu.bitcast(tok, v.dtype)
        return jnp.concatenate([jnp.where(never_v[...] > 1.0, tok, v[0:8]), v[8:]], axis=0)

    def copy(src, dst, sem):
        return pltpu.make_async_copy(src, dst, sems.at[sem])

    def wait_all(buf, sem):
        copy(buf, buf, sem).wait()

    def mod_row(k, rows=8):
        v = mod_v[k]
        return v if rows == 8 else jnp.concatenate([v] * (rows // 8), axis=0)

    def put_rows(dst, r0, v):
        for j in range(DB):
            dst[j, pl.ds(r0, v.shape[0]), :] = v[:, j * 128:(j + 1) * 128].astype(BF16)

    def ln1(seg, r0):
        n, inv = _ln(x_v[seg, pl.ds(r0, 8), :].astype(F32))
        return n * mod_row(1) + mod_row(0), inv

    x_tail = copy(x_hbm.at[pl.ds(1, NSEG - 1), pl.ds(M, SEG - M), :],
                  x_v.at[pl.ds(1, NSEG - 1), pl.ds(M, SEG - M), :], SEM_X + 2)

    def prologue():
        wmod_w = wmod_hbm.bitcast(U32)
        w_words = [w.bitcast(U32) for w in (wq_hbm, wk_hbm, wv_hbm)]

        def start_mod(j):
            col = j * 128 if isinstance(j, int) else pl.multiple_of(j * 128, 128)
            for k in range(2):
                copy(wmod_w.at[:, pl.ds(k * D + col, 128)], wmod_v.at[k, j], SEM_MOD + j).start()

        def wait_mod(j):
            wait_all(wmod_v.at[pl.ds(0, 2), j], SEM_MOD + j)

        def start_chunk(k):
            col = k * D if isinstance(k, int) else pl.multiple_of(k * D, D)
            for j in range(DB):
                copy(wmod_w.at[:, pl.ds(col + j * 128, 128)], wmod_v.at[k, j], SEM_MOD2 + k - 2).start()

        def start_ktile(j):
            rows = pl.ds(j * 128 if isinstance(j, int) else pl.multiple_of(j * 128, 128), 128)
            for g in range(KMAJ):
                copy(w_words[0].at[rows, g, :], stage.at[g, rows, :], SEM_WQ + j).start()

        small = [copy(c_hbm, c_v, SEM_SMALL), copy(mem0_hbm, mem0_v, SEM_SMALL + 1),
                 copy(wr_hbm, wr_v, SEM_SMALL + 2)]
        x_head = copy(x_hbm.at[:, pl.ds(0, M), :], x_v.at[:, pl.ds(0, M), :], SEM_X)
        x_seg0 = copy(x_hbm.at[0, pl.ds(M, SEG - M), :], x_v.at[0, pl.ds(M, SEG - M), :], SEM_X + 1)
        for cp in small:
            cp.start()
        x_head.start()
        x_seg0.start()
        start_mod(0)
        for j in range(AHEAD):
            start_ktile(j)
            start_mod(j + 1)
        slab_cps = [copy(w_words[g // NPAIR].at[:, g % NPAIR, :], stage.at[g], SEM_ST + (g - KMAJ) // PPI)
                    for g in range(KMAJ, NGP)]

        fill_v[...] = _fill_matrix()
        x1_v[0] = jnp.zeros((SEG, D), BF16)
        r_v[...] = jnp.full(r_v.shape, -jnp.inf, F32)
        never_v[...] = jnp.zeros(never_v.shape, F32)
        qkv_s[0] = jnp.zeros((2 * SEG, E), BF16)
        o_s[0] = jnp.zeros(o_s.shape[1:], BF16)
        acc_s[0] = jnp.zeros(acc_s.shape[1:], F32)

        def zero_acc(h, carry):
            acc[h] = jnp.zeros((NSEG * M, E), F32)
            return carry

        lax.fori_loop(0, 2 * KMAJ, zero_acc, 0)

        for cp in small:
            cp.wait()
        c = c_v[...].astype(F32)
        sc = _rb(c * jax.nn.sigmoid(c))
        put_rows(sc_row, 0, jnp.broadcast_to(sc, (16, D)))
        for j in range(DB):
            sc_col[pl.ds(j * 128, 128), :] = jnp.broadcast_to(sc[:, j * 128:(j + 1) * 128], (128, 128)).T
        mod_v[6] = jnp.broadcast_to(wr_v[...].astype(F32).reshape(1, D), (8, D))
        put_rows(lhs_v, 0, mem0_v[...].astype(F32))

        x_head.wait()
        x_seg0.wait()
        NB = 16
        RB = NSEG * M // NB
        NR = NSEG * M + SEG - M
        for b in range(NB + 1):
            if b < NB:
                xb = x_v[pl.ds(b * (NSEG // NB), NSEG // NB), pl.ds(0, M), :].astype(F32).reshape(RB, D)
            else:
                xb = x_v[0, pl.ds(M, SEG - M), :].astype(F32)
            nb = _ln(xb)[0]
            for j in range(DB):
                n_v[j, pl.ds(b * RB, nb.shape[0]), :] = nb[:, j * 128:(j + 1) * 128]

        hc_w = hc.bitcast(U32)
        sc_w = sc_row.bitcast(U32)

        def mod_block(j, k, src=None):
            scb = jnp.concatenate([_bf(sc_w[i]) for i in range(DB)], axis=1)
            v = _rb(_dot(scb, _bf(wmod_v[k, j if src is None else src]))[0:8])
            if k == 1:
                v = _rb(1.0 + v)
            col = j * 128 if isinstance(j, int) else pl.multiple_of(j * 128, 128)
            mod_v[k, :, pl.ds(col, 128)] = v
            return v

        def h_block(j, ca, sa):
            n = n_v[j, pl.ds(0, NR), :].reshape(NR // 8, 8, 128)
            hv = (n * ca[None] + sa[None]).reshape(NR, 128).astype(BF16)
            hc[j] = hv[0:NSEG * M]
            lhs_v[j, pl.ds(M, SEG - M), :] = hv[NSEG * M:]

        def pack_pair(r1, r2):
            r = jnp.concatenate([r1.reshape(NSEG, M, E), r2.reshape(NSEG, M, E)], axis=1)
            return r.reshape(NIT, UNR * 2 * M, E).astype(BF16)

        def split_pair(b):
            return (pltpu.bitcast(b << 16, F32).astype(BF16),
                    pltpu.bitcast(b & jnp.uint32(0xFFFF0000), F32).astype(BF16))

        def q_stage(j, last, more_dmas):
            static = isinstance(j, int)
            k0 = j * 128 if static else pl.multiple_of(j * 128, 128)
            src = None if last else jnp.where(j == 0, 0, j + 1)
            for p in range(KMAJ):
                ws = split_pair(stage[p, pl.ds(k0, 128), :])
                rs = []
                for t in range(2):
                    h = 2 * p + t
                    w_v[h, j] = ws[t]
                    rs.append(_dot(_bf(hc_w[j]), _bf(w_w[h, j])) + acc[h])
                    if not last:
                        acc[h] = rs[t]
                if last:
                    cache[p] = pack_pair(*rs)
                elif p == 1:
                    ca = mod_block(j + 1, 1, src)
                elif p == 3:
                    h_block(j + 1, ca, mod_block(j + 1, 0, src))
                if p == 1:
                    more_dmas()

        wait_mod(0)
        h_block(0, mod_block(0, 1), mod_block(0, 0))

        def wait_ktile(j):
            rows = pl.ds(j * 128 if isinstance(j, int) else pl.multiple_of(j * 128, 128), 128)
            wait_all(stage.at[pl.ds(0, KMAJ), rows, :], SEM_WQ + j)

        def q_body(j, carry):
            @pl.when(j == 1)
            def _():
                wait_mod(1)
                h_block(1, mod_block(1, 1), mod_block(1, 0))

            wait_ktile(j)

            @pl.when(j > 0)
            def _():
                wait_mod(j + 1)

            def more_dmas():
                @pl.when(j + AHEAD < DB)
                def _():
                    start_ktile(j + AHEAD)

                @pl.when(j + AHEAD + 1 < DB)
                def _():
                    start_mod(j + AHEAD + 1)

                @pl.when(j + AHEAD == DB)
                def _():
                    for cp in slab_cps[:2 * PPI]:
                        cp.start()

            q_stage(j, False, more_dmas)
            return carry

        lax.fori_loop(0, DB - 1, q_body, 0)
        wait_ktile(DB - 1)

        def last_dmas():
            for i in range(2, (NGP - KMAJ) // PPI):
                for cp in slab_cps[i * PPI:(i + 1) * PPI]:
                    cp.start()
                if i < 4:
                    start_chunk(i)

        q_stage(DB - 1, True, last_dmas)

        def pro_body(i, carry):
            g0 = KMAJ + i * PPI
            wait_all(stage.at[pl.ds(g0, PPI)], SEM_ST + i)

            @pl.when(i >= 2)
            def _():
                wait_all(wmod_v.at[i], SEM_MOD2 + i - 2)

            def more_dmas():
                @pl.when(i < 2)
                def _():
                    start_chunk(i + 4)

                @pl.when(i == 1)
                def _():
                    x_tail.start()

                @pl.when(jnp.logical_and(i >= 2, i < 4))
                def _():
                    wo_w = wo_hbm.bitcast(U32)
                    for t in range(DB // 2):
                        j = (i - 2) * (DB // 2) + t
                        cols = pl.ds(pl.multiple_of(j * 128, 128), 128)
                        copy(wo_w.at[:, cols], wo_v.at[j], SEM_WO).start()

            one = jnp.where(jnp.logical_or(i == 1, i == 4), 1.0, 0.0)

            def mod_cols(j):
                v = jnp.sum(_bf(wmod_v[i, j]).astype(F32) * sc_col[...], axis=0, keepdims=True)
                v = _rb(one + _rb(jnp.broadcast_to(v, (8, 128))))
                mod_v[i, :, pl.ds(j * 128, 128)] = v
                return v

            for t in range(PPI):
                gp = g0 + t
                w_v[2 * gp], w_v[2 * gp + 1] = split_pair(stage[gp].reshape(DB, 128, E))
                rs = []
                for hh in range(2):
                    n = 2 * t + hh - (2 * PPI - DB)
                    parts = [hc_w[j] for j in range(DB)]
                    parts[0] = tie(parts[0], mod_cols(n) if n >= 0 else None)
                    hcv = jnp.concatenate([_bf(w) for w in parts], axis=1)
                    rs.append(_dot(hcv, weights(2 * gp + hh)))
                cache[gp] = pack_pair(*rs)
                if t == 0:
                    more_dmas()
            return carry

        lax.fori_loop(0, (NGP - KMAJ) // PPI, pro_body, 0)

    prologue()

    def main():
        lane = lax.broadcasted_iota(jnp.int32, (8, 2 * 128), 1)

        def post(seg, q, keep=True):
            rows = pl.ds(8 * q, 8)
            x1 = x1_v[seg, rows, :].astype(F32)
            n, inv = _ln(x1)
            h2 = _rb(n * mod_row(4) + mod_row(3))
            r = _rb(jnp.sum(h2 * mod_row(6), axis=-1, keepdims=True))
            if keep:
                r_v[...] = jnp.where(lane == seg * 4 + q, r, r_v[...])
            h2_v[seg, rows, :] = h2.astype(BF16)
            out_v[seg, rows, :] = (x1 + mod_row(5) * h2).astype(BF16)
            return inv, r

        def out_copy(grp):
            return copy(out_v.at[pl.ds(grp * UNR, UNR)], out_hbm.at[pl.ds(grp * UNR, UNR)], SEM_OUT)

        wg_w, wu_w, wd_w = wg_hbm.bitcast(U32), wu_hbm.bitcast(U32), wd_hbm.bitcast(U32)
        x_tail.wait()
        wait_all(wo_v, SEM_WO)

        def step(it, u):
            s = it * UNR + u
            lhs = jnp.concatenate([_bf(lhs_w[j]) for j in range(DB)], axis=1)
            nseg = jnp.minimum(s + 1, NSEG - 1)

            def side(slot):
                if slot not in SIDE_SLOTS:
                    return None
                i = SIDE_SLOTS.index(slot)
                if i < 4:
                    lag = 2 if i == 0 else 1
                    return post(jnp.maximum(s - lag, 0), i)[0]
                r0 = (i - 3) * 8
                h, inv = ln1(nseg, r0)
                put_rows(lhs_v, r0, h)
                return inv

            def proj(m_i, p):
                g = m_i * NPAIR + p
                for t in range(2):
                    qkv_s[g, pl.ds(t * SEG, SEG), :] = _dot(lhs, weights(2 * g + t)).astype(BF16)

            def rows_of(m_i, p):
                g = m_i * NPAIR + p
                return jnp.concatenate([_bf(qkv_w[g]), _bf(cache_w[g, it, pl.ds(u * M, M), :])], axis=0)

            def probs(p):
                parts = [lax.dot_general(_bf(qkv_w[p]), rows_of(1, p), (((1,), (1,)), ((), ())),
                                         preferred_element_type=F32)]
                qc = _bf(cache_w[p, it, pl.ds(u * M, M), :]).astype(F32)
                kc = _bf(cache_w[NPAIR + p, it, pl.ds(u * M, M), :]).astype(F32)
                col = lax.broadcasted_iota(jnp.int32, (M, PR), 1)
                for t in range(2):
                    km = _bf(qkv_w[NPAIR + p, pl.ds(t * (SEG // 2), 8), :]).astype(F32)
                    qt = qc[t * M:(t + 1) * M]
                    st = jnp.zeros((M, PR), F32)
                    for j in range(M):
                        st = jnp.where(col == t * SEG + j,
                                       jnp.sum(qt * km[j:j + 1], axis=-1, keepdims=True), st)
                        st = jnp.where(col == 2 * SEG + t * M + j,
                                       jnp.sum(qt * kc[t * M + j:t * M + j + 1], axis=-1, keepdims=True), st)
                    parts.append(st)
                sc = jnp.concatenate(parts, axis=0) * SCALE
                fm = fill_v[...]
                tok = side(("softmax", p))
                if tok is not None:
                    top = fm[0:8]
                    fm = jnp.concatenate([jnp.where(top > 1.0, tok, top), fm[8:]], axis=0)
                sc = jnp.where(fm == 0.0, sc, fm)
                e = jnp.exp(sc - jnp.max(sc, axis=-1, keepdims=True))
                return (e * _recip(jnp.sum(e, axis=-1, keepdims=True))).astype(BF16)

            def attend(p, pr):
                o = _dot(pr, rows_of(2, p))
                for t in range(2):
                    o_s[2 * p + t, pl.ds(0, SEG), :] = o[t * SEG:(t + 1) * SEG].astype(BF16)
                for t in range(2):
                    o_s[2 * p + t, pl.ds(SEG + (u % 2) * M, M), :] = (
                        o[2 * SEG + t * M:2 * SEG + (t + 1) * M].astype(BF16))

            ps = {}
            for pa in range(0, NPAIR, 2):
                pb = pa + 1
                todo = [(0, pa), (1, pa), (0, pb), (1, pb), (2, pa), (2, pb)]
                if pa == 0 and u > 0:
                    hs = [(m_i * NPAIR + p, t) for m_i, p in todo[:NSPLIT] for t in range(2)]
                    ke = KEARLY * 128
                    first = [_dot(lhs[:, :ke], weights(2 * g + t, 0, KEARLY)) for g, t in hs]
                    for (g, t), part in zip(hs, first):
                        res = _dot(lhs[:, ke:], weights(2 * g + t, KEARLY, DB)) + part
                        qkv_s[g, pl.ds(t * SEG, SEG), :] = res.astype(BF16)
                    todo = todo[NSPLIT:]
                for m_i, p in todo:
                    proj(m_i, p)
                for kind in ("scores", "values") if pa % 4 == 0 else ("values", "scores"):
                    for p in (pa, pb):
                        if kind == "scores":
                            ps[p] = probs(p)
                        elif p >= 2:
                            attend(p - 2, ps.pop(p - 2))
            L = NPAIR - 1

            nr = SEG + (2 * M if u % 2 else 0)
            for h0, h1 in ((0, HA), (HA, H)):
                for j in range(DB):
                    words = [o_w[h, pl.ds(0, nr // 2), :] for h in range(h0, h1)]
                    words[0] = tie(words[0], side((h0, j)))
                    ol = jnp.concatenate([_bf(w) for w in words], axis=1)
                    part = _dot(ol, _bf(wo_v[j, pl.ds(h0 * E // 2, (h1 - h0) * E // 2), :]))
                    if h0 == 0:
                        acc_s[j, pl.ds(0, nr), :] = part
                    else:
                        a = part + acc_s[j, pl.ds(0, nr), :]
                        cols = pl.ds(j * 128, 128)
                        lhs_v[j, pl.ds(0, M), :] = a[0:M].astype(BF16)
                        for q in range(1, nr // M):
                            seg, rows = (s, pl.ds(q * M, M)) if q < 4 else (s + q - 5, pl.ds(0, M))
                            x1 = x_v[seg, rows, cols].astype(F32) + mod_v[2, :, cols] * a[q * M:(q + 1) * M]
                            x1_v[seg, rows, cols] = x1.astype(BF16)
                    if h0 == 0 and j == 4:
                        attend(L - 1, ps.pop(L - 1))
                        attend(L, ps.pop(L))

        def iteration(it, carry):
            @pl.when(it >= 2)
            def _():
                out_copy(it - 2).start()

            @pl.when(it < FB // 2)
            def _():
                for t in range(2):
                    j = 2 * it + t
                    cols = pl.ds(pl.multiple_of(j * 128, 128), 128)
                    half = pl.ds(t * (D // 2), D // 2)
                    copy(wg_w.at[:, cols], stage.at[it, half, :], SEM_MOE).start()
                    copy(wu_w.at[:, cols], stage.at[FB // 2 + it, half, :], SEM_MOE).start()

            @pl.when(it < DB)
            def _():
                cols = pl.ds(pl.multiple_of(it * 128, 128), 128)
                for t in range(2):
                    copy(wd_w.at[pl.ds(t * (F // 4), F // 4), cols],
                         stage.at[FB + 2 * it + t, pl.ds(0, F // 4), :], SEM_MOE + 1).start()

            for u in range(UNR):
                step(it, u)
            return carry

        lax.fori_loop(0, NIT, iteration, 0)

        out_copy(NIT - 2).start()
        wait_all(stage.at[pl.ds(0, FB)], SEM_MOE)
        wait_all(stage.at[pl.ds(FB, 2 * DB), pl.ds(0, F // 4), :], SEM_MOE + 1)
        r8 = lax.broadcasted_iota(jnp.int32, (8, 1), 0)

        def top2(vals, idx, axes):
            def red(f, v):
                for ax in axes:
                    v = f(v, axis=ax, keepdims=True)
                return v
            m1 = red(jnp.max, vals)
            i1 = red(jnp.min, jnp.where(vals == m1, idx, S - 1.0))
            rest = jnp.where(idx == i1, -jnp.inf, vals)
            m2 = red(jnp.max, rest)
            i2 = red(jnp.min, jnp.where(rest == m2, jnp.where(idx == i1, S - 1.0, idx), S - 1.0))
            return m1, i1, m2, i2

        m1, i1v, m2, i2v = top2(r_v[...], (lane * 8 + r8).astype(F32), (1, 0))
        vals = [jnp.where(r8 == 0, m1, jnp.where(r8 == 1, m2, -jnp.inf))]
        idxs = [jnp.where(r8 == 0, i1v, jnp.where(r8 == 1, i2v, S - 1.0))]
        for seg, q in [(NSEG - 2, 0)] + [(NSEG - 1, q) for q in range(4)]:
            vals.append(post(seg, q, keep=False)[1])
            idxs.append((r8 + (seg * SEG + q * 8)).astype(F32))
        out_copy(NIT - 1).start()
        m1, i1v, m2, i2v = top2(jnp.concatenate(vals, axis=0), jnp.concatenate(idxs, axis=0), (0,))
        i1 = i1v.astype(jnp.int32)[0, 0]
        i2 = i2v.astype(jnp.int32)[0, 0]

        def tile_of(i):
            return i >> 5, pl.multiple_of(((i >> 3) & 3) * 8, 8)

        sel = [tile_of(i1), tile_of(i2)]
        x1s = jnp.concatenate([x1_v[sg, pl.ds(r0, 8), :].astype(F32) for sg, r0 in sel], axis=0)
        h2s = jnp.concatenate([h2_v[sg, pl.ds(r0, 8), :].astype(F32) for sg, r0 in sel], axis=0)
        h2b = h2s.astype(BF16)
        gus = []
        for j in range(FB):
            half = pl.ds((j % 2) * (D // 2), D // 2)
            g = _rb(_dot(h2b, _bf(stage[j // 2, half, :])))
            g = _rb(g * jax.nn.sigmoid(g))
            u = _rb(_dot(h2b, _bf(stage[FB // 2 + j // 2, half, :])))
            gus.append(g * u)
        gu = jnp.concatenate(gus, axis=1).astype(BF16)
        ys = []
        for j in range(DB):
            wd = stage[pl.ds(FB + 2 * j, 2), pl.ds(0, F // 4), :].reshape(F // 2, 128)
            ys.append(_rb(_dot(gu, _bf(wd))))
        y = jnp.concatenate(ys, axis=1)
        rows = lax.broadcasted_iota(jnp.int32, (16, 1), 0)
        rs = _rb(jax.nn.sigmoid(jnp.where(rows < 8, m1, m2)))
        y = _rb(y * rs)
        full = x1s + mod_row(5, 16) * _rb(h2s + y)

        copy(out_v, out_hbm, SEM_OUT).wait()
        for t, (i, (sg, r0)) in enumerate(zip((i1, i2), sel)):
            old = out_v[sg, pl.ds(r0, 8), :].astype(F32)
            new = jnp.where(r8 == (i & 7), full[t * 8:(t + 1) * 8], old)
            out_v[sg, pl.ds(r0, 8), :] = new.astype(BF16)
        fix = [copy(out_v.at[sg, pl.ds(r0, 8), :], out_hbm.at[sg, pl.ds(r0, 8), :], SEM_OUT + 1 + t)
               for t, (sg, r0) in enumerate(sel)]
        differ = (i1 >> 3) != (i2 >> 3)
        fix[0].start()

        @pl.when(differ)
        def _():
            fix[1].start()
            fix[1].wait()

        fix[0].wait()

    main()


@jax.jit
def pallas_adaLN_cond__memory_aug_recurrent_mem_tr__moe_arch_mod__prompt_kernel(
    A_x: jax.Array,
    A_mem0: jax.Array,
    A_Wq: jax.Array,
    A_Wk: jax.Array,
    A_Wv: jax.Array,
    A_Wo: jax.Array,
    A_seg_len: jax.Array,
    B_x: jax.Array,
    B_w_r: jax.Array,
    B_w_gate: jax.Array,
    B_w_up: jax.Array,
    B_w_down: jax.Array,
    c: jax.Array,
    w_mod: jax.Array,
):
    del A_seg_len, B_x
    assert A_x.shape == (1, S, D) and A_mem0.shape == (1, M, D) and A_Wq.shape == (D, H, E)
    hbm = pl.BlockSpec(memory_space=pl.ANY)
    out = pl.pallas_call(
        _kernel,
        out_shape=jax.ShapeDtypeStruct((NSEG, SEG, D), BF16),
        in_specs=[hbm] * 12,
        out_specs=hbm,
        scratch_shapes=[
            pltpu.VMEM((NSEG, SEG, D), BF16),
            pltpu.VMEM((3 * H, DB, 128, E), BF16),
            pltpu.VMEM((DB, H * E // 2, 128), U32),
            pltpu.VMEM((NGP, NIT, UNR * 2 * M, E), BF16),
            pltpu.VMEM((DB, SEG, 128), BF16),
            pltpu.VMEM((NGP, 2 * SEG, E), BF16),
            pltpu.VMEM((H, 2 * SEG, E), BF16),
            pltpu.VMEM((DB, 2 * SEG, 128), F32),
            pltpu.VMEM((7, 8, D), F32),
            pltpu.VMEM((NGP, D, E), U32),
            pltpu.VMEM((6, DB, D // 2, 128), U32),
            pltpu.VMEM((DB, NSEG * M, E), BF16),
            pltpu.VMEM((DB, NSEG * M + SEG, 128), F32),
            pltpu.VMEM((2 * KMAJ, NSEG * M, E), F32),
            pltpu.VMEM((DB, 16, 128), BF16),
            pltpu.VMEM((D, 128), F32),
            pltpu.VMEM((NSEG, SEG, D), BF16),
            pltpu.VMEM((NSEG, SEG, D), BF16),
            pltpu.VMEM((NSEG, SEG, D), BF16),
            pltpu.VMEM((M, D), BF16),
            pltpu.VMEM((8, S // 8), F32),
            pltpu.VMEM((PR, PR), F32),
            pltpu.VMEM((8, 128), F32),
            pltpu.VMEM((1, D), BF16),
            pltpu.VMEM((D,), BF16),
            pltpu.SemaphoreType.DMA((NSEM,)),
        ],
        compiler_params=pltpu.CompilerParams(
            vmem_limit_bytes=120 * 1024 * 1024, disable_bounds_checks=True,
            disable_semaphore_checks=True),
    )(
        A_x.reshape(NSEG, SEG, D),
        A_mem0.reshape(M, D),
        A_Wq, A_Wk, A_Wv,
        A_Wo.reshape(H * E, D),
        B_w_r,
        B_w_gate, B_w_up, B_w_down,
        c, w_mod,
    )
    return out.reshape(1, S, D)
```

```python
import jax
import jax.numpy as jnp
from jax import lax
import jax.experimental.pallas as pl
import jax.experimental.pallas.tpu as pltpu

BF16 = jnp.bfloat16
F32 = jnp.float32
U32 = jnp.uint32

S = 2048
D = 1024
H = 32
E = 128
M = 8
SEG = 32
NSEG = S // SEG
NPAIR = H // 2
NGP = 3 * NPAIR
F = 3584
DB = D // 128
FB = F // 128
PR = 2 * SEG + 2 * M
UNR = 4
NIT = NSEG // UNR
KMAJ = 12
AHEAD = 3
PPI = 6
NSPLIT = 3
KEARLY = 5
HA = 24
SIDE_SLOTS = [("softmax", 8), (0, 2), (0, 5), (0, 7)]
EPS = 1e-5
SCALE = E ** (-0.5)

SEM_SMALL = 0
SEM_X = SEM_SMALL + 3
SEM_MOD = SEM_X + 2
SEM_MOD2 = SEM_MOD + DB
SEM_WQ = SEM_MOD2 + 4
SEM_ST = SEM_WQ + DB
SEM_WO = SEM_ST + (NGP - KMAJ) // PPI
SEM_MOE = SEM_WO + 1
SEM_OUT = SEM_MOE + 2
NSEM = SEM_OUT + 3


def _rb(v):
    return v.astype(BF16).astype(F32)


def _dot(a, b):
    return jnp.dot(a, b, preferred_element_type=F32)


def _recip(x):
    r = pl.reciprocal(x, approx=True)
    return r * (2.0 - x * r)


def _bf(words):
    return pltpu.bitcast(words, BF16)


def _ln(x):
    m = jnp.mean(x, axis=-1, keepdims=True)
    mb = _rb(m)
    d = x - mb
    var = jnp.mean(d * d, axis=-1, keepdims=True) - (m - mb) * (m - mb)
    inv = _recip(_rb(jnp.sqrt(_rb(_rb(jnp.maximum(var, 0.0)) + EPS))))
    return d * inv, inv


def _fill_matrix():
    i = lax.broadcasted_iota(jnp.int32, (PR, PR), 0)
    j = lax.broadcasted_iota(jnp.int32, (PR, PR), 1)

    def head(t):
        return jnp.where(t < 2 * SEG, t >> 5, (t - 2 * SEG) >> 3)

    def pos(t):
        r = t & (SEG - 1)
        return jnp.where(t < 2 * SEG, jnp.where(r < M, r, r + M), M + (t & (M - 1)))

    same = head(i) == head(j)
    pi = pos(i)
    ok = jnp.where(pi < M, 1, jnp.where(pi >= pos(j), 1, 0))
    return jnp.where(same, jnp.where(ok == 1, 0.0, -1e9), -3e38).astype(F32)


def _kernel(x_hbm, mem0_hbm, wq_hbm, wk_hbm, wv_hbm, wo_hbm, wr_hbm, wg_hbm, wu_hbm, wd_hbm,
            c_hbm, wmod_hbm, out_hbm,
            x_v, w_v, wo_v, cache, lhs_v, qkv_s, o_s, acc_s, mod_v, ab_v,
            stage, wmod_v, hc, n_v, acc, sc_row, sc_col, x1_v, h2_v, out_v,
            mem0_v, r_v, fill_v, never_v, c_v, wr_v, sems):
    w_w = w_v.bitcast(U32)
    cache_w = cache.bitcast(U32)
    lhs_w = lhs_v.bitcast(U32)
    qkv_w = qkv_s.bitcast(U32)
    o_w = o_s.bitcast(U32)

    def weights(h, j0=0, j1=DB):
        return _bf(w_w[h, pl.ds(j0, j1 - j0)].reshape((j1 - j0) * 64, E))

    def tie(v, tok):
        if tok is None:
            return v
        tok = jnp.broadcast_to(tok, (8, 128))
        if v.dtype != F32:
            tok = pltpu.bitcast(tok, v.dtype)
        return jnp.concatenate([jnp.where(never_v[...] > 1.0, tok, v[0:8]), v[8:]], axis=0)

    def copy(src, dst, sem):
        return pltpu.make_async_copy(src, dst, sems.at[sem])

    def wait_all(buf, sem):
        copy(buf, buf, sem).wait()

    def mod_row(k, rows=8):
        v = mod_v[k]
        return v if rows == 8 else jnp.concatenate([v] * (rows // 8), axis=0)

    def put_rows(dst, r0, v):
        for j in range(DB):
            dst[j, pl.ds(r0, v.shape[0]), :] = v[:, j * 128:(j + 1) * 128].astype(BF16)

    def prologue():
        wmod_w = wmod_hbm.bitcast(U32)
        w_words = [w.bitcast(U32) for w in (wq_hbm, wk_hbm, wv_hbm)]

        def start_mod(j):
            col = j * 128 if isinstance(j, int) else pl.multiple_of(j * 128, 128)
            for k in range(2):
                copy(wmod_w.at[:, pl.ds(k * D + col, 128)], wmod_v.at[k, j], SEM_MOD + j).start()

        def wait_mod(j):
            wait_all(wmod_v.at[pl.ds(0, 2), j], SEM_MOD + j)

        def start_chunk(k):
            col = k * D if isinstance(k, int) else pl.multiple_of(k * D, D)
            for j in range(DB):
                copy(wmod_w.at[:, pl.ds(col + j * 128, 128)], wmod_v.at[k, j], SEM_MOD2 + k - 2).start()

        def start_ktile(j):
            rows = pl.ds(j * 128 if isinstance(j, int) else pl.multiple_of(j * 128, 128), 128)
            for g in range(KMAJ):
                copy(w_words[0].at[rows, g, :], stage.at[g, rows, :], SEM_WQ + j).start()

        small = [copy(c_hbm, c_v, SEM_SMALL), copy(mem0_hbm, mem0_v, SEM_SMALL + 1),
                 copy(wr_hbm, wr_v, SEM_SMALL + 2)]
        x_head = copy(x_hbm.at[:, pl.ds(0, M), :], x_v.at[:, pl.ds(0, M), :], SEM_X)
        x_tail = copy(x_hbm.at[:, pl.ds(M, SEG - M), :], x_v.at[:, pl.ds(M, SEG - M), :], SEM_X + 1)
        for cp in small:
            cp.start()
        x_head.start()
        start_mod(0)
        for j in range(AHEAD):
            start_ktile(j)
            start_mod(j + 1)
        slab_cps = [copy(w_words[g // NPAIR].at[:, g % NPAIR, :], stage.at[g], SEM_ST + (g - KMAJ) // PPI)
                    for g in range(KMAJ, NGP)]

        fill_v[...] = _fill_matrix()
        x1_v[0] = jnp.zeros((SEG, D), BF16)
        r_v[...] = jnp.full(r_v.shape, -jnp.inf, F32)
        never_v[...] = jnp.zeros(never_v.shape, F32)
        qkv_s[0] = jnp.zeros((2 * SEG, E), BF16)
        o_s[0] = jnp.zeros(o_s.shape[1:], BF16)
        acc_s[0] = jnp.zeros(acc_s.shape[1:], F32)

        def zero_acc(h, carry):
            acc[h] = jnp.zeros((NSEG * M, E), F32)
            return carry

        lax.fori_loop(0, 2 * KMAJ, zero_acc, 0)

        for cp in small:
            cp.wait()
        c = c_v[...].astype(F32)
        sc = _rb(c * jax.nn.sigmoid(c))
        put_rows(sc_row, 0, jnp.broadcast_to(sc, (16, D)))
        for j in range(DB):
            sc_col[pl.ds(j * 128, 128), :] = jnp.broadcast_to(sc[:, j * 128:(j + 1) * 128], (128, 128)).T
        mod_v[6] = jnp.broadcast_to(wr_v[...].astype(F32).reshape(1, D), (8, D))
        put_rows(lhs_v.at[0], 0, mem0_v[...].astype(F32))

        x_head.wait()
        NB = 16
        RB = NSEG * M // NB
        for b in range(NB):
            xb = x_v[pl.ds(b * (NSEG // NB), NSEG // NB), pl.ds(0, M), :].astype(F32).reshape(RB, D)
            nb = _ln(xb)[0]
            for j in range(DB):
                n_v[j, pl.ds(b * RB, RB), :] = nb[:, j * 128:(j + 1) * 128]

        hc_w = hc.bitcast(U32)
        sc_w = sc_row.bitcast(U32)

        def mod_block(j, k, src=None):
            scb = jnp.concatenate([_bf(sc_w[i]) for i in range(DB)], axis=1)
            v = _rb(_dot(scb, _bf(wmod_v[k, j if src is None else src]))[0:8])
            if k == 1:
                v = _rb(1.0 + v)
            col = j * 128 if isinstance(j, int) else pl.multiple_of(j * 128, 128)
            ab_v[k, :, pl.ds(col, 128)] = v
            return v

        def h_block(j, ca, sa):
            n = n_v[j].reshape(NSEG, M, 128)
            hc[j] = (n * ca[None] + sa[None]).reshape(NSEG * M, 128).astype(BF16)

        def pack_pair(r1, r2):
            r = jnp.concatenate([r1.reshape(NSEG, M, E), r2.reshape(NSEG, M, E)], axis=1)
            return r.reshape(NIT, UNR * 2 * M, E).astype(BF16)

        def split_pair(b):
            return (pltpu.bitcast(b << 16, F32).astype(BF16),
                    pltpu.bitcast(b & jnp.uint32(0xFFFF0000), F32).astype(BF16))

        def q_stage(j, last, more_dmas):
            static = isinstance(j, int)
            k0 = j * 128 if static else pl.multiple_of(j * 128, 128)
            src = None if last else jnp.where(j == 0, 0, j + 1)
            for p in range(KMAJ):
                ws = split_pair(stage[p, pl.ds(k0, 128), :])
                rs = []
                for t in range(2):
                    h = 2 * p + t
                    w_v[h, j] = ws[t]
                    rs.append(_dot(_bf(hc_w[j]), _bf(w_w[h, j])) + acc[h])
                    if not last:
                        acc[h] = rs[t]
                if last:
                    cache[p] = pack_pair(*rs)
                elif p == 1:
                    ca = mod_block(j + 1, 1, src)
                elif p == 3:
                    h_block(j + 1, ca, mod_block(j + 1, 0, src))
                if p == 1:
                    more_dmas()

        wait_mod(0)
        h_block(0, mod_block(0, 1), mod_block(0, 0))

        def wait_ktile(j):
            rows = pl.ds(j * 128 if isinstance(j, int) else pl.multiple_of(j * 128, 128), 128)
            wait_all(stage.at[pl.ds(0, KMAJ), rows, :], SEM_WQ + j)

        def q_body(j, carry):
            @pl.when(j == 1)
            def _():
                wait_mod(1)
                h_block(1, mod_block(1, 1), mod_block(1, 0))

            wait_ktile(j)

            @pl.when(j > 0)
            def _():
                wait_mod(j + 1)

            def more_dmas():
                @pl.when(j + AHEAD < DB)
                def _():
                    start_ktile(j + AHEAD)

                @pl.when(j + AHEAD + 1 < DB)
                def _():
                    start_mod(j + AHEAD + 1)

                @pl.when(j + AHEAD == DB)
                def _():
                    for cp in slab_cps[:2 * PPI]:
                        cp.start()

            q_stage(j, False, more_dmas)
            return carry

        lax.fori_loop(0, DB - 1, q_body, 0)
        wait_ktile(DB - 1)

        def last_dmas():
            for i in range(2, 5):
                for cp in slab_cps[i * PPI:(i + 1) * PPI]:
                    cp.start()
                if i < 4:
                    start_chunk(i)
                if i == 2:
                    x_tail.start()

        q_stage(DB - 1, True, last_dmas)

        def pro_body(i, carry):
            g0 = KMAJ + i * PPI
            wait_all(stage.at[pl.ds(g0, PPI)], SEM_ST + i)

            @pl.when(i >= 2)
            def _():
                wait_all(wmod_v.at[i], SEM_MOD2 + i - 2)

            @pl.when(i == 2)
            def _():
                x_tail.wait()

            def more_dmas():
                @pl.when(i < 2)
                def _():
                    start_chunk(i + 4)

                @pl.when(i == 0)
                def _():
                    for cp in slab_cps[5 * PPI:]:
                        cp.start()

                @pl.when(jnp.logical_and(i >= 2, i < 4))
                def _():
                    wo_w = wo_hbm.bitcast(U32)
                    for t in range(DB // 2):
                        j = (i - 2) * (DB // 2) + t
                        cols = pl.ds(pl.multiple_of(j * 128, 128), 128)
                        copy(wo_w.at[:, cols], wo_v.at[j], SEM_WO).start()

            one = jnp.where(jnp.logical_or(i == 1, i == 4), 1.0, 0.0)

            def mod_cols(j):
                v = jnp.sum(_bf(wmod_v[i, j]).astype(F32) * sc_col[...], axis=0, keepdims=True)
                v = _rb(one + _rb(jnp.broadcast_to(v, (8, 128))))
                mod_v[i, :, pl.ds(j * 128, 128)] = v
                return v

            def ln_rows(n):
                seg = jnp.maximum(i - 2, 0) * (NSEG // 4) + n // 3
                r0 = (n % 3 + 1) * 8
                src = pl.multiple_of(jnp.where(i >= 2, r0, 0), 8)
                nrm, inv = _ln(x_v[seg, pl.ds(src, 8), :].astype(F32))
                put_rows(lhs_v.at[seg], r0, nrm * ab_v[1] + ab_v[0])
                return inv

            LPD = 3 * (NSEG // 4) // (2 * PPI)
            for t in range(PPI):
                gp = g0 + t
                w_v[2 * gp], w_v[2 * gp + 1] = split_pair(stage[gp].reshape(DB, 128, E))
                rs = []
                for hh in range(2):
                    n = 2 * t + hh - (2 * PPI - DB)
                    parts = [hc_w[j] for j in range(DB)]
                    parts[0] = tie(parts[0], mod_cols(n) if n >= 0 else None)
                    parts[-1] = tie(parts[-1], sum(ln_rows((2 * t + hh) * LPD + k) for k in range(LPD)))
                    hcv = jnp.concatenate([_bf(w) for w in parts], axis=1)
                    rs.append(_dot(hcv, weights(2 * gp + hh)))
                cache[gp] = pack_pair(*rs)
                if t == 0:
                    more_dmas()
            return carry

        lax.fori_loop(0, (NGP - KMAJ) // PPI, pro_body, 0)

    prologue()

    def main():
        lane = lax.broadcasted_iota(jnp.int32, (8, 2 * 128), 1)

        def post(seg, q, keep=True):
            rows = pl.ds(8 * q, 8)
            x1 = x1_v[seg, rows, :].astype(F32)
            n, inv = _ln(x1)
            h2 = _rb(n * mod_row(4) + mod_row(3))
            r = _rb(jnp.sum(h2 * mod_row(6), axis=-1, keepdims=True))
            if keep:
                r_v[...] = jnp.where(lane == seg * 4 + q, r, r_v[...])
            h2_v[seg, rows, :] = h2.astype(BF16)
            out_v[seg, rows, :] = (x1 + mod_row(5) * h2).astype(BF16)
            return inv, r

        def out_copy(grp):
            return copy(out_v.at[pl.ds(grp * UNR, UNR)], out_hbm.at[pl.ds(grp * UNR, UNR)], SEM_OUT)

        wg_w, wu_w, wd_w = wg_hbm.bitcast(U32), wu_hbm.bitcast(U32), wd_hbm.bitcast(U32)
        wait_all(wo_v, SEM_WO)

        def step(it, u):
            s = it * UNR + u
            lhs = jnp.concatenate([_bf(lhs_w[s, j]) for j in range(DB)], axis=1)

            def side(slot):
                if slot not in SIDE_SLOTS:
                    return None
                q = SIDE_SLOTS.index(slot)
                return post(jnp.maximum(s - (2 if q == 0 else 1), 0), q)[0]

            def proj(m_i, p):
                g = m_i * NPAIR + p
                for t in range(2):
                    qkv_s[g, pl.ds(t * SEG, SEG), :] = _dot(lhs, weights(2 * g + t)).astype(BF16)

            def rows_of(m_i, p):
                g = m_i * NPAIR + p
                return jnp.concatenate([_bf(qkv_w[g]), _bf(cache_w[g, it, pl.ds(u * M, M), :])], axis=0)

            def probs(p):
                parts = [lax.dot_general(_bf(qkv_w[p]), rows_of(1, p), (((1,), (1,)), ((), ())),
                                         preferred_element_type=F32)]
                qc = _bf(cache_w[p, it, pl.ds(u * M, M), :]).astype(F32)
                kc = _bf(cache_w[NPAIR + p, it, pl.ds(u * M, M), :]).astype(F32)
                col = lax.broadcasted_iota(jnp.int32, (M, PR), 1)
                for t in range(2):
                    km = _bf(qkv_w[NPAIR + p, pl.ds(t * (SEG // 2), 8), :]).astype(F32)
                    qt = qc[t * M:(t + 1) * M]
                    st = jnp.zeros((M, PR), F32)
                    for j in range(M):
                        st = jnp.where(col == t * SEG + j,
                                       jnp.sum(qt * km[j:j + 1], axis=-1, keepdims=True), st)
                        st = jnp.where(col == 2 * SEG + t * M + j,
                                       jnp.sum(qt * kc[t * M + j:t * M + j + 1], axis=-1, keepdims=True), st)
                    parts.append(st)
                sc = jnp.concatenate(parts, axis=0) * SCALE
                fm = fill_v[...]
                tok = side(("softmax", p))
                if tok is not None:
                    top = fm[0:8]
                    fm = jnp.concatenate([jnp.where(top > 1.0, tok, top), fm[8:]], axis=0)
                sc = jnp.where(fm == 0.0, sc, fm)
                e = jnp.exp(sc - jnp.max(sc, axis=-1, keepdims=True))
                return (e * _recip(jnp.sum(e, axis=-1, keepdims=True))).astype(BF16)

            def attend(p, pr):
                o = _dot(pr, rows_of(2, p))
                for t in range(2):
                    o_s[2 * p + t, pl.ds(0, SEG), :] = o[t * SEG:(t + 1) * SEG].astype(BF16)
                for t in range(2):
                    o_s[2 * p + t, pl.ds(SEG + (u % 2) * M, M), :] = (
                        o[2 * SEG + t * M:2 * SEG + (t + 1) * M].astype(BF16))

            ps = {}
            for pa in range(0, NPAIR, 2):
                pb = pa + 1
                todo = [(0, pa), (1, pa), (0, pb), (1, pb), (2, pa), (2, pb)]
                if pa == 0 and u > 0:
                    hs = [(m_i * NPAIR + p, t) for m_i, p in todo[:NSPLIT] for t in range(2)]
                    ke = KEARLY * 128
                    first = [_dot(lhs[:, :ke], weights(2 * g + t, 0, KEARLY)) for g, t in hs]
                    for (g, t), part in zip(hs, first):
                        res = _dot(lhs[:, ke:], weights(2 * g + t, KEARLY, DB)) + part
                        qkv_s[g, pl.ds(t * SEG, SEG), :] = res.astype(BF16)
                    todo = todo[NSPLIT:]
                for m_i, p in todo:
                    proj(m_i, p)
                for kind in ("scores", "values") if pa % 4 == 0 else ("values", "scores"):
                    for p in (pa, pb):
                        if kind == "scores":
                            ps[p] = probs(p)
                        elif p >= 2:
                            attend(p - 2, ps.pop(p - 2))
            L = NPAIR - 1

            nxt = s + 1 if u < UNR - 1 else jnp.where(it < NIT - 1, s + 1, 0)
            nr = SEG + (2 * M if u % 2 else 0)
            for h0, h1 in ((0, HA), (HA, H)):
                for j in range(DB):
                    words = [o_w[h, pl.ds(0, nr // 2), :] for h in range(h0, h1)]
                    words[0] = tie(words[0], side((h0, j)))
                    ol = jnp.concatenate([_bf(w) for w in words], axis=1)
                    part = _dot(ol, _bf(wo_v[j, pl.ds(h0 * E // 2, (h1 - h0) * E // 2), :]))
                    if h0 == 0:
                        acc_s[j, pl.ds(0, nr), :] = part
                    else:
                        a = part + acc_s[j, pl.ds(0, nr), :]
                        cols = pl.ds(j * 128, 128)
                        lhs_v[nxt, j, pl.ds(0, M), :] = a[0:M].astype(BF16)
                        for q in range(1, nr // M):
                            seg, rows = (s, pl.ds(q * M, M)) if q < 4 else (s + q - 5, pl.ds(0, M))
                            x1 = x_v[seg, rows, cols].astype(F32) + mod_v[2, :, cols] * a[q * M:(q + 1) * M]
                            x1_v[seg, rows, cols] = x1.astype(BF16)
                    if h0 == 0 and j == 4:
                        attend(L - 1, ps.pop(L - 1))
                        attend(L, ps.pop(L))

        def iteration(it, carry):
            @pl.when(it >= 2)
            def _():
                out_copy(it - 2).start()

            @pl.when(it < FB // 2)
            def _():
                for t in range(2):
                    j = 2 * it + t
                    cols = pl.ds(pl.multiple_of(j * 128, 128), 128)
                    half = pl.ds(t * (D // 2), D // 2)
                    copy(wg_w.at[:, cols], stage.at[it, half, :], SEM_MOE).start()
                    copy(wu_w.at[:, cols], stage.at[FB // 2 + it, half, :], SEM_MOE).start()

            @pl.when(it < DB)
            def _():
                cols = pl.ds(pl.multiple_of(it * 128, 128), 128)
                for t in range(2):
                    copy(wd_w.at[pl.ds(t * (F // 4), F // 4), cols],
                         stage.at[FB + 2 * it + t, pl.ds(0, F // 4), :], SEM_MOE + 1).start()

            for u in range(UNR):
                step(it, u)
            return carry

        lax.fori_loop(0, NIT, iteration, 0)

        out_copy(NIT - 2).start()
        wait_all(stage.at[pl.ds(0, FB)], SEM_MOE)
        wait_all(stage.at[pl.ds(FB, 2 * DB), pl.ds(0, F // 4), :], SEM_MOE + 1)
        r8 = lax.broadcasted_iota(jnp.int32, (8, 1), 0)

        def top2(vals, idx, axes):
            def red(f, v):
                for ax in axes:
                    v = f(v, axis=ax, keepdims=True)
                return v
            m1 = red(jnp.max, vals)
            i1 = red(jnp.min, jnp.where(vals == m1, idx, S - 1.0))
            rest = jnp.where(idx == i1, -jnp.inf, vals)
            m2 = red(jnp.max, rest)
            i2 = red(jnp.min, jnp.where(rest == m2, jnp.where(idx == i1, S - 1.0, idx), S - 1.0))
            return m1, i1, m2, i2

        m1, i1v, m2, i2v = top2(r_v[...], (lane * 8 + r8).astype(F32), (1, 0))
        vals = [jnp.where(r8 == 0, m1, jnp.where(r8 == 1, m2, -jnp.inf))]
        idxs = [jnp.where(r8 == 0, i1v, jnp.where(r8 == 1, i2v, S - 1.0))]
        for seg, q in [(NSEG - 2, 0)] + [(NSEG - 1, q) for q in range(4)]:
            vals.append(post(seg, q, keep=False)[1])
            idxs.append((r8 + (seg * SEG + q * 8)).astype(F32))
        out_copy(NIT - 1).start()
        m1, i1v, m2, i2v = top2(jnp.concatenate(vals, axis=0), jnp.concatenate(idxs, axis=0), (0,))
        i1 = i1v.astype(jnp.int32)[0, 0]
        i2 = i2v.astype(jnp.int32)[0, 0]

        def tile_of(i):
            return i >> 5, pl.multiple_of(((i >> 3) & 3) * 8, 8)

        sel = [tile_of(i1), tile_of(i2)]
        x1s = jnp.concatenate([x1_v[sg, pl.ds(r0, 8), :].astype(F32) for sg, r0 in sel], axis=0)
        h2s = jnp.concatenate([h2_v[sg, pl.ds(r0, 8), :].astype(F32) for sg, r0 in sel], axis=0)
        h2b = h2s.astype(BF16)
        gus = []
        for j in range(FB):
            half = pl.ds((j % 2) * (D // 2), D // 2)
            g = _rb(_dot(h2b, _bf(stage[j // 2, half, :])))
            g = _rb(g * jax.nn.sigmoid(g))
            u = _rb(_dot(h2b, _bf(stage[FB // 2 + j // 2, half, :])))
            gus.append(g * u)
        gu = jnp.concatenate(gus, axis=1).astype(BF16)
        ys = []
        for j in range(DB):
            wd = stage[pl.ds(FB + 2 * j, 2), pl.ds(0, F // 4), :].reshape(F // 2, 128)
            ys.append(_rb(_dot(gu, _bf(wd))))
        y = jnp.concatenate(ys, axis=1)
        rows = lax.broadcasted_iota(jnp.int32, (16, 1), 0)
        rs = _rb(jax.nn.sigmoid(jnp.where(rows < 8, m1, m2)))
        y = _rb(y * rs)
        full = x1s + mod_row(5, 16) * _rb(h2s + y)

        copy(out_v, out_hbm, SEM_OUT).wait()
        for t, (i, (sg, r0)) in enumerate(zip((i1, i2), sel)):
            old = out_v[sg, pl.ds(r0, 8), :].astype(F32)
            new = jnp.where(r8 == (i & 7), full[t * 8:(t + 1) * 8], old)
            out_v[sg, pl.ds(r0, 8), :] = new.astype(BF16)
        fix = [copy(out_v.at[sg, pl.ds(r0, 8), :], out_hbm.at[sg, pl.ds(r0, 8), :], SEM_OUT + 1 + t)
               for t, (sg, r0) in enumerate(sel)]
        differ = (i1 >> 3) != (i2 >> 3)
        fix[0].start()

        @pl.when(differ)
        def _():
            fix[1].start()
            fix[1].wait()

        fix[0].wait()

    main()


@jax.jit
def pallas_adaLN_cond__memory_aug_recurrent_mem_tr__moe_arch_mod__prompt_kernel(
    A_x: jax.Array,
    A_mem0: jax.Array,
    A_Wq: jax.Array,
    A_Wk: jax.Array,
    A_Wv: jax.Array,
    A_Wo: jax.Array,
    A_seg_len: jax.Array,
    B_x: jax.Array,
    B_w_r: jax.Array,
    B_w_gate: jax.Array,
    B_w_up: jax.Array,
    B_w_down: jax.Array,
    c: jax.Array,
    w_mod: jax.Array,
):
    del A_seg_len, B_x
    assert A_x.shape == (1, S, D) and A_mem0.shape == (1, M, D) and A_Wq.shape == (D, H, E)
    hbm = pl.BlockSpec(memory_space=pl.ANY)
    out = pl.pallas_call(
        _kernel,
        out_shape=jax.ShapeDtypeStruct((NSEG, SEG, D), BF16),
        in_specs=[hbm] * 12,
        out_specs=hbm,
        scratch_shapes=[
            pltpu.VMEM((NSEG, SEG, D), BF16),
            pltpu.VMEM((3 * H, DB, 128, E), BF16),
            pltpu.VMEM((DB, H * E // 2, 128), U32),
            pltpu.VMEM((NGP, NIT, UNR * 2 * M, E), BF16),
            pltpu.VMEM((NSEG, DB, SEG, 128), BF16),
            pltpu.VMEM((NGP, 2 * SEG, E), BF16),
            pltpu.VMEM((H, 2 * SEG, E), BF16),
            pltpu.VMEM((DB, 2 * SEG, 128), F32),
            pltpu.VMEM((7, 8, D), F32),
            pltpu.VMEM((2, 8, D), F32),
            pltpu.VMEM((NGP, D, E), U32),
            pltpu.VMEM((6, DB, D // 2, 128), U32),
            pltpu.VMEM((DB, NSEG * M, E), BF16),
            pltpu.VMEM((DB, NSEG * M, 128), F32),
            pltpu.VMEM((2 * KMAJ, NSEG * M, E), F32),
            pltpu.VMEM((DB, 16, 128), BF16),
            pltpu.VMEM((D, 128), F32),
            pltpu.VMEM((NSEG, SEG, D), BF16),
            pltpu.VMEM((NSEG, SEG, D), BF16),
            pltpu.VMEM((NSEG, SEG, D), BF16),
            pltpu.VMEM((M, D), BF16),
            pltpu.VMEM((8, S // 8), F32),
            pltpu.VMEM((PR, PR), F32),
            pltpu.VMEM((8, 128), F32),
            pltpu.VMEM((1, D), BF16),
            pltpu.VMEM((D,), BF16),
            pltpu.SemaphoreType.DMA((NSEM,)),
        ],
        compiler_params=pltpu.CompilerParams(
            vmem_limit_bytes=120 * 1024 * 1024, disable_bounds_checks=True,
            disable_semaphore_checks=True),
    )(
        A_x.reshape(NSEG, SEG, D),
        A_mem0.reshape(M, D),
        A_Wq, A_Wk, A_Wv,
        A_Wo.reshape(H * E, D),
        B_w_r,
        B_w_gate, B_w_up, B_w_down,
        c, w_mod,
    )
    return out.reshape(1, S, D)
```

```python
import jax
import jax.numpy as jnp
from jax import lax
import jax.experimental.pallas as pl
import jax.experimental.pallas.tpu as pltpu

BF16 = jnp.bfloat16
F32 = jnp.float32
U32 = jnp.uint32

S = 2048
D = 1024
H = 32
E = 128
M = 8
SEG = 32
NSEG = S // SEG
NPAIR = H // 2
NGP = 3 * NPAIR
F = 3584
DB = D // 128
FB = F // 128
PR = 2 * SEG + 2 * M
UNR = 4
NIT = NSEG // UNR
KMAJ = 12
AHEAD = 3
PPI = 6
NSPLIT = 3
KEARLY = 5
HA = 24
SIDE_SLOTS = [("softmax", 8), (0, 2), (0, 5), (0, 7)]
H_SLOTS = (6, 8)
EPS = 1e-5
SCALE = E ** (-0.5)

SEM_SMALL = 0
SEM_X = SEM_SMALL + 3
SEM_MOD = SEM_X + 2
SEM_MOD2 = SEM_MOD + DB
SEM_WQ = SEM_MOD2 + 4
SEM_ST = SEM_WQ + DB
SEM_WO = SEM_ST + (NGP - KMAJ) // PPI
SEM_MOE = SEM_WO + 1
SEM_OUT = SEM_MOE + 2
NSEM = SEM_OUT + 3


def _rb(v):
    return v.astype(BF16).astype(F32)


def _dot(a, b):
    return jnp.dot(a, b, preferred_element_type=F32)


def _recip(x):
    r = pl.reciprocal(x, approx=True)
    return r * (2.0 - x * r)


def _bf(words):
    return pltpu.bitcast(words, BF16)


def _ln(x):
    m = jnp.mean(x, axis=-1, keepdims=True)
    mb = _rb(m)
    d = x - mb
    var = jnp.mean(d * d, axis=-1, keepdims=True) - (m - mb) * (m - mb)
    inv = _recip(_rb(jnp.sqrt(_rb(_rb(jnp.maximum(var, 0.0)) + EPS))))
    return d * inv, inv


def _fill_matrix():
    i = lax.broadcasted_iota(jnp.int32, (PR, PR), 0)
    j = lax.broadcasted_iota(jnp.int32, (PR, PR), 1)

    def head(t):
        return jnp.where(t < 2 * SEG, t >> 5, (t - 2 * SEG) >> 3)

    def pos(t):
        r = t & (SEG - 1)
        return jnp.where(t < 2 * SEG, jnp.where(r < M, r, r + M), M + (t & (M - 1)))

    same = head(i) == head(j)
    pi = pos(i)
    ok = jnp.where(pi < M, 1, jnp.where(pi >= pos(j), 1, 0))
    return jnp.where(same, jnp.where(ok == 1, 0.0, -1e9), -3e38).astype(F32)


def _kernel(x_hbm, mem0_hbm, wq_hbm, wk_hbm, wv_hbm, wo_hbm, wr_hbm, wg_hbm, wu_hbm, wd_hbm,
            c_hbm, wmod_hbm, out_hbm,
            x_v, w_v, wo_v, cache, lhs_v, qkv_s, o_s, acc_s, mod_v, ab_v,
            stage, wmod_v, hc, n_v, acc, sc_row, sc_col, x1_v, h2_v, out_v,
            mem0_v, r_v, fill_v, never_v, c_v, wr_v, sems):
    w_w = w_v.bitcast(U32)
    cache_w = cache.bitcast(U32)
    lhs_w = lhs_v.bitcast(U32)
    qkv_w = qkv_s.bitcast(U32)
    o_w = o_s.bitcast(U32)

    def weights(h, j0=0, j1=DB):
        return _bf(w_w[h, pl.ds(j0, j1 - j0)].reshape((j1 - j0) * 64, E))

    def tie(v, tok, r0=0):
        if tok is None:
            return v
        tok = jnp.broadcast_to(tok, (8, 128))
        if v.dtype != F32:
            tok = pltpu.bitcast(tok, v.dtype)
        parts = [v[:r0], jnp.where(never_v[...] > 1.0, tok, v[r0:r0 + 8]), v[r0 + 8:]]
        return jnp.concatenate([x for x in parts if x.shape[0]], axis=0)

    def copy(src, dst, sem):
        return pltpu.make_async_copy(src, dst, sems.at[sem])

    def wait_all(buf, sem):
        copy(buf, buf, sem).wait()

    def mod_row(k, rows=8):
        v = mod_v[k]
        return v if rows == 8 else jnp.concatenate([v] * (rows // 8), axis=0)

    def put_rows(dst, r0, v):
        for j in range(DB):
            dst[j, pl.ds(r0, v.shape[0]), :] = v[:, j * 128:(j + 1) * 128].astype(BF16)

    def prologue():
        wmod_w = wmod_hbm.bitcast(U32)
        w_words = [w.bitcast(U32) for w in (wq_hbm, wk_hbm, wv_hbm)]

        def start_mod(j):
            col = j * 128 if isinstance(j, int) else pl.multiple_of(j * 128, 128)
            for k in range(2):
                copy(wmod_w.at[:, pl.ds(k * D + col, 128)], wmod_v.at[k, j], SEM_MOD + j).start()

        def wait_mod(j):
            wait_all(wmod_v.at[pl.ds(0, 2), j], SEM_MOD + j)

        def start_chunk(k):
            col = k * D if isinstance(k, int) else pl.multiple_of(k * D, D)
            for j in range(DB):
                copy(wmod_w.at[:, pl.ds(col + j * 128, 128)], wmod_v.at[k, j], SEM_MOD2 + k - 2).start()

        def start_ktile(j):
            rows = pl.ds(j * 128 if isinstance(j, int) else pl.multiple_of(j * 128, 128), 128)
            for g in range(KMAJ):
                copy(w_words[0].at[rows, g, :], stage.at[g, rows, :], SEM_WQ + j).start()

        small = [copy(c_hbm, c_v, SEM_SMALL), copy(mem0_hbm, mem0_v, SEM_SMALL + 1),
                 copy(wr_hbm, wr_v, SEM_SMALL + 2)]
        x_head = copy(x_hbm.at[:, pl.ds(0, M), :], x_v.at[:, pl.ds(0, M), :], SEM_X)
        x_tail = copy(x_hbm.at[:, pl.ds(M, SEG - M), :], x_v.at[:, pl.ds(M, SEG - M), :], SEM_X + 1)
        for cp in small:
            cp.start()
        x_head.start()
        start_mod(0)
        for j in range(AHEAD):
            start_ktile(j)
            start_mod(j + 1)
        slab_cps = [copy(w_words[g // NPAIR].at[:, g % NPAIR, :], stage.at[g], SEM_ST + (g - KMAJ) // PPI)
                    for g in range(KMAJ, NGP)]

        fill_v[...] = _fill_matrix()
        x1_v[0] = jnp.zeros((SEG, D), BF16)
        r_v[...] = jnp.full(r_v.shape, -jnp.inf, F32)
        never_v[...] = jnp.zeros(never_v.shape, F32)
        qkv_s[0] = jnp.zeros((2 * SEG, E), BF16)
        o_s[0] = jnp.zeros(o_s.shape[1:], BF16)
        acc_s[0] = jnp.zeros(acc_s.shape[1:], F32)

        def zero_acc(h, carry):
            acc[h] = jnp.zeros((NSEG * M, E), F32)
            return carry

        lax.fori_loop(0, 2 * KMAJ, zero_acc, 0)

        for cp in small:
            cp.wait()
        c = c_v[...].astype(F32)
        sc = _rb(c * jax.nn.sigmoid(c))
        put_rows(sc_row, 0, jnp.broadcast_to(sc, (16, D)))
        for j in range(DB):
            sc_col[pl.ds(j * 128, 128), :] = jnp.broadcast_to(sc[:, j * 128:(j + 1) * 128], (128, 128)).T
        mod_v[6] = jnp.broadcast_to(wr_v[...].astype(F32).reshape(1, D), (8, D))
        put_rows(lhs_v.at[0], 0, mem0_v[...].astype(F32))

        x_head.wait()
        NB = 16
        RB = NSEG * M // NB
        for b in range(NB):
            xb = x_v[pl.ds(b * (NSEG // NB), NSEG // NB), pl.ds(0, M), :].astype(F32).reshape(RB, D)
            nb = _ln(xb)[0]
            for j in range(DB):
                n_v[j, pl.ds(b * RB, RB), :] = nb[:, j * 128:(j + 1) * 128]

        hc_w = hc.bitcast(U32)
        sc_w = sc_row.bitcast(U32)

        def mod_block(j, k, src=None):
            scb = jnp.concatenate([_bf(sc_w[i]) for i in range(DB)], axis=1)
            v = _rb(_dot(scb, _bf(wmod_v[k, j if src is None else src]))[0:8])
            if k == 1:
                v = _rb(1.0 + v)
            col = j * 128 if isinstance(j, int) else pl.multiple_of(j * 128, 128)
            ab_v[k, :, pl.ds(col, 128)] = v
            return v

        def h_block(j, ca, sa, r0=0, nr=NSEG * M):
            n = n_v[j, pl.ds(r0, nr), :].reshape(nr // M, M, 128)
            hc[j, pl.ds(r0, nr), :] = (n * ca[None] + sa[None]).reshape(nr, 128).astype(BF16)

        def pack_pair(r1, r2):
            r = jnp.concatenate([r1.reshape(NSEG, M, E), r2.reshape(NSEG, M, E)], axis=1)
            return r.reshape(NIT, UNR * 2 * M, E).astype(BF16)

        def split_pair(b):
            return (pltpu.bitcast(b << 16, F32).astype(BF16),
                    pltpu.bitcast(b & jnp.uint32(0xFFFF0000), F32).astype(BF16))

        def q_stage(j, last, more_dmas):
            static = isinstance(j, int)
            k0 = j * 128 if static else pl.multiple_of(j * 128, 128)
            src = None if last else jnp.where(j == 0, 0, j + 1)
            for p in range(KMAJ):
                ws = split_pair(stage[p, pl.ds(k0, 128), :])
                rs = []
                for t in range(2):
                    h = 2 * p + t
                    w_v[h, j] = ws[t]
                    rs.append(_dot(_bf(hc_w[j]), _bf(w_w[h, j])) + acc[h])
                    if not last:
                        acc[h] = rs[t]
                if last:
                    cache[p] = pack_pair(*rs)
                elif p == 1:
                    ca = mod_block(j + 1, 1, src)
                elif p == 3:
                    sa = mod_block(j + 1, 0, src)
                elif p in H_SLOTS:
                    nr = NSEG * M // len(H_SLOTS)
                    h_block(j + 1, tie(ca, rs[0][0:8]), sa, H_SLOTS.index(p) * nr, nr)
                if p == 1:
                    more_dmas()

        wait_mod(0)
        h_block(0, mod_block(0, 1), mod_block(0, 0))

        def wait_ktile(j):
            rows = pl.ds(j * 128 if isinstance(j, int) else pl.multiple_of(j * 128, 128), 128)
            wait_all(stage.at[pl.ds(0, KMAJ), rows, :], SEM_WQ + j)

        def q_body(j, carry):
            @pl.when(j == 1)
            def _():
                wait_mod(1)
                h_block(1, mod_block(1, 1), mod_block(1, 0))

            wait_ktile(j)

            @pl.when(j > 0)
            def _():
                wait_mod(j + 1)

            def more_dmas():
                @pl.when(j + AHEAD < DB)
                def _():
                    start_ktile(j + AHEAD)

                @pl.when(j + AHEAD + 1 < DB)
                def _():
                    start_mod(j + AHEAD + 1)

                @pl.when(j + AHEAD == DB)
                def _():
                    for cp in slab_cps[:2 * PPI]:
                        cp.start()

            q_stage(j, False, more_dmas)
            return carry

        lax.fori_loop(0, DB - 1, q_body, 0)
        wait_ktile(DB - 1)

        def last_dmas():
            for i in range(2, 5):
                for cp in slab_cps[i * PPI:(i + 1) * PPI]:
                    cp.start()
                if i < 4:
                    start_chunk(i)
                if i == 2:
                    x_tail.start()

        q_stage(DB - 1, True, last_dmas)

        def pro_body(i, carry):
            g0 = KMAJ + i * PPI
            wait_all(stage.at[pl.ds(g0, PPI)], SEM_ST + i)

            @pl.when(i >= 2)
            def _():
                wait_all(wmod_v.at[i], SEM_MOD2 + i - 2)

            @pl.when(i == 2)
            def _():
                x_tail.wait()

            def more_dmas():
                @pl.when(i < 2)
                def _():
                    start_chunk(i + 4)

                @pl.when(i == 0)
                def _():
                    for cp in slab_cps[5 * PPI:]:
                        cp.start()

                @pl.when(jnp.logical_and(i >= 2, i < 4))
                def _():
                    wo_w = wo_hbm.bitcast(U32)
                    for t in range(DB // 2):
                        j = (i - 2) * (DB // 2) + t
                        cols = pl.ds(pl.multiple_of(j * 128, 128), 128)
                        copy(wo_w.at[:, cols], wo_v.at[j], SEM_WO).start()

            one = jnp.where(jnp.logical_or(i == 1, i == 4), 1.0, 0.0)

            def mod_cols(j):
                v = jnp.sum(_bf(wmod_v[i, j]).astype(F32) * sc_col[...], axis=0, keepdims=True)
                v = _rb(one + _rb(jnp.broadcast_to(v, (8, 128))))
                mod_v[i, :, pl.ds(j * 128, 128)] = v
                return v

            def ln_rows(n):
                seg = jnp.maximum(i - 2, 0) * (NSEG // 4) + n // 3
                r0 = (n % 3 + 1) * 8
                src = pl.multiple_of(jnp.where(i >= 2, r0, 0), 8)
                nrm, inv = _ln(x_v[seg, pl.ds(src, 8), :].astype(F32))
                put_rows(lhs_v.at[seg], r0, nrm * ab_v[1] + ab_v[0])
                return inv

            LPD = 3 * (NSEG // 4) // (2 * PPI)
            for t in range(PPI):
                gp = g0 + t
                w_v[2 * gp], w_v[2 * gp + 1] = split_pair(stage[gp].reshape(DB, 128, E))
                rs = []
                for hh in range(2):
                    n = 2 * t + hh - (2 * PPI - DB)
                    parts = [hc_w[j] for j in range(DB)]
                    parts[0] = tie(parts[0], mod_cols(n) if n >= 0 else None)
                    for k in range(LPD):
                        parts[-1] = tie(parts[-1], ln_rows((2 * t + hh) * LPD + k),
                                        k * (NSEG * M // 2 // LPD))
                    hcv = jnp.concatenate([_bf(w) for w in parts], axis=1)
                    rs.append(_dot(hcv, weights(2 * gp + hh)))
                cache[gp] = pack_pair(*rs)
                if t == 0:
                    more_dmas()
            return carry

        lax.fori_loop(0, (NGP - KMAJ) // PPI, pro_body, 0)

    prologue()

    def main():
        lane = lax.broadcasted_iota(jnp.int32, (8, 2 * 128), 1)

        def post(seg, q, keep=True):
            rows = pl.ds(8 * q, 8)
            x1 = x1_v[seg, rows, :].astype(F32)
            n, inv = _ln(x1)
            h2 = _rb(n * mod_row(4) + mod_row(3))
            r = _rb(jnp.sum(h2 * mod_row(6), axis=-1, keepdims=True))
            if keep:
                r_v[...] = jnp.where(lane == seg * 4 + q, r, r_v[...])
            h2_v[seg, rows, :] = h2.astype(BF16)
            out_v[seg, rows, :] = (x1 + mod_row(5) * h2).astype(BF16)
            return inv, r

        def out_copy(grp):
            return copy(out_v.at[pl.ds(grp * UNR, UNR)], out_hbm.at[pl.ds(grp * UNR, UNR)], SEM_OUT)

        wg_w, wu_w, wd_w = wg_hbm.bitcast(U32), wu_hbm.bitcast(U32), wd_hbm.bitcast(U32)
        wait_all(wo_v, SEM_WO)

        def step(it, u):
            s = it * UNR + u
            lhs = jnp.concatenate([_bf(lhs_w[s, j]) for j in range(DB)], axis=1)

            def side(slot):
                if slot not in SIDE_SLOTS:
                    return None
                q = SIDE_SLOTS.index(slot)
                return post(jnp.maximum(s - (2 if q == 0 else 1), 0), q)[0]

            def proj(m_i, p):
                g = m_i * NPAIR + p
                for t in range(2):
                    qkv_s[g, pl.ds(t * SEG, SEG), :] = _dot(lhs, weights(2 * g + t)).astype(BF16)

            def rows_of(m_i, p):
                g = m_i * NPAIR + p
                return jnp.concatenate([_bf(qkv_w[g]), _bf(cache_w[g, it, pl.ds(u * M, M), :])], axis=0)

            def probs(p):
                parts = [lax.dot_general(_bf(qkv_w[p]), rows_of(1, p), (((1,), (1,)), ((), ())),
                                         preferred_element_type=F32)]
                qc = _bf(cache_w[p, it, pl.ds(u * M, M), :]).astype(F32)
                kc = _bf(cache_w[NPAIR + p, it, pl.ds(u * M, M), :]).astype(F32)
                col = lax.broadcasted_iota(jnp.int32, (M, PR), 1)
                for t in range(2):
                    km = _bf(qkv_w[NPAIR + p, pl.ds(t * (SEG // 2), 8), :]).astype(F32)
                    qt = qc[t * M:(t + 1) * M]
                    st = jnp.zeros((M, PR), F32)
                    for j in range(M):
                        st = jnp.where(col == t * SEG + j,
                                       jnp.sum(qt * km[j:j + 1], axis=-1, keepdims=True), st)
                        st = jnp.where(col == 2 * SEG + t * M + j,
                                       jnp.sum(qt * kc[t * M + j:t * M + j + 1], axis=-1, keepdims=True), st)
                    parts.append(st)
                sc = jnp.concatenate(parts, axis=0) * SCALE
                fm = fill_v[...]
                tok = side(("softmax", p))
                if tok is not None:
                    top = fm[0:8]
                    fm = jnp.concatenate([jnp.where(top > 1.0, tok, top), fm[8:]], axis=0)
                sc = jnp.where(fm == 0.0, sc, fm)
                e = jnp.exp(sc - jnp.max(sc, axis=-1, keepdims=True))
                return (e * _recip(jnp.sum(e, axis=-1, keepdims=True))).astype(BF16)

            def attend(p, pr):
                o = _dot(pr, rows_of(2, p))
                for t in range(2):
                    o_s[2 * p + t, pl.ds(0, SEG), :] = o[t * SEG:(t + 1) * SEG].astype(BF16)
                for t in range(2):
                    o_s[2 * p + t, pl.ds(SEG + (u % 2) * M, M), :] = (
                        o[2 * SEG + t * M:2 * SEG + (t + 1) * M].astype(BF16))

            ps = {}
            for pa in range(0, NPAIR, 2):
                pb = pa + 1
                todo = [(0, pa), (1, pa), (0, pb), (1, pb), (2, pa), (2, pb)]
                if pa == 0 and u > 0:
                    hs = [(m_i * NPAIR + p, t) for m_i, p in todo[:NSPLIT] for t in range(2)]
                    ke = KEARLY * 128
                    first = [_dot(lhs[:, :ke], weights(2 * g + t, 0, KEARLY)) for g, t in hs]
                    for (g, t), part in zip(hs, first):
                        res = _dot(lhs[:, ke:], weights(2 * g + t, KEARLY, DB)) + part
                        qkv_s[g, pl.ds(t * SEG, SEG), :] = res.astype(BF16)
                    todo = todo[NSPLIT:]
                for m_i, p in todo:
                    proj(m_i, p)
                for kind in ("scores", "values") if pa % 4 == 0 else ("values", "scores"):
                    for p in (pa, pb):
                        if kind == "scores":
                            ps[p] = probs(p)
                        elif p >= 2:
                            attend(p - 2, ps.pop(p - 2))
            L = NPAIR - 1

            nxt = s + 1 if u < UNR - 1 else jnp.where(it < NIT - 1, s + 1, 0)
            nr = SEG + (2 * M if u % 2 else 0)
            for h0, h1 in ((0, HA), (HA, H)):
                for j in range(DB):
                    words = [o_w[h, pl.ds(0, nr // 2), :] for h in range(h0, h1)]
                    words[0] = tie(words[0], side((h0, j)))
                    ol = jnp.concatenate([_bf(w) for w in words], axis=1)
                    part = _dot(ol, _bf(wo_v[j, pl.ds(h0 * E // 2, (h1 - h0) * E // 2), :]))
                    if h0 == 0:
                        acc_s[j, pl.ds(0, nr), :] = part
                    else:
                        a = part + acc_s[j, pl.ds(0, nr), :]
                        cols = pl.ds(j * 128, 128)
                        lhs_v[nxt, j, pl.ds(0, M), :] = a[0:M].astype(BF16)
                        for q in range(1, nr // M):
                            seg, rows = (s, pl.ds(q * M, M)) if q < 4 else (s + q - 5, pl.ds(0, M))
                            x1 = x_v[seg, rows, cols].astype(F32) + mod_v[2, :, cols] * a[q * M:(q + 1) * M]
                            x1_v[seg, rows, cols] = x1.astype(BF16)
                    if h0 == 0 and j == 4:
                        attend(L - 1, ps.pop(L - 1))
                        attend(L, ps.pop(L))

        def iteration(it, carry):
            @pl.when(it >= 2)
            def _():
                out_copy(it - 2).start()

            @pl.when(it < FB // 2)
            def _():
                for t in range(2):
                    j = 2 * it + t
                    cols = pl.ds(pl.multiple_of(j * 128, 128), 128)
                    half = pl.ds(t * (D // 2), D // 2)
                    copy(wg_w.at[:, cols], stage.at[it, half, :], SEM_MOE).start()
                    copy(wu_w.at[:, cols], stage.at[FB // 2 + it, half, :], SEM_MOE).start()

            @pl.when(it < DB)
            def _():
                cols = pl.ds(pl.multiple_of(it * 128, 128), 128)
                for t in range(2):
                    copy(wd_w.at[pl.ds(t * (F // 4), F // 4), cols],
                         stage.at[FB + 2 * it + t, pl.ds(0, F // 4), :], SEM_MOE + 1).start()

            for u in range(UNR):
                step(it, u)
            return carry

        lax.fori_loop(0, NIT, iteration, 0)

        out_copy(NIT - 2).start()
        wait_all(stage.at[pl.ds(0, FB)], SEM_MOE)
        wait_all(stage.at[pl.ds(FB, 2 * DB), pl.ds(0, F // 4), :], SEM_MOE + 1)
        r8 = lax.broadcasted_iota(jnp.int32, (8, 1), 0)

        def top2(vals, idx, axes):
            def red(f, v):
                for ax in axes:
                    v = f(v, axis=ax, keepdims=True)
                return v
            m1 = red(jnp.max, vals)
            i1 = red(jnp.min, jnp.where(vals == m1, idx, S - 1.0))
            rest = jnp.where(idx == i1, -jnp.inf, vals)
            m2 = red(jnp.max, rest)
            i2 = red(jnp.min, jnp.where(rest == m2, jnp.where(idx == i1, S - 1.0, idx), S - 1.0))
            return m1, i1, m2, i2

        m1, i1v, m2, i2v = top2(r_v[...], (lane * 8 + r8).astype(F32), (1, 0))
        vals = [jnp.where(r8 == 0, m1, jnp.where(r8 == 1, m2, -jnp.inf))]
        idxs = [jnp.where(r8 == 0, i1v, jnp.where(r8 == 1, i2v, S - 1.0))]
        for seg, q in [(NSEG - 2, 0)] + [(NSEG - 1, q) for q in range(4)]:
            vals.append(post(seg, q, keep=False)[1])
            idxs.append((r8 + (seg * SEG + q * 8)).astype(F32))
        out_copy(NIT - 1).start()
        m1, i1v, m2, i2v = top2(jnp.concatenate(vals, axis=0), jnp.concatenate(idxs, axis=0), (0,))
        i1 = i1v.astype(jnp.int32)[0, 0]
        i2 = i2v.astype(jnp.int32)[0, 0]

        def tile_of(i):
            return i >> 5, pl.multiple_of(((i >> 3) & 3) * 8, 8)

        sel = [tile_of(i1), tile_of(i2)]
        x1s = jnp.concatenate([x1_v[sg, pl.ds(r0, 8), :].astype(F32) for sg, r0 in sel], axis=0)
        h2s = jnp.concatenate([h2_v[sg, pl.ds(r0, 8), :].astype(F32) for sg, r0 in sel], axis=0)
        h2b = h2s.astype(BF16)
        gus = []
        for j in range(FB):
            half = pl.ds((j % 2) * (D // 2), D // 2)
            g = _rb(_dot(h2b, _bf(stage[j // 2, half, :])))
            g = _rb(g * jax.nn.sigmoid(g))
            u = _rb(_dot(h2b, _bf(stage[FB // 2 + j // 2, half, :])))
            gus.append(g * u)
        gu = jnp.concatenate(gus, axis=1).astype(BF16)
        ys = []
        for j in range(DB):
            wd = stage[pl.ds(FB + 2 * j, 2), pl.ds(0, F // 4), :].reshape(F // 2, 128)
            ys.append(_rb(_dot(gu, _bf(wd))))
        y = jnp.concatenate(ys, axis=1)
        rows = lax.broadcasted_iota(jnp.int32, (16, 1), 0)
        rs = _rb(jax.nn.sigmoid(jnp.where(rows < 8, m1, m2)))
        y = _rb(y * rs)
        full = x1s + mod_row(5, 16) * _rb(h2s + y)

        copy(out_v, out_hbm, SEM_OUT).wait()
        for t, (i, (sg, r0)) in enumerate(zip((i1, i2), sel)):
            old = out_v[sg, pl.ds(r0, 8), :].astype(F32)
            new = jnp.where(r8 == (i & 7), full[t * 8:(t + 1) * 8], old)
            out_v[sg, pl.ds(r0, 8), :] = new.astype(BF16)
        fix = [copy(out_v.at[sg, pl.ds(r0, 8), :], out_hbm.at[sg, pl.ds(r0, 8), :], SEM_OUT + 1 + t)
               for t, (sg, r0) in enumerate(sel)]
        differ = (i1 >> 3) != (i2 >> 3)
        fix[0].start()

        @pl.when(differ)
        def _():
            fix[1].start()
            fix[1].wait()

        fix[0].wait()

    main()


@jax.jit
def pallas_adaLN_cond__memory_aug_recurrent_mem_tr__moe_arch_mod__prompt_kernel(
    A_x: jax.Array,
    A_mem0: jax.Array,
    A_Wq: jax.Array,
    A_Wk: jax.Array,
    A_Wv: jax.Array,
    A_Wo: jax.Array,
    A_seg_len: jax.Array,
    B_x: jax.Array,
    B_w_r: jax.Array,
    B_w_gate: jax.Array,
    B_w_up: jax.Array,
    B_w_down: jax.Array,
    c: jax.Array,
    w_mod: jax.Array,
):
    del A_seg_len, B_x
    assert A_x.shape == (1, S, D) and A_mem0.shape == (1, M, D) and A_Wq.shape == (D, H, E)
    hbm = pl.BlockSpec(memory_space=pl.ANY)
    out = pl.pallas_call(
        _kernel,
        out_shape=jax.ShapeDtypeStruct((NSEG, SEG, D), BF16),
        in_specs=[hbm] * 12,
        out_specs=hbm,
        scratch_shapes=[
            pltpu.VMEM((NSEG, SEG, D), BF16),
            pltpu.VMEM((3 * H, DB, 128, E), BF16),
            pltpu.VMEM((DB, H * E // 2, 128), U32),
            pltpu.VMEM((NGP, NIT, UNR * 2 * M, E), BF16),
            pltpu.VMEM((NSEG, DB, SEG, 128), BF16),
            pltpu.VMEM((NGP, 2 * SEG, E), BF16),
            pltpu.VMEM((H, 2 * SEG, E), BF16),
            pltpu.VMEM((DB, 2 * SEG, 128), F32),
            pltpu.VMEM((7, 8, D), F32),
            pltpu.VMEM((2, 8, D), F32),
            pltpu.VMEM((NGP, D, E), U32),
            pltpu.VMEM((6, DB, D // 2, 128), U32),
            pltpu.VMEM((DB, NSEG * M, E), BF16),
            pltpu.VMEM((DB, NSEG * M, 128), F32),
            pltpu.VMEM((2 * KMAJ, NSEG * M, E), F32),
            pltpu.VMEM((DB, 16, 128), BF16),
            pltpu.VMEM((D, 128), F32),
            pltpu.VMEM((NSEG, SEG, D), BF16),
            pltpu.VMEM((NSEG, SEG, D), BF16),
            pltpu.VMEM((NSEG, SEG, D), BF16),
            pltpu.VMEM((M, D), BF16),
            pltpu.VMEM((8, S // 8), F32),
            pltpu.VMEM((PR, PR), F32),
            pltpu.VMEM((8, 128), F32),
            pltpu.VMEM((1, D), BF16),
            pltpu.VMEM((D,), BF16),
            pltpu.SemaphoreType.DMA((NSEM,)),
        ],
        compiler_params=pltpu.CompilerParams(
            vmem_limit_bytes=120 * 1024 * 1024, disable_bounds_checks=True,
            disable_semaphore_checks=True),
    )(
        A_x.reshape(NSEG, SEG, D),
        A_mem0.reshape(M, D),
        A_Wq, A_Wk, A_Wv,
        A_Wo.reshape(H * E, D),
        B_w_r,
        B_w_gate, B_w_up, B_w_down,
        c, w_mod,
    )
    return out.reshape(1, S, D)
```

```python
import jax
import jax.numpy as jnp
from jax import lax
import jax.experimental.pallas as pl
import jax.experimental.pallas.tpu as pltpu

BF16 = jnp.bfloat16
F32 = jnp.float32
U32 = jnp.uint32

S = 2048
D = 1024
H = 32
E = 128
M = 8
SEG = 32
NSEG = S // SEG
NPAIR = H // 2
NGP = 3 * NPAIR
F = 3584
DB = D // 128
FB = F // 128
PR = 2 * SEG + 2 * M
UNR = 4
NIT = NSEG // UNR
KMAJ = 12
AHEAD = 3
PPI = 6
NSPLIT = 3
KEARLY = 5
HA = 24
SIDE_SLOTS = [("softmax", 8), (0, 2), (0, 5), (0, 7)]
MOD_SLOTS = (11, 7)
H_SLOTS = (6, 8)
EPS = 1e-5
SCALE = E ** (-0.5)

SEM_SMALL = 0
SEM_X = SEM_SMALL + 3
SEM_MOD = SEM_X + 2
SEM_MOD2 = SEM_MOD + DB
SEM_WQ = SEM_MOD2 + 4
SEM_ST = SEM_WQ + DB
SEM_WO = SEM_ST + (NGP - KMAJ) // PPI
SEM_MOE = SEM_WO + 1
SEM_OUT = SEM_MOE + 2
NSEM = SEM_OUT + 3


def _rb(v):
    return v.astype(BF16).astype(F32)


def _dot(a, b):
    return jnp.dot(a, b, preferred_element_type=F32)


def _recip(x):
    r = pl.reciprocal(x, approx=True)
    return r * (2.0 - x * r)


def _bf(words):
    return pltpu.bitcast(words, BF16)


def _ln(x):
    m = jnp.mean(x, axis=-1, keepdims=True)
    mb = _rb(m)
    d = x - mb
    var = jnp.mean(d * d, axis=-1, keepdims=True) - (m - mb) * (m - mb)
    inv = _recip(_rb(jnp.sqrt(_rb(_rb(jnp.maximum(var, 0.0)) + EPS))))
    return d * inv, inv


def _fill_matrix():
    i = lax.broadcasted_iota(jnp.int32, (PR, PR), 0)
    j = lax.broadcasted_iota(jnp.int32, (PR, PR), 1)

    def head(t):
        return jnp.where(t < 2 * SEG, t >> 5, (t - 2 * SEG) >> 3)

    def pos(t):
        r = t & (SEG - 1)
        return jnp.where(t < 2 * SEG, jnp.where(r < M, r, r + M), M + (t & (M - 1)))

    same = head(i) == head(j)
    pi = pos(i)
    ok = jnp.where(pi < M, 1, jnp.where(pi >= pos(j), 1, 0))
    return jnp.where(same, jnp.where(ok == 1, 0.0, -1e9), -3e38).astype(F32)


def _kernel(x_hbm, mem0_hbm, wq_hbm, wk_hbm, wv_hbm, wo_hbm, wr_hbm, wg_hbm, wu_hbm, wd_hbm,
            c_hbm, wmod_hbm, out_hbm,
            x_v, w_v, wo_v, cache, lhs_v, qkv_s, o_s, acc_s, mod_v, ab_v,
            stage, wmod_v, hc, n_v, acc, sc_row, sc_col, x1_v, h2_v, out_v,
            mem0_v, r_v, fill_v, never_v, c_v, wr_v, sems):
    w_w = w_v.bitcast(U32)
    cache_w = cache.bitcast(U32)
    lhs_w = lhs_v.bitcast(U32)
    qkv_w = qkv_s.bitcast(U32)
    o_w = o_s.bitcast(U32)

    def weights(h, j0=0, j1=DB):
        return _bf(w_w[h, pl.ds(j0, j1 - j0)].reshape((j1 - j0) * 64, E))

    def tie(v, tok, r0=0):
        if tok is None:
            return v
        tok = jnp.broadcast_to(tok, (8, 128))
        if v.dtype != F32:
            tok = pltpu.bitcast(tok, v.dtype)
        parts = [v[:r0], jnp.where(never_v[...] > 1.0, tok, v[r0:r0 + 8]), v[r0 + 8:]]
        return jnp.concatenate([x for x in parts if x.shape[0]], axis=0)

    def copy(src, dst, sem):
        return pltpu.make_async_copy(src, dst, sems.at[sem])

    def wait_all(buf, sem):
        copy(buf, buf, sem).wait()

    def mod_row(k, rows=8):
        v = mod_v[k]
        return v if rows == 8 else jnp.concatenate([v] * (rows // 8), axis=0)

    def put_rows(dst, r0, v):
        for j in range(DB):
            dst[j, pl.ds(r0, v.shape[0]), :] = v[:, j * 128:(j + 1) * 128].astype(BF16)

    def prologue():
        wmod_w = wmod_hbm.bitcast(U32)
        w_words = [w.bitcast(U32) for w in (wq_hbm, wk_hbm, wv_hbm)]

        def start_mod(j):
            col = j * 128 if isinstance(j, int) else pl.multiple_of(j * 128, 128)
            for k in range(2):
                copy(wmod_w.at[:, pl.ds(k * D + col, 128)], wmod_v.at[k, j], SEM_MOD + j).start()

        def wait_mod(j):
            wait_all(wmod_v.at[pl.ds(0, 2), j], SEM_MOD + j)

        def start_chunk(k):
            col = k * D if isinstance(k, int) else pl.multiple_of(k * D, D)
            for j in range(DB):
                copy(wmod_w.at[:, pl.ds(col + j * 128, 128)], wmod_v.at[k, j], SEM_MOD2 + k - 2).start()

        def start_ktile(j):
            rows = pl.ds(j * 128 if isinstance(j, int) else pl.multiple_of(j * 128, 128), 128)
            for g in range(KMAJ):
                copy(w_words[0].at[rows, g, :], stage.at[g, rows, :], SEM_WQ + j).start()

        small = [copy(c_hbm, c_v, SEM_SMALL), copy(mem0_hbm, mem0_v, SEM_SMALL + 1),
                 copy(wr_hbm, wr_v, SEM_SMALL + 2)]
        x_head = copy(x_hbm.at[:, pl.ds(0, M), :], x_v.at[:, pl.ds(0, M), :], SEM_X)
        x_tail = copy(x_hbm.at[:, pl.ds(M, SEG - M), :], x_v.at[:, pl.ds(M, SEG - M), :], SEM_X + 1)
        for cp in small:
            cp.start()
        x_head.start()
        start_mod(0)
        for j in range(AHEAD):
            start_ktile(j)
            start_mod(j + 1)
        slab_cps = [copy(w_words[g // NPAIR].at[:, g % NPAIR, :], stage.at[g], SEM_ST + (g - KMAJ) // PPI)
                    for g in range(KMAJ, NGP)]

        fill_v[...] = _fill_matrix()
        x1_v[0] = jnp.zeros((SEG, D), BF16)
        r_v[...] = jnp.full(r_v.shape, -jnp.inf, F32)
        never_v[...] = jnp.zeros(never_v.shape, F32)
        qkv_s[0] = jnp.zeros((2 * SEG, E), BF16)
        o_s[0] = jnp.zeros(o_s.shape[1:], BF16)
        acc_s[0] = jnp.zeros(acc_s.shape[1:], F32)

        def zero_acc(h, carry):
            acc[h] = jnp.zeros((NSEG * M, E), F32)
            return carry

        lax.fori_loop(0, 2 * KMAJ, zero_acc, 0)

        for cp in small:
            cp.wait()
        c = c_v[...].astype(F32)
        sc = _rb(c * jax.nn.sigmoid(c))
        put_rows(sc_row, 0, jnp.broadcast_to(sc, (16, D)))
        for j in range(DB):
            sc_col[pl.ds(j * 128, 128), :] = jnp.broadcast_to(sc[:, j * 128:(j + 1) * 128], (128, 128)).T
        mod_v[6] = jnp.broadcast_to(wr_v[...].astype(F32).reshape(1, D), (8, D))
        put_rows(lhs_v.at[0], 0, mem0_v[...].astype(F32))

        x_head.wait()
        NB = 16
        RB = NSEG * M // NB
        for b in range(NB):
            xb = x_v[pl.ds(b * (NSEG // NB), NSEG // NB), pl.ds(0, M), :].astype(F32).reshape(RB, D)
            nb = _ln(xb)[0]
            for j in range(DB):
                n_v[j, pl.ds(b * RB, RB), :] = nb[:, j * 128:(j + 1) * 128]

        hc_w = hc.bitcast(U32)
        sc_w = sc_row.bitcast(U32)

        def mod_vpu(k, j):
            v = jnp.sum(_bf(wmod_v[k, j]).astype(F32) * sc_col[...], axis=0, keepdims=True)
            return _rb(jnp.broadcast_to(v, (8, 128)))

        def mod_block(j, k, src=None):
            if src is None:
                scb = jnp.concatenate([_bf(sc_w[i]) for i in range(DB)], axis=1)
                v = _rb(_dot(scb, _bf(wmod_v[k, j]))[0:8])
            else:
                v = mod_vpu(k, src)
            if k == 1:
                v = _rb(1.0 + v)
            col = j * 128 if isinstance(j, int) else pl.multiple_of(j * 128, 128)
            ab_v[k, :, pl.ds(col, 128)] = v
            return v

        def h_block(j, ca, sa, r0=0, nr=NSEG * M):
            n = n_v[j, pl.ds(r0, nr), :].reshape(nr // M, M, 128)
            hc[j, pl.ds(r0, nr), :] = (n * ca[None] + sa[None]).reshape(nr, 128).astype(BF16)

        def pack_pair(r1, r2):
            r = jnp.concatenate([r1.reshape(NSEG, M, E), r2.reshape(NSEG, M, E)], axis=1)
            return r.reshape(NIT, UNR * 2 * M, E).astype(BF16)

        def split_pair(b):
            return (pltpu.bitcast(b << 16, F32).astype(BF16),
                    pltpu.bitcast(b & jnp.uint32(0xFFFF0000), F32).astype(BF16))

        def q_stage(j, last, more_dmas):
            static = isinstance(j, int)
            k0 = j * 128 if static else pl.multiple_of(j * 128, 128)
            src = None if last else jnp.where(j == 0, 0, j + 1)
            mods = {}
            for p in range(KMAJ):
                ws = split_pair(stage[p, pl.ds(k0, 128), :])
                rs = []
                for t in range(2):
                    h = 2 * p + t
                    w_v[h, j] = ws[t]
                    lw = hc_w[j]
                    if not last and h in MOD_SLOTS:
                        k = MOD_SLOTS.index(h)
                        mods[k] = mod_block(j + 1, k, src)
                        lw = tie(lw, mods[k], NSEG * M // 4)
                    rs.append(_dot(_bf(lw), _bf(w_w[h, j])) + acc[h])
                    if not last:
                        acc[h] = rs[t]
                if last:
                    cache[p] = pack_pair(*rs)
                elif p in H_SLOTS:
                    nr = NSEG * M // len(H_SLOTS)
                    h_block(j + 1, tie(mods[1], rs[0][0:8]), mods[0], H_SLOTS.index(p) * nr, nr)
                if p == (1 if last else KMAJ - 3):
                    more_dmas()

        wait_mod(0)
        h_block(0, mod_block(0, 1), mod_block(0, 0))

        def wait_ktile(j):
            rows = pl.ds(j * 128 if isinstance(j, int) else pl.multiple_of(j * 128, 128), 128)
            wait_all(stage.at[pl.ds(0, KMAJ), rows, :], SEM_WQ + j)

        def q_body(j, carry):
            @pl.when(j == 1)
            def _():
                wait_mod(1)
                h_block(1, mod_block(1, 1), mod_block(1, 0))

            wait_ktile(j)

            @pl.when(j > 0)
            def _():
                wait_mod(j + 1)

            def more_dmas():
                @pl.when(j + AHEAD < DB)
                def _():
                    start_ktile(j + AHEAD)

                @pl.when(j + AHEAD + 1 < DB)
                def _():
                    start_mod(j + AHEAD + 1)

                @pl.when(j + AHEAD == DB - 1)
                def _():
                    for cp in slab_cps[:2 * PPI]:
                        cp.start()

            q_stage(j, False, more_dmas)
            return carry

        lax.fori_loop(0, DB - 1, q_body, 0)
        wait_ktile(DB - 1)

        def last_dmas():
            for i in range(2, 5):
                for cp in slab_cps[i * PPI:(i + 1) * PPI]:
                    cp.start()
                if i < 4:
                    start_chunk(i)
                if i == 2:
                    x_tail.start()

        q_stage(DB - 1, True, last_dmas)

        def pro_body(i, carry):
            g0 = KMAJ + i * PPI
            wait_all(stage.at[pl.ds(g0, PPI)], SEM_ST + i)

            @pl.when(i >= 2)
            def _():
                wait_all(wmod_v.at[i], SEM_MOD2 + i - 2)

            @pl.when(i == 2)
            def _():
                x_tail.wait()

            def more_dmas():
                @pl.when(i < 2)
                def _():
                    start_chunk(i + 4)

                @pl.when(i == 0)
                def _():
                    for cp in slab_cps[5 * PPI:]:
                        cp.start()

                @pl.when(jnp.logical_and(i >= 2, i < 4))
                def _():
                    wo_w = wo_hbm.bitcast(U32)
                    for t in range(DB // 2):
                        j = (i - 2) * (DB // 2) + t
                        cols = pl.ds(pl.multiple_of(j * 128, 128), 128)
                        copy(wo_w.at[:, cols], wo_v.at[j], SEM_WO).start()

            one = jnp.where(jnp.logical_or(i == 1, i == 4), 1.0, 0.0)

            def mod_cols(j):
                v = _rb(one + mod_vpu(i, j))
                mod_v[i, :, pl.ds(j * 128, 128)] = v
                return v

            def ln_rows(n):
                seg = jnp.maximum(i - 2, 0) * (NSEG // 4) + n // 3
                r0 = (n % 3 + 1) * 8
                src = pl.multiple_of(jnp.where(i >= 2, r0, 0), 8)
                nrm, inv = _ln(x_v[seg, pl.ds(src, 8), :].astype(F32))
                put_rows(lhs_v.at[seg], r0, nrm * ab_v[1] + ab_v[0])
                return inv

            LPD = 3 * (NSEG // 4) // (2 * PPI)
            for t in range(PPI):
                gp = g0 + t
                w_v[2 * gp], w_v[2 * gp + 1] = split_pair(stage[gp].reshape(DB, 128, E))
                rs = []
                for hh in range(2):
                    n = 2 * t + hh - (2 * PPI - DB)
                    parts = [hc_w[j] for j in range(DB)]
                    parts[0] = tie(parts[0], mod_cols(n) if n >= 0 else None)
                    for k in range(LPD):
                        parts[-1] = tie(parts[-1], ln_rows((2 * t + hh) * LPD + k),
                                        k * (NSEG * M // 2 // LPD))
                    hcv = jnp.concatenate([_bf(w) for w in parts], axis=1)
                    rs.append(_dot(hcv, weights(2 * gp + hh)))
                cache[gp] = pack_pair(*rs)
                if t == 0:
                    more_dmas()
            return carry

        lax.fori_loop(0, (NGP - KMAJ) // PPI, pro_body, 0)

    prologue()

    def main():
        lane = lax.broadcasted_iota(jnp.int32, (8, 2 * 128), 1)

        def post(seg, q, keep=True):
            rows = pl.ds(8 * q, 8)
            x1 = x1_v[seg, rows, :].astype(F32)
            n, inv = _ln(x1)
            h2 = _rb(n * mod_row(4) + mod_row(3))
            r = _rb(jnp.sum(h2 * mod_row(6), axis=-1, keepdims=True))
            if keep:
                r_v[...] = jnp.where(lane == seg * 4 + q, r, r_v[...])
            h2_v[seg, rows, :] = h2.astype(BF16)
            out_v[seg, rows, :] = (x1 + mod_row(5) * h2).astype(BF16)
            return inv, r

        def out_copy(grp):
            return copy(out_v.at[pl.ds(grp * UNR, UNR)], out_hbm.at[pl.ds(grp * UNR, UNR)], SEM_OUT)

        wg_w, wu_w, wd_w = wg_hbm.bitcast(U32), wu_hbm.bitcast(U32), wd_hbm.bitcast(U32)
        wait_all(wo_v, SEM_WO)

        def step(it, u):
            s = it * UNR + u
            lhs = jnp.concatenate([_bf(lhs_w[s, j]) for j in range(DB)], axis=1)

            def side(slot):
                if slot not in SIDE_SLOTS:
                    return None
                q = SIDE_SLOTS.index(slot)
                return post(jnp.maximum(s - (2 if q == 0 else 1), 0), q)[0]

            def proj(m_i, p):
                g = m_i * NPAIR + p
                for t in range(2):
                    qkv_s[g, pl.ds(t * SEG, SEG), :] = _dot(lhs, weights(2 * g + t)).astype(BF16)

            def rows_of(m_i, p):
                g = m_i * NPAIR + p
                return jnp.concatenate([_bf(qkv_w[g]), _bf(cache_w[g, it, pl.ds(u * M, M), :])], axis=0)

            def probs(p):
                parts = [lax.dot_general(_bf(qkv_w[p]), rows_of(1, p), (((1,), (1,)), ((), ())),
                                         preferred_element_type=F32)]
                qc = _bf(cache_w[p, it, pl.ds(u * M, M), :]).astype(F32)
                kc = _bf(cache_w[NPAIR + p, it, pl.ds(u * M, M), :]).astype(F32)
                col = lax.broadcasted_iota(jnp.int32, (M, PR), 1)
                for t in range(2):
                    km = _bf(qkv_w[NPAIR + p, pl.ds(t * (SEG // 2), 8), :]).astype(F32)
                    qt = qc[t * M:(t + 1) * M]
                    st = jnp.zeros((M, PR), F32)
                    for j in range(M):
                        st = jnp.where(col == t * SEG + j,
                                       jnp.sum(qt * km[j:j + 1], axis=-1, keepdims=True), st)
                        st = jnp.where(col == 2 * SEG + t * M + j,
                                       jnp.sum(qt * kc[t * M + j:t * M + j + 1], axis=-1, keepdims=True), st)
                    parts.append(st)
                sc = jnp.concatenate(parts, axis=0) * SCALE
                fm = fill_v[...]
                tok = side(("softmax", p))
                if tok is not None:
                    top = fm[0:8]
                    fm = jnp.concatenate([jnp.where(top > 1.0, tok, top), fm[8:]], axis=0)
                sc = jnp.where(fm == 0.0, sc, fm)
                e = jnp.exp(sc - jnp.max(sc, axis=-1, keepdims=True))
                return (e * _recip(jnp.sum(e, axis=-1, keepdims=True))).astype(BF16)

            def attend(p, pr):
                o = _dot(pr, rows_of(2, p))
                for t in range(2):
                    o_s[2 * p + t, pl.ds(0, SEG), :] = o[t * SEG:(t + 1) * SEG].astype(BF16)
                for t in range(2):
                    o_s[2 * p + t, pl.ds(SEG + (u % 2) * M, M), :] = (
                        o[2 * SEG + t * M:2 * SEG + (t + 1) * M].astype(BF16))

            ps = {}
            for pa in range(0, NPAIR, 2):
                pb = pa + 1
                todo = [(0, pa), (1, pa), (0, pb), (1, pb), (2, pa), (2, pb)]
                if pa == 0 and u > 0:
                    hs = [(m_i * NPAIR + p, t) for m_i, p in todo[:NSPLIT] for t in range(2)]
                    ke = KEARLY * 128
                    first = [_dot(lhs[:, :ke], weights(2 * g + t, 0, KEARLY)) for g, t in hs]
                    for (g, t), part in zip(hs, first):
                        res = _dot(lhs[:, ke:], weights(2 * g + t, KEARLY, DB)) + part
                        qkv_s[g, pl.ds(t * SEG, SEG), :] = res.astype(BF16)
                    todo = todo[NSPLIT:]
                for m_i, p in todo:
                    proj(m_i, p)
                for kind in ("scores", "values") if pa % 4 == 0 else ("values", "scores"):
                    for p in (pa, pb):
                        if kind == "scores":
                            ps[p] = probs(p)
                        elif p >= 2:
                            attend(p - 2, ps.pop(p - 2))
            L = NPAIR - 1

            nxt = s + 1 if u < UNR - 1 else jnp.where(it < NIT - 1, s + 1, 0)
            nr = SEG + (2 * M if u % 2 else 0)
            for h0, h1 in ((0, HA), (HA, H)):
                for j in range(DB):
                    words = [o_w[h, pl.ds(0, nr // 2), :] for h in range(h0, h1)]
                    words[0] = tie(words[0], side((h0, j)))
                    ol = jnp.concatenate([_bf(w) for w in words], axis=1)
                    part = _dot(ol, _bf(wo_v[j, pl.ds(h0 * E // 2, (h1 - h0) * E // 2), :]))
                    if h0 == 0:
                        acc_s[j, pl.ds(0, nr), :] = part
                    else:
                        a = part + acc_s[j, pl.ds(0, nr), :]
                        cols = pl.ds(j * 128, 128)
                        lhs_v[nxt, j, pl.ds(0, M), :] = a[0:M].astype(BF16)
                        for q in range(1, nr // M):
                            seg, rows = (s, pl.ds(q * M, M)) if q < 4 else (s + q - 5, pl.ds(0, M))
                            x1 = x_v[seg, rows, cols].astype(F32) + mod_v[2, :, cols] * a[q * M:(q + 1) * M]
                            x1_v[seg, rows, cols] = x1.astype(BF16)
                    if h0 == 0 and j == 4:
                        attend(L - 1, ps.pop(L - 1))
                        attend(L, ps.pop(L))

        def iteration(it, carry):
            @pl.when(it >= 2)
            def _():
                out_copy(it - 2).start()

            @pl.when(it < FB // 2)
            def _():
                for t in range(2):
                    j = 2 * it + t
                    cols = pl.ds(pl.multiple_of(j * 128, 128), 128)
                    half = pl.ds(t * (D // 2), D // 2)
                    copy(wg_w.at[:, cols], stage.at[it, half, :], SEM_MOE).start()
                    copy(wu_w.at[:, cols], stage.at[FB // 2 + it, half, :], SEM_MOE).start()

            @pl.when(it < DB)
            def _():
                cols = pl.ds(pl.multiple_of(it * 128, 128), 128)
                for t in range(2):
                    copy(wd_w.at[pl.ds(t * (F // 4), F // 4), cols],
                         stage.at[FB + 2 * it + t, pl.ds(0, F // 4), :], SEM_MOE + 1).start()

            for u in range(UNR):
                step(it, u)
            return carry

        lax.fori_loop(0, NIT, iteration, 0)

        out_copy(NIT - 2).start()
        wait_all(stage.at[pl.ds(0, FB)], SEM_MOE)
        wait_all(stage.at[pl.ds(FB, 2 * DB), pl.ds(0, F // 4), :], SEM_MOE + 1)
        r8 = lax.broadcasted_iota(jnp.int32, (8, 1), 0)

        def top2(vals, idx, axes):
            def red(f, v):
                for ax in axes:
                    v = f(v, axis=ax, keepdims=True)
                return v
            m1 = red(jnp.max, vals)
            i1 = red(jnp.min, jnp.where(vals == m1, idx, S - 1.0))
            rest = jnp.where(idx == i1, -jnp.inf, vals)
            m2 = red(jnp.max, rest)
            i2 = red(jnp.min, jnp.where(rest == m2, jnp.where(idx == i1, S - 1.0, idx), S - 1.0))
            return m1, i1, m2, i2

        m1, i1v, m2, i2v = top2(r_v[...], (lane * 8 + r8).astype(F32), (1, 0))
        vals = [jnp.where(r8 == 0, m1, jnp.where(r8 == 1, m2, -jnp.inf))]
        idxs = [jnp.where(r8 == 0, i1v, jnp.where(r8 == 1, i2v, S - 1.0))]
        for seg, q in [(NSEG - 2, 0)] + [(NSEG - 1, q) for q in range(4)]:
            vals.append(post(seg, q, keep=False)[1])
            idxs.append((r8 + (seg * SEG + q * 8)).astype(F32))
        out_copy(NIT - 1).start()
        m1, i1v, m2, i2v = top2(jnp.concatenate(vals, axis=0), jnp.concatenate(idxs, axis=0), (0,))
        i1 = i1v.astype(jnp.int32)[0, 0]
        i2 = i2v.astype(jnp.int32)[0, 0]

        def tile_of(i):
            return i >> 5, pl.multiple_of(((i >> 3) & 3) * 8, 8)

        sel = [tile_of(i1), tile_of(i2)]
        x1s = jnp.concatenate([x1_v[sg, pl.ds(r0, 8), :].astype(F32) for sg, r0 in sel], axis=0)
        h2s = jnp.concatenate([h2_v[sg, pl.ds(r0, 8), :].astype(F32) for sg, r0 in sel], axis=0)
        h2b = h2s.astype(BF16)
        gus = []
        for j in range(FB):
            half = pl.ds((j % 2) * (D // 2), D // 2)
            g = _rb(_dot(h2b, _bf(stage[j // 2, half, :])))
            g = _rb(g * jax.nn.sigmoid(g))
            u = _rb(_dot(h2b, _bf(stage[FB // 2 + j // 2, half, :])))
            gus.append(g * u)
        gu = jnp.concatenate(gus, axis=1).astype(BF16)
        ys = []
        for j in range(DB):
            wd = stage[pl.ds(FB + 2 * j, 2), pl.ds(0, F // 4), :].reshape(F // 2, 128)
            ys.append(_rb(_dot(gu, _bf(wd))))
        y = jnp.concatenate(ys, axis=1)
        rows = lax.broadcasted_iota(jnp.int32, (16, 1), 0)
        rs = _rb(jax.nn.sigmoid(jnp.where(rows < 8, m1, m2)))
        y = _rb(y * rs)
        full = x1s + mod_row(5, 16) * _rb(h2s + y)

        copy(out_v, out_hbm, SEM_OUT).wait()
        for t, (i, (sg, r0)) in enumerate(zip((i1, i2), sel)):
            old = out_v[sg, pl.ds(r0, 8), :].astype(F32)
            new = jnp.where(r8 == (i & 7), full[t * 8:(t + 1) * 8], old)
            out_v[sg, pl.ds(r0, 8), :] = new.astype(BF16)
        fix = [copy(out_v.at[sg, pl.ds(r0, 8), :], out_hbm.at[sg, pl.ds(r0, 8), :], SEM_OUT + 1 + t)
               for t, (sg, r0) in enumerate(sel)]
        differ = (i1 >> 3) != (i2 >> 3)
        fix[0].start()

        @pl.when(differ)
        def _():
            fix[1].start()
            fix[1].wait()

        fix[0].wait()

    main()


@jax.jit
def pallas_adaLN_cond__memory_aug_recurrent_mem_tr__moe_arch_mod__prompt_kernel(
    A_x: jax.Array,
    A_mem0: jax.Array,
    A_Wq: jax.Array,
    A_Wk: jax.Array,
    A_Wv: jax.Array,
    A_Wo: jax.Array,
    A_seg_len: jax.Array,
    B_x: jax.Array,
    B_w_r: jax.Array,
    B_w_gate: jax.Array,
    B_w_up: jax.Array,
    B_w_down: jax.Array,
    c: jax.Array,
    w_mod: jax.Array,
):
    del A_seg_len, B_x
    assert A_x.shape == (1, S, D) and A_mem0.shape == (1, M, D) and A_Wq.shape == (D, H, E)
    hbm = pl.BlockSpec(memory_space=pl.ANY)
    out = pl.pallas_call(
        _kernel,
        out_shape=jax.ShapeDtypeStruct((NSEG, SEG, D), BF16),
        in_specs=[hbm] * 12,
        out_specs=hbm,
        scratch_shapes=[
            pltpu.VMEM((NSEG, SEG, D), BF16),
            pltpu.VMEM((3 * H, DB, 128, E), BF16),
            pltpu.VMEM((DB, H * E // 2, 128), U32),
            pltpu.VMEM((NGP, NIT, UNR * 2 * M, E), BF16),
            pltpu.VMEM((NSEG, DB, SEG, 128), BF16),
            pltpu.VMEM((NGP, 2 * SEG, E), BF16),
            pltpu.VMEM((H, 2 * SEG, E), BF16),
            pltpu.VMEM((DB, 2 * SEG, 128), F32),
            pltpu.VMEM((7, 8, D), F32),
            pltpu.VMEM((2, 8, D), F32),
            pltpu.VMEM((NGP, D, E), U32),
            pltpu.VMEM((6, DB, D // 2, 128), U32),
            pltpu.VMEM((DB, NSEG * M, E), BF16),
            pltpu.VMEM((DB, NSEG * M, 128), F32),
            pltpu.VMEM((2 * KMAJ, NSEG * M, E), F32),
            pltpu.VMEM((DB, 16, 128), BF16),
            pltpu.VMEM((D, 128), F32),
            pltpu.VMEM((NSEG, SEG, D), BF16),
            pltpu.VMEM((NSEG, SEG, D), BF16),
            pltpu.VMEM((NSEG, SEG, D), BF16),
            pltpu.VMEM((M, D), BF16),
            pltpu.VMEM((8, S // 8), F32),
            pltpu.VMEM((PR, PR), F32),
            pltpu.VMEM((8, 128), F32),
            pltpu.VMEM((1, D), BF16),
            pltpu.VMEM((D,), BF16),
            pltpu.SemaphoreType.DMA((NSEM,)),
        ],
        compiler_params=pltpu.CompilerParams(
            vmem_limit_bytes=120 * 1024 * 1024, disable_bounds_checks=True,
            disable_semaphore_checks=True),
    )(
        A_x.reshape(NSEG, SEG, D),
        A_mem0.reshape(M, D),
        A_Wq, A_Wk, A_Wv,
        A_Wo.reshape(H * E, D),
        B_w_r,
        B_w_gate, B_w_up, B_w_down,
        c, w_mod,
    )
    return out.reshape(1, S, D)
```

```python
import jax
import jax.numpy as jnp
from jax import lax
import jax.experimental.pallas as pl
import jax.experimental.pallas.tpu as pltpu

BF16 = jnp.bfloat16
F32 = jnp.float32
U32 = jnp.uint32

S = 2048
D = 1024
H = 32
E = 128
M = 8
SEG = 32
NSEG = S // SEG
NPAIR = H // 2
NGP = 3 * NPAIR
F = 3584
DB = D // 128
FB = F // 128
PR = 2 * SEG + 2 * M
UNR = 4
NIT = NSEG // UNR
KMAJ = 12
AHEAD = 3
PPI = 6
NSPLIT = 3
KEARLY = 5
HA = 24
SIDE_SLOTS = [("softmax", 8), (0, 2), (0, 5), (0, 7)]
MOD_SLOTS = (11, 7)
H_SLOTS = (6, 8)
EPS = 1e-5
SCALE = E ** (-0.5)

SEM_SMALL = 0
SEM_X = SEM_SMALL + 3
SEM_MOD = SEM_X + 2
SEM_MOD2 = SEM_MOD + DB
SEM_WQ = SEM_MOD2 + 4
SEM_ST = SEM_WQ + DB
SEM_WO = SEM_ST + (NGP - KMAJ) // PPI
SEM_MOE = SEM_WO + 1
SEM_OUT = SEM_MOE + 2
NSEM = SEM_OUT + 3


def _rb(v):
    return v.astype(BF16).astype(F32)


def _dot(a, b):
    return jnp.dot(a, b, preferred_element_type=F32)


def _recip(x):
    r = pl.reciprocal(x, approx=True)
    return r * (2.0 - x * r)


def _bf(words):
    return pltpu.bitcast(words, BF16)


def _ln(x):
    m = jnp.mean(x, axis=-1, keepdims=True)
    mb = _rb(m)
    d = x - mb
    var = jnp.mean(d * d, axis=-1, keepdims=True) - (m - mb) * (m - mb)
    inv = _recip(_rb(jnp.sqrt(_rb(_rb(jnp.maximum(var, 0.0)) + EPS))))
    return d * inv, inv


def _fill_matrix():
    i = lax.broadcasted_iota(jnp.int32, (PR, PR), 0)
    j = lax.broadcasted_iota(jnp.int32, (PR, PR), 1)

    def head(t):
        return jnp.where(t < 2 * SEG, t >> 5, (t - 2 * SEG) >> 3)

    def pos(t):
        r = t & (SEG - 1)
        return jnp.where(t < 2 * SEG, jnp.where(r < M, r, r + M), M + (t & (M - 1)))

    same = head(i) == head(j)
    pi = pos(i)
    ok = jnp.where(pi < M, 1, jnp.where(pi >= pos(j), 1, 0))
    return jnp.where(same, jnp.where(ok == 1, 0.0, -1e9), -3e38).astype(F32)


def _kernel(x_hbm, mem0_hbm, wq_hbm, wk_hbm, wv_hbm, wo_hbm, wr_hbm, wg_hbm, wu_hbm, wd_hbm,
            c_hbm, wmod_hbm, out_hbm,
            x_v, w_v, wo_v, cache, lhs_v, qkv_s, o_s, acc_s, mod_v, ab_v,
            stage, wmod_v, hc, n_v, acc, sc_row, sc_col, x1_v, h2_v, out_v,
            mem0_v, r_v, fill_v, never_v, c_v, wr_v, sems):
    w_w = w_v.bitcast(U32)
    cache_w = cache.bitcast(U32)
    lhs_w = lhs_v.bitcast(U32)
    qkv_w = qkv_s.bitcast(U32)
    o_w = o_s.bitcast(U32)

    def weights(h, j0=0, j1=DB):
        return _bf(w_w[h, pl.ds(j0, j1 - j0)].reshape((j1 - j0) * 64, E))

    def tie(v, tok, r0=0):
        if tok is None:
            return v
        tok = jnp.broadcast_to(tok, (8, 128))
        if v.dtype != F32:
            tok = pltpu.bitcast(tok, v.dtype)
        parts = [jnp.where(never_v[...] > 1.0, tok, v[r0:r0 + 8])]
        if r0 > 0:
            parts.insert(0, v[:r0])
        if r0 + 8 < v.shape[0]:
            parts.append(v[r0 + 8:])
        return jnp.concatenate(parts, axis=0)

    def copy(src, dst, sem):
        return pltpu.make_async_copy(src, dst, sems.at[sem])

    def wait_all(buf, sem):
        copy(buf, buf, sem).wait()

    def mod_row(k, rows=8):
        v = mod_v[k]
        return v if rows == 8 else jnp.concatenate([v] * (rows // 8), axis=0)

    def put_rows(dst, r0, v):
        for j in range(DB):
            dst[j, pl.ds(r0, v.shape[0]), :] = v[:, j * 128:(j + 1) * 128].astype(BF16)

    def prologue():
        wmod_w = wmod_hbm.bitcast(U32)
        w_words = [w.bitcast(U32) for w in (wq_hbm, wk_hbm, wv_hbm)]

        def start_mod(j):
            col = j * 128 if isinstance(j, int) else pl.multiple_of(j * 128, 128)
            for k in range(2):
                copy(wmod_w.at[:, pl.ds(k * D + col, 128)], wmod_v.at[k, j], SEM_MOD + j).start()

        def wait_mod(j):
            wait_all(wmod_v.at[pl.ds(0, 2), j], SEM_MOD + j)

        def start_chunk(k):
            col = k * D if isinstance(k, int) else pl.multiple_of(k * D, D)
            for j in range(DB):
                copy(wmod_w.at[:, pl.ds(col + j * 128, 128)], wmod_v.at[k, j], SEM_MOD2 + k - 2).start()

        def start_ktile(j):
            rows = pl.ds(j * 128 if isinstance(j, int) else pl.multiple_of(j * 128, 128), 128)
            for g in range(KMAJ):
                copy(w_words[0].at[rows, g, :], stage.at[g, rows, :], SEM_WQ + j).start()

        small = [copy(c_hbm, c_v, SEM_SMALL), copy(mem0_hbm, mem0_v, SEM_SMALL + 1),
                 copy(wr_hbm, wr_v, SEM_SMALL + 2)]
        x_head = copy(x_hbm.at[:, pl.ds(0, M), :], x_v.at[:, pl.ds(0, M), :], SEM_X)
        x_tail = copy(x_hbm.at[:, pl.ds(M, SEG - M), :], x_v.at[:, pl.ds(M, SEG - M), :], SEM_X + 1)
        for cp in small:
            cp.start()
        x_head.start()
        start_mod(0)
        for j in range(AHEAD):
            start_ktile(j)
            start_mod(j + 1)
        slab_cps = [copy(w_words[g // NPAIR].at[:, g % NPAIR, :], stage.at[g], SEM_ST + (g - KMAJ) // PPI)
                    for g in range(KMAJ, NGP)]

        fill_v[...] = _fill_matrix()
        x1_v[0] = jnp.zeros((SEG, D), BF16)
        r_v[...] = jnp.full(r_v.shape, -jnp.inf, F32)
        never_v[...] = jnp.zeros(never_v.shape, F32)
        qkv_s[0] = jnp.zeros((2 * SEG, E), BF16)
        o_s[0] = jnp.zeros(o_s.shape[1:], BF16)
        acc_s[0] = jnp.zeros(acc_s.shape[1:], F32)

        def zero_acc(h, carry):
            acc[h] = jnp.zeros((NSEG * M, E), F32)
            return carry

        lax.fori_loop(0, 2 * KMAJ, zero_acc, 0)

        for cp in small:
            cp.wait()
        c = c_v[...].astype(F32)
        sc = _rb(c * jax.nn.sigmoid(c))
        put_rows(sc_row, 0, jnp.broadcast_to(sc, (16, D)))
        for j in range(DB):
            sc_col[pl.ds(j * 128, 128), :] = jnp.broadcast_to(sc[:, j * 128:(j + 1) * 128], (128, 128)).T
        mod_v[6] = jnp.broadcast_to(wr_v[...].astype(F32).reshape(1, D), (8, D))
        put_rows(lhs_v.at[0], 0, mem0_v[...].astype(F32))

        x_head.wait()
        NB = 16
        RB = NSEG * M // NB
        for b in range(NB):
            xb = x_v[pl.ds(b * (NSEG // NB), NSEG // NB), pl.ds(0, M), :].astype(F32).reshape(RB, D)
            nb = _ln(xb)[0]
            for j in range(DB):
                n_v[j, pl.ds(b * RB, RB), :] = nb[:, j * 128:(j + 1) * 128]

        hc_w = hc.bitcast(U32)
        sc_w = sc_row.bitcast(U32)

        def mod_vpu(k, j):
            v = jnp.sum(_bf(wmod_v[k, j]).astype(F32) * sc_col[...], axis=0, keepdims=True)
            return _rb(jnp.broadcast_to(v, (8, 128)))

        def mod_block(j, k, src=None):
            if src is None:
                scb = jnp.concatenate([_bf(sc_w[i]) for i in range(DB)], axis=1)
                v = _rb(_dot(scb, _bf(wmod_v[k, j]))[0:8])
            else:
                v = mod_vpu(k, src)
            if k == 1:
                v = _rb(1.0 + v)
            col = j * 128 if isinstance(j, int) else pl.multiple_of(j * 128, 128)
            ab_v[k, :, pl.ds(col, 128)] = v
            return v

        def h_block(j, ca, sa, r0=0, nr=NSEG * M):
            n = n_v[j, pl.ds(r0, nr), :].reshape(nr // M, M, 128)
            hc[j, pl.ds(r0, nr), :] = (n * ca[None] + sa[None]).reshape(nr, 128).astype(BF16)

        def pack_pair(r1, r2):
            r = jnp.concatenate([r1.reshape(NSEG, M, E), r2.reshape(NSEG, M, E)], axis=1)
            return r.reshape(NIT, UNR * 2 * M, E).astype(BF16)

        def split_pair(b):
            return (pltpu.bitcast(b << 16, F32).astype(BF16),
                    pltpu.bitcast(b & jnp.uint32(0xFFFF0000), F32).astype(BF16))

        def q_stage(j, last, more_dmas):
            static = isinstance(j, int)
            k0 = j * 128 if static else pl.multiple_of(j * 128, 128)
            src = None if last else jnp.where(j == 0, 0, j + 1)
            mods = {}
            for p in range(KMAJ):
                ws = split_pair(stage[p, pl.ds(k0, 128), :])
                rs = []
                for t in range(2):
                    h = 2 * p + t
                    w_v[h, j] = ws[t]
                    lw = hc_w[j]
                    if not last and h in MOD_SLOTS:
                        k = MOD_SLOTS.index(h)
                        mods[k] = mod_block(j + 1, k, src)
                        lw = tie(lw, mods[k], NSEG * M // 4)
                    rs.append(_dot(_bf(lw), _bf(w_w[h, j])) + acc[h])
                    if not last:
                        acc[h] = rs[t]
                if last:
                    cache[p] = pack_pair(*rs)
                elif p in H_SLOTS:
                    nr = NSEG * M // len(H_SLOTS)
                    h_block(j + 1, tie(mods[1], rs[0][0:8]), mods[0], H_SLOTS.index(p) * nr, nr)
                if p == (1 if last else KMAJ - 3):
                    more_dmas()

        wait_mod(0)
        h_block(0, mod_block(0, 1), mod_block(0, 0))

        def wait_ktile(j):
            rows = pl.ds(j * 128 if isinstance(j, int) else pl.multiple_of(j * 128, 128), 128)
            wait_all(stage.at[pl.ds(0, KMAJ), rows, :], SEM_WQ + j)

        def q_body(j, carry):
            @pl.when(j == 1)
            def _():
                wait_mod(1)
                h_block(1, mod_block(1, 1), mod_block(1, 0))

            wait_ktile(j)

            @pl.when(j > 0)
            def _():
                wait_mod(j + 1)

            def more_dmas():
                @pl.when(j + AHEAD < DB)
                def _():
                    start_ktile(j + AHEAD)

                @pl.when(j + AHEAD + 1 < DB)
                def _():
                    start_mod(j + AHEAD + 1)

                @pl.when(j + AHEAD == DB - 1)
                def _():
                    for cp in slab_cps[:2 * PPI]:
                        cp.start()

            q_stage(j, False, more_dmas)
            return carry

        lax.fori_loop(0, DB - 1, q_body, 0)
        wait_ktile(DB - 1)

        def last_dmas():
            for i in range(2, 5):
                for cp in slab_cps[i * PPI:(i + 1) * PPI]:
                    cp.start()
                if i < 4:
                    start_chunk(i)
                if i == 2:
                    x_tail.start()

        q_stage(DB - 1, True, last_dmas)

        def pro_body(i, carry):
            g0 = KMAJ + i * PPI
            wait_all(stage.at[pl.ds(g0, PPI)], SEM_ST + i)

            @pl.when(i >= 2)
            def _():
                wait_all(wmod_v.at[i], SEM_MOD2 + i - 2)

            @pl.when(i == 2)
            def _():
                x_tail.wait()

            def more_dmas():
                @pl.when(i < 2)
                def _():
                    start_chunk(i + 4)

                @pl.when(i == 0)
                def _():
                    for cp in slab_cps[5 * PPI:]:
                        cp.start()

                @pl.when(jnp.logical_and(i >= 2, i < 4))
                def _():
                    wo_w = wo_hbm.bitcast(U32)
                    for t in range(DB // 2):
                        j = (i - 2) * (DB // 2) + t
                        cols = pl.ds(pl.multiple_of(j * 128, 128), 128)
                        copy(wo_w.at[:, cols], wo_v.at[j], SEM_WO).start()

            one = jnp.where(jnp.logical_or(i == 1, i == 4), 1.0, 0.0)

            def mod_cols(j):
                v = _rb(one + mod_vpu(i, j))
                mod_v[i, :, pl.ds(j * 128, 128)] = v
                return v

            def ln_rows(n):
                seg = jnp.maximum(i - 2, 0) * (NSEG // 4) + n // 3
                r0 = (n % 3 + 1) * 8
                src = pl.multiple_of(jnp.where(i >= 2, r0, 0), 8)
                nrm, inv = _ln(x_v[seg, pl.ds(src, 8), :].astype(F32))
                put_rows(lhs_v.at[seg], r0, nrm * ab_v[1] + ab_v[0])
                return inv

            LPD = 3 * (NSEG // 4) // (2 * PPI)
            for t in range(PPI):
                gp = g0 + t
                w_v[2 * gp], w_v[2 * gp + 1] = split_pair(stage[gp].reshape(DB, 128, E))
                rs = []
                for hh in range(2):
                    n = 2 * t + hh - (2 * PPI - DB)
                    parts = [hc_w[j] for j in range(DB)]
                    parts[0] = tie(parts[0], mod_cols(n) if n >= 0 else None)
                    for k in range(LPD):
                        parts[-1] = tie(parts[-1], ln_rows((2 * t + hh) * LPD + k),
                                        k * (NSEG * M // 2 // LPD))
                    hcv = jnp.concatenate([_bf(w) for w in parts], axis=1)
                    rs.append(_dot(hcv, weights(2 * gp + hh)))
                cache[gp] = pack_pair(*rs)
                if t == 0:
                    more_dmas()
            return carry

        lax.fori_loop(0, (NGP - KMAJ) // PPI, pro_body, 0)

    prologue()

    def main():
        lane = lax.broadcasted_iota(jnp.int32, (8, 2 * 128), 1)

        def post(seg, q, keep=True):
            rows = pl.ds(8 * q, 8)
            x1 = x1_v[seg, rows, :].astype(F32)
            n, inv = _ln(x1)
            h2 = _rb(n * mod_row(4) + mod_row(3))
            r = _rb(jnp.sum(h2 * mod_row(6), axis=-1, keepdims=True))
            if keep:
                r_v[...] = jnp.where(lane == seg * 4 + q, r, r_v[...])
            h2_v[seg, rows, :] = h2.astype(BF16)
            out_v[seg, rows, :] = (x1 + mod_row(5) * h2).astype(BF16)
            return inv, r

        def out_copy(grp):
            return copy(out_v.at[pl.ds(grp * UNR, UNR)], out_hbm.at[pl.ds(grp * UNR, UNR)], SEM_OUT)

        wg_w, wu_w, wd_w = wg_hbm.bitcast(U32), wu_hbm.bitcast(U32), wd_hbm.bitcast(U32)
        wait_all(wo_v, SEM_WO)

        def step(it, u):
            s = it * UNR + u
            lhs = jnp.concatenate([_bf(lhs_w[s, j]) for j in range(DB)], axis=1)

            def side(slot):
                if slot not in SIDE_SLOTS:
                    return None
                q = SIDE_SLOTS.index(slot)
                return post(jnp.maximum(s - (2 if q == 0 else 1), 0), q)[0]

            def proj(m_i, p):
                g = m_i * NPAIR + p
                for t in range(2):
                    qkv_s[g, pl.ds(t * SEG, SEG), :] = _dot(lhs, weights(2 * g + t)).astype(BF16)

            def rows_of(m_i, p):
                g = m_i * NPAIR + p
                return jnp.concatenate([_bf(qkv_w[g]), _bf(cache_w[g, it, pl.ds(u * M, M), :])], axis=0)

            def probs(p):
                parts = [lax.dot_general(_bf(qkv_w[p]), rows_of(1, p), (((1,), (1,)), ((), ())),
                                         preferred_element_type=F32)]
                qc = _bf(cache_w[p, it, pl.ds(u * M, M), :]).astype(F32)
                kc = _bf(cache_w[NPAIR + p, it, pl.ds(u * M, M), :]).astype(F32)
                col = lax.broadcasted_iota(jnp.int32, (M, PR), 1)
                for t in range(2):
                    km = _bf(qkv_w[NPAIR + p, pl.ds(t * (SEG // 2), 8), :]).astype(F32)
                    qt = qc[t * M:(t + 1) * M]
                    st = jnp.zeros((M, PR), F32)
                    for j in range(M):
                        st = jnp.where(col == t * SEG + j,
                                       jnp.sum(qt * km[j:j + 1], axis=-1, keepdims=True), st)
                        st = jnp.where(col == 2 * SEG + t * M + j,
                                       jnp.sum(qt * kc[t * M + j:t * M + j + 1], axis=-1, keepdims=True), st)
                    parts.append(st)
                sc = jnp.concatenate(parts, axis=0) * SCALE
                fm = fill_v[...]
                tok = side(("softmax", p))
                if tok is not None:
                    top = fm[0:8]
                    fm = jnp.concatenate([jnp.where(top > 1.0, tok, top), fm[8:]], axis=0)
                sc = jnp.where(fm == 0.0, sc, fm)
                e = jnp.exp(sc - jnp.max(sc, axis=-1, keepdims=True))
                return (e * _recip(jnp.sum(e, axis=-1, keepdims=True))).astype(BF16)

            def attend(p, pr):
                o = _dot(pr, rows_of(2, p))
                for t in range(2):
                    o_s[2 * p + t, pl.ds(0, SEG), :] = o[t * SEG:(t + 1) * SEG].astype(BF16)
                for t in range(2):
                    o_s[2 * p + t, pl.ds(SEG + (u % 2) * M, M), :] = (
                        o[2 * SEG + t * M:2 * SEG + (t + 1) * M].astype(BF16))

            ps = {}
            for pa in range(0, NPAIR, 2):
                pb = pa + 1
                todo = [(0, pa), (1, pa), (0, pb), (1, pb), (2, pa), (2, pb)]
                if pa == 0 and u > 0:
                    hs = [(m_i * NPAIR + p, t) for m_i, p in todo[:NSPLIT] for t in range(2)]
                    ke = KEARLY * 128
                    first = [_dot(lhs[:, :ke], weights(2 * g + t, 0, KEARLY)) for g, t in hs]
                    for (g, t), part in zip(hs, first):
                        res = _dot(lhs[:, ke:], weights(2 * g + t, KEARLY, DB)) + part
                        qkv_s[g, pl.ds(t * SEG, SEG), :] = res.astype(BF16)
                    todo = todo[NSPLIT:]
                for m_i, p in todo:
                    proj(m_i, p)
                for kind in ("scores", "values") if pa % 4 == 0 else ("values", "scores"):
                    for p in (pa, pb):
                        if kind == "scores":
                            ps[p] = probs(p)
                        elif p >= 2:
                            attend(p - 2, ps.pop(p - 2))
            L = NPAIR - 1

            nxt = s + 1 if u < UNR - 1 else jnp.where(it < NIT - 1, s + 1, 0)
            nr = SEG + (2 * M if u % 2 else 0)
            for h0, h1 in ((0, HA), (HA, H)):
                for j in range(DB):
                    words = [o_w[h, pl.ds(0, nr // 2), :] for h in range(h0, h1)]
                    words[0] = tie(words[0], side((h0, j)))
                    ol = jnp.concatenate([_bf(w) for w in words], axis=1)
                    part = _dot(ol, _bf(wo_v[j, pl.ds(h0 * E // 2, (h1 - h0) * E // 2), :]))
                    if h0 == 0:
                        acc_s[j, pl.ds(0, nr), :] = part
                    else:
                        a = part + acc_s[j, pl.ds(0, nr), :]
                        cols = pl.ds(j * 128, 128)
                        lhs_v[nxt, j, pl.ds(0, M), :] = a[0:M].astype(BF16)
                        for q in range(1, nr // M):
                            seg, rows = (s, pl.ds(q * M, M)) if q < 4 else (s + q - 5, pl.ds(0, M))
                            x1 = x_v[seg, rows, cols].astype(F32) + mod_v[2, :, cols] * a[q * M:(q + 1) * M]
                            x1_v[seg, rows, cols] = x1.astype(BF16)
                    if h0 == 0 and j == 4:
                        attend(L - 1, ps.pop(L - 1))
                        attend(L, ps.pop(L))

        def iteration(it, carry):
            @pl.when(it >= 2)
            def _():
                out_copy(it - 2).start()

            @pl.when(it < FB // 2)
            def _():
                for t in range(2):
                    j = 2 * it + t
                    cols = pl.ds(pl.multiple_of(j * 128, 128), 128)
                    half = pl.ds(t * (D // 2), D // 2)
                    copy(wg_w.at[:, cols], stage.at[it, half, :], SEM_MOE).start()
                    copy(wu_w.at[:, cols], stage.at[FB // 2 + it, half, :], SEM_MOE).start()

            @pl.when(it < DB)
            def _():
                cols = pl.ds(pl.multiple_of(it * 128, 128), 128)
                for t in range(2):
                    copy(wd_w.at[pl.ds(t * (F // 4), F // 4), cols],
                         stage.at[FB + 2 * it + t, pl.ds(0, F // 4), :], SEM_MOE + 1).start()

            for u in range(UNR):
                step(it, u)
            return carry

        lax.fori_loop(0, NIT, iteration, 0)

        out_copy(NIT - 2).start()
        wait_all(stage.at[pl.ds(0, FB)], SEM_MOE)
        wait_all(stage.at[pl.ds(FB, 2 * DB), pl.ds(0, F // 4), :], SEM_MOE + 1)
        r8 = lax.broadcasted_iota(jnp.int32, (8, 1), 0)

        def top2(vals, idx, axes):
            def red(f, v):
                for ax in axes:
                    v = f(v, axis=ax, keepdims=True)
                return v
            m1 = red(jnp.max, vals)
            i1 = red(jnp.min, jnp.where(vals == m1, idx, S - 1.0))
            rest = jnp.where(idx == i1, -jnp.inf, vals)
            m2 = red(jnp.max, rest)
            i2 = red(jnp.min, jnp.where(rest == m2, jnp.where(idx == i1, S - 1.0, idx), S - 1.0))
            return m1, i1, m2, i2

        m1, i1v, m2, i2v = top2(r_v[...], (lane * 8 + r8).astype(F32), (1, 0))
        vals = [jnp.where(r8 == 0, m1, jnp.where(r8 == 1, m2, -jnp.inf))]
        idxs = [jnp.where(r8 == 0, i1v, jnp.where(r8 == 1, i2v, S - 1.0))]
        for seg, q in [(NSEG - 2, 0)] + [(NSEG - 1, q) for q in range(4)]:
            vals.append(post(seg, q, keep=False)[1])
            idxs.append((r8 + (seg * SEG + q * 8)).astype(F32))
        out_copy(NIT - 1).start()
        m1, i1v, m2, i2v = top2(jnp.concatenate(vals, axis=0), jnp.concatenate(idxs, axis=0), (0,))
        i1 = i1v.astype(jnp.int32)[0, 0]
        i2 = i2v.astype(jnp.int32)[0, 0]

        def tile_of(i):
            return i >> 5, pl.multiple_of(((i >> 3) & 3) * 8, 8)

        sel = [tile_of(i1), tile_of(i2)]
        x1s = jnp.concatenate([x1_v[sg, pl.ds(r0, 8), :].astype(F32) for sg, r0 in sel], axis=0)
        h2s = jnp.concatenate([h2_v[sg, pl.ds(r0, 8), :].astype(F32) for sg, r0 in sel], axis=0)
        h2b = h2s.astype(BF16)
        gus = []
        for j in range(FB):
            half = pl.ds((j % 2) * (D // 2), D // 2)
            g = _rb(_dot(h2b, _bf(stage[j // 2, half, :])))
            g = _rb(g * jax.nn.sigmoid(g))
            u = _rb(_dot(h2b, _bf(stage[FB // 2 + j // 2, half, :])))
            gus.append(g * u)
        gu = jnp.concatenate(gus, axis=1).astype(BF16)
        ys = []
        for j in range(DB):
            wd = stage[pl.ds(FB + 2 * j, 2), pl.ds(0, F // 4), :].reshape(F // 2, 128)
            ys.append(_rb(_dot(gu, _bf(wd))))
        y = jnp.concatenate(ys, axis=1)
        rows = lax.broadcasted_iota(jnp.int32, (16, 1), 0)
        rs = _rb(jax.nn.sigmoid(jnp.where(rows < 8, m1, m2)))
        y = _rb(y * rs)
        full = x1s + mod_row(5, 16) * _rb(h2s + y)

        copy(out_v, out_hbm, SEM_OUT).wait()
        for t, (i, (sg, r0)) in enumerate(zip((i1, i2), sel)):
            old = out_v[sg, pl.ds(r0, 8), :].astype(F32)
            new = jnp.where(r8 == (i & 7), full[t * 8:(t + 1) * 8], old)
            out_v[sg, pl.ds(r0, 8), :] = new.astype(BF16)
        fix = [copy(out_v.at[sg, pl.ds(r0, 8), :], out_hbm.at[sg, pl.ds(r0, 8), :], SEM_OUT + 1 + t)
               for t, (sg, r0) in enumerate(sel)]
        differ = (i1 >> 3) != (i2 >> 3)
        fix[0].start()

        @pl.when(differ)
        def _():
            fix[1].start()
            fix[1].wait()

        fix[0].wait()

    main()


@jax.jit
def pallas_adaLN_cond__memory_aug_recurrent_mem_tr__moe_arch_mod__prompt_kernel(
    A_x: jax.Array,
    A_mem0: jax.Array,
    A_Wq: jax.Array,
    A_Wk: jax.Array,
    A_Wv: jax.Array,
    A_Wo: jax.Array,
    A_seg_len: jax.Array,
    B_x: jax.Array,
    B_w_r: jax.Array,
    B_w_gate: jax.Array,
    B_w_up: jax.Array,
    B_w_down: jax.Array,
    c: jax.Array,
    w_mod: jax.Array,
):
    del A_seg_len, B_x
    assert A_x.shape == (1, S, D) and A_mem0.shape == (1, M, D) and A_Wq.shape == (D, H, E)
    hbm = pl.BlockSpec(memory_space=pl.ANY)
    out = pl.pallas_call(
        _kernel,
        out_shape=jax.ShapeDtypeStruct((NSEG, SEG, D), BF16),
        in_specs=[hbm] * 12,
        out_specs=hbm,
        scratch_shapes=[
            pltpu.VMEM((NSEG, SEG, D), BF16),
            pltpu.VMEM((3 * H, DB, 128, E), BF16),
            pltpu.VMEM((DB, H * E // 2, 128), U32),
            pltpu.VMEM((NGP, NIT, UNR * 2 * M, E), BF16),
            pltpu.VMEM((NSEG, DB, SEG, 128), BF16),
            pltpu.VMEM((NGP, 2 * SEG, E), BF16),
            pltpu.VMEM((H, 2 * SEG, E), BF16),
            pltpu.VMEM((DB, 2 * SEG, 128), F32),
            pltpu.VMEM((7, 8, D), F32),
            pltpu.VMEM((2, 8, D), F32),
            pltpu.VMEM((NGP, D, E), U32),
            pltpu.VMEM((6, DB, D // 2, 128), U32),
            pltpu.VMEM((DB, NSEG * M, E), BF16),
            pltpu.VMEM((DB, NSEG * M, 128), F32),
            pltpu.VMEM((2 * KMAJ, NSEG * M, E), F32),
            pltpu.VMEM((DB, 16, 128), BF16),
            pltpu.VMEM((D, 128), F32),
            pltpu.VMEM((NSEG, SEG, D), BF16),
            pltpu.VMEM((NSEG, SEG, D), BF16),
            pltpu.VMEM((NSEG, SEG, D), BF16),
            pltpu.VMEM((M, D), BF16),
            pltpu.VMEM((8, S // 8), F32),
            pltpu.VMEM((PR, PR), F32),
            pltpu.VMEM((8, 128), F32),
            pltpu.VMEM((1, D), BF16),
            pltpu.VMEM((D,), BF16),
            pltpu.SemaphoreType.DMA((NSEM,)),
        ],
        compiler_params=pltpu.CompilerParams(
            vmem_limit_bytes=120 * 1024 * 1024, disable_bounds_checks=True,
            disable_semaphore_checks=True),
    )(
        A_x.reshape(NSEG, SEG, D),
        A_mem0.reshape(M, D),
        A_Wq, A_Wk, A_Wv,
        A_Wo.reshape(H * E, D),
        B_w_r,
        B_w_gate, B_w_up, B_w_down,
        c, w_mod,
    )
    return out.reshape(1, S, D)
```

```python
import jax
import jax.numpy as jnp
from jax import lax
import jax.experimental.pallas as pl
import jax.experimental.pallas.tpu as pltpu

BF16 = jnp.bfloat16
F32 = jnp.float32
U32 = jnp.uint32

S = 2048
D = 1024
H = 32
E = 128
M = 8
SEG = 32
NSEG = S // SEG
NPAIR = H // 2
NGP = 3 * NPAIR
F = 3584
DB = D // 128
FB = F // 128
PR = 2 * SEG + 2 * M
UNR = 4
NIT = NSEG // UNR
KMAJ = 12
AHEAD = 3
PPI = 6
NSPLIT = 3
KEARLY = 6
HA = 24
SIDE_SLOTS = [("softmax", 8), (0, 2), (0, 5), (0, 7)]
MOD_SLOTS = (11, 7)
H_SLOTS = (6, 8)
EPS = 1e-5
SCALE = E ** (-0.5)

SEM_SMALL = 0
SEM_X = SEM_SMALL + 3
SEM_MOD = SEM_X + 2
SEM_MOD2 = SEM_MOD + DB
SEM_WQ = SEM_MOD2 + 4
SEM_ST = SEM_WQ + DB
SEM_WO = SEM_ST + (NGP - KMAJ) // PPI
SEM_MOE = SEM_WO + 1
SEM_OUT = SEM_MOE + 2
NSEM = SEM_OUT + 3


def _rb(v):
    return v.astype(BF16).astype(F32)


def _dot(a, b):
    return jnp.dot(a, b, preferred_element_type=F32)


def _recip(x):
    r = pl.reciprocal(x, approx=True)
    return r * (2.0 - x * r)


def _bf(words):
    return pltpu.bitcast(words, BF16)


def _ln(x):
    m = jnp.mean(x, axis=-1, keepdims=True)
    mb = _rb(m)
    d = x - mb
    var = jnp.mean(d * d, axis=-1, keepdims=True) - (m - mb) * (m - mb)
    inv = _recip(_rb(jnp.sqrt(_rb(_rb(jnp.maximum(var, 0.0)) + EPS))))
    return d * inv, inv


def _fill_matrix():
    i = lax.broadcasted_iota(jnp.int32, (PR, PR), 0)
    j = lax.broadcasted_iota(jnp.int32, (PR, PR), 1)

    def head(t):
        return jnp.where(t < 2 * SEG, t >> 5, (t - 2 * SEG) >> 3)

    def pos(t):
        r = t & (SEG - 1)
        return jnp.where(t < 2 * SEG, jnp.where(r < M, r, r + M), M + (t & (M - 1)))

    same = head(i) == head(j)
    pi = pos(i)
    ok = jnp.where(pi < M, 1, jnp.where(pi >= pos(j), 1, 0))
    return jnp.where(same, jnp.where(ok == 1, 0.0, -1e9), -3e38).astype(F32)


def _kernel(x_hbm, mem0_hbm, wq_hbm, wk_hbm, wv_hbm, wo_hbm, wr_hbm, wg_hbm, wu_hbm, wd_hbm,
            c_hbm, wmod_hbm, out_hbm,
            x_v, w_v, wo_v, cache, lhs_v, qkv_s, o_s, acc_s, mod_v, ab_v,
            stage, wmod_v, hc, n_v, acc, sc_row, sc_col, x1_v, h2_v, out_v,
            mem0_v, r_v, fill_v, never_v, c_v, wr_v, sems):
    w_w = w_v.bitcast(U32)
    cache_w = cache.bitcast(U32)
    lhs_w = lhs_v.bitcast(U32)
    qkv_w = qkv_s.bitcast(U32)
    o_w = o_s.bitcast(U32)

    def weights(h, j0=0, j1=DB):
        return _bf(w_w[h, pl.ds(j0, j1 - j0)].reshape((j1 - j0) * 64, E))

    def tie(v, tok, r0=0):
        if tok is None:
            return v
        tok = jnp.broadcast_to(tok, (8, 128))
        if v.dtype != F32:
            tok = pltpu.bitcast(tok, v.dtype)
        parts = [jnp.where(never_v[...] > 1.0, tok, v[r0:r0 + 8])]
        if r0 > 0:
            parts.insert(0, v[:r0])
        if r0 + 8 < v.shape[0]:
            parts.append(v[r0 + 8:])
        return jnp.concatenate(parts, axis=0)

    def copy(src, dst, sem):
        return pltpu.make_async_copy(src, dst, sems.at[sem])

    def wait_all(buf, sem):
        copy(buf, buf, sem).wait()

    def mod_row(k, rows=8):
        v = mod_v[k]
        return v if rows == 8 else jnp.concatenate([v] * (rows // 8), axis=0)

    def put_rows(dst, r0, v):
        for j in range(DB):
            dst[j, pl.ds(r0, v.shape[0]), :] = v[:, j * 128:(j + 1) * 128].astype(BF16)

    def prologue():
        wmod_w = wmod_hbm.bitcast(U32)
        w_words = [w.bitcast(U32) for w in (wq_hbm, wk_hbm, wv_hbm)]

        def start_mod(j):
            col = j * 128 if isinstance(j, int) else pl.multiple_of(j * 128, 128)
            for k in range(2):
                copy(wmod_w.at[:, pl.ds(k * D + col, 128)], wmod_v.at[k, j], SEM_MOD + j).start()

        def wait_mod(j):
            wait_all(wmod_v.at[pl.ds(0, 2), j], SEM_MOD + j)

        def start_chunk(k):
            col = k * D if isinstance(k, int) else pl.multiple_of(k * D, D)
            for j in range(DB):
                copy(wmod_w.at[:, pl.ds(col + j * 128, 128)], wmod_v.at[k, j], SEM_MOD2 + k - 2).start()

        def start_ktile(j):
            rows = pl.ds(j * 128 if isinstance(j, int) else pl.multiple_of(j * 128, 128), 128)
            for g in range(KMAJ):
                copy(w_words[0].at[rows, g, :], stage.at[g, rows, :], SEM_WQ + j).start()

        small = [copy(c_hbm, c_v, SEM_SMALL), copy(mem0_hbm, mem0_v, SEM_SMALL + 1),
                 copy(wr_hbm, wr_v, SEM_SMALL + 2)]
        x_head = copy(x_hbm.at[:, pl.ds(0, M), :], x_v.at[:, pl.ds(0, M), :], SEM_X)
        x_tail = copy(x_hbm.at[:, pl.ds(M, SEG - M), :], x_v.at[:, pl.ds(M, SEG - M), :], SEM_X + 1)
        for cp in small:
            cp.start()
        x_head.start()
        start_mod(0)
        for j in range(AHEAD):
            start_ktile(j)
            start_mod(j + 1)
        slab_cps = [copy(w_words[g // NPAIR].at[:, g % NPAIR, :], stage.at[g], SEM_ST + (g - KMAJ) // PPI)
                    for g in range(KMAJ, NGP)]

        fill_v[...] = _fill_matrix()
        x1_v[0] = jnp.zeros((SEG, D), BF16)
        r_v[...] = jnp.full(r_v.shape, -jnp.inf, F32)
        never_v[...] = jnp.zeros(never_v.shape, F32)
        qkv_s[0] = jnp.zeros((2 * SEG, E), BF16)
        o_s[0] = jnp.zeros(o_s.shape[1:], BF16)
        acc_s[0] = jnp.zeros(acc_s.shape[1:], F32)

        def zero_acc(h, carry):
            acc[h] = jnp.zeros((NSEG * M, E), F32)
            return carry

        lax.fori_loop(0, 2 * KMAJ, zero_acc, 0)

        for cp in small:
            cp.wait()
        c = c_v[...].astype(F32)
        sc = _rb(c * jax.nn.sigmoid(c))
        put_rows(sc_row, 0, jnp.broadcast_to(sc, (16, D)))
        for j in range(DB):
            sc_col[pl.ds(j * 128, 128), :] = jnp.broadcast_to(sc[:, j * 128:(j + 1) * 128], (128, 128)).T
        mod_v[6] = jnp.broadcast_to(wr_v[...].astype(F32).reshape(1, D), (8, D))
        put_rows(lhs_v.at[0], 0, mem0_v[...].astype(F32))

        x_head.wait()
        NB = 16
        RB = NSEG * M // NB
        for b in range(NB):
            xb = x_v[pl.ds(b * (NSEG // NB), NSEG // NB), pl.ds(0, M), :].astype(F32).reshape(RB, D)
            nb = _ln(xb)[0]
            for j in range(DB):
                n_v[j, pl.ds(b * RB, RB), :] = nb[:, j * 128:(j + 1) * 128]

        hc_w = hc.bitcast(U32)
        sc_w = sc_row.bitcast(U32)

        def mod_vpu(k, j):
            v = jnp.sum(_bf(wmod_v[k, j]).astype(F32) * sc_col[...], axis=0, keepdims=True)
            return _rb(jnp.broadcast_to(v, (8, 128)))

        def mod_block(j, k, src=None):
            if src is None:
                scb = jnp.concatenate([_bf(sc_w[i]) for i in range(DB)], axis=1)
                v = _rb(_dot(scb, _bf(wmod_v[k, j]))[0:8])
            else:
                v = mod_vpu(k, src)
            if k == 1:
                v = _rb(1.0 + v)
            col = j * 128 if isinstance(j, int) else pl.multiple_of(j * 128, 128)
            ab_v[k, :, pl.ds(col, 128)] = v
            return v

        def h_block(j, ca, sa, r0=0, nr=NSEG * M):
            n = n_v[j, pl.ds(r0, nr), :].reshape(nr // M, M, 128)
            hc[j, pl.ds(r0, nr), :] = (n * ca[None] + sa[None]).reshape(nr, 128).astype(BF16)

        def pack_pair(r1, r2):
            r = jnp.concatenate([r1.reshape(NSEG, M, E), r2.reshape(NSEG, M, E)], axis=1)
            return r.reshape(NIT, UNR * 2 * M, E).astype(BF16)

        def split_pair(b):
            return (pltpu.bitcast(b << 16, F32).astype(BF16),
                    pltpu.bitcast(b & jnp.uint32(0xFFFF0000), F32).astype(BF16))

        def q_stage(j, last, more_dmas):
            static = isinstance(j, int)
            k0 = j * 128 if static else pl.multiple_of(j * 128, 128)
            src = None if last else jnp.where(j == 0, 0, j + 1)
            mods = {}
            for p in range(KMAJ):
                ws = split_pair(stage[p, pl.ds(k0, 128), :])
                rs = []
                for t in range(2):
                    h = 2 * p + t
                    w_v[h, j] = ws[t]
                    lw = hc_w[j]
                    if not last and h in MOD_SLOTS:
                        k = MOD_SLOTS.index(h)
                        mods[k] = mod_block(j + 1, k, src)
                        lw = tie(lw, mods[k], NSEG * M // 4)
                    rs.append(_dot(_bf(lw), _bf(w_w[h, j])) + acc[h])
                    if not last:
                        acc[h] = rs[t]
                if last:
                    cache[p] = pack_pair(*rs)
                elif p in H_SLOTS:
                    nr = NSEG * M // len(H_SLOTS)
                    h_block(j + 1, tie(mods[1], rs[0][0:8]), mods[0], H_SLOTS.index(p) * nr, nr)
                if p == (1 if last else KMAJ - 3):
                    more_dmas()

        wait_mod(0)
        h_block(0, mod_block(0, 1), mod_block(0, 0))

        def wait_ktile(j):
            rows = pl.ds(j * 128 if isinstance(j, int) else pl.multiple_of(j * 128, 128), 128)
            wait_all(stage.at[pl.ds(0, KMAJ), rows, :], SEM_WQ + j)

        def q_body(j, carry):
            @pl.when(j == 1)
            def _():
                wait_mod(1)
                h_block(1, mod_block(1, 1), mod_block(1, 0))

            wait_ktile(j)

            @pl.when(j > 0)
            def _():
                wait_mod(j + 1)

            def more_dmas():
                @pl.when(j + AHEAD < DB)
                def _():
                    start_ktile(j + AHEAD)

                @pl.when(j + AHEAD + 1 < DB)
                def _():
                    start_mod(j + AHEAD + 1)

                @pl.when(j + AHEAD == DB - 1)
                def _():
                    for cp in slab_cps[:2 * PPI]:
                        cp.start()

            q_stage(j, False, more_dmas)
            return carry

        lax.fori_loop(0, DB - 1, q_body, 0)
        wait_ktile(DB - 1)

        def last_dmas():
            for i in range(2, 5):
                for cp in slab_cps[i * PPI:(i + 1) * PPI]:
                    cp.start()
                if i < 4:
                    start_chunk(i)
                if i == 2:
                    x_tail.start()

        q_stage(DB - 1, True, last_dmas)

        def pro_body(i, carry):
            g0 = KMAJ + i * PPI
            wait_all(stage.at[pl.ds(g0, PPI)], SEM_ST + i)

            @pl.when(i >= 2)
            def _():
                wait_all(wmod_v.at[i], SEM_MOD2 + i - 2)

            @pl.when(i == 2)
            def _():
                x_tail.wait()

            def more_dmas():
                @pl.when(i < 2)
                def _():
                    start_chunk(i + 4)

                @pl.when(i == 0)
                def _():
                    for cp in slab_cps[5 * PPI:]:
                        cp.start()

                @pl.when(jnp.logical_and(i >= 2, i < 4))
                def _():
                    wo_w = wo_hbm.bitcast(U32)
                    for t in range(DB // 2):
                        j = (i - 2) * (DB // 2) + t
                        cols = pl.ds(pl.multiple_of(j * 128, 128), 128)
                        copy(wo_w.at[:, cols], wo_v.at[j], SEM_WO).start()

            one = jnp.where(jnp.logical_or(i == 1, i == 4), 1.0, 0.0)

            def mod_cols(j):
                v = _rb(one + mod_vpu(i, j))
                mod_v[i, :, pl.ds(j * 128, 128)] = v
                return v

            def ln_rows(n):
                seg = jnp.maximum(i - 2, 0) * (NSEG // 4) + n // 3
                r0 = (n % 3 + 1) * 8
                src = pl.multiple_of(jnp.where(i >= 2, r0, 0), 8)
                nrm, inv = _ln(x_v[seg, pl.ds(src, 8), :].astype(F32))
                put_rows(lhs_v.at[seg], r0, nrm * ab_v[1] + ab_v[0])
                return inv

            LPD = 3 * (NSEG // 4) // (2 * PPI)
            for t in range(PPI):
                gp = g0 + t
                w_v[2 * gp], w_v[2 * gp + 1] = split_pair(stage[gp].reshape(DB, 128, E))
                rs = []
                for hh in range(2):
                    n = 2 * t + hh - (2 * PPI - DB)
                    parts = [hc_w[j] for j in range(DB)]
                    parts[0] = tie(parts[0], mod_cols(n) if n >= 0 else None)
                    for k in range(LPD):
                        parts[-1] = tie(parts[-1], ln_rows((2 * t + hh) * LPD + k),
                                        k * (NSEG * M // 2 // LPD))
                    hcv = jnp.concatenate([_bf(w) for w in parts], axis=1)
                    rs.append(_dot(hcv, weights(2 * gp + hh)))
                cache[gp] = pack_pair(*rs)
                if t == 0:
                    more_dmas()
            return carry

        lax.fori_loop(0, (NGP - KMAJ) // PPI, pro_body, 0)

    prologue()

    def main():
        lane = lax.broadcasted_iota(jnp.int32, (8, 2 * 128), 1)

        def post(seg, q, keep=True):
            rows = pl.ds(8 * q, 8)
            x1 = x1_v[seg, rows, :].astype(F32)
            n, inv = _ln(x1)
            h2 = _rb(n * mod_row(4) + mod_row(3))
            r = _rb(jnp.sum(h2 * mod_row(6), axis=-1, keepdims=True))
            if keep:
                r_v[...] = jnp.where(lane == seg * 4 + q, r, r_v[...])
            h2_v[seg, rows, :] = h2.astype(BF16)
            out_v[seg, rows, :] = (x1 + mod_row(5) * h2).astype(BF16)
            return inv, r

        def out_copy(grp):
            return copy(out_v.at[pl.ds(grp * UNR, UNR)], out_hbm.at[pl.ds(grp * UNR, UNR)], SEM_OUT)

        wg_w, wu_w, wd_w = wg_hbm.bitcast(U32), wu_hbm.bitcast(U32), wd_hbm.bitcast(U32)
        wait_all(wo_v, SEM_WO)

        def step(it, u):
            s = it * UNR + u
            lhs = jnp.concatenate([_bf(lhs_w[s, j]) for j in range(DB)], axis=1)

            def side(slot):
                if slot not in SIDE_SLOTS:
                    return None
                q = SIDE_SLOTS.index(slot)
                return post(jnp.maximum(s - (2 if q == 0 else 1), 0), q)[0]

            def proj(m_i, p):
                g = m_i * NPAIR + p
                for t in range(2):
                    qkv_s[g, pl.ds(t * SEG, SEG), :] = _dot(lhs, weights(2 * g + t)).astype(BF16)

            def rows_of(m_i, p):
                g = m_i * NPAIR + p
                return jnp.concatenate([_bf(qkv_w[g]), _bf(cache_w[g, it, pl.ds(u * M, M), :])], axis=0)

            def probs(p):
                parts = [lax.dot_general(_bf(qkv_w[p]), rows_of(1, p), (((1,), (1,)), ((), ())),
                                         preferred_element_type=F32)]
                qc = _bf(cache_w[p, it, pl.ds(u * M, M), :]).astype(F32)
                kc = _bf(cache_w[NPAIR + p, it, pl.ds(u * M, M), :]).astype(F32)
                col = lax.broadcasted_iota(jnp.int32, (M, PR), 1)

                def scores8(q, keys):
                    xs = [jnp.sum(q * keys[j:j + 1], axis=-1, keepdims=True) for j in range(M)]
                    bit = 1
                    while len(xs) > 1:
                        xs = [jnp.where((col & bit) == 0, xs[i], xs[i + 1]) for i in range(0, len(xs), 2)]
                        bit *= 2
                    return xs[0]

                for t in range(2):
                    km = _bf(qkv_w[NPAIR + p, pl.ds(t * (SEG // 2), 8), :]).astype(F32)
                    qt = qc[t * M:(t + 1) * M]
                    parts.append(jnp.where(col < 2 * SEG, scores8(qt, km),
                                           scores8(qt, kc[t * M:(t + 1) * M])))
                sc = jnp.concatenate(parts, axis=0) * SCALE
                fm = fill_v[...]
                tok = side(("softmax", p))
                if tok is not None:
                    top = fm[0:8]
                    fm = jnp.concatenate([jnp.where(top > 1.0, tok, top), fm[8:]], axis=0)
                sc = jnp.where(fm == 0.0, sc, fm)
                e = jnp.exp(sc - jnp.max(sc, axis=-1, keepdims=True))
                return (e * _recip(jnp.sum(e, axis=-1, keepdims=True))).astype(BF16)

            def attend(p, pr):
                o = _dot(pr, rows_of(2, p))
                for t in range(2):
                    o_s[2 * p + t, pl.ds(0, SEG), :] = o[t * SEG:(t + 1) * SEG].astype(BF16)
                for t in range(2):
                    o_s[2 * p + t, pl.ds(SEG + (u % 2) * M, M), :] = (
                        o[2 * SEG + t * M:2 * SEG + (t + 1) * M].astype(BF16))

            ps = {}
            for pa in range(0, NPAIR, 2):
                pb = pa + 1
                todo = [(0, pa), (1, pa), (0, pb), (1, pb), (2, pa), (2, pb)]
                if pa == 0 and u > 0:
                    hs = [(m_i * NPAIR + p, t) for m_i, p in todo[:NSPLIT] for t in range(2)]
                    ke = KEARLY * 128
                    first = [_dot(lhs[:, :ke], weights(2 * g + t, 0, KEARLY)) for g, t in hs]
                    for (g, t), part in zip(hs, first):
                        res = _dot(lhs[:, ke:], weights(2 * g + t, KEARLY, DB)) + part
                        qkv_s[g, pl.ds(t * SEG, SEG), :] = res.astype(BF16)
                    todo = todo[NSPLIT:]
                for m_i, p in todo:
                    proj(m_i, p)
                for kind in ("scores", "values") if pa % 4 == 0 else ("values", "scores"):
                    for p in (pa, pb):
                        if kind == "scores":
                            ps[p] = probs(p)
                        elif p >= 2:
                            attend(p - 2, ps.pop(p - 2))
            L = NPAIR - 1

            nxt = s + 1 if u < UNR - 1 else jnp.where(it < NIT - 1, s + 1, 0)
            nr = SEG + (2 * M if u % 2 else 0)
            for h0, h1 in ((0, HA), (HA, H)):
                for j in range(DB):
                    words = [o_w[h, pl.ds(0, nr // 2), :] for h in range(h0, h1)]
                    words[0] = tie(words[0], side((h0, j)))
                    ol = jnp.concatenate([_bf(w) for w in words], axis=1)
                    part = _dot(ol, _bf(wo_v[j, pl.ds(h0 * E // 2, (h1 - h0) * E // 2), :]))
                    if h0 == 0:
                        acc_s[j, pl.ds(0, nr), :] = part
                    else:
                        a = part + acc_s[j, pl.ds(0, nr), :]
                        cols = pl.ds(j * 128, 128)
                        lhs_v[nxt, j, pl.ds(0, M), :] = a[0:M].astype(BF16)
                        for q in range(1, nr // M):
                            seg, rows = (s, pl.ds(q * M, M)) if q < 4 else (s + q - 5, pl.ds(0, M))
                            x1 = x_v[seg, rows, cols].astype(F32) + mod_v[2, :, cols] * a[q * M:(q + 1) * M]
                            x1_v[seg, rows, cols] = x1.astype(BF16)
                    if h0 == 0 and j == (2 if u % 2 else 3):
                        attend(L - 1, ps.pop(L - 1))
                        attend(L, ps.pop(L))

        def iteration(it, carry):
            @pl.when(it >= 2)
            def _():
                out_copy(it - 2).start()

            @pl.when(it < FB // 2)
            def _():
                for t in range(2):
                    j = 2 * it + t
                    cols = pl.ds(pl.multiple_of(j * 128, 128), 128)
                    half = pl.ds(t * (D // 2), D // 2)
                    copy(wg_w.at[:, cols], stage.at[it, half, :], SEM_MOE).start()
                    copy(wu_w.at[:, cols], stage.at[FB // 2 + it, half, :], SEM_MOE).start()

            @pl.when(it < DB)
            def _():
                cols = pl.ds(pl.multiple_of(it * 128, 128), 128)
                for t in range(2):
                    copy(wd_w.at[pl.ds(t * (F // 4), F // 4), cols],
                         stage.at[FB + 2 * it + t, pl.ds(0, F // 4), :], SEM_MOE + 1).start()

            for u in range(UNR):
                step(it, u)
            return carry

        lax.fori_loop(0, NIT, iteration, 0)

        out_copy(NIT - 2).start()
        wait_all(stage.at[pl.ds(0, FB)], SEM_MOE)
        wait_all(stage.at[pl.ds(FB, 2 * DB), pl.ds(0, F // 4), :], SEM_MOE + 1)
        r8 = lax.broadcasted_iota(jnp.int32, (8, 1), 0)

        def top2(vals, idx, axes):
            def red(f, v):
                for ax in axes:
                    v = f(v, axis=ax, keepdims=True)
                return v
            m1 = red(jnp.max, vals)
            i1 = red(jnp.min, jnp.where(vals == m1, idx, S - 1.0))
            rest = jnp.where(idx == i1, -jnp.inf, vals)
            m2 = red(jnp.max, rest)
            i2 = red(jnp.min, jnp.where(rest == m2, jnp.where(idx == i1, S - 1.0, idx), S - 1.0))
            return m1, i1, m2, i2

        m1, i1v, m2, i2v = top2(r_v[...], (lane * 8 + r8).astype(F32), (1, 0))
        vals = [jnp.where(r8 == 0, m1, jnp.where(r8 == 1, m2, -jnp.inf))]
        idxs = [jnp.where(r8 == 0, i1v, jnp.where(r8 == 1, i2v, S - 1.0))]
        for seg, q in [(NSEG - 2, 0)] + [(NSEG - 1, q) for q in range(4)]:
            vals.append(post(seg, q, keep=False)[1])
            idxs.append((r8 + (seg * SEG + q * 8)).astype(F32))
        out_copy(NIT - 1).start()
        m1, i1v, m2, i2v = top2(jnp.concatenate(vals, axis=0), jnp.concatenate(idxs, axis=0), (0,))
        i1 = i1v.astype(jnp.int32)[0, 0]
        i2 = i2v.astype(jnp.int32)[0, 0]

        def tile_of(i):
            return i >> 5, pl.multiple_of(((i >> 3) & 3) * 8, 8)

        sel = [tile_of(i1), tile_of(i2)]
        x1s = jnp.concatenate([x1_v[sg, pl.ds(r0, 8), :].astype(F32) for sg, r0 in sel], axis=0)
        h2s = jnp.concatenate([h2_v[sg, pl.ds(r0, 8), :].astype(F32) for sg, r0 in sel], axis=0)
        h2b = h2s.astype(BF16)
        gus = []
        for j in range(FB):
            half = pl.ds((j % 2) * (D // 2), D // 2)
            g = _rb(_dot(h2b, _bf(stage[j // 2, half, :])))
            g = _rb(g * jax.nn.sigmoid(g))
            u = _rb(_dot(h2b, _bf(stage[FB // 2 + j // 2, half, :])))
            gus.append(g * u)
        gu = jnp.concatenate(gus, axis=1).astype(BF16)
        ys = []
        for j in range(DB):
            wd = stage[pl.ds(FB + 2 * j, 2), pl.ds(0, F // 4), :].reshape(F // 2, 128)
            ys.append(_rb(_dot(gu, _bf(wd))))
        y = jnp.concatenate(ys, axis=1)
        rows = lax.broadcasted_iota(jnp.int32, (16, 1), 0)
        rs = _rb(jax.nn.sigmoid(jnp.where(rows < 8, m1, m2)))
        y = _rb(y * rs)
        full = x1s + mod_row(5, 16) * _rb(h2s + y)

        copy(out_v, out_hbm, SEM_OUT).wait()
        for t, (i, (sg, r0)) in enumerate(zip((i1, i2), sel)):
            old = out_v[sg, pl.ds(r0, 8), :].astype(F32)
            new = jnp.where(r8 == (i & 7), full[t * 8:(t + 1) * 8], old)
            out_v[sg, pl.ds(r0, 8), :] = new.astype(BF16)
        fix = [copy(out_v.at[sg, pl.ds(r0, 8), :], out_hbm.at[sg, pl.ds(r0, 8), :], SEM_OUT + 1 + t)
               for t, (sg, r0) in enumerate(sel)]
        differ = (i1 >> 3) != (i2 >> 3)
        fix[0].start()

        @pl.when(differ)
        def _():
            fix[1].start()
            fix[1].wait()

        fix[0].wait()

    main()


@jax.jit
def pallas_adaLN_cond__memory_aug_recurrent_mem_tr__moe_arch_mod__prompt_kernel(
    A_x: jax.Array,
    A_mem0: jax.Array,
    A_Wq: jax.Array,
    A_Wk: jax.Array,
    A_Wv: jax.Array,
    A_Wo: jax.Array,
    A_seg_len: jax.Array,
    B_x: jax.Array,
    B_w_r: jax.Array,
    B_w_gate: jax.Array,
    B_w_up: jax.Array,
    B_w_down: jax.Array,
    c: jax.Array,
    w_mod: jax.Array,
):
    del A_seg_len, B_x
    assert A_x.shape == (1, S, D) and A_mem0.shape == (1, M, D) and A_Wq.shape == (D, H, E)
    hbm = pl.BlockSpec(memory_space=pl.ANY)
    out = pl.pallas_call(
        _kernel,
        out_shape=jax.ShapeDtypeStruct((NSEG, SEG, D), BF16),
        in_specs=[hbm] * 12,
        out_specs=hbm,
        scratch_shapes=[
            pltpu.VMEM((NSEG, SEG, D), BF16),
            pltpu.VMEM((3 * H, DB, 128, E), BF16),
            pltpu.VMEM((DB, H * E // 2, 128), U32),
            pltpu.VMEM((NGP, NIT, UNR * 2 * M, E), BF16),
            pltpu.VMEM((NSEG, DB, SEG, 128), BF16),
            pltpu.VMEM((NGP, 2 * SEG, E), BF16),
            pltpu.VMEM((H, 2 * SEG, E), BF16),
            pltpu.VMEM((DB, 2 * SEG, 128), F32),
            pltpu.VMEM((7, 8, D), F32),
            pltpu.VMEM((2, 8, D), F32),
            pltpu.VMEM((NGP, D, E), U32),
            pltpu.VMEM((6, DB, D // 2, 128), U32),
            pltpu.VMEM((DB, NSEG * M, E), BF16),
            pltpu.VMEM((DB, NSEG * M, 128), F32),
            pltpu.VMEM((2 * KMAJ, NSEG * M, E), F32),
            pltpu.VMEM((DB, 16, 128), BF16),
            pltpu.VMEM((D, 128), F32),
            pltpu.VMEM((NSEG, SEG, D), BF16),
            pltpu.VMEM((NSEG, SEG, D), BF16),
            pltpu.VMEM((NSEG, SEG, D), BF16),
            pltpu.VMEM((M, D), BF16),
            pltpu.VMEM((8, S // 8), F32),
            pltpu.VMEM((PR, PR), F32),
            pltpu.VMEM((8, 128), F32),
            pltpu.VMEM((1, D), BF16),
            pltpu.VMEM((D,), BF16),
            pltpu.SemaphoreType.DMA((NSEM,)),
        ],
        compiler_params=pltpu.CompilerParams(
            vmem_limit_bytes=120 * 1024 * 1024, disable_bounds_checks=True,
            disable_semaphore_checks=True),
    )(
        A_x.reshape(NSEG, SEG, D),
        A_mem0.reshape(M, D),
        A_Wq, A_Wk, A_Wv,
        A_Wo.reshape(H * E, D),
        B_w_r,
        B_w_gate, B_w_up, B_w_down,
        c, w_mod,
    )
    return out.reshape(1, S, D)
```
